```python
import jax
import jax.numpy as jnp

def _softmax(x, axis=-1):
    return jax.nn.softmax(x, axis=axis)
def _gelu(x):
    return jax.nn.gelu(x, approximate=True)
def _silu(x):
    return jax.nn.silu(x)
def _sigmoid(x):
    return jax.nn.sigmoid(x)
def _layernorm(x, axis=-1, eps=1e-5):
    m = jnp.mean(x, axis=axis, keepdims=True)
    v = jnp.var(x, axis=axis, keepdims=True)
    return (x - m) / jnp.sqrt(v + eps)
def _scatter_add(tgt, idx, src, axis=0):
    return tgt.at[idx].add(src)
def _segment_sum(src, seg, n):
    return jax.ops.segment_sum(src, seg, n)
class _Rng:
    def __init__(self, key):
        self._k = key
    def _next(self):
        self._k, sub = jax.random.split(self._k)
        return sub
    def normal(self, shape):
        return jax.random.normal(self._next(), shape, dtype=jnp.bfloat16)
    def randint(self, lo, hi, shape):
        return jax.random.randint(self._next(), shape, lo, hi, dtype=jnp.int32)
    def uniform(self, shape, lo=0.0, hi=1.0):
        return jax.random.uniform(self._next(), shape, jnp.bfloat16, lo, hi)
    def permutation(self, n):
        return jax.random.permutation(self._next(), n)


kernel_name = 'gated_mix__compressed_kv_cla__moe_arch_mod__prompt'

def setup_inputs():
    _rng = _Rng(jax.random.key(int.from_bytes(__import__("os").urandom(4), "little")))
    _w = (lambda a: (lambda t: t.astype(jnp.bfloat16) if jnp.issubdtype(t.dtype, jnp.floating) else t)(jnp.asarray(a)))
    def _A_setup():
        B, H, Sq, Sk, D, M = 1, 16, 2048, 2048, 256, 448
        Dc = 4 * D
        return {
            "x": _w((lambda *s: _rng.normal(s) * 0.05)(B, Sq, M)),
            "c_kv": _w((lambda *s: _rng.normal(s) * 0.05)(B, Sk, Dc)),
            "w_q": _w((lambda *s: _rng.normal(s) * 0.05)(M, H, D) * (M ** -0.5)),
            "w_uk": _w((lambda *s: _rng.normal(s) * 0.05)(Dc, H, D) * (Dc ** -0.5)),
            "w_uv": _w((lambda *s: _rng.normal(s) * 0.05)(Dc, H, D) * (Dc ** -0.5)),
            "w_o": _w((lambda *s: _rng.normal(s) * 0.05)(H, D, M) * ((H * D) ** -0.5)),
        }
    _A_in = _A_setup()

    def _B_setup():
        B, S, D, F, C = 1, 2048, 448, 1792, 2
        return {
            "x": _w((lambda *s: _rng.normal(s) * 0.05)(B, S, D)),
            "w_r": _w((lambda *s: _rng.normal(s) * 0.05)(D)),
            "w_gate": _w((lambda *s: _rng.normal(s) * 0.05)(D, F)),
            "w_up": _w((lambda *s: _rng.normal(s) * 0.05)(D, F)),
            "w_down": _w((lambda *s: _rng.normal(s) * 0.05)(F, D)),
        }
    _B_in = _B_setup()

    return {
        "A_x": _A_in["x"],
        "A_c_kv": _A_in["c_kv"],
        "A_w_q": _A_in["w_q"],
        "A_w_uk": _A_in["w_uk"],
        "A_w_uv": _A_in["w_uv"],
        "A_w_o": _A_in["w_o"],
        "B_x": _B_in["x"],
        "B_w_r": _B_in["w_r"],
        "B_w_gate": _B_in["w_gate"],
        "B_w_up": _B_in["w_up"],
        "B_w_down": _B_in["w_down"],
        "gate_w": _w((lambda *s: _rng.normal(s) * 0.05)(448)),
    }

def reference(A_x, A_c_kv, A_w_q, A_w_uk, A_w_uv, A_w_o, B_x, B_w_r, B_w_gate, B_w_up, B_w_down, gate_w):
    def _A_ref(x, c_kv, w_q, w_uk, w_uv, w_o):
        B, Sq, M = x.shape[0], x.shape[1], x.shape[2]
        Sk = c_kv.shape[1]
        H, D = w_q.shape[1], w_q.shape[2]
        q = jnp.einsum("bqm,mhd->bhqd", x, w_q)
        k = jnp.einsum("bkc,chd->bhkd", c_kv, w_uk)
        v = jnp.einsum("bkc,chd->bhkd", c_kv, w_uv)
        scores = jnp.einsum("bhqd,bhkd->bhqk", q, k) * (D ** -0.5)
        off = Sk - Sq
        qi = jnp.arange(Sq)[:, None]
        kj = jnp.arange(Sk)[None, :]
        cmask = kj <= (qi + off)
        scores = jnp.where(cmask[None, None], scores, -1e9)
        p = _softmax(scores, axis=-1)
        ctx = jnp.einsum("bhqk,bhkd->bhqd", p, v)
        return jnp.einsum("bhqd,hdm->bqm", ctx, w_o)

    def _B_ref(x, w_r, w_gate, w_up, w_down):
        B, S, D = x.shape
        C = 2
        r = x @ w_r
        idx = jnp.argsort(-r, axis=-1)[:, :C]
        idx_e = jnp.repeat(idx.reshape(B, C, 1), D, axis=2)
        x_sel = jnp.take_along_axis(x, idx_e, axis=1)
        g = _silu(x_sel @ w_gate)
        u = x_sel @ w_up
        y = (g * u) @ w_down
        r_sel = _sigmoid(jnp.take_along_axis(r, idx, axis=1))
        y = y * r_sel.reshape(B, C, 1)
        b_off = (jnp.arange(B) * S).reshape(B, 1)
        flat_idx = (idx + b_off).reshape(B * C)
        zero = (x * 0.0).reshape(B * S, D)
        upd = _scatter_add(zero, flat_idx, y.reshape(B * C, D), axis=0)
        return x + upd.reshape(B, S, D)

    x = A_x
    g = _sigmoid((x * gate_w).sum(-1, keepdims=True))
    a = _A_ref(x, A_c_kv, A_w_q, A_w_uk, A_w_uv, A_w_o)
    b = _B_ref(x, B_w_r, B_w_gate, B_w_up, B_w_down)
    return g * a + (1 - g) * b
```

```python
import functools, math
import jax, jax.numpy as jnp
from jax import lax
from jax.experimental import pallas as pl
from jax.experimental.pallas import tpu as pltpu

S, M, H, D, DC, F = 2048, 448, 16, 256, 1024, 1792
NP = H // 2
NT = (((1,), (1,)), ((), ()))
LOG2E = math.log2(math.e)
bf = jnp.bfloat16
f32 = jnp.float32
u32 = jnp.uint32
NEG = -1e30

SEM_XT, SEM_C, SEM_WO, SEM_FFN, SEM_VEC, SEM_OUT, SEM_KV, SEM_WQ = 0, 1, 2, 3, 6, 8, 12, 16
NSEM = 24


def _lo(x):
    return pltpu.bitcast(x << 16, f32).astype(bf)


def _hi(x):
    return pltpu.bitcast(x & jnp.uint32(0xFFFF0000), f32).astype(bf)


def _sel(x, sh):
    return pltpu.bitcast((x << sh) & jnp.uint32(0xFFFF0000), f32).astype(bf)


def kernel(xt_hbm, c_hbm, wq_hbm, wk_hbm, wv_hbm, wo_hbm, wr_hbm, wg_hbm, wu_hbm, wd_hbm, gw_hbm,
           o_hbm,
           xt_s, x_s, c_s, wq_p, wkv_p, wo_s, q_s, k_s, v_s, acc_s, wg_s, wu_s, wd_s,
           wr_s, gw_s, rg_s, out_s, sem, *, tq, cfg):
    mk = pltpu.make_async_copy
    wq32 = wq_hbm.bitcast(u32)
    wk32 = wk_hbm.bitcast(u32)
    wv32 = wv_hbm.bitcast(u32)
    cp_xt = mk(xt_hbm, xt_s, sem.at[SEM_XT])
    cp_wq = lambda j: mk(wq32.at[:, j, :], wq_p.at[j], sem.at[SEM_WQ + j])
    cp_wr = mk(wr_hbm, wr_s, sem.at[SEM_VEC])
    cp_gw = mk(gw_hbm, gw_s, sem.at[SEM_VEC + 1])

    def cp_kv(j):
        slot = j % 2
        return [mk(wk32.at[:, j, :], wkv_p.at[slot, 0], sem.at[SEM_KV + 2 * slot]),
                mk(wv32.at[:, j, :], wkv_p.at[slot, 1], sem.at[SEM_KV + 2 * slot + 1])]
    cp_c = mk(c_hbm, c_s, sem.at[SEM_C])
    cp_wo = mk(wo_hbm, wo_s, sem.at[SEM_WO])
    cp_ffn = [mk(wg_hbm, wg_s, sem.at[SEM_FFN]), mk(wu_hbm, wu_s, sem.at[SEM_FFN + 1]), mk(wd_hbm, wd_s, sem.at[SEM_FFN + 2])]

    cp_xt.start()
    cp_wr.start()
    cp_gw.start()
    cp_wq(0).start()
    acc_s[...] = jnp.zeros_like(acc_s)
    cp_xt.wait()
    for j in range(1, NP):
        cp_wq(j).start()
    cp_c.start()
    for cp in cp_kv(0):
        cp.start()
    cp_wo.start()
    for cp in cp_ffn:
        cp.start()

    x_s[...] = xt_s[...].T
    cp_wr.wait()
    cp_gw.wait()
    row8 = lax.broadcasted_iota(jnp.int32, (8, M), 0)
    lhs = jnp.where(row8 == 0, wr_s[...].reshape(1, M).astype(f32), gw_s[...].reshape(1, M).astype(f32)).astype(bf)
    rg_s[...] = jnp.dot(lhs, xt_s[...], preferred_element_type=f32)

    def qbody(j, carry):
        cp_wq(j).wait()
        w32 = wq_p[j]
        w = jnp.concatenate([_lo(w32), _hi(w32)], axis=1)
        q = (jnp.dot(x_s[...], w, preferred_element_type=f32) * (D ** -0.5 * LOG2E)).astype(bf)
        for e in range(2):
            for t in range(2):
                q_s[2 * j + e, t] = q[:, (2 * e + t) * 128:(2 * e + t + 1) * 128]
        return carry
    lax.fori_loop(0, NP, qbody, 0)

    cp_c.wait()
    cp_wo.wait()

    nq = S // tq
    row = lax.broadcasted_iota(jnp.int32, (tq, tq), 0)
    col = lax.broadcasted_iota(jnp.int32, (tq, tq), 1)
    tri = col <= row

    def head(h, carry):
        j = h // 2
        slot = j % 2

        @pl.when(h % 2 == 0)
        def _():
            for cp in cp_kv(j):
                cp.wait()

            @pl.when(j + 1 < NP)
            def _():
                for cp in cp_kv(j + 1):
                    cp.start()

        sh = (16 * (1 - h % 2)).astype(u32)
        wk = _sel(wkv_p[slot, 0], sh)
        wv = _sel(wkv_p[slot, 1], sh)
        wo = wo_s[h]

        def vproj():
            v = jnp.dot(c_s[...], wv, preferred_element_type=f32).astype(bf)
            for t in range(2):
                v_s[t] = v[:, t * 128:(t + 1) * 128]

        def rows2(ref, a, b):
            return jnp.concatenate([ref[t, a:b, :] for t in range(2)], axis=1)

        def qk(i):
            L = (i + 1) * tq
            q = jnp.concatenate([q_s[h, t, i * tq:(i + 1) * tq, :] for t in range(2)], axis=1)
            sd = lax.dot_general(q, rows2(k_s, L - tq, L), NT, preferred_element_type=f32)
            sd = jnp.where(tri, sd, NEG)
            if i == 0:
                return (sd,)
            so = lax.dot_general(q, rows2(k_s, 0, L - tq), NT, preferred_element_type=f32)
            return (so, sd)

        def sm_pv(i, ss):
            L = (i + 1) * tq
            m = functools.reduce(jnp.maximum, [jnp.max(s, axis=1, keepdims=True) for s in ss])
            ps = [jnp.exp2(s - m) for s in ss]
            l = functools.reduce(jnp.add, [jnp.sum(p, axis=1, keepdims=True) for p in ps])
            p = jnp.concatenate([p.astype(bf) for p in ps], axis=1) if len(ps) > 1 else ps[0].astype(bf)
            ctx = jnp.dot(p, rows2(v_s, 0, L), preferred_element_type=f32)
            r0 = pl.reciprocal(l, approx=True)
            r = r0 * (2.0 - l * r0)
            return (ctx * r).astype(bf)

        def oproj(i, ctx):
            acc_s[:, i * tq:(i + 1) * tq] += lax.dot_general(wo, ctx, NT, preferred_element_type=f32)

        kc = cfg.get('kc', 2)
        ns = cfg.get('ns', 4)
        od = cfg.get('od', 2)
        step = S // kc
        for a in range(0, S, step):
            k = jnp.dot(c_s[a:a + step, :], wk, preferred_element_type=f32).astype(bf)
            for t in range(2):
                k_s[t, a:a + step, :] = k[:, t * 128:(t + 1) * 128]
        sss = {i: qk(i) for i in range(ns)}
        vproj()
        ctxs = {}
        sss[ns] = qk(ns)
        for i in range(ns):
            ctxs[i] = sm_pv(i, sss.pop(i))
        done = 0
        for i in range(ns, nq):
            if i + 1 < nq:
                sss[i + 1] = qk(i + 1)
            ctxs[i] = sm_pv(i, sss.pop(i))
            n = 0
            while done <= i - od and n < 2:
                oproj(done, ctxs.pop(done)); done += 1; n += 1
        while done < nq:
            oproj(done, ctxs.pop(done)); done += 1
        return carry

    lax.fori_loop(0, H, head, 0)

    r = rg_s[0:1, :]
    rb = r.astype(bf).astype(f32)
    lane = lax.broadcasted_iota(jnp.int32, (1, S), 1)
    m1 = jnp.max(rb, axis=1, keepdims=True)
    i1 = jnp.min(jnp.where(rb == m1, lane, S), axis=1, keepdims=True)
    rb2 = jnp.where(lane == i1, -jnp.inf, rb)
    m2 = jnp.max(rb2, axis=1, keepdims=True)
    i2 = jnp.min(jnp.where(jnp.logical_and(rb2 == m2, lane != i1), lane, S), axis=1, keepdims=True)
    rows = lax.broadcasted_iota(jnp.int32, (16, S), 0)
    lanes = lax.broadcasted_iota(jnp.int32, (16, S), 1)
    sel = jnp.where(rows == 0, i1, jnp.where(rows == 1, i2, -1))
    onehot = (lanes == sel).astype(f32).astype(bf)
    xs = jnp.dot(onehot, x_s[...], preferred_element_type=f32).astype(bf)
    for cp in cp_ffn:
        cp.wait()
    gg = jnp.dot(xs, wg_s[...], preferred_element_type=f32)
    uu = jnp.dot(xs, wu_s[...], preferred_element_type=f32)
    hh = (gg * jax.nn.sigmoid(gg) * uu)
    rcol = lax.broadcasted_iota(jnp.int32, (16, 1), 0)
    rsel = jax.nn.sigmoid(jnp.where(rcol == 0, m1, m2))
    hh = hh.astype(bf)
    yT = lax.dot_general(wd_s[...], hh, NT, preferred_element_type=f32)
    y1 = yT[:, 0:1] * rsel[0:1, :]
    y2 = yT[:, 1:2] * rsel[1:2, :]
    g = jax.nn.sigmoid(rg_s[1:2, :])
    CW = 512
    cps = []
    for b in range(S // CW):
        sl = slice(b * CW, (b + 1) * CW)
        ln = lane[:, sl]
        upd = jnp.where(ln == i1, y1, 0.0) + jnp.where(ln == i2, y2, 0.0)
        gb = g[:, sl]
        out_s[:, sl] = (gb * acc_s[:, sl] + (1.0 - gb) * (xt_s[:, sl].astype(f32) + upd)).astype(bf)
        cp = mk(out_s.at[:, pl.ds(b * CW, CW)], o_hbm.at[:, pl.ds(b * CW, CW)], sem.at[SEM_OUT + b])
        cp.start()
        cps.append(cp)
    for cp in cps:
        cp.wait()


def make(tq=128, **cfg):
    name = "k3_" + "_".join([str(tq)] + [f"{k}{int(v)}" for k, v in sorted(cfg.items())])

    @jax.jit
    def f(A_x, A_c_kv, A_w_q, A_w_uk, A_w_uv, A_w_o, B_x, B_w_r, B_w_gate, B_w_up, B_w_down, gate_w):
        xt = A_x[0].T
        c = A_c_kv[0]
        woT = A_w_o.transpose(0, 2, 1)
        wdT = B_w_down.T
        V = pltpu.VMEM
        outT = pl.pallas_call(
            functools.partial(kernel, tq=tq, cfg=cfg),
            in_specs=[pl.BlockSpec(memory_space=pl.ANY)] * 11,
            out_specs=pl.BlockSpec(memory_space=pl.ANY),
            out_shape=jax.ShapeDtypeStruct((M, S), bf),
            scratch_shapes=[
                V((M, S), bf), V((S, M), bf), V((S, DC), bf),
                V((NP, M, D), u32), V((2, 2, DC, D), u32), V((H, M, D), bf),
                V((H, 2, S, 128), bf), V((2, S, 128), bf), V((2, S, 128), bf), V((M, S), f32),
                V((M, F), bf), V((M, F), bf), V((M, F), bf),
                V((M,), bf), V((M,), bf), V((8, S), f32), V((M, S), bf),
                pltpu.SemaphoreType.DMA((NSEM,)),
            ],
            compiler_params=pltpu.CompilerParams(vmem_limit_bytes=110 * 1024 * 1024),
            name=name,
        )(xt, c, A_w_q, A_w_uk, A_w_uv, woT, B_w_r, B_w_gate, B_w_up, wdT, gate_w)
        return outT.T[None]
    return f


_impl = make(**{'tq': 128, 'od': 3, 'ns': 3})


@jax.jit
def pallas_gated_mix__compressed_kv_cla__moe_arch_mod__prompt_kernel(
    A_x: jax.Array,
    A_c_kv: jax.Array,
    A_w_q: jax.Array,
    A_w_uk: jax.Array,
    A_w_uv: jax.Array,
    A_w_o: jax.Array,
    B_x: jax.Array,
    B_w_r: jax.Array,
    B_w_gate: jax.Array,
    B_w_up: jax.Array,
    B_w_down: jax.Array,
    gate_w: jax.Array,
):
    return _impl(A_x, A_c_kv, A_w_q, A_w_uk, A_w_uv, A_w_o, B_x, B_w_r, B_w_gate, B_w_up, B_w_down, gate_w)
```

```python
import functools, math
import jax, jax.numpy as jnp
from jax import lax
from jax.experimental import pallas as pl
from jax.experimental.pallas import tpu as pltpu

S, M, H, D, DC, F = 2048, 448, 16, 256, 1024, 1792
NP = H // 2
NT = (((1,), (1,)), ((), ()))
LOG2E = math.log2(math.e)
bf = jnp.bfloat16
f32 = jnp.float32
u32 = jnp.uint32
NEG = -1e30

SEM_C, SEM_WO, SEM_FFN, SEM_VEC, SEM_KV, SEM_WQ, SEM_OUT, SEM_XT = 1, 2, 3, 6, 8, 12, 20, 28
NSEM = 44


def _lo(x):
    return pltpu.bitcast(x << 16, f32).astype(bf)


def _hi(x):
    return pltpu.bitcast(x & jnp.uint32(0xFFFF0000), f32).astype(bf)


def _sel(x, sh):
    return pltpu.bitcast((x << sh) & jnp.uint32(0xFFFF0000), f32).astype(bf)


PROGS = {
    0: "Q0 Q1 Q2 V Q3 P0 P1 P2 Q4 P3 Q5 P4 D0 Q6 P5 Q7 P6 D2 Q8 P7 Q9 P8 D4 Q10 P9 Q11 P10 D6 Q12 P11 Q13 P12 D8 Q14 P13 Q15 P14 D10 P15 D12 D14",
    1: "Q0 Q1 Q2 V Q3 P0 P1 P2 Q4 P3 Q5 P4 D0 Q6 P5 Q7 P6 D2 Q8 P7 Q9 P8 D4 Q10 P9 Q11 P10 D6 Q12 P11 Q13 P12 D8 Q14 P13 Q15 P14 D10 P15 D12 S14 S15",
    2: "Q0 Q1 Q15 V Q14 P0 P1 P15 Q13 P14 D0 Q12 P13 Q11 P12 D14 Q10 P11 Q9 P10 D12 Q8 P9 Q7 P8 D10 Q6 P7 Q5 P6 D8 Q4 P5 Q3 P4 Q2 P3 D6 P2 D4 S3 S2",
    3: "Q0 Q1 Q2 V Q3 P0 P1 P2 Q4 P3 Q5 P4 D0 Q6 P5 Q7 P6 D2 Q8 P7 Q9 P8 D4 Q10 P9 Q11 P10 D6 Q12 P11 Q13 P12 Q14 D8 Q15 P13 D10 P14 P15 D12 S14 S15",
}


def make_prog(nq, cfg):
    if 'prog' in cfg:
        return [(t[0], int(t[1:] or 0)) for t in PROGS[cfg['prog']].split()]
    ns = cfg.get('ns', 3)
    od = cfg.get('od', 3)
    mode = cfg.get('mode', 0)
    hold = cfg.get('hold', 0)
    if mode == 0:
        main = list(range(ns, nq))
    else:
        main = list(range(nq - 1, ns - 1, -1))
    prog = [('Q', i) for i in range(ns)]
    if mode == 1:
        prog += [('Q', main[0]), ('V', 0), ('Q', main[1])]
    else:
        prog += [('V', 0), ('Q', main[0])]
    prog += [('P', i) for i in range(ns)]
    ready = list(range(ns))
    qdone = 2 if mode == 1 else 1
    for n, i in enumerate(main):
        last = n == len(main) - 1
        if qdone < len(main) and qdone <= n + 1:
            prog.append(('Q', main[qdone])); qdone += 1
        if last:
            while len(ready) > cfg.get('tail', 2):
                prog.append(('O', ready.pop(0)))
        prog.append(('P', i))
        ready.append(i)
        k = 0
        lim = od + (hold if n >= len(main) - 1 - hold else 0)
        while len(ready) > lim and k < 2 and not last:
            prog.append(('O', ready.pop(0))); k += 1
    prog += [('O', i) for i in ready]
    return prog


def kernel(xt_hbm, c_hbm, wq_hbm, wk_hbm, wv_hbm, wo_hbm, wr_hbm, wg_hbm, wu_hbm, wd_hbm, gw_hbm,
           o_hbm,
           xt_s, x_s, c_s, wq_p, wkv_p, wo_s, q_s, k_s, v_s, acc_s, wg_s, wu_s, wd_s,
           wr_s, gw_s, g_s, out_s, r_s, grow_s, xs_s, rsel_s, idx_s, sem, *, tq, cfg):
    mk = pltpu.make_async_copy
    wq32 = wq_hbm.bitcast(u32)
    wk32 = wk_hbm.bitcast(u32)
    wv32 = wv_hbm.bitcast(u32)
    cp_wq = lambda j: mk(wq32.at[:, j, :], wq_p.at[j], sem.at[SEM_WQ + j])
    cp_wr = mk(wr_hbm, wr_s, sem.at[SEM_VEC])
    cp_gw = mk(gw_hbm, gw_s, sem.at[SEM_VEC + 1])

    def cp_kv(j):
        slot = j % 2
        return [mk(wk32.at[:, j, :], wkv_p.at[slot, 0], sem.at[SEM_KV + 2 * slot]),
                mk(wv32.at[:, j, :], wkv_p.at[slot, 1], sem.at[SEM_KV + 2 * slot + 1])]
    cp_c = mk(c_hbm, c_s, sem.at[SEM_C])
    cp_wo = mk(wo_hbm, wo_s, sem.at[SEM_WO])
    cp_ffn = [mk(wg_hbm, wg_s, sem.at[SEM_FFN]), mk(wu_hbm, wu_s, sem.at[SEM_FFN + 1]), mk(wd_hbm, wd_s, sem.at[SEM_FFN + 2])]

    OW = cfg.get('ow', 256)
    cp_out = lambda b: mk(out_s.at[:, pl.ds(b * OW, OW)], o_hbm.at[:, pl.ds(b * OW, OW)], sem.at[SEM_OUT + b])

    XC = cfg.get('xc', 256)
    NXC = S // XC
    cp_xtc = lambda k: mk(xt_hbm.at[:, pl.ds(k * XC, XC)], xt_s.at[:, pl.ds(k * XC, XC)], sem.at[SEM_XT + k])
    cp_wq(0).start()
    for k in range(NXC):
        cp_xtc(k).start()
        if k == 0:
            cp_wr.start()
            cp_gw.start()
    for j in range(1, NP):
        cp_wq(j).start()
    for cp in cp_ffn:
        cp.start()
    cp_c.start()
    for cp in cp_kv(0):
        cp.start()
    cp_wo.start()

    def qw(j):
        w32 = wq_p[j]
        return jnp.concatenate([_lo(w32), _hi(w32)], axis=1)

    def qdot(j, w, r0, r1, n0, n1):
        q = (jnp.dot(x_s[r0:r1, :], w[:, n0 * 128:n1 * 128], preferred_element_type=f32) * (D ** -0.5 * LOG2E)).astype(bf)
        for n in range(n0, n1):
            q_s[2 * j + n // 2, n % 2, r0:r1, :] = q[:, (n - n0) * 128:(n - n0 + 1) * 128]

    def qinter(j, w, sops, rc=256):
        sops = list(sops)
        for n in range(4):
            for r0 in range(0, S, rc):
                if sops:
                    sops.pop(0)()
                qdot(j, w, r0, r0 + rc, n, n + 1)
        assert not sops

    row8 = lax.broadcasted_iota(jnp.int32, (8, M), 0)

    def tr(k):
        x_s[k * XC:(k + 1) * XC, :] = xt_s[:, k * XC:(k + 1) * XC].T

    def route(n):
        lhs = jnp.where(row8 == 0, wr_s[...].reshape(1, M).astype(f32), gw_s[...].reshape(1, M).astype(f32)).astype(bf)
        grow_s[n] = jnp.dot(lhs, xt_s[:, n * 128:(n + 1) * 128], preferred_element_type=f32)

    segs = cfg.get('segs', (2, 5, 8))
    cp_wq(0).wait()
    tdone = qdone = rdone = 0
    for si, e in enumerate(segs):
        for k in range(tdone, e):
            cp_xtc(k).wait()
        last = si == len(segs) - 1
        if last:
            cp_wr.wait()
            cp_gw.wait()
        w = qw(0)
        qe = e if last else e - 1
        while tdone < e or qdone < qe:
            if tdone < e:
                tr(tdone); tdone += 1
            if qdone < min(qe, tdone - (1 if tdone < e or si == 0 else 0)) or (tdone == e and qdone < qe):
                if last and rdone < S // 128:
                    for n in range(4):
                        for hh_ in range(2):
                            route(rdone); rdone += 1
                            r0 = qdone * XC + hh_ * (XC // 2)
                            qdot(0, w, r0, r0 + XC // 2, n, n + 1)
                else:
                    qdot(0, w, qdone * XC, (qdone + 1) * XC, 0, 4)
                qdone += 1
    r_all = jnp.concatenate([grow_s[n][0:1, :] for n in range(S // 128)], axis=1)
    rb = r_all.astype(bf).astype(f32)
    lane = lax.broadcasted_iota(jnp.int32, (1, S), 1)
    m1 = jnp.max(rb, axis=1, keepdims=True)
    i1 = jnp.minimum(jnp.min(jnp.where(rb == m1, lane, S)), S - 1)
    rb2 = jnp.where(lane == i1, -jnp.inf, rb)
    m2 = jnp.max(rb2, axis=1, keepdims=True)
    i2 = jnp.minimum(jnp.min(jnp.where(jnp.logical_and(rb2 == m2, lane != i1), lane, S)), S - 1)
    row16 = lax.broadcasted_iota(jnp.int32, (16, M), 0)

    def xrow(i):
        blk = x_s[pl.ds(pl.multiple_of((i // 16) * 16, 16), 16), :].astype(f32)
        return jnp.sum(jnp.where(row16 == i % 16, blk, 0.0), axis=0, keepdims=True)
    xs_s[...] = jnp.where(row16 == 0, xrow(i1), jnp.where(row16 == 1, xrow(i2), 0.0)).astype(bf)
    rcol = lax.broadcasted_iota(jnp.int32, (16, 128), 0)
    rsel_s[...] = jax.nn.sigmoid(jnp.where(rcol == 0, m1, m2))
    idx_s[0] = i1
    idx_s[1] = i2

    def qbody(j, carry):
        cp_wq(j).wait()
        qdot(j, qw(j), 0, S, 0, 4)
        return carry
    lax.fori_loop(1, NP - 1, qbody, 0)

    for cp in cp_ffn:
        cp.wait()
    cp_wq(NP - 1).wait()
    for n in range(S // 128):
        g8 = jax.nn.sigmoid(grow_s[n])
        g_s[n * 128:(n + 1) * 128, :] = g8.T
        grow_s[n] = g8
        acc_s[n] = (1.0 - g8[1:2, :]) * xt_s[:, n * 128:(n + 1) * 128].astype(f32)
    xs = xs_s[...]
    ggs, uus, ys, hh = [], [], {}, []
    sops = []
    for n in range(F // 128):
        sops.append(lambda n=n: ggs.append(jnp.dot(xs, wg_s[:, n * 128:(n + 1) * 128], preferred_element_type=f32)))
        sops.append(lambda n=n: uus.append(jnp.dot(xs, wu_s[:, n * 128:(n + 1) * 128], preferred_element_type=f32)))

    def act():
        gg = jnp.concatenate(ggs, axis=1)
        uu = jnp.concatenate(uus, axis=1)
        hh.append((gg * jax.nn.sigmoid(gg) * uu).astype(bf))
    sops += [act] + [lambda: None] * 3
    for n0 in range(0, M, 128):
        for k0 in range(0, F, 512):
            def f(n0=n0, k0=k0):
                k1, n1 = min(k0 + 512, F), min(n0 + 128, M)
                t = lax.dot_general(hh[0][:, k0:k1], wd_s[n0:n1, k0:k1], NT, preferred_element_type=f32)
                ys[n0] = t if n0 not in ys else ys[n0] + t
            sops.append(f)
    qinter(NP - 1, qw(NP - 1), sops, rc=128)
    y = jnp.concatenate([ys[n0] for n0 in range(0, M, 128)] + [jnp.zeros((16, 512 - M), f32)], axis=1) * rsel_s[:, 0:1]
    yT = y.T
    lane128 = lax.broadcasted_iota(jnp.int32, (1, 128), 1)
    for e in range(2):
        i = idx_s[e]
        t = i // 128
        acc_s[t] += jnp.where(lane128 == i % 128, (1.0 - grow_s[t][1:2, :]) * yT[:M, e:e + 1], 0.0)

    cp_c.wait()
    cp_wo.wait()

    nq = S // tq
    row = lax.broadcasted_iota(jnp.int32, (tq, tq), 0)
    col = lax.broadcasted_iota(jnp.int32, (tq, tq), 1)
    tri = col <= row

    def head(h, carry):
        j = h // 2
        slot = j % 2

        @pl.when(h % 2 == 0)
        def _():
            for cp in cp_kv(j):
                cp.wait()

            @pl.when(j + 1 < NP)
            def _():
                for cp in cp_kv(j + 1):
                    cp.start()

        sh = (16 * (1 - h % 2)).astype(u32)
        wk = _sel(wkv_p[slot, 0], sh)
        wv = _sel(wkv_p[slot, 1], sh)
        wo = wo_s[h]

        kv = {}

        def rows2(ref, a, b):
            return jnp.concatenate([ref[t, a:b, :] for t in range(2)], axis=1)

        def getk(a, b):
            return kv['k'][a:b, :] if cfg.get('kval', 1) else rows2(k_s, a, b)

        def getv(a, b):
            return kv['v'][a:b, :] if cfg.get('kval', 1) else rows2(v_s, a, b)

        def vproj():
            v = jnp.dot(c_s[...], wv, preferred_element_type=f32).astype(bf)
            if cfg.get('kval', 1):
                kv['v'] = v
            else:
                for t in range(2):
                    v_s[t] = v[:, t * 128:(t + 1) * 128]

        def qk(i):
            L = (i + 1) * tq
            q = jnp.concatenate([q_s[h, t, i * tq:(i + 1) * tq, :] for t in range(2)], axis=1)
            s = lax.dot_general(q, getk(0, L), NT, preferred_element_type=f32)
            sd = jnp.where(tri, s[:, L - tq:], NEG)
            if i == 0:
                return sd
            return jnp.concatenate([s[:, :L - tq], sd], axis=1)

        def sm_pv(i, s):
            L = (i + 1) * tq
            m = jnp.max(s, axis=1, keepdims=True)
            if cfg.get('chain', 1):
                nacc = None
                ps = []
                for j in range(L // 128):
                    p = jnp.exp2(s[:, j * 128:(j + 1) * 128] - m)
                    if nacc is None:
                        nacc = -p
                    else:
                        p = jnp.maximum(p, nacc)
                        nacc = nacc - p
                    ps.append(p)
                l = -jnp.sum(nacc, axis=1, keepdims=True)
                p = jnp.concatenate(ps, axis=1)
            else:
                p = jnp.exp2(s - m)
                l = None if cfg.get('lbf', 0) else jnp.sum(p, axis=1, keepdims=True)
            pb = p.astype(bf)
            if l is None:
                l = jnp.sum(pb.astype(f32), axis=1, keepdims=True)
            ctx = jnp.dot(pb, getv(0, L), preferred_element_type=f32)
            r0 = pl.reciprocal(l, approx=True)
            r = r0 * (2.0 - l * r0) * g_s[i * tq:(i + 1) * tq, 1:2]
            return (ctx * r).astype(bf)

        def oproj(i, ctx):
            acc_s[:, i * tq:(i + 1) * tq] += lax.dot_general(wo, ctx, NT, preferred_element_type=f32)

        odone = set()

        def fin(blocks):
            odone.update(blocks)
            b = blocks[0] * tq // OW
            if all(bb in odone for bb in range(b * OW // tq, (b + 1) * OW // tq)):
                @pl.when(h == H - 1)
                def _():
                    cp_out(b).start()

        def oproj2(i, ctx):
            d = lax.dot_general(wo, ctx, NT, preferred_element_type=f32)
            for e in range(2):
                a = acc_s[i + e] + d[:, e * tq:(e + 1) * tq]
                acc_s[i + e] = a
                out_s[:, (i + e) * tq:(i + e + 1) * tq] = a.astype(bf)
            fin([i, i + 1])

        def oprojs(i, ctx):
            for a0 in (0, M // 2):
                a = acc_s[i, a0:a0 + M // 2, :] + lax.dot_general(wo[a0:a0 + M // 2], ctx, NT, preferred_element_type=f32)
                acc_s[i, a0:a0 + M // 2, :] = a
                out_s[a0:a0 + M // 2, i * tq:(i + 1) * tq] = a.astype(bf)
            fin([i])

        kc = cfg.get('kc', 2)
        ns = cfg.get('ns', 4)
        od = cfg.get('od', 2)
        step = S // kc
        ks = []
        for a in range(0, S, step):
            k = jnp.dot(c_s[a:a + step, :], wk, preferred_element_type=f32).astype(bf)
            if cfg.get('kval', 1):
                ks.append(k)
            else:
                for t in range(2):
                    k_s[t, a:a + step, :] = k[:, t * 128:(t + 1) * 128]
        if cfg.get('kval', 1):
            kv['k'] = jnp.concatenate(ks, axis=0)
        prog = make_prog(nq, cfg)
        sss, ctxs = {}, {}
        for op, i in prog:
            if op == 'Q':
                sss[i] = qk(i)
            elif op == 'V':
                vproj()
            elif op == 'P':
                ctxs[i] = sm_pv(i, sss.pop(i))
            elif op == 'O':
                oproj(i, ctxs.pop(i))
            elif op == 'D':
                oproj2(i, jnp.concatenate([ctxs.pop(i), ctxs.pop(i + 1)], axis=0))
            elif op == 'S':
                oprojs(i, ctxs.pop(i))
        return carry

    lax.fori_loop(0, H, head, 0)

    for b in range(S // OW):
        cp_out(b).wait()


def make(tq=128, **cfg):
    name = "k9_" + "_".join([str(tq)] + [f"{k}{v}" for k, v in sorted(cfg.items())]).replace(" ", "").replace("(", "").replace(")", "").replace(",", "x")

    @jax.jit
    def f(A_x, A_c_kv, A_w_q, A_w_uk, A_w_uv, A_w_o, B_x, B_w_r, B_w_gate, B_w_up, B_w_down, gate_w):
        xt = A_x[0].T
        c = A_c_kv[0]
        woT = A_w_o.transpose(0, 2, 1)
        wdT = B_w_down.T
        V = pltpu.VMEM
        outT = pl.pallas_call(
            functools.partial(kernel, tq=tq, cfg=cfg),
            in_specs=[pl.BlockSpec(memory_space=pl.ANY)] * 11,
            out_specs=pl.BlockSpec(memory_space=pl.ANY),
            out_shape=jax.ShapeDtypeStruct((M, S), bf),
            scratch_shapes=[
                V((M, S), bf), V((S, M), bf), V((S, DC), bf),
                V((NP, M, D), u32), V((2, 2, DC, D), u32), V((H, M, D), bf),
                V((H, 2, S, 128), bf), V((2, S, 128), bf), V((2, S, 128), bf), V((S // 128, M, 128), f32),
                V((M, F), bf), V((M, F), bf), V((M, F), bf),
                V((M,), bf), V((M,), bf), V((S, 8), f32), V((M, S), bf),
                V((1, S), f32), V((S // 128, 8, 128), f32), V((16, M), bf), V((16, 128), f32), pltpu.SMEM((2,), jnp.int32),
                pltpu.SemaphoreType.DMA((NSEM,)),
            ],
            compiler_params=pltpu.CompilerParams(vmem_limit_bytes=110 * 1024 * 1024),
            name=name,
        )(xt, c, A_w_q, A_w_uk, A_w_uv, woT, B_w_r, B_w_gate, B_w_up, wdT, gate_w)
        return outT.T[None]
    return f


_impl = make(**{'chain': 0, 'prog': 2, 'lbf': 1})


@jax.jit
def pallas_gated_mix__compressed_kv_cla__moe_arch_mod__prompt_kernel(
    A_x: jax.Array,
    A_c_kv: jax.Array,
    A_w_q: jax.Array,
    A_w_uk: jax.Array,
    A_w_uv: jax.Array,
    A_w_o: jax.Array,
    B_x: jax.Array,
    B_w_r: jax.Array,
    B_w_gate: jax.Array,
    B_w_up: jax.Array,
    B_w_down: jax.Array,
    gate_w: jax.Array,
):
    return _impl(A_x, A_c_kv, A_w_q, A_w_uk, A_w_uv, A_w_o, B_x, B_w_r, B_w_gate, B_w_up, B_w_down, gate_w)
```

```python
import functools, math
import jax, jax.numpy as jnp
from jax import lax
from jax.experimental import pallas as pl
from jax.experimental.pallas import tpu as pltpu

S, M, H, D, DC, F = 2048, 448, 16, 256, 1024, 1792
NP = H // 2
HS, HC, HM = S // 2, DC // 2, M // 2
T = 128
NQ = S // T
NT = (((1,), (1,)), ((), ()))
QSCALE = D ** -0.5 * math.log2(math.e)
bf = jnp.bfloat16
f32 = jnp.float32
u32 = jnp.uint32
NEG = -1e30

SEM_C, SEM_WO, SEM_FFN, SEM_VEC, SEM_KV, SEM_WQ, SEM_OUT, SEM_XT = 1, 2, 3, 6, 8, 12, 20, 28
NSEM = 44

PROGS = {
    10: "R0 R7 V R6 P0 P1 P15 P14 D0 R5 P13 P12 D14 R4 P11 P10 D12 R3 P9 P8 D10 R2 P7 P6 D8 R1 P5 P4 D6 P3 P2 D4 S3 S2",
    11: "R0 R7 V R6 P0 P1 P15 P14 R5 D0 P13 P12 R4 D14 P11 P10 R3 D12 P9 P8 R2 D10 P7 P6 R1 D8 P5 P4 D6 P3 P2 D4 S3 S2",
    12: "R0 R7 V R6 P0 P1 P14 P15 D0 R5 P12 P13 D14 R4 P10 P11 D12 R3 P8 P9 D10 R2 P6 P7 D8 R1 P4 P5 D6 P2 P3 D4 S2 S3",
    2: "Q0 Q1 Q15 V Q14 P0 P1 P15 Q13 P14 D0 Q12 P13 Q11 P12 D14 Q10 P11 Q9 P10 D12 Q8 P9 Q7 P8 D10 Q6 P7 Q5 P6 D8 Q4 P5 Q3 P4 Q2 P3 D6 P2 D4 S3 S2",
    4: "Q0 Q1 Q15 V Q14 P0 P1 P15 Q13 P14 D0 Q12 P13 Q11 P12 D14 Q10 P11 Q9 P10 D12 Q8 P9 Q7 P8 D10 Q6 P7 Q5 P6 D8 Q4 P5 Q3 P4 Q2 P3 D6 P2 D4 D2",
}


def _merge(a, b):
    out, i, j = [], 0, 0
    while i < len(a) or j < len(b):
        if j >= len(b) or (i < len(a) and i * len(b) <= j * len(a)):
            out.append(a[i]); i += 1
        else:
            out.append(b[j]); j += 1
    return out


def fine_prog(cfg):
    pc = cfg.get('pc', 2)
    if cfg.get('dfirst', 0):
        R = lambda I: [('d', I, 0)] + [('r', I, J) for J in range(I)]
    else:
        R = lambda I: [('r', I, J) for J in range(I)] + [('d', I, 0)]
    P1 = lambda i: [('p', i, c) for c in range(0, i + 1, pc)]
    if cfg.get('pab', 0):
        P = lambda I: _merge(P1(2 * I + 1), P1(2 * I))
    else:
        P = (lambda I: P1(2 * I + 1) + P1(2 * I)) if cfg.get('bfirst', 0) else (lambda I: P1(2 * I) + P1(2 * I + 1))
    nch = cfg.get('nch', 2)
    io = (1, 3, 4, 6, 0, 2, 5)
    MM = lambda r1s, ch: [('m', (r1, r2, ch), 0) for r1 in r1s for r2 in io]
    K5, V2 = (1, 3, 4, 6, 0), (2, 5)
    r7 = lambda js: [('r', 7, J) for J in js]
    if nch == 1:
        V = MM(V2, 0)
        nv = cfg.get('nv', 10)
        prog = MM(K5, 0) + V[:1] + _merge(R(0) + R(7), V[1:nv]) + V[nv:]
    else:
        h_ = nch // 2
        KA = sum([MM(K5, ch) for ch in range(h_)], [])
        KB = sum([MM(K5, ch) for ch in range(h_, nch)], [])
        VA = sum([MM(V2, ch) for ch in range(h_)], [])
        VB = sum([MM(V2, ch) for ch in range(h_, nch)], [])
        k0 = int(len(KB) * cfg.get('k0', 0.2))
        v0 = int(len(VA) * cfg.get('v0', 0.2))
        prog = (KA + KB[:k0] + _merge([('d', 0, 0)] + r7((0, 2, 4, 6)), KB[k0:]) + VA[:v0]
                + _merge(r7((1, 3, 5)) + [('d', 7, 0)], VA[v0:]) + VB)
    order = [7, 6, 5, 4, 3, 2, 1]
    pend = [0]
    for n, I in enumerate(order):
        ps = P(I)
        if n == 0:
            ps = P(0) + ps
        nxt = R(order[n + 1]) if n + 1 < len(order) else []
        k = max(1, int(round(len(ps) * cfg.get('rf', 1.0))))
        body = _merge(nxt, ps[:k]) + ps[k:]
        dpos = cfg.get('dpos', 0.9)
        if n > 0:
            k = int(len(body) * dpos)
            body = body[:k] + [('D', 2 * pend.pop(0), 0)] + body[k:]
        prog += body
        pend.append(I)
    last = pend.pop()
    prog += [('D', 2 * I, 0) for I in pend]
    prog += [('S', 2 * last + 1, 0), ('S', 2 * last, 0)] if cfg.get('bfirst', 0) else [('S', 2 * last, 0), ('S', 2 * last + 1, 0)]
    return prog


def _lo32(x):
    return pltpu.bitcast(x << 16, f32)


def _hi32(x):
    return pltpu.bitcast(x & jnp.uint32(0xFFFF0000), f32)


def _lhs_terms(a11, a12, a21, a22):
    return [a11 + a22, a21 + a22, a11, a22, a11 + a12, a21 - a11, a12 - a22]


def _rhs_terms(b11, b12, b21, b22):
    return [b11 + b22, b11, b12 - b22, b21 - b11, b22, b11 + b12, b21 + b22]


def _strassen(mm, var=0):
    if var == 0:
        m1 = mm(0); m4 = mm(3); m5 = mm(4); m7 = mm(6); m3 = mm(2); m2 = mm(1); m6 = mm(5)
        return m1 + m4 - m5 + m7, m3 + m5, m2 + m4, m1 + m3 - m2 + m6
    if var == 1:
        m2 = mm(1); m3 = mm(2); m4 = mm(3); m5 = mm(4); m1 = mm(0); m7 = mm(6); m6 = mm(5)
        return (m4 - m5) + (m1 + m7), m3 + m5, m2 + m4, (m3 - m2) + (m1 + m6)


def _lhs_terms2(a11, a12, a21, a22):
    h21 = 0.5 * a21
    q21 = 0.25 * a21
    h22 = 0.5 * a22
    s1 = a11 + a22
    v = a12 + q21
    hs = 0.5 * s1
    return [s1, q21 + h22, a11 + h21, h22 - q21, v + hs, h21 - a11, v - hs]


def _rhs_terms2(b11, b12, b21, b22):
    h21 = 0.5 * b21
    t1 = b11 + b22
    v = b12 + 0.5 * h21
    ht = 0.5 * t1
    return [t1, b11 + h21, v - ht, h21 - b11, b22 - h21, v + ht, b22 + h21]


def _left2(m):
    s = m[3] + m[1]
    t = m[0] + (m[3] - m[1])
    return t + (m[6] - m[4]), s, t, s + (m[6] + m[4])


def _comb2(m):
    c11, s, t, se = _left2(m)
    return c11, se + (m[2] - m[5]), s, t + (m[2] + m[5])


def _left1(m):
    return (m[3] - m[4]) + (m[0] + m[6]), m[1] + m[3], m[0] - m[1], m[4]


def _comb1(m):
    return (m[3] - m[4]) + (m[0] + m[6]), m[2] + m[4], m[1] + m[3], (m[2] - m[1]) + (m[0] + m[5])


def _zero_like_dep(v):
    return (pltpu.bitcast(v[0:8, 0:128], u32) >> 16) >> 16


def _dep_u32(vals):
    ts = []
    for v in vals:
        v = pltpu.bitcast(v, u32) if v.dtype != u32 else v
        r, c = v.shape
        for r0 in range(0, r, 8):
            for c0 in range(0, c - T + 1, T):
                ts.append(v[r0:r0 + 8, c0:c0 + T])
    W = 4
    acc = ts[:W]
    for i, t in enumerate(ts[W:]):
        acc[i % W] = acc[i % W] | t
    while len(acc) > 1:
        acc = [acc[i] | acc[i + 1] if i + 1 < len(acc) else acc[i] for i in range(0, len(acc), 2)]
    return (acc[0] >> 16) >> 16


def _feed(a, z):
    if z is None:
        return a
    a32 = pltpu.bitcast(a, u32)
    top = a32[0:8, :T] | z
    if a32.shape[1] > T:
        top = jnp.concatenate([top, a32[0:8, T:]], axis=1)
    return pltpu.bitcast(jnp.concatenate([top, a32[8:]], axis=0), bf)


def kernel(xt_hbm, c_hbm, wq_hbm, wk_hbm, wv_hbm, wo_hbm, wr_hbm, wg_hbm, wu_hbm, wd_hbm, gw_hbm,
           o_hbm,
           xt_s, x_s, xa_s, c_s, sa_s, wq_p, wkv_p, wo_s, q_s, qa_s, acc_s, wg_s, wu_s, wd_s,
           wr_s, gw_s, out_s, g_s, xs_s, rsel_s, idx_s, s_s, sem, *, cfg):
    mk = pltpu.make_async_copy
    wq32 = wq_hbm.bitcast(u32)
    wk32 = wk_hbm.bitcast(u32)
    wv32 = wv_hbm.bitcast(u32)
    cp_wq = lambda j: mk(wq32.at[:, j, :], wq_p.at[j], sem.at[SEM_WQ + j])
    cp_wr = mk(wr_hbm, wr_s, sem.at[SEM_VEC])
    cp_gw = mk(gw_hbm, gw_s, sem.at[SEM_VEC + 1])

    def cp_kv(j):
        slot = j % 2
        return [mk(wk32.at[:, j, :], wkv_p.at[slot, 0], sem.at[SEM_KV + 2 * slot]),
                mk(wv32.at[:, j, :], wkv_p.at[slot, 1], sem.at[SEM_KV + 2 * slot + 1])]
    cp_c = mk(c_hbm, c_s, sem.at[SEM_C])
    cp_wo = mk(wo_hbm, wo_s, sem.at[SEM_WO])
    cp_ffn = [mk(wg_hbm, wg_s, sem.at[SEM_FFN]), mk(wu_hbm, wu_s, sem.at[SEM_FFN + 1]), mk(wd_hbm, wd_s, sem.at[SEM_FFN + 2])]
    OW = 256
    cp_out = lambda b: mk(out_s.at[:, pl.ds(b * OW, OW)], o_hbm.at[:, pl.ds(b * OW, OW)], sem.at[SEM_OUT + b])
    XC = 256
    NXC = S // XC
    cp_xtc = lambda k: mk(xt_hbm.at[:, pl.ds(k * XC, XC)], xt_s.at[:, pl.ds(k * XC, XC)], sem.at[SEM_XT + k])

    cp_wq(0).start()
    for k in range(NXC):
        cp_xtc(k).start()
    cp_wr.start()
    cp_gw.start()
    for j in range(1, NP):
        cp_wq(j).start()
    for cp in cp_ffn:
        cp.start()
    cp_c.start()
    for cp in cp_kv(0):
        cp.start()
    cp_wo.start()

    sq = cfg.get('sq', 1)
    sqk = cfg.get('sqk', 1)

    def store_q(j, e, r0, q):
        qs = q * QSCALE
        for t in range(2):
            q_s[2 * j + e, t, r0:r0 + q.shape[0], :] = qs[:, t * T:(t + 1) * T].astype(bf)
        if sqk:
            for p0 in range(0, q.shape[0], 2 * T):
                if r0 + p0 == 0:
                    continue
                qa, qc = qs[p0:p0 + T], qs[p0 + T:p0 + 2 * T]
                k = 0
                for i, v in enumerate(_lhs_terms(qa[:, :T], qa[:, T:], qc[:, :T], qc[:, T:])):
                    if i not in (2, 3):
                        qa_s[2 * j + e, k, (r0 + p0) // 2:(r0 + p0) // 2 + T, :] = v.astype(bf)
                        k += 1

    def qplain(j, w, r0, r1, n0, n1, z=None):
        wn = w[:, n0 * T:n1 * T]
        qf = (jnp.dot(_feed(x_s[0, r0:r1, :], z), wn[:HM], preferred_element_type=f32)
              + jnp.dot(x_s[1, r0:r1, :], wn[HM:], preferred_element_type=f32))
        return qf

    def qplain_blk(j, w, r0, small=None):
        if small is None:
            qf = qplain(j, w, r0, r0 + 2 * T, 0, 4)
        else:
            cols = []
            for n in range(4):
                cols.append(jnp.concatenate([qplain(j, w, r0 + u * T, r0 + (u + 1) * T, n, n + 1, small()) for u in range(2)], axis=0))
            qf = jnp.concatenate(cols, axis=1)
        store_q(j, 0, r0, qf[:, :D]); store_q(j, 1, r0, qf[:, D:])

    def qw(j):
        w32 = wq_p[j]
        return jnp.concatenate([_lo32(w32).astype(bf), _hi32(w32).astype(bf)], axis=1)

    def q_rhs(j):
        w32 = wq_p[j]
        lo, hi = _lo32(w32), _hi32(w32)
        return [t.astype(bf) for t in _rhs_terms(lo[:HM], hi[:HM], lo[HM:], hi[HM:])]

    def q_lhs(i, r0, r1):
        if i == 2:
            return x_s[0, r0:r1, :]
        if i == 3:
            return x_s[1, HS + r0:HS + r1, :]
        return xa_s[i, r0:r1, :]

    def qstr(j, ts, r0, r1, pre=None, post=None):
        def mm(i):
            if pre is None:
                return jnp.dot(q_lhs(i, r0, r1), ts[i], preferred_element_type=f32)
            return jnp.concatenate([jnp.dot(_feed(q_lhs(i, u, u + T), pre()), ts[i], preferred_element_type=f32)
                                    for u in range(r0, r1, T)], axis=0)
        c11, c12, c21, c22 = _strassen(mm)
        store_q(j, 0, r0, c11); store_q(j, 1, r0, c12); store_q(j, 0, HS + r0, c21); store_q(j, 1, HS + r0, c22)

    RB = 16

    def xprep(r0):
        a = [x_s[e, h0 + r0:h0 + r0 + RB, :].astype(f32) for h0 in (0, HS) for e in (0, 1)]
        outs = []
        for i, v in enumerate(_lhs_terms(*a)):
            if i not in (2, 3):
                vb = v.astype(bf)
                xa_s[i, r0:r0 + RB, :] = vb
                outs.append(pltpu.bitcast(vb, u32))
        return outs

    row8 = lax.broadcasted_iota(jnp.int32, (8, M), 0)

    def tr(k):
        for e in range(2):
            x_s[e, k * XC:(k + 1) * XC, :] = xt_s[e * HM:(e + 1) * HM, k * XC:(k + 1) * XC].T

    def route(n):
        lhs = jnp.where(row8 == 0, wr_s[...].reshape(1, M).astype(f32), gw_s[...].reshape(1, M).astype(f32)).astype(bf)
        g_s[n] = jnp.dot(lhs, xt_s[:, n * T:(n + 1) * T], preferred_element_type=f32)

    segs = cfg.get('segs', (2, 4, 8))
    cp_wq(0).wait()
    tdone = qdone = rdone = 0
    xdone = 0
    nsmall = (segs[-1] - segs[-2] + 1) * 8
    ksm = 0
    st = dict(r=0, k=0, x=0)

    def small0():
        if st['r'] < NQ:
            route(st['r']); st['r'] += 1
        st['k'] += 1
        x0 = cfg.get('x0', 12)
        outs = []
        if sq and st['k'] > x0:
            tgt = min(HS // RB, (st['k'] - x0) * (HS // RB) // (nsmall - x0))
            while st['x'] < tgt:
                outs += xprep(st['x'] * RB); st['x'] += 1
        return _dep_u32(outs) if outs else None
    for si, e in enumerate(segs):
        for k in range(tdone, e):
            cp_xtc(k).wait()
        last = si == len(segs) - 1
        if last:
            cp_wr.wait()
            cp_gw.wait()
            while tdone < e:
                tr(tdone); tdone += 1
        w = qw(0)
        qe = e if last else e - 1
        while tdone < e or qdone < qe:
            if tdone < e:
                tr(tdone); tdone += 1
            if qdone < min(qe, tdone - (1 if tdone < e or si == 0 else 0)) or (tdone == e and qdone < qe):
                qplain_blk(0, w, qdone * XC, small0 if last else None)
                qdone += 1
    assert not sq or st['x'] == HS // RB

    r_all = jnp.concatenate([g_s[n][0:1, :] for n in range(NQ)], axis=1)
    rb = r_all.astype(bf).astype(f32)
    lane = lax.broadcasted_iota(jnp.int32, (1, S), 1)
    m1 = jnp.max(rb, axis=1, keepdims=True)
    i1 = jnp.minimum(jnp.min(jnp.where(rb == m1, lane, S)), S - 1)
    rb2 = jnp.where(lane == i1, -jnp.inf, rb)
    m2 = jnp.max(rb2, axis=1, keepdims=True)
    i2 = jnp.minimum(jnp.min(jnp.where(jnp.logical_and(rb2 == m2, lane != i1), lane, S)), S - 1)
    row16 = lax.broadcasted_iota(jnp.int32, (16, HM), 0)

    def xrow(e, i):
        blk = x_s[e, pl.ds(pl.multiple_of((i // 16) * 16, 16), 16), :].astype(f32)
        return jnp.sum(jnp.where(row16 == i % 16, blk, 0.0), axis=0, keepdims=True)
    for e in range(2):
        xs_s[e] = jnp.where(row16 == 0, xrow(e, i1), jnp.where(row16 == 1, xrow(e, i2), 0.0)).astype(bf)
    rcol = lax.broadcasted_iota(jnp.int32, (16, T), 0)
    rsel_s[...] = jax.nn.sigmoid(jnp.where(rcol == 0, m1, m2))
    idx_s[0] = i1
    idx_s[1] = i2

    def qbody(j, carry):
        cp_wq(j).wait()
        if sq:
            qstr(j, q_rhs(j), 0, HS)
        else:
            raise NotImplementedError
        return carry
    lax.fori_loop(1, NP - 1, qbody, 0)

    for cp in cp_ffn:
        cp.wait()
    cp_wq(NP - 1).wait()
    cp_c.wait()

    QS, QC = S // 4, DC // 4

    dps = cfg.get('dps', 1)
    dpo, dpi = cfg.get('dpo', dps), cfg.get('dpi', dps)
    lo_, li_ = (_lhs_terms2 if dpo else _lhs_terms), (_lhs_terms2 if dpi else _lhs_terms)

    def cprep(t):
        r0, c0 = (t // 2) * RB, (t % 2) * T
        blk = lambda i, k: c_s[i * QS + r0:i * QS + r0 + RB, k * QC + c0:k * QC + c0 + T].astype(f32)
        inner = [[[blk(2 * i1 + i2, 2 * k1 + k2) for i1 in range(2) for k1 in range(2)] for k2 in range(2)] for i2 in range(2)]
        outer = [[lo_(*inner[i2][k2]) for k2 in range(2)] for i2 in range(2)]
        outs = []
        for r1 in range(7):
            for r2, v in enumerate(li_(outer[0][0][r1], outer[0][1][r1], outer[1][0][r1], outer[1][1][r1])):
                o = pltpu.bitcast(v.astype(bf), u32)
                sa_s[7 * r1 + r2, r0 // 2:(r0 + RB) // 2, c0:c0 + T] = o
                outs.append(o)
        return outs

    def binit(n):
        g8 = jax.nn.sigmoid(g_s[n])
        g_s[n] = g8
        a = (1.0 - g8[1:2, :]) * xt_s[:, n * T:(n + 1) * T].astype(f32)
        acc_s[n] = a
        return [a]

    ggs, uus, ys, hh = [], [], {}, []
    sops = []

    def xdot(w_s, n):
        return (jnp.dot(xs_s[0], w_s[:HM, n * T:(n + 1) * T], preferred_element_type=f32)
                + jnp.dot(xs_s[1], w_s[HM:, n * T:(n + 1) * T], preferred_element_type=f32))
    for n in range(F // T):
        sops.append(lambda n=n: ggs.append(xdot(wg_s, n)))
        sops.append(lambda n=n: uus.append(xdot(wu_s, n)))

    def act():
        gg = jnp.concatenate(ggs, axis=1)
        uu = jnp.concatenate(uus, axis=1)
        hh.append((gg * jax.nn.sigmoid(gg) * uu).astype(bf))
    sops += [act] + [lambda: None] * 3
    for n0 in range(0, M, T):
        for k0 in range(0, F, 512):
            def f(n0=n0, k0=k0):
                k1, n1 = min(k0 + 512, F), min(n0 + T, M)
                t = lax.dot_general(hh[0][:, k0:k1], wd_s[n0:n1, k0:k1], NT, preferred_element_type=f32)
                ys[n0] = t if n0 not in ys else ys[n0] + t
            sops.append(f)
    cnt = [0, 0]
    ndots = 56 if sq else 64
    c0 = cfg.get('c0', 2)

    def pre():
        if sops:
            sops.pop(0)()
        k = cnt[0]
        cnt[0] += 1
        outs = []
        while k >= c0 and cnt[1] < min(HS // RB, (k + 1 - c0) * (HS // RB) // (ndots - c0)):
            outs += cprep(cnt[1]); cnt[1] += 1
        if k % 3 == 2 and k // 3 < NQ:
            outs += binit(k // 3)
        return _dep_u32(outs) if outs else None
    if sq:
        ts = q_rhs(NP - 1)
        for r0 in range(0, HS, 2 * T):
            qstr(NP - 1, ts, r0, r0 + 2 * T, pre)
    assert not sops and cnt[1] == HS // RB
    y = jnp.concatenate([ys[n0] for n0 in range(0, M, T)] + [jnp.zeros((16, 512 - M), f32)], axis=1) * rsel_s[:, 0:1]
    yT = y.T
    lane128 = lax.broadcasted_iota(jnp.int32, (1, T), 1)
    for e in range(2):
        i = idx_s[e]
        t = i // T
        acc_s[t] += jnp.where(lane128 == i % T, (1.0 - g_s[t][1:2, :]) * yT[:M, e:e + 1], 0.0)

    cp_wo.wait()

    tri = lax.broadcasted_iota(jnp.int32, (T, T), 1) <= lax.broadcasted_iota(jnp.int32, (T, T), 0)
    prog = fine_prog(cfg)

    def head(h, carry):
        j = h // 2
        slot = j % 2

        @pl.when(h % 2 == 0)
        def _():
            for cp in cp_kv(j):
                cp.wait()

            @pl.when(j + 1 < NP)
            def _():
                for cp in cp_kv(j + 1):
                    cp.start()

        sh = (16 * (1 - h % 2)).astype(u32)

        wf = [pltpu.bitcast((wkv_p[slot, m] << sh) & jnp.uint32(0xFFFF0000), f32) for m in range(2)]
        ro_, ri_ = (_rhs_terms2 if dpo else _rhs_terms), (_rhs_terms2 if dpi else _rhs_terms)
        if dps and cfg.get('bb', 0):
            BR = cfg.get('br', 16)
            cols = {}
            for r0 in range(0, QC, BR):
                b = {(k, jj): wf[jj // 2][k * QC + r0:k * QC + r0 + BR, (jj % 2) * T:(jj % 2 + 1) * T]
                     for k in range(4) for jj in range(4)}
                for st in (2, 1):
                    for k in range(4):
                        for jj in range(4):
                            if not k & st:
                                b[k, jj] = b[k, jj] + 0.5 * b[k + st, jj]
                    for k in range(4):
                        for jj in range(4):
                            if jj & st:
                                b[k, jj] = b[k, jj] - 0.5 * b[k, jj - st]
                for key, v in b.items():
                    cols.setdefault(key, []).append(v)
            bp = {key: jnp.concatenate(v, axis=0) for key, v in cols.items()}
            tq = [[_rhs_terms(bp[k2, j2], bp[k2, 2 + j2], bp[2 + k2, j2], bp[2 + k2, 2 + j2]) for j2 in range(2)] for k2 in range(2)]
            tinner = [[u.astype(bf) for u in _rhs_terms(tq[0][0][r1], tq[0][1][r1], tq[1][0][r1], tq[1][1][r1])] for r1 in range(7)]
            touter = None
        else:
            touter = ro_(wf[0][:HC], wf[1][:HC], wf[0][HC:], wf[1][HC:])
            tinner = [[u.astype(bf) for u in ri_(t[:QC, :T], t[:QC, T:], t[QC:, :T], t[QC:, T:])] for t in touter]
        nch = cfg.get('nch', 2)
        CR = QS // nch
        pres, mo, kblk, vblk, part = {}, {}, {}, {}, {}
        force = []
        cs_in = (1.0, 0.5, 2.0, 1.0) if dpi else (1.0,) * 4
        cs_out = (1.0, 0.5, 2.0, 1.0) if dpo else (1.0,) * 4

        def scaled(v, c):
            return v if c == 1.0 else v * c

        def pmm(r1, r2, ch):
            a = pltpu.bitcast(sa_s[7 * r1 + r2, ch * CR // 2:(ch + 1) * CR // 2, :], bf)
            fk = cfg.get('fk', 0)
            for it in list(force):
                it[0] -= 1
                if it[0] == 0:
                    a = _feed(a, _dep_u32(it[1]))
                    force.remove(it)
            fb = cfg.get('fb', 0)
            seq = (1, 3, 4, 6, 0, 2, 5)
            p1, p2 = seq.index(r1), seq.index(r2)
            if fb and ch == 0 and p1 + 1 < 7 and fb <= p2 < fb + 4:
                t = touter[seq[p1 + 1]]
                q = p2 - fb
                a = _feed(a, _dep_u32([t[(q // 2) * QC:(q // 2 + 1) * QC, (q % 2) * T:(q % 2 + 1) * T]]))
            pres[r1, r2, ch] = jnp.dot(a, tinner[r1][r2], preferred_element_type=f32)
            if all((r1, q, ch) in pres for q in range(7)):
                m = {q: pres.pop((r1, q, ch)) for q in range(7)}
                mo[r1, ch] = _comb2(m) if dpi else _comb1(m)
                if fk:
                    if cfg.get('fsp', 0):
                        for b4 in range(4):
                            force.append([fk + b4, [mo[r1, ch][b4]]])
                    else:
                        force.append([fk, list(mo[r1, ch])])
                if (ch, 0) not in kblk and all((q, ch) in mo for q in (0, 1, 3, 4, 6)):
                    for b4 in range(4):
                        m = {q: mo[q, ch][b4] for q in (0, 1, 3, 4, 6)}
                        c11, c21, p22, p12 = _left2(m) if dpo else _left1(m)
                        kblk[ch, b4] = (scaled(c11, cs_in[b4]), scaled(c21, cs_in[b4] * cs_out[2]))
                        part[ch, b4] = (p12, p22)
                if all((q, ch) in mo for q in range(7)):
                    for b4 in range(4):
                        p12, p22 = part[ch, b4]
                        m2, m5 = mo[2, ch][b4], mo[5, ch][b4]
                        c12 = p12 + (m2 - m5) if dpo else p12 + m2
                        vblk[ch, b4] = (scaled(c12, cs_in[b4] * cs_out[1]), scaled(p22 + (m2 + m5), cs_in[b4]))

        def rows_of(blk, t0, t1):
            out = []
            for t in range(t0, t1):
                i, u = t // 4, t % 4
                ch, off = u * T // CR, u * T % CR
                out.append(jnp.concatenate([blk[ch, 2 * (i % 2) + j2][i // 2][off:off + T] for j2 in range(2)], axis=1))
            return out[0] if len(out) == 1 else jnp.concatenate(out, axis=0)

        def ktile(t):
            if t not in kv['k']:
                kv['k'][t] = rows_of(kblk, t, t + 1).astype(bf)
            return kv['k'][t]

        def kterms(J):
            if J not in kv['ks']:
                ka, kb = rows_of(kblk, 2 * J, 2 * J + 1), rows_of(kblk, 2 * J + 1, 2 * J + 2)
                kv['ks'][J] = [t.astype(bf) for t in _rhs_terms(ka[:, :T], kb[:, :T], ka[:, T:], kb[:, T:])]
            return kv['ks'][J]

        wo = wo_s[h]
        if cfg.get('so', 1):
            wof = wo.astype(f32)
            wos = [t.astype(bf) for t in _lhs_terms(wof[:HM, :T], wof[:HM, T:], wof[HM:, :T], wof[HM:, T:])]

        kv = dict(k={}, ks={}, v={})

        stile = {}
        sm = {}
        rmax = {}

        def qtiles(I):
            return [q_s[h, t, i * T:(i + 1) * T, :] for i in (2 * I, 2 * I + 1) for t in range(2)]

        def rpiece(I, J):
            q4 = qtiles(I)
            qx = [qa_s[h, k, I * T:(I + 1) * T, :] for k in range(5)]
            lhs = [qx[0], qx[1], q4[0], q4[3], qx[2], qx[3], qx[4]]
            cs = _strassen(lambda i: lax.dot_general(lhs[i], kterms(J)[i], NT, preferred_element_type=f32), cfg.get('sv', 0))
            if cfg.get('ss', 0):
                sl = I % 2
                for (u, v), c in zip(((0, 0), (0, 1), (1, 0), (1, 1)), cs):
                    s_s[sl, u, 2 * J + v] = c
                if cfg.get('ss', 0) == 1:
                    cs = [s_s[sl, u, 2 * J + v] for u in range(2) for v in range(2)]
                for (u, v) in ((0, 0), (0, 1), (1, 0), (1, 1)):
                    stile[2 * I + u, 2 * J + v] = s_s[sl, u, 2 * J + v]
            else:
                for (u, v), c in zip(((0, 0), (0, 1), (1, 0), (1, 1)), cs):
                    stile[2 * I + u, 2 * J + v] = c
            for u in range(2):
                mx = jnp.maximum(cs[2 * u], cs[2 * u + 1])
                rmax[2 * I + u] = mx if 2 * I + u not in rmax else jnp.maximum(rmax[2 * I + u], mx)

        def dpiece(I):
            a, b = 2 * I, 2 * I + 1
            q4 = qtiles(I)
            qa = jnp.concatenate(q4[0:2], axis=1)
            qb = jnp.concatenate(q4[2:4], axis=1)
            d1 = lax.dot_general(jnp.concatenate([qa, qb], axis=0), ktile(a), NT, preferred_element_type=f32)
            d2 = lax.dot_general(qb, ktile(b), NT, preferred_element_type=f32)
            stile[a, a] = jnp.where(tri, d1[:T], NEG)
            stile[b, a] = d1[T:]
            stile[b, b] = jnp.where(tri, d2, NEG)

        def pchunk(i, c):
            pc = cfg.get('pc', 2)
            if c == 0:
                I = i // 2
                mx = functools.reduce(jnp.maximum, ([rmax[i]] if I > 0 else []) + [stile[i, t] for t in range(2 * I, i + 1)])
                sm[i] = dict(m=jnp.max(mx, axis=1, keepdims=True), l=None, ctx=None)
            st_ = sm[i]
            c1 = min(c + pc, i + 1)
            pe = jnp.exp2(jnp.concatenate([stile.pop((i, t)) for t in range(c, c1)], axis=1) - st_['m'])
            pz = pe
            lf = cfg.get('lf', 0)
            hist = st_.setdefault('hist', [])
            if lf and len(hist) >= lf:
                z = _dep_u32([hist[-lf]])
                top = pltpu.bitcast(pltpu.bitcast(pe[0:8, :T], u32) | z, f32)
                if pe.shape[1] > T:
                    top = jnp.concatenate([top, pe[0:8, T:]], axis=1)
                pz = jnp.concatenate([top, pe[8:]], axis=0)
            pb = pz.astype(bf)
            pf = pb.astype(f32) if cfg.get('lbf', 1) else pe
            for t in range(c1 - c):
                st_['l'] = pf[:, t * T:(t + 1) * T] if st_['l'] is None else st_['l'] + pf[:, t * T:(t + 1) * T]
            hist.append(st_['l'])
            if (c, c1) not in kv['v']:
                kv['v'][c, c1] = rows_of(vblk, c, c1).astype(bf)
            d = jnp.dot(pb, kv['v'][c, c1], preferred_element_type=f32)
            st_['ctx'] = d if st_['ctx'] is None else st_['ctx'] + d

        def ctx_of(i):
            st_ = sm.pop(i)
            l = jnp.sum(st_['l'], axis=1, keepdims=True)
            r0 = pl.reciprocal(l, approx=True)
            return st_['ctx'] * (r0 * (2.0 - l * r0))

        odone = set()

        def accum(i, a0, d):
            a1 = a0 + d.shape[0]
            a = acc_s[i, a0:a1, :] + g_s[i][1:2, :] * d
            acc_s[i, a0:a1, :] = a
            out_s[a0:a1, i * T:(i + 1) * T] = a.astype(bf)

        def fin(blocks):
            odone.update(blocks)
            b = blocks[0] * T // OW
            if all(bb in odone for bb in range(b * OW // T, (b + 1) * OW // T)):
                @pl.when(h == H - 1)
                def _():
                    cp_out(b).start()

        def oproj2(i, ca, cb):
            if cfg.get('so', 1):
                ts = _rhs_terms(ca[:, :T], cb[:, :T], ca[:, T:], cb[:, T:])
                c11, c12, c21, c22 = _strassen(
                    lambda k: lax.dot_general(wos[k], ts[k].astype(bf), NT, preferred_element_type=f32))
                accum(i, 0, c11); accum(i + 1, 0, c12); accum(i, HM, c21); accum(i + 1, HM, c22)
            else:
                d = lax.dot_general(wo, jnp.concatenate([ca, cb], axis=0).astype(bf), NT, preferred_element_type=f32)
                accum(i, 0, d[:, :T]); accum(i + 1, 0, d[:, T:])
            fin([i, i + 1])

        def oprojs(i, ctx):
            cb = ctx.astype(bf)
            for a0 in (0, HM):
                accum(i, a0, lax.dot_general(wo[a0:a0 + HM], cb, NT, preferred_element_type=f32))
            fin([i])

        for op, i, c in prog:
            if op == 'r':
                rpiece(i, c)
            elif op == 'd':
                dpiece(i)
            elif op == 'm':
                pmm(*i)
            elif op == 'p':
                pchunk(i, c)
            elif op == 'D':
                oproj2(i, ctx_of(i), ctx_of(i + 1))
            elif op == 'S':
                oprojs(i, ctx_of(i))
        return carry

    lax.fori_loop(0, H, head, 0)
    for b in range(S // OW):
        cp_out(b).wait()


def make(**cfg):
    name = ("k19_" + "_".join([f"{k}{v}" for k, v in sorted(cfg.items())])).replace(" ", "").replace("(", "").replace(")", "").replace(",", "x")

    @jax.jit
    def f(A_x, A_c_kv, A_w_q, A_w_uk, A_w_uv, A_w_o, B_x, B_w_r, B_w_gate, B_w_up, B_w_down, gate_w):
        xt = A_x[0].T
        c = A_c_kv[0]
        woT = A_w_o.transpose(0, 2, 1)
        wdT = B_w_down.T
        V = pltpu.VMEM
        outT = pl.pallas_call(
            functools.partial(kernel, cfg=cfg),
            in_specs=[pl.BlockSpec(memory_space=pl.ANY)] * 11,
            out_specs=pl.BlockSpec(memory_space=pl.ANY),
            out_shape=jax.ShapeDtypeStruct((M, S), bf),
            scratch_shapes=[
                V((M, S), bf), V((2, S, HM), bf), V((7, HS, HM), bf), V((S, DC), bf), V((49, S // 8, DC // 4), u32),
                V((NP, M, D), u32), V((2, 2, DC, D), u32), V((H, M, D), bf),
                V((H, 2, S, T), bf), V((H, 5, HS, T), bf), V((NQ, M, T), f32),
                V((M, F), bf), V((M, F), bf), V((M, F), bf),
                V((M,), bf), V((M,), bf), V((M, S), bf),
                V((NQ, 8, T), f32), V((2, 16, HM), bf), V((16, T), f32), pltpu.SMEM((2,), jnp.int32), V((2, 2, NQ, T, T), f32),
                pltpu.SemaphoreType.DMA((NSEM,)),
            ],
            compiler_params=pltpu.CompilerParams(vmem_limit_bytes=110 * 1024 * 1024),
            name=name,
        )(xt, c, A_w_q, A_w_uk, A_w_uv, woT, B_w_r, B_w_gate, B_w_up, wdT, gate_w)
        return outT.T[None]
    return f


_impl = make(**{'so': 0, 'sv': 1, 'rf': 0.9, 'ss': 1, 'nch': 1, 'dpo': 1, 'dpi': 0, 'nv': 8})


@jax.jit
def pallas_gated_mix__compressed_kv_cla__moe_arch_mod__prompt_kernel(
    A_x: jax.Array,
    A_c_kv: jax.Array,
    A_w_q: jax.Array,
    A_w_uk: jax.Array,
    A_w_uv: jax.Array,
    A_w_o: jax.Array,
    B_x: jax.Array,
    B_w_r: jax.Array,
    B_w_gate: jax.Array,
    B_w_up: jax.Array,
    B_w_down: jax.Array,
    gate_w: jax.Array,
):
    return _impl(A_x, A_c_kv, A_w_q, A_w_uk, A_w_uv, A_w_o, B_x, B_w_r, B_w_gate, B_w_up, B_w_down, gate_w)
```

```python
import functools, math
import jax, jax.numpy as jnp
from jax import lax
from jax.experimental import pallas as pl
from jax.experimental.pallas import tpu as pltpu

S, M, H, D, DC, F = 2048, 448, 16, 256, 1024, 1792
NP = H // 2
HS, HC, HM = S // 2, DC // 2, M // 2
T = 128
NQ = S // T
NT = (((1,), (1,)), ((), ()))
QSCALE = D ** -0.5 * math.log2(math.e)
bf = jnp.bfloat16
f32 = jnp.float32
u32 = jnp.uint32
NEG = -1e30

SEM_WO, SEM_FFN, SEM_VEC, SEM_KV, SEM_WQ, SEM_OUT, SEM_XT, SEM_C = 2, 3, 6, 8, 12, 20, 28, 36
NSEM = 44

PROGS = {
    10: "R0 R7 V R6 P0 P1 P15 P14 D0 R5 P13 P12 D14 R4 P11 P10 D12 R3 P9 P8 D10 R2 P7 P6 D8 R1 P5 P4 D6 P3 P2 D4 S3 S2",
    11: "R0 R7 V R6 P0 P1 P15 P14 R5 D0 P13 P12 R4 D14 P11 P10 R3 D12 P9 P8 R2 D10 P7 P6 R1 D8 P5 P4 D6 P3 P2 D4 S3 S2",
    12: "R0 R7 V R6 P0 P1 P14 P15 D0 R5 P12 P13 D14 R4 P10 P11 D12 R3 P8 P9 D10 R2 P6 P7 D8 R1 P4 P5 D6 P2 P3 D4 S2 S3",
    2: "Q0 Q1 Q15 V Q14 P0 P1 P15 Q13 P14 D0 Q12 P13 Q11 P12 D14 Q10 P11 Q9 P10 D12 Q8 P9 Q7 P8 D10 Q6 P7 Q5 P6 D8 Q4 P5 Q3 P4 Q2 P3 D6 P2 D4 S3 S2",
    4: "Q0 Q1 Q15 V Q14 P0 P1 P15 Q13 P14 D0 Q12 P13 Q11 P12 D14 Q10 P11 Q9 P10 D12 Q8 P9 Q7 P8 D10 Q6 P7 Q5 P6 D8 Q4 P5 Q3 P4 Q2 P3 D6 P2 D4 D2",
}


def _merge(a, b):
    out, i, j = [], 0, 0
    while i < len(a) or j < len(b):
        if j >= len(b) or (i < len(a) and i * len(b) <= j * len(a)):
            out.append(a[i]); i += 1
        else:
            out.append(b[j]); j += 1
    return out


def fine_prog(cfg):
    pc = cfg.get('pc', 2)
    if cfg.get('dfirst', 0):
        R = lambda I: [('d', I, 0)] + [('r', I, J) for J in range(I)]
    else:
        R = lambda I: [('r', I, J) for J in range(I)] + [('d', I, 0)]
    P1 = lambda i: [('p', i, c) for c in range(0, i + 1, pc)]
    if cfg.get('pab', 0):
        P = lambda I: _merge(P1(2 * I + 1), P1(2 * I))
    else:
        P = (lambda I: P1(2 * I + 1) + P1(2 * I)) if cfg.get('bfirst', 0) else (lambda I: P1(2 * I) + P1(2 * I + 1))
    nch = cfg.get('nch', 2)
    io = (1, 3, 4, 6, 0, 2, 5)
    MM = lambda r1s, ch: [('m', (r1, r2, ch), 0) for r1 in r1s for r2 in io]
    K5, V2 = (1, 3, 4, 6, 0), (2, 5)
    r7 = lambda js: [('r', 7, J) for J in js]
    if nch == 1:
        V = MM(V2, 0)
        nv = cfg.get('nv', 10)
        prog = MM(K5, 0) + V[:1] + _merge(R(0) + R(7), V[1:nv]) + V[nv:]
    else:
        h_ = nch // 2
        KA = sum([MM(K5, ch) for ch in range(h_)], [])
        KB = sum([MM(K5, ch) for ch in range(h_, nch)], [])
        VA = sum([MM(V2, ch) for ch in range(h_)], [])
        VB = sum([MM(V2, ch) for ch in range(h_, nch)], [])
        k0 = int(len(KB) * cfg.get('k0', 0.2))
        v0 = int(len(VA) * cfg.get('v0', 0.2))
        prog = (KA + KB[:k0] + _merge([('d', 0, 0)] + r7((0, 2, 4, 6)), KB[k0:]) + VA[:v0]
                + _merge(r7((1, 3, 5)) + [('d', 7, 0)], VA[v0:]) + VB)
    order = [7, 6, 5, 4, 3, 2, 1]
    pend = [0]
    for n, I in enumerate(order):
        ps = P(I)
        if n == 0:
            ps = P(0) + ps
        nxt = R(order[n + 1]) if n + 1 < len(order) else []
        k = max(1, int(round(len(ps) * cfg.get('rf', 1.0))))
        body = _merge(nxt, ps[:k]) + ps[k:]
        dpos = cfg.get('dpos', 0.9)
        if n > 0:
            k = int(len(body) * dpos)
            body = body[:k] + [('D', 2 * pend.pop(0), 0)] + body[k:]
        prog += body
        pend.append(I)
    last = pend.pop()
    prog += [('D', 2 * I, 0) for I in pend]
    prog += [('S', 2 * last + 1, 0), ('S', 2 * last, 0)] if cfg.get('bfirst', 0) else [('S', 2 * last, 0), ('S', 2 * last + 1, 0)]
    return prog


def _lo32(x):
    return pltpu.bitcast(x << 16, f32)


def _hi32(x):
    return pltpu.bitcast(x & jnp.uint32(0xFFFF0000), f32)


def _lhs_terms(a11, a12, a21, a22):
    return [a11 + a22, a21 + a22, a11, a22, a11 + a12, a21 - a11, a12 - a22]


def _rhs_terms(b11, b12, b21, b22):
    return [b11 + b22, b11, b12 - b22, b21 - b11, b22, b11 + b12, b21 + b22]


def _strassen(mm, var=0):
    if var == 0:
        m1 = mm(0); m4 = mm(3); m5 = mm(4); m7 = mm(6); m3 = mm(2); m2 = mm(1); m6 = mm(5)
        return m1 + m4 - m5 + m7, m3 + m5, m2 + m4, m1 + m3 - m2 + m6
    if var == 1:
        m2 = mm(1); m3 = mm(2); m4 = mm(3); m5 = mm(4); m1 = mm(0); m7 = mm(6); m6 = mm(5)
        return (m4 - m5) + (m1 + m7), m3 + m5, m2 + m4, (m3 - m2) + (m1 + m6)


def _lhs_terms2(a11, a12, a21, a22):
    h21 = 0.5 * a21
    q21 = 0.25 * a21
    h22 = 0.5 * a22
    s1 = a11 + a22
    v = a12 + q21
    hs = 0.5 * s1
    return [s1, q21 + h22, a11 + h21, h22 - q21, v + hs, h21 - a11, v - hs]


def _rhs_terms2(b11, b12, b21, b22):
    h21 = 0.5 * b21
    t1 = b11 + b22
    v = b12 + 0.5 * h21
    ht = 0.5 * t1
    return [t1, b11 + h21, v - ht, h21 - b11, b22 - h21, v + ht, b22 + h21]


def _left2(m):
    s = m[3] + m[1]
    t = m[0] + (m[3] - m[1])
    return t + (m[6] - m[4]), s, t, s + (m[6] + m[4])


def _comb2(m):
    c11, s, t, se = _left2(m)
    return c11, se + (m[2] - m[5]), s, t + (m[2] + m[5])


def _left1(m):
    return (m[3] - m[4]) + (m[0] + m[6]), m[1] + m[3], m[0] - m[1], m[4]


def _comb1(m):
    return (m[3] - m[4]) + (m[0] + m[6]), m[2] + m[4], m[1] + m[3], (m[2] - m[1]) + (m[0] + m[5])


def _zero_like_dep(v):
    return (pltpu.bitcast(v[0:8, 0:128], u32) >> 16) >> 16


def _dep_u32(vals):
    ts = []
    for v in vals:
        v = pltpu.bitcast(v, u32) if v.dtype != u32 else v
        r, c = v.shape
        for r0 in range(0, r, 8):
            for c0 in range(0, c - T + 1, T):
                ts.append(v[r0:r0 + 8, c0:c0 + T])
    W = 4
    acc = ts[:W]
    for i, t in enumerate(ts[W:]):
        acc[i % W] = acc[i % W] | t
    while len(acc) > 1:
        acc = [acc[i] | acc[i + 1] if i + 1 < len(acc) else acc[i] for i in range(0, len(acc), 2)]
    return (acc[0] >> 16) >> 16


def _feed(a, z):
    if z is None:
        return a
    a32 = pltpu.bitcast(a, u32)
    top = a32[0:8, :T] | z
    if a32.shape[1] > T:
        top = jnp.concatenate([top, a32[0:8, T:]], axis=1)
    return pltpu.bitcast(jnp.concatenate([top, a32[8:]], axis=0), bf)


def _vregs(vals):
    ts = []
    for v in vals:
        v = pltpu.bitcast(v, u32) if v.dtype != u32 else v
        r, c = v.shape
        for r0 in range(0, r, 8):
            for c0 in range(0, c - T + 1, T):
                ts.append(v[r0:r0 + 8, c0:c0 + T])
    return ts


class _Pacer:
    def __init__(self, thunks, per, first, last):
        self.thunks, self.pool, self.k = list(thunks), [], 0
        self.tot, self.first, self.last, self.done = per * len(self.thunks), first, last, 0

    def __call__(self):
        k = self.k
        self.k += 1
        if k < self.first:
            return None
        goal = min(self.tot, -(-(k + 1 - self.first) * self.tot // (self.last - self.first)))
        want = goal - self.done
        while len(self.pool) < want and self.thunks:
            self.pool.extend(_vregs(self.thunks.pop(0)()))
        outs, self.pool = self.pool[:want], self.pool[want:]
        self.done += len(outs)
        return _dep_u32(outs) if outs else None

    def finished(self):
        return not self.thunks and not self.pool


class _Feeder:
    def __init__(self):
        self.q, self.k = [], 0

    def add(self, vals, lag):
        self.q += [(self.k + lag, t) for t in _vregs(vals)]

    def __call__(self, rate):
        self.k += 1
        n = 0
        while n < min(rate, len(self.q)) and self.q[n][0] <= self.k:
            n += 1
        outs, self.q = [t for _, t in self.q[:n]], self.q[n:]
        return _dep_u32(outs) if outs else None


def _or(*zs):
    zs = [z for z in zs if z is not None]
    return functools.reduce(lambda a, b: a | b, zs) if zs else None


def kernel(xt_hbm, c_hbm, wq_hbm, wk_hbm, wv_hbm, wo_hbm, wr_hbm, wg_hbm, wu_hbm, wd_hbm, gw_hbm,
           o_hbm,
           xt_s, x_s, xa_s, c_s, sa_s, wq_p, wkv_p, wo_s, q_s, qa_s, acc_s, wg_s, wu_s, wd_s,
           wr_s, gw_s, out_s, g_s, xs_s, rsel_s, idx_s, s_s, sem, *, cfg):
    mk = pltpu.make_async_copy
    wq32 = wq_hbm.bitcast(u32)
    wk32 = wk_hbm.bitcast(u32)
    wv32 = wv_hbm.bitcast(u32)
    cp_wq = lambda j: mk(wq32.at[:, j, :], wq_p.at[j], sem.at[SEM_WQ + j])
    cp_wr = mk(wr_hbm, wr_s, sem.at[SEM_VEC])
    cp_gw = mk(gw_hbm, gw_s, sem.at[SEM_VEC + 1])

    def cp_kv(j):
        slot = j % 2
        return [mk(wk32.at[:, j, :], wkv_p.at[slot, 0], sem.at[SEM_KV + 2 * slot]),
                mk(wv32.at[:, j, :], wkv_p.at[slot, 1], sem.at[SEM_KV + 2 * slot + 1])]
    QS, QC = S // 4, DC // 4
    RB = 16
    NG = cfg.get('ng', 5)
    CRW = NG * RB

    def cp_c(j):
        r0 = (j - 1) * CRW
        n = CRW if not isinstance(j, int) or j < NP - 1 else QS - r0
        return [mk(c_hbm.at[pl.ds(i * QS + r0, n)], c_s.at[pl.ds(i * QS + r0, n)], sem.at[SEM_C + j]) for i in range(4)]
    cp_wo = mk(wo_hbm, wo_s, sem.at[SEM_WO])
    cp_ffn = [mk(wg_hbm, wg_s, sem.at[SEM_FFN]), mk(wu_hbm, wu_s, sem.at[SEM_FFN + 1]), mk(wd_hbm, wd_s, sem.at[SEM_FFN + 2])]
    OW = 256
    cp_out = lambda b: mk(out_s.at[:, pl.ds(b * OW, OW)], o_hbm.at[:, pl.ds(b * OW, OW)], sem.at[SEM_OUT + b])
    XC = 256
    NXC = S // XC
    cp_xtc = lambda k: mk(xt_hbm.at[:, pl.ds(k * XC, XC)], xt_s.at[:, pl.ds(k * XC, XC)], sem.at[SEM_XT + k])

    cp_wq(0).start()
    for k in range(NXC):
        cp_xtc(k).start()
    cp_wr.start()
    cp_gw.start()
    for j in range(1, NP):
        cp_wq(j).start()
        for cp in cp_c(j):
            cp.start()
    for cp in cp_ffn:
        cp.start()
    for cp in cp_kv(0):
        cp.start()
    cp_wo.start()

    sq = cfg.get('sq', 1)
    sqk = cfg.get('sqk', 1)

    def store_q(j, e, r0, q):
        qs = q * QSCALE
        for t in range(2):
            q_s[2 * j + e, t, r0:r0 + q.shape[0], :] = qs[:, t * T:(t + 1) * T].astype(bf)
        if sqk:
            for p0 in range(0, q.shape[0], 2 * T):
                if r0 + p0 == 0:
                    continue
                qa, qc = qs[p0:p0 + T], qs[p0 + T:p0 + 2 * T]
                k = 0
                for i, v in enumerate(_lhs_terms(qa[:, :T], qa[:, T:], qc[:, :T], qc[:, T:])):
                    if i not in (2, 3):
                        qa_s[2 * j + e, k, (r0 + p0) // 2:(r0 + p0) // 2 + T, :] = v.astype(bf)
                        k += 1

    def qplain(j, w, r0, r1, n0, n1, z=None):
        wn = w[:, n0 * T:n1 * T]
        qf = (jnp.dot(_feed(x_s[0, r0:r1, :], z), wn[:HM], preferred_element_type=f32)
              + jnp.dot(x_s[1, r0:r1, :], wn[HM:], preferred_element_type=f32))
        return qf

    def qplain_blk(j, w, r0, small=None):
        if small is None:
            qf = qplain(j, w, r0, r0 + 2 * T, 0, 4)
        else:
            cols = []
            for n in range(4):
                cols.append(jnp.concatenate([qplain(j, w, r0 + u * T, r0 + (u + 1) * T, n, n + 1, small()) for u in range(2)], axis=0))
            qf = jnp.concatenate(cols, axis=1)
        store_q(j, 0, r0, qf[:, :D]); store_q(j, 1, r0, qf[:, D:])

    def qw(j):
        w32 = wq_p[j]
        return jnp.concatenate([_lo32(w32).astype(bf), _hi32(w32).astype(bf)], axis=1)

    def q_rhs(j):
        w32 = wq_p[j]
        lo, hi = _lo32(w32), _hi32(w32)
        return [t.astype(bf) for t in _rhs_terms(lo[:HM], hi[:HM], lo[HM:], hi[HM:])]

    def q_lhs(i, r0, r1):
        if i == 2:
            return x_s[0, r0:r1, :]
        if i == 3:
            return x_s[1, HS + r0:HS + r1, :]
        return xa_s[i, r0:r1, :]

    def qstr(j, ts, r0, r1, pre=None, step=T):
        def mm(i):
            if pre is None:
                return jnp.dot(q_lhs(i, r0, r1), ts[i], preferred_element_type=f32)
            return jnp.concatenate([jnp.dot(_feed(q_lhs(i, u, u + step), pre()), ts[i], preferred_element_type=f32)
                                    for u in range(r0, r1, step)], axis=0)
        c11, c12, c21, c22 = _strassen(mm)
        store_q(j, 0, r0, c11); store_q(j, 1, r0, c12); store_q(j, 0, HS + r0, c21); store_q(j, 1, HS + r0, c22)

    def xprep(r0):
        a = [x_s[e, h0 + r0:h0 + r0 + RB, :].astype(f32) for h0 in (0, HS) for e in (0, 1)]
        outs = []
        for i, v in enumerate(_lhs_terms(*a)):
            if i not in (2, 3):
                vb = v.astype(bf)
                xa_s[i, r0:r0 + RB, :] = vb
                outs.append(pltpu.bitcast(vb, u32))
        return outs

    row8 = lax.broadcasted_iota(jnp.int32, (8, M), 0)

    def tr(k):
        for e in range(2):
            x_s[e, k * XC:(k + 1) * XC, :] = xt_s[e * HM:(e + 1) * HM, k * XC:(k + 1) * XC].T

    def route(n):
        lhs = jnp.where(row8 == 0, wr_s[...].reshape(1, M).astype(f32), gw_s[...].reshape(1, M).astype(f32)).astype(bf)
        g_s[n] = jnp.dot(lhs, xt_s[:, n * T:(n + 1) * T], preferred_element_type=f32)

    segs = cfg.get('segs', (2, 4, 8))
    cp_wq(0).wait()
    tdone = qdone = rdone = 0
    xdone = 0
    nsmall = (segs[-1] - segs[-2] + 1) * 8
    ksm = 0
    st = dict(r=0)
    xp = _Pacer([functools.partial(xprep, r0) for r0 in range(0, HS, RB)], 5, cfg.get('x0', 12), nsmall)

    def small0():
        if st['r'] < NQ:
            route(st['r']); st['r'] += 1
        return xp()
    for si, e in enumerate(segs):
        for k in range(tdone, e):
            cp_xtc(k).wait()
        last = si == len(segs) - 1
        if last:
            cp_wr.wait()
            cp_gw.wait()
            while tdone < e:
                tr(tdone); tdone += 1
        w = qw(0)
        qe = e if last else e - 1
        while tdone < e or qdone < qe:
            if tdone < e:
                tr(tdone); tdone += 1
            if qdone < min(qe, tdone - (1 if tdone < e or si == 0 else 0)) or (tdone == e and qdone < qe):
                qplain_blk(0, w, qdone * XC, small0 if last else None)
                qdone += 1
    assert xp.finished()

    r_all = jnp.concatenate([g_s[n][0:1, :] for n in range(NQ)], axis=1)
    rb = r_all.astype(bf).astype(f32)
    lane = lax.broadcasted_iota(jnp.int32, (1, S), 1)
    m1 = jnp.max(rb, axis=1, keepdims=True)
    i1 = jnp.minimum(jnp.min(jnp.where(rb == m1, lane, S)), S - 1)
    rb2 = jnp.where(lane == i1, -jnp.inf, rb)
    m2 = jnp.max(rb2, axis=1, keepdims=True)
    i2 = jnp.minimum(jnp.min(jnp.where(jnp.logical_and(rb2 == m2, lane != i1), lane, S)), S - 1)
    row16 = lax.broadcasted_iota(jnp.int32, (16, HM), 0)

    def xrow(e, i):
        blk = x_s[e, pl.ds(pl.multiple_of((i // 16) * 16, 16), 16), :].astype(f32)
        return jnp.sum(jnp.where(row16 == i % 16, blk, 0.0), axis=0, keepdims=True)
    for e in range(2):
        xs_s[e] = jnp.where(row16 == 0, xrow(e, i1), jnp.where(row16 == 1, xrow(e, i2), 0.0)).astype(bf)
    rcol = lax.broadcasted_iota(jnp.int32, (16, T), 0)
    rsel_s[...] = jax.nn.sigmoid(jnp.where(rcol == 0, m1, m2))
    idx_s[0] = i1
    idx_s[1] = i2

    dps = cfg.get('dps', 1)
    dpo, dpi = cfg.get('dpo', dps), cfg.get('dpi', dps)
    lo_, li_ = (_lhs_terms2 if dpo else _lhs_terms), (_lhs_terms2 if dpi else _lhs_terms)

    def cprep(g, c0):
        if isinstance(g, int):
            rows = lambda i: pl.ds(i * QS + g * RB, RB)
            orow = pl.ds(g * RB // 2, RB // 2)
        else:
            rows = lambda i: pl.ds(pl.multiple_of(i * QS + g * RB, RB), RB)
            orow = pl.ds(pl.multiple_of(g * (RB // 2), RB // 2), RB // 2)
        blk = lambda i, k: c_s[rows(i), k * QC + c0:k * QC + c0 + T].astype(f32)
        inner = [[[blk(2 * i1 + i2, 2 * k1 + k2) for i1 in range(2) for k1 in range(2)] for k2 in range(2)] for i2 in range(2)]
        outer = [[lo_(*inner[i2][k2]) for k2 in range(2)] for i2 in range(2)]
        outs = []
        for r1 in range(7):
            for r2, v in enumerate(li_(outer[0][0][r1], outer[0][1][r1], outer[1][0][r1], outer[1][1][r1])):
                o = pltpu.bitcast(v.astype(bf), u32)
                sa_s[7 * r1 + r2, orow, c0:c0 + T] = o
                outs.append(o)
        return outs

    def qbody(j, carry):
        cp_wq(j).wait()
        for cp in cp_c(j):
            cp.wait()
        QR = cfg.get('qr', 128)
        cpz = _Pacer([functools.partial(cprep, (j - 1) * NG + t // 2, (t % 2) * T) for t in range(2 * NG)], 49,
                     cfg.get('l0', 1), 7 * HS // QR)
        qstr(j, q_rhs(j), 0, HS, cpz, QR)
        assert cpz.finished()
        return carry
    lax.fori_loop(1, NP - 1, qbody, 0)

    for cp in cp_ffn:
        cp.wait()
    cp_wq(NP - 1).wait()
    for cp in cp_c(NP - 1):
        cp.wait()

    def binit(n):
        g8 = jax.nn.sigmoid(g_s[n])
        g_s[n] = g8
        a = (1.0 - g8[1:2, :]) * xt_s[:, n * T:(n + 1) * T].astype(f32)
        acc_s[n] = a
        return [a]

    ggs, uus, ys, hh = [], [], {}, []
    sops = []

    def xdot(w_s, n):
        return (jnp.dot(xs_s[0], w_s[:HM, n * T:(n + 1) * T], preferred_element_type=f32)
                + jnp.dot(xs_s[1], w_s[HM:, n * T:(n + 1) * T], preferred_element_type=f32))
    for n in range(F // T):
        sops.append(lambda n=n: ggs.append(xdot(wg_s, n)))
        sops.append(lambda n=n: uus.append(xdot(wu_s, n)))

    def act():
        gg = jnp.concatenate(ggs, axis=1)
        uu = jnp.concatenate(uus, axis=1)
        hh.append((gg * jax.nn.sigmoid(gg) * uu).astype(bf))
    sops += [act] + [lambda: None] * 3
    for n0 in range(0, M, T):
        for k0 in range(0, F, 512):
            def f(n0=n0, k0=k0):
                k1, n1 = min(k0 + 512, F), min(n0 + T, M)
                t = lax.dot_general(hh[0][:, k0:k1], wd_s[n0:n1, k0:k1], NT, preferred_element_type=f32)
                ys[n0] = t if n0 not in ys else ys[n0] + t
            sops.append(f)
    ndots = 56
    nrest = 2 * (QS // RB - (NP - 2) * NG)
    cp7 = _Pacer([functools.partial(cprep, (NP - 2) * NG + t // 2, (t % 2) * T) for t in range(nrest)], 49, cfg.get('c0', 2), ndots)
    bp7 = _Pacer([functools.partial(binit, n) for n in range(NQ)], M // 8, 1, ndots - cfg.get('b1', 4))

    def pre():
        if sops:
            sops.pop(0)()
        return _or(cp7(), bp7())
    if sq:
        ts = q_rhs(NP - 1)
        for r0 in range(0, HS, 2 * T):
            qstr(NP - 1, ts, r0, r0 + 2 * T, pre)
    assert not sops and cp7.finished() and bp7.finished()
    y = jnp.concatenate([ys[n0] for n0 in range(0, M, T)] + [jnp.zeros((16, 512 - M), f32)], axis=1) * rsel_s[:, 0:1]
    yT = y.T
    lane128 = lax.broadcasted_iota(jnp.int32, (1, T), 1)
    for e in range(2):
        i = idx_s[e]
        t = i // T
        acc_s[t] += jnp.where(lane128 == i % T, (1.0 - g_s[t][1:2, :]) * yT[:M, e:e + 1], 0.0)

    cp_wo.wait()

    tri = lax.broadcasted_iota(jnp.int32, (T, T), 1) <= lax.broadcasted_iota(jnp.int32, (T, T), 0)
    prog = fine_prog(cfg)

    def head(h, carry):
        j = h // 2
        slot = j % 2

        @pl.when(h % 2 == 0)
        def _():
            for cp in cp_kv(j):
                cp.wait()

            @pl.when(j + 1 < NP)
            def _():
                for cp in cp_kv(j + 1):
                    cp.start()

        sh = (16 * (1 - h % 2)).astype(u32)

        wf = [pltpu.bitcast((wkv_p[slot, m] << sh) & jnp.uint32(0xFFFF0000), f32) for m in range(2)]
        ro_, ri_ = (_rhs_terms2 if dpo else _rhs_terms), (_rhs_terms2 if dpi else _rhs_terms)
        if dps and cfg.get('bb', 0):
            BR = cfg.get('br', 16)
            cols = {}
            for r0 in range(0, QC, BR):
                b = {(k, jj): wf[jj // 2][k * QC + r0:k * QC + r0 + BR, (jj % 2) * T:(jj % 2 + 1) * T]
                     for k in range(4) for jj in range(4)}
                for st in (2, 1):
                    for k in range(4):
                        for jj in range(4):
                            if not k & st:
                                b[k, jj] = b[k, jj] + 0.5 * b[k + st, jj]
                    for k in range(4):
                        for jj in range(4):
                            if jj & st:
                                b[k, jj] = b[k, jj] - 0.5 * b[k, jj - st]
                for key, v in b.items():
                    cols.setdefault(key, []).append(v)
            bp = {key: jnp.concatenate(v, axis=0) for key, v in cols.items()}
            tq = [[_rhs_terms(bp[k2, j2], bp[k2, 2 + j2], bp[2 + k2, j2], bp[2 + k2, 2 + j2]) for j2 in range(2)] for k2 in range(2)]
            tinner = [[u.astype(bf) for u in _rhs_terms(tq[0][0][r1], tq[0][1][r1], tq[1][0][r1], tq[1][1][r1])] for r1 in range(7)]
            touter = None
        else:
            touter = ro_(wf[0][:HC], wf[1][:HC], wf[0][HC:], wf[1][HC:])
            tinner = [[u.astype(bf) for u in ri_(t[:QC, :T], t[:QC, T:], t[QC:, :T], t[QC:, T:])] for t in touter]
        CR = QS
        pres, mo, kblk, vblk, acc_o = {}, {}, {}, {}, {}
        fd = _Feeder()
        plag, prate, PR = cfg.get('plag', 6), cfg.get('prate', 0), cfg.get('pr', 128)
        SEQ = (1, 3, 4, 6, 0, 2, 5)

        def pmm(r1, r2, ch):
            res = []
            for u in range(0, QS, PR):
                a = pltpu.bitcast(sa_s[7 * r1 + r2, u // 2:(u + PR) // 2, :], bf)
                res.append(jnp.dot(_feed(a, fd(prate) if prate else None), tinner[r1][r2], preferred_element_type=f32))
            m = pres.setdefault(r1, {})
            m[r2] = jnp.concatenate(res, axis=0)
            new = []
            if r2 == 3:
                m['c21'] = m[1] + m[3]; new = ['c21']
            elif r2 == 6:
                m['a'] = (m[3] - m[4]) + m[6]; new = ['a']
            elif r2 == 2:
                m['c11'] = m['a'] + m[0]; m['c12'] = m[2] + m[4]; m['b'] = (m[0] - m[1]) + m[2]; new = ['c11', 'c12', 'b']
            elif r2 == 5:
                m['c22'] = m['b'] + m[5]; new = ['c22']
            for key in new:
                if key[0] != 'c':
                    if cfg.get('fab', 1):
                        fd.add([m[key]], plag)
                    continue
                b4 = ('c11', 'c12', 'c21', 'c22').index(key)
                o, A = m[key], acc_o.setdefault(b4, {})
                if r1 == 1:
                    A['o2'] = o; out = [o]
                elif r1 == 3:
                    A['s'] = o + A['o2']; A['d'] = o - A['o2']
                    A['k1'] = A['s'] * 2.0; out = [A['k1'], A['d']]
                elif r1 == 4:
                    A['f'] = A['d'] - o; A['e'] = A['s'] + o; out = [A['f'], A['e']]
                elif r1 == 6:
                    A['f'] = A['f'] + o; A['e'] = A['e'] + o; out = [A['f'], A['e']]
                elif r1 == 0:
                    kblk[0, b4] = (o + A['f'], A['k1']); A['t'] = o + A['d']; out = [kblk[0, b4][0], A['t']]
                elif r1 == 2:
                    A['e'] = A['e'] + o; A['t'] = A['t'] + o; out = [A['e'], A['t']]
                else:
                    vblk[0, b4] = ((A['e'] - o) * 0.5, A['t'] + o); out = list(vblk[0, b4])
                fd.add(out, plag)
            if cfg.get('fb', 0) and r2 == SEQ[cfg['fb'] - 1] and r1 != 5:
                fd.add([touter[SEQ[SEQ.index(r1) + 1]]], 0)

        def rows_of(blk, t0, t1):
            out = []
            for t in range(t0, t1):
                i, u = t // 4, t % 4
                ch, off = u * T // CR, u * T % CR
                out.append(jnp.concatenate([blk[ch, 2 * (i % 2) + j2][i // 2][off:off + T] for j2 in range(2)], axis=1))
            return out[0] if len(out) == 1 else jnp.concatenate(out, axis=0)

        def ktile(t):
            if t not in kv['k']:
                kv['k'][t] = rows_of(kblk, t, t + 1).astype(bf)
            return kv['k'][t]

        def kterms(J):
            if J not in kv['ks']:
                ka, kb = rows_of(kblk, 2 * J, 2 * J + 1), rows_of(kblk, 2 * J + 1, 2 * J + 2)
                kv['ks'][J] = [t.astype(bf) for t in _rhs_terms(ka[:, :T], kb[:, :T], ka[:, T:], kb[:, T:])]
            return kv['ks'][J]

        wo = wo_s[h]
        if cfg.get('so', 1):
            wof = wo.astype(f32)
            wos = [t.astype(bf) for t in _lhs_terms(wof[:HM, :T], wof[:HM, T:], wof[HM:, :T], wof[HM:, T:])]

        kv = dict(k={}, ks={}, v={})

        stile = {}
        sm = {}
        rmax = {}

        def qtiles(I):
            return [q_s[h, t, i * T:(i + 1) * T, :] for i in (2 * I, 2 * I + 1) for t in range(2)]

        def rpiece(I, J):
            q4 = qtiles(I)
            qx = [qa_s[h, k, I * T:(I + 1) * T, :] for k in range(5)]
            lhs = [qx[0], qx[1], q4[0], q4[3], qx[2], qx[3], qx[4]]
            rrate = cfg.get('rrate', 0)
            cs = _strassen(lambda i: lax.dot_general(_feed(lhs[i], fd(rrate) if rrate else None), kterms(J)[i], NT,
                                                     preferred_element_type=f32), cfg.get('sv', 0))
            if cfg.get('ss', 0):
                sl = I % 2
                for (u, v), c in zip(((0, 0), (0, 1), (1, 0), (1, 1)), cs):
                    s_s[sl, u, 2 * J + v] = c
                if cfg.get('ss', 0) == 1:
                    cs = [s_s[sl, u, 2 * J + v] for u in range(2) for v in range(2)]
                for (u, v) in ((0, 0), (0, 1), (1, 0), (1, 1)):
                    stile[2 * I + u, 2 * J + v] = s_s[sl, u, 2 * J + v]
            else:
                for (u, v), c in zip(((0, 0), (0, 1), (1, 0), (1, 1)), cs):
                    stile[2 * I + u, 2 * J + v] = c
            for u in range(2):
                mx = jnp.maximum(cs[2 * u], cs[2 * u + 1])
                rmax[2 * I + u] = mx if 2 * I + u not in rmax else jnp.maximum(rmax[2 * I + u], mx)
                if cfg.get('fr', 0):
                    fd.add([rmax[2 * I + u]], cfg['fr'])

        def dpiece(I):
            a, b = 2 * I, 2 * I + 1
            q4 = qtiles(I)
            qa = jnp.concatenate(q4[0:2], axis=1)
            qb = jnp.concatenate(q4[2:4], axis=1)
            d1 = lax.dot_general(jnp.concatenate([qa, qb], axis=0), ktile(a), NT, preferred_element_type=f32)
            d2 = lax.dot_general(qb, ktile(b), NT, preferred_element_type=f32)
            stile[a, a] = jnp.where(tri, d1[:T], NEG)
            stile[b, a] = d1[T:]
            stile[b, b] = jnp.where(tri, d2, NEG)

        def pchunk(i, c):
            pc = cfg.get('pc', 2)
            if c == 0:
                I = i // 2
                mx = functools.reduce(jnp.maximum, ([rmax[i]] if I > 0 else []) + [stile[i, t] for t in range(2 * I, i + 1)])
                sm[i] = dict(m=jnp.max(mx, axis=1, keepdims=True), l=None, ctx=None)
            st_ = sm[i]
            c1 = min(c + pc, i + 1)
            pe = jnp.exp2(jnp.concatenate([stile.pop((i, t)) for t in range(c, c1)], axis=1) - st_['m'])
            pz = pe
            lf = cfg.get('lf', 0)
            hist = st_.setdefault('hist', [])
            if lf and len(hist) >= lf:
                z = _dep_u32([hist[-lf]])
                top = pltpu.bitcast(pltpu.bitcast(pe[0:8, :T], u32) | z, f32)
                if pe.shape[1] > T:
                    top = jnp.concatenate([top, pe[0:8, T:]], axis=1)
                pz = jnp.concatenate([top, pe[8:]], axis=0)
            pb = pz.astype(bf)
            pf = pb.astype(f32) if cfg.get('lbf', 1) else pe
            for t in range(c1 - c):
                st_['l'] = pf[:, t * T:(t + 1) * T] if st_['l'] is None else st_['l'] + pf[:, t * T:(t + 1) * T]
            hist.append(st_['l'])
            if (c, c1) not in kv['v']:
                kv['v'][c, c1] = rows_of(vblk, c, c1).astype(bf)
            d = jnp.dot(pb, kv['v'][c, c1], preferred_element_type=f32)
            st_['ctx'] = d if st_['ctx'] is None else st_['ctx'] + d

        def ctx_of(i):
            st_ = sm.pop(i)
            l = jnp.sum(st_['l'], axis=1, keepdims=True)
            r0 = pl.reciprocal(l, approx=True)
            return st_['ctx'] * (r0 * (2.0 - l * r0))

        odone = set()

        def accum(i, a0, d):
            a1 = a0 + d.shape[0]
            a = acc_s[i, a0:a1, :] + g_s[i][1:2, :] * d
            acc_s[i, a0:a1, :] = a
            out_s[a0:a1, i * T:(i + 1) * T] = a.astype(bf)

        def fin(blocks):
            odone.update(blocks)
            b = blocks[0] * T // OW
            if all(bb in odone for bb in range(b * OW // T, (b + 1) * OW // T)):
                @pl.when(h == H - 1)
                def _():
                    cp_out(b).start()

        def oproj2(i, ca, cb):
            if cfg.get('so', 1):
                ts = _rhs_terms(ca[:, :T], cb[:, :T], ca[:, T:], cb[:, T:])
                c11, c12, c21, c22 = _strassen(
                    lambda k: lax.dot_general(wos[k], ts[k].astype(bf), NT, preferred_element_type=f32))
                accum(i, 0, c11); accum(i + 1, 0, c12); accum(i, HM, c21); accum(i + 1, HM, c22)
            else:
                d = lax.dot_general(wo, jnp.concatenate([ca, cb], axis=0).astype(bf), NT, preferred_element_type=f32)
                accum(i, 0, d[:, :T]); accum(i + 1, 0, d[:, T:])
            fin([i, i + 1])

        def oprojs(i, ctx):
            cb = ctx.astype(bf)
            for a0 in (0, HM):
                accum(i, a0, lax.dot_general(wo[a0:a0 + HM], cb, NT, preferred_element_type=f32))
            fin([i])

        for op, i, c in prog:
            if op == 'r':
                rpiece(i, c)
            elif op == 'd':
                dpiece(i)
            elif op == 'm':
                pmm(*i)
            elif op == 'p':
                pchunk(i, c)
            elif op == 'D':
                oproj2(i, ctx_of(i), ctx_of(i + 1))
            elif op == 'S':
                oprojs(i, ctx_of(i))
        return carry

    lax.fori_loop(0, H, head, 0)
    for b in range(S // OW):
        cp_out(b).wait()


def make(**cfg):
    name = ("k23_" + "_".join([f"{k}{v}" for k, v in sorted(cfg.items())])).replace(" ", "").replace("(", "").replace(")", "").replace(",", "x")

    @jax.jit
    def f(A_x, A_c_kv, A_w_q, A_w_uk, A_w_uv, A_w_o, B_x, B_w_r, B_w_gate, B_w_up, B_w_down, gate_w):
        xt = A_x[0].T
        c = A_c_kv[0]
        woT = A_w_o.transpose(0, 2, 1)
        wdT = B_w_down.T
        V = pltpu.VMEM
        outT = pl.pallas_call(
            functools.partial(kernel, cfg=cfg),
            in_specs=[pl.BlockSpec(memory_space=pl.ANY)] * 11,
            out_specs=pl.BlockSpec(memory_space=pl.ANY),
            out_shape=jax.ShapeDtypeStruct((M, S), bf),
            scratch_shapes=[
                V((M, S), bf), V((2, S, HM), bf), V((7, HS, HM), bf), V((S, DC), bf), V((49, S // 8, DC // 4), u32),
                V((NP, M, D), u32), V((2, 2, DC, D), u32), V((H, M, D), bf),
                V((H, 2, S, T), bf), V((H, 5, HS, T), bf), V((NQ, M, T), f32),
                V((M, F), bf), V((M, F), bf), V((M, F), bf),
                V((M,), bf), V((M,), bf), V((M, S), bf),
                V((NQ, 8, T), f32), V((2, 16, HM), bf), V((16, T), f32), pltpu.SMEM((2,), jnp.int32), V((2, 2, NQ, T, T), f32),
                pltpu.SemaphoreType.DMA((NSEM,)),
            ],
            compiler_params=pltpu.CompilerParams(vmem_limit_bytes=110 * 1024 * 1024),
            name=name,
        )(xt, c, A_w_q, A_w_uk, A_w_uv, woT, B_w_r, B_w_gate, B_w_up, wdT, gate_w)
        return outT.T[None]
    return f


_impl = make(**{'so': 0, 'sv': 1, 'rf': 0.9, 'ss': 1, 'nch': 1, 'dpo': 1, 'dpi': 0, 'nv': 6, 'b1': 8, 'pr': 512})


@jax.jit
def pallas_gated_mix__compressed_kv_cla__moe_arch_mod__prompt_kernel(
    A_x: jax.Array,
    A_c_kv: jax.Array,
    A_w_q: jax.Array,
    A_w_uk: jax.Array,
    A_w_uv: jax.Array,
    A_w_o: jax.Array,
    B_x: jax.Array,
    B_w_r: jax.Array,
    B_w_gate: jax.Array,
    B_w_up: jax.Array,
    B_w_down: jax.Array,
    gate_w: jax.Array,
):
    return _impl(A_x, A_c_kv, A_w_q, A_w_uk, A_w_uv, A_w_o, B_x, B_w_r, B_w_gate, B_w_up, B_w_down, gate_w)
```

```python
import functools
import math

import jax
import jax.numpy as jnp
from jax import lax
from jax.experimental import pallas as pl
from jax.experimental.pallas import tpu as pltpu

S, M, H, D, DC, F = 2048, 448, 16, 256, 1024, 1792
T = 128
NP, NQ = H // 2, S // T
HS, HM, HC = S // 2, M // 2, DC // 2
QS, QC = S // 4, DC // 4
RB = 16
XC, OW = 256, 256
NG = 5
NT = (((1,), (1,)), ((), ()))
QSCALE = D ** -0.5 * math.log2(math.e)
NEG = -1e30
bf, f32, u32 = jnp.bfloat16, jnp.float32, jnp.uint32
HI = 0xFFFF0000

SEM_WO, SEM_FFN, SEM_VEC, SEM_KV, SEM_WQ, SEM_OUT, SEM_XT, SEM_C, NSEM = 0, 1, 4, 6, 8, 16, 24, 32, 40
SEQ = (1, 3, 4, 6, 0, 2, 5)


def _lhs_terms(a11, a12, a21, a22):
    return [a11 + a22, a21 + a22, a11, a22, a11 + a12, a21 - a11, a12 - a22]


def _rhs_terms(b11, b12, b21, b22):
    return [b11 + b22, b11, b12 - b22, b21 - b11, b22, b11 + b12, b21 + b22]


def _strassen(mm):
    m2, m3, m4, m5, m1, m7, m6 = [mm(i) for i in (1, 2, 3, 4, 0, 6, 5)]
    return (m4 - m5) + (m1 + m7), m3 + m5, m2 + m4, (m3 - m2) + (m1 + m6)


def _lhs_terms2(a11, a12, a21, a22):
    h21, q21, h22 = 0.5 * a21, 0.25 * a21, 0.5 * a22
    s1 = a11 + a22
    v, hs = a12 + q21, 0.5 * s1
    return [s1, q21 + h22, a11 + h21, h22 - q21, v + hs, h21 - a11, v - hs]


def _rhs_terms2(b11, b12, b21, b22):
    h21 = 0.5 * b21
    t1 = b11 + b22
    v, ht = b12 + 0.5 * h21, 0.5 * t1
    return [t1, b11 + h21, v - ht, h21 - b11, b22 - h21, v + ht, b22 + h21]


def _vregs(vals):
    ts = []
    for v in vals:
        v = v if v.dtype == u32 else pltpu.bitcast(v, u32)
        ts += [v[r:r + 8, c:c + T] for r in range(0, v.shape[0], 8) for c in range(0, v.shape[1] - T + 1, T)]
    return ts


def _zero_from(ts):
    acc = ts[:4]
    for i, t in enumerate(ts[4:]):
        acc[i % 4] = acc[i % 4] | t
    while len(acc) > 1:
        acc = [acc[i] | acc[i + 1] if i + 1 < len(acc) else acc[i] for i in range(0, len(acc), 2)]
    return (acc[0] >> 16) >> 16


def _feed(a, *zs):
    zs = [z for z in zs if z is not None]
    if not zs:
        return a
    a32 = pltpu.bitcast(a, u32)
    top = functools.reduce(lambda p, q: p | q, zs, a32[0:8, :T])
    if a32.shape[1] > T:
        top = jnp.concatenate([top, a32[0:8, T:]], axis=1)
    return pltpu.bitcast(jnp.concatenate([top, a32[8:]], axis=0), bf)


class _Pacer:
    def __init__(self, thunks, per, first, last):
        self.thunks, self.pool, self.k, self.done = list(thunks), [], 0, 0
        self.tot, self.first, self.last = per * len(self.thunks), first, last

    def __call__(self):
        self.k += 1
        if self.k <= self.first:
            return None
        want = min(self.tot, -(-(self.k - self.first) * self.tot // (self.last - self.first))) - self.done
        while len(self.pool) < want and self.thunks:
            self.pool += _vregs(self.thunks.pop(0)())
        outs, self.pool = self.pool[:want], self.pool[want:]
        self.done += len(outs)
        return _zero_from(outs) if outs else None

    def finished(self):
        return not self.thunks and not self.pool


def _merge(a, b):
    out, i, j = [], 0, 0
    while i < len(a) or j < len(b):
        if j >= len(b) or (i < len(a) and i * len(b) <= j * len(a)):
            out.append(a[i]); i += 1
        else:
            out.append(b[j]); j += 1
    return out


def _head_program():
    R = lambda I: [('r', I, J) for J in range(I)] + [('d', I, 0)]
    P = lambda I: [('p', i, c) for i in (2 * I, 2 * I + 1) for c in range(0, i + 1, 2)]
    MM = lambda r1s: [('m', r1, r2) for r1 in r1s for r2 in SEQ]
    V = MM(SEQ[5:])
    nv = 10
    prog = MM(SEQ[:5]) + V[:1] + _merge(R(0) + R(7), V[1:nv]) + V[nv:]
    pend = [0]
    for I in range(7, 0, -1):
        ps = (P(0) if I == 7 else []) + P(I)
        k = max(1, int(round(len(ps) * 0.9)))
        body = _merge(R(I - 1) if I > 1 else [], ps[:k]) + ps[k:]
        if I < 7:
            k = int(len(body) * 0.9)
            body = body[:k] + [('D', 2 * pend.pop(0), 0)] + body[k:]
        prog += body
        pend.append(I)
    return prog + [('D', 2 * pend[0], 0), ('S', 2, 0), ('S', 3, 0)]


def _dot(a, b):
    return jnp.dot(a, b, preferred_element_type=f32)


def _dot_nt(a, b):
    return lax.dot_general(a, b, NT, preferred_element_type=f32)


def _unpack(w32, sh):
    return pltpu.bitcast((w32 << sh) & jnp.uint32(HI), f32)


def _kernel(xt_hbm, c_hbm, wq_hbm, wk_hbm, wv_hbm, wo_hbm, wr_hbm, wg_hbm, wu_hbm, wd_hbm, gw_hbm, o_hbm,
            xt_s, x_s, xa_s, c_s, ca_s, wq_p, wkv_p, wo_s, q_s, qa_s, acc_s, wg_s, wu_s, wd_s,
            wr_s, gw_s, out_s, g_s, xs_s, rsel_s, idx_s, s_s, t0_s, sem):
    mk = pltpu.make_async_copy
    wq32, wk32, wv32 = wq_hbm.bitcast(u32), wk_hbm.bitcast(u32), wv_hbm.bitcast(u32)
    cp_wq = lambda j: mk(wq32.at[:, j, :], wq_p.at[j], sem.at[SEM_WQ + j])
    cp_kv = lambda j, m: mk((wk32, wv32)[m].at[:, j, :], wkv_p.at[j & 1, m], sem.at[SEM_KV + m])
    cp_xt = lambda k: mk(xt_hbm.at[:, pl.ds(k * XC, XC)], xt_s.at[:, pl.ds(k * XC, XC)], sem.at[SEM_XT + k])
    cp_out = lambda b: mk(out_s.at[:, pl.ds(b * OW, OW)], o_hbm.at[:, pl.ds(b * OW, OW)], sem.at[SEM_OUT + b])
    cp_vec = [mk(wr_hbm, wr_s, sem.at[SEM_VEC]), mk(gw_hbm, gw_s, sem.at[SEM_VEC + 1])]
    cp_ffn = [mk(src, dst, sem.at[SEM_FFN + n]) for n, (src, dst) in
              enumerate(((wg_hbm, wg_s), (wu_hbm, wu_s), (wd_hbm, wd_s)))]
    cp_wo = mk(wo_hbm, wo_s, sem.at[SEM_WO])

    def cp_c(j):
        r0 = (j - 1) * NG * RB
        n = QS - r0 if isinstance(j, int) and j == NP - 1 else NG * RB
        return [mk(c_hbm.at[pl.ds(i * QS + r0, n)], c_s.at[pl.ds(i * QS + r0, n)], sem.at[SEM_C + j])
                for i in range(4)]

    cp_wq(0).start()
    for k in range(S // XC):
        cp_xt(k).start()
    for cp in cp_vec:
        cp.start()
    for j in range(1, NP):
        cp_wq(j).start()
        for cp in cp_c(j):
            cp.start()
    for cp in cp_ffn + [cp_kv(0, 0), cp_kv(0, 1), cp_wo]:
        cp.start()

    def store_q(j, e, r0, q):
        q = q * QSCALE
        for t in range(2):
            q_s[2 * j + e, t, r0:r0 + q.shape[0], :] = q[:, t * T:(t + 1) * T].astype(bf)
        for p0 in range(0, q.shape[0], 2 * T):
            if r0 + p0 > 0:
                qa, qb = q[p0:p0 + T], q[p0 + T:p0 + 2 * T]
                terms = _lhs_terms(qa[:, :T], qa[:, T:], qb[:, :T], qb[:, T:])
                for k, i in enumerate((0, 1, 4, 5, 6)):
                    qa_s[2 * j + e, k, (r0 + p0) // 2:(r0 + p0) // 2 + T, :] = terms[i].astype(bf)

    def q_plain(w, r0, hook=None):
        prod = lambda a, b, wn, z: _dot(_feed(x_s[0, a:b, :], z), wn[:HM]) + _dot(x_s[1, a:b, :], wn[HM:])
        if hook is None:
            qf = prod(r0, r0 + 2 * T, w, None)
        else:
            qf = jnp.concatenate([jnp.concatenate(
                [prod(r0 + u * T, r0 + (u + 1) * T, w[:, n * T:(n + 1) * T], hook()) for u in range(2)], axis=0)
                for n in range(4)], axis=1)
        store_q(0, 0, r0, qf[:, :D])
        store_q(0, 1, r0, qf[:, D:])

    def q_rhs(j):
        lo, hi = pltpu.bitcast(wq_p[j] << 16, f32), pltpu.bitcast(wq_p[j] & jnp.uint32(HI), f32)
        return [t.astype(bf) for t in _rhs_terms(lo[:HM], hi[:HM], lo[HM:], hi[HM:])]

    def q_strassen(j, ts, r0, r1, hook):
        def lhs(i, u):
            if i in (2, 3):
                return x_s[i - 2, (i - 2) * HS + u:(i - 2) * HS + u + T, :]
            return xa_s[i - 2 * (i > 3), u:u + T, :]
        cs = _strassen(lambda i: jnp.concatenate(
            [_dot(_feed(lhs(i, u), *hook()), ts[i]) for u in range(r0, r1, T)], axis=0))
        for n, c in enumerate(cs):
            store_q(j, n % 2, (n // 2) * HS + r0, c)

    def x_prep(r0):
        a = [x_s[e, h0 + r0:h0 + r0 + RB, :].astype(f32) for h0 in (0, HS) for e in (0, 1)]
        terms = _lhs_terms(*a)
        outs = []
        for k, i in enumerate((0, 1, 4, 5, 6)):
            v = terms[i].astype(bf)
            xa_s[k, r0:r0 + RB, :] = v
            outs.append(pltpu.bitcast(v, u32))
        return outs

    def c_prep(g, c0):
        al = (lambda v, m: v) if isinstance(g, int) else pl.multiple_of
        blk = lambda i, k: c_s[pl.ds(al(i * QS + g * RB, RB), RB), k * QC + c0:k * QC + c0 + T].astype(f32)
        outer = [_lhs_terms2(*[blk(2 * i1 + i2, 2 * k1 + k2) for i1 in range(2) for k1 in range(2)])
                 for i2 in range(2) for k2 in range(2)]
        outs = []
        for r1 in range(7):
            for r2, v in enumerate(_lhs_terms(*[o[r1] for o in outer])):
                outs.append(pltpu.bitcast(v.astype(bf), u32))
                ca_s[7 * r1 + r2, pl.ds(al(g * (RB // 2), RB // 2), RB // 2), c0:c0 + T] = outs[-1]
        return outs

    def c_pacer(g0, ng, first, last):
        return _Pacer([functools.partial(c_prep, g0 + t // 2, (t % 2) * T) for t in range(2 * ng)], 49, first, last)

    def transpose(k):
        for e in range(2):
            x_s[e, k * XC:(k + 1) * XC, :] = xt_s[e * HM:(e + 1) * HM, k * XC:(k + 1) * XC].T

    def q_w0():
        return jnp.concatenate([pltpu.bitcast(wq_p[0] << 16, f32).astype(bf),
                                pltpu.bitcast(wq_p[0] & jnp.uint32(HI), f32).astype(bf)], axis=1)

    cp_wq(0).wait()
    cp_xt(0).wait()
    cp_xt(1).wait()
    transpose(0)
    transpose(1)
    q_plain(q_w0(), 0)
    cp_xt(2).wait()
    cp_xt(3).wait()
    w0 = q_w0()
    transpose(2)
    q_plain(w0, XC)
    transpose(3)
    q_plain(w0, 2 * XC)
    for k in range(4, S // XC):
        cp_xt(k).wait()
    for cp in cp_vec:
        cp.wait()
    for k in range(4, S // XC):
        transpose(k)
    row8 = lax.broadcasted_iota(jnp.int32, (8, M), 0)
    x_pace = _Pacer([functools.partial(x_prep, r0) for r0 in range(0, HS, RB)], 5, 12, 40)
    routed = []

    def hook0():
        n = len(routed)
        if n < NQ:
            rg = jnp.where(row8 == 0, wr_s[...].reshape(1, M).astype(f32), gw_s[...].reshape(1, M).astype(f32))
            g_s[n] = _dot(rg.astype(bf), xt_s[:, n * T:(n + 1) * T])
            routed.append(n)
        return x_pace()
    w0 = q_w0()
    for k in range(3, S // XC):
        q_plain(w0, k * XC, hook0)
    assert x_pace.finished()

    rb = jnp.concatenate([g_s[n][0:1, :] for n in range(NQ)], axis=1).astype(bf).astype(f32)
    lane = lax.broadcasted_iota(jnp.int32, (1, S), 1)
    m1 = jnp.max(rb, axis=1, keepdims=True)
    i1 = jnp.minimum(jnp.min(jnp.where(rb == m1, lane, S)), S - 1)
    rb2 = jnp.where(lane == i1, -jnp.inf, rb)
    m2 = jnp.max(rb2, axis=1, keepdims=True)
    i2 = jnp.minimum(jnp.min(jnp.where(jnp.logical_and(rb2 == m2, lane != i1), lane, S)), S - 1)
    row16 = lax.broadcasted_iota(jnp.int32, (16, HM), 0)

    def x_row(e, i):
        blk = x_s[e, pl.ds(pl.multiple_of((i // 16) * 16, 16), 16), :].astype(f32)
        return jnp.sum(jnp.where(row16 == i % 16, blk, 0.0), axis=0, keepdims=True)
    for e in range(2):
        xs_s[e] = jnp.where(row16 == 0, x_row(e, i1), jnp.where(row16 == 1, x_row(e, i2), 0.0)).astype(bf)
    rsel_s[...] = jax.nn.sigmoid(jnp.where(lax.broadcasted_iota(jnp.int32, (16, T), 0) == 0, m1, m2))
    idx_s[0] = i1
    idx_s[1] = i2

    def q_body(j, carry):
        cp_wq(j).wait()
        for cp in cp_c(j):
            cp.wait()
        pace = c_pacer((j - 1) * NG, NG, 1, 56)
        q_strassen(j, q_rhs(j), 0, HS, lambda: (pace(),))
        assert pace.finished()
        return carry
    lax.fori_loop(1, NP - 1, q_body, 0)

    for cp in cp_ffn + [cp_wq(NP - 1)] + cp_c(NP - 1):
        cp.wait()

    def residual(n):
        g8 = jax.nn.sigmoid(g_s[n])
        g_s[n] = g8
        a = (1.0 - g8[1:2, :]) * xt_s[:, n * T:(n + 1) * T].astype(f32)
        acc_s[n] = a
        return [a]

    gs, us, ys, hid = [], [], {}, []
    xs_dot = lambda w_s, n: (_dot(xs_s[0], w_s[:HM, n * T:(n + 1) * T]) + _dot(xs_s[1], w_s[HM:, n * T:(n + 1) * T]))

    def swiglu():
        gg, uu = jnp.concatenate(gs, axis=1), jnp.concatenate(us, axis=1)
        hid.append((gg * jax.nn.sigmoid(gg) * uu).astype(bf))

    def down(n0, k0):
        t = _dot_nt(hid[0][:, k0:min(k0 + 512, F)], wd_s[n0:min(n0 + T, M), k0:min(k0 + 512, F)])
        ys[n0] = ys[n0] + t if n0 in ys else t
    side = []
    for n in range(F // T):
        side += [lambda n=n: gs.append(xs_dot(wg_s, n)), lambda n=n: us.append(xs_dot(wu_s, n))]
    side += [swiglu] + [lambda: None] * 3
    side += [functools.partial(down, n0, k0) for n0 in range(0, M, T) for k0 in range(0, F, 512)]
    c_pace = c_pacer((NP - 2) * NG, QS // RB - (NP - 2) * NG, 2, 56)
    r_pace = _Pacer([functools.partial(residual, n) for n in range(NQ)], M // 8, 1, 48)

    def hook7():
        if side:
            side.pop(0)()
        return c_pace(), r_pace()
    ts7 = q_rhs(NP - 1)
    for r0 in range(0, HS, 2 * T):
        q_strassen(NP - 1, ts7, r0, r0 + 2 * T, hook7)
    assert not side and c_pace.finished() and r_pace.finished()
    y = jnp.concatenate([ys[n0] for n0 in range(0, M, T)] + [jnp.zeros((16, 512 - M), f32)], axis=1)
    yt = (y * rsel_s[:, 0:1]).T
    lane128 = lax.broadcasted_iota(jnp.int32, (1, T), 1)
    for e in range(2):
        i = idx_s[e]
        acc_s[i // T] += jnp.where(lane128 == i % T, (1.0 - g_s[i // T][1:2, :]) * yt[:M, e:e + 1], 0.0)

    cp_wo.wait()
    cp_kv(0, 0).wait()
    cp_kv(1, 0).start()

    def first_terms(hn):
        w = _unpack(wkv_p[(hn >> 1) & 1, 0, :, :T], (16 * (1 - (hn & 1))).astype(u32))
        t = w[:HC] + 0.5 * w[HC:]
        outs = [pltpu.bitcast(v.astype(bf), u32) for v in (t[:QC], t[QC:] - t[:QC])]
        for n, o in enumerate(outs):
            t0_s[n] = o
        return outs
    first_terms(jnp.int32(0))

    tri = lax.broadcasted_iota(jnp.int32, (T, T), 1) <= lax.broadcasted_iota(jnp.int32, (T, T), 0)
    prog = _head_program()

    def head(h, carry):
        par, slot = h & 1, (h >> 1) & 1
        for m in range(2):
            @pl.when(jnp.logical_and(h < H - 1, par == 1 - m))
            def _():
                cp_kv((h + 1) >> 1, m).wait()

        sh = (16 * (1 - par)).astype(u32)
        rhs = []
        for r1 in range(7):
            wk, wv = [_unpack(wkv_p[slot, m], sh + (h >> (8 + r1)).astype(u32)) for m in range(2)]
            t = _rhs_terms2(wk[:HC], wv[:HC], wk[HC:], wv[HC:])[r1]
            rhs.append([u.astype(bf) for u in _rhs_terms(t[:QC, :T], t[:QC, T:], t[QC:, :T], t[QC:, T:])])
        rhs[1][1], rhs[1][3] = [pltpu.bitcast(t0_s[n], bf) for n in range(2)]
        t_pace = _Pacer([lambda: first_terms(jnp.minimum(h + 1, H - 1))], 32, 196 - 14, 196)
        prods, outer, kblk, vblk = {}, [{} for _ in range(4)], {}, {}

        def kv_product(r1, r2):
            m = prods.setdefault(r1, {})
            m[r2] = _dot(pltpu.bitcast(ca_s[7 * r1 + r2], bf), rhs[r1][r2])
            new = {}
            if r2 == 3:
                new = {2: m[1] + m[3]}
            elif r2 == 2:
                new = {0: ((m[3] - m[4]) + m[6]) + m[0], 1: m[2] + m[4]}
            elif r2 == 5:
                new = {3: ((m[0] - m[1]) + m[2]) + m[5]}
            for b, o in new.items():
                a = outer[b]
                if r1 == 1:
                    a['p1'] = o
                elif r1 == 3:
                    a['e'], a['d'] = o + a['p1'], o - a['p1']
                    a['k1'] = a['e'] * 2.0
                elif r1 == 4:
                    a['f'], a['e'] = a['d'] - o, a['e'] + o
                elif r1 == 6:
                    a['f'], a['e'] = a['f'] + o, a['e'] + o
                elif r1 == 0:
                    kblk[b], a['t'] = (o + a['f'], a['k1']), o + a['d']
                elif r1 == 2:
                    a['e'], a['t'] = a['e'] + o, a['t'] + o
                else:
                    vblk[b] = ((a['e'] - o) * 0.5, a['t'] + o)

        def rows(blk, t0, t1):
            return jnp.concatenate([jnp.concatenate(
                [blk[2 * (t // 4 % 2) + j2][t // 8][t % 4 * T:(t % 4 + 1) * T] for j2 in range(2)], axis=1)
                for t in range(t0, t1)], axis=0)

        @functools.cache
        def k_tile(t):
            return rows(kblk, t, t + 1).astype(bf)

        @functools.cache
        def k_terms(J):
            ka, kb = rows(kblk, 2 * J, 2 * J + 1), rows(kblk, 2 * J + 1, 2 * J + 2)
            return [t.astype(bf) for t in _rhs_terms(ka[:, :T], kb[:, :T], ka[:, T:], kb[:, T:])]

        @functools.cache
        def v_tiles(c0, c1):
            return rows(vblk, c0, c1).astype(bf)

        scores, rmax, soft, o_done = {}, {}, {}, set()
        q_tiles = lambda I: [q_s[h, t, i * T:(i + 1) * T, :] for i in (2 * I, 2 * I + 1) for t in range(2)]

        def score_block(I, J):
            q4, qx = q_tiles(I), [qa_s[h, k, I * T:(I + 1) * T, :] for k in range(5)]
            lhs = [qx[0], qx[1], q4[0], q4[3], qx[2], qx[3], qx[4]]
            cs = _strassen(lambda i: _dot_nt(_feed(lhs[i], t_pace()), k_terms(J)[i]))
            for n, c in enumerate(cs):
                s_s[I % 2, n // 2, 2 * J + n % 2] = c
            for u in range(2):
                sa, sb = s_s[I % 2, u, 2 * J], s_s[I % 2, u, 2 * J + 1]
                scores[2 * I + u, 2 * J] = s_s[I % 2, u, 2 * J]
                scores[2 * I + u, 2 * J + 1] = s_s[I % 2, u, 2 * J + 1]
                mx = jnp.maximum(sa, sb)
                rmax[2 * I + u] = jnp.maximum(rmax[2 * I + u], mx) if 2 * I + u in rmax else mx

        def score_diag(I):
            a, b = 2 * I, 2 * I + 1
            q4 = q_tiles(I)
            qa, qb = jnp.concatenate(q4[0:2], axis=1), jnp.concatenate(q4[2:4], axis=1)
            d1 = _dot_nt(jnp.concatenate([qa, qb], axis=0), k_tile(a))
            d2 = _dot_nt(qb, k_tile(b))
            scores[a, a], scores[b, a], scores[b, b] = jnp.where(tri, d1[:T], NEG), d1[T:], jnp.where(tri, d2, NEG)

        def pv_chunk(i, c0):
            if c0 == 0:
                mx = functools.reduce(jnp.maximum, ([rmax[i]] if i > 1 else [])
                                      + [scores[i, t] for t in range(i // 2 * 2, i + 1)])
                soft[i] = dict(m=jnp.max(mx, axis=1, keepdims=True), l=None, ctx=None)
            st = soft[i]
            c1 = min(c0 + 2, i + 1)
            p = jnp.exp2(jnp.concatenate([scores.pop((i, t)) for t in range(c0, c1)], axis=1) - st['m']).astype(bf)
            pf = p.astype(f32)
            for t in range(c1 - c0):
                st['l'] = pf[:, t * T:(t + 1) * T] if st['l'] is None else st['l'] + pf[:, t * T:(t + 1) * T]
            d = _dot(p, v_tiles(c0, c1))
            st['ctx'] = d if st['ctx'] is None else st['ctx'] + d

        def context(i):
            st = soft.pop(i)
            l = jnp.sum(st['l'], axis=1, keepdims=True)
            r = pl.reciprocal(l, approx=True)
            return st['ctx'] * (r * (2.0 - l * r))

        def accumulate(i, a0, d):
            a = acc_s[i, a0:a0 + d.shape[0], :] + g_s[i][1:2, :] * d
            acc_s[i, a0:a0 + d.shape[0], :] = a
            out_s[a0:a0 + d.shape[0], i * T:(i + 1) * T] = a.astype(bf)

        def out_proj(blocks):
            wo = wo_s[h]
            ctx = jnp.concatenate([context(i) for i in blocks], axis=0).astype(bf)
            if len(blocks) == 2:
                d = _dot_nt(wo, ctx)
                accumulate(blocks[0], 0, d[:, :T])
                accumulate(blocks[1], 0, d[:, T:])
            else:
                for a0 in (0, HM):
                    accumulate(blocks[0], a0, _dot_nt(wo[a0:a0 + HM], ctx))
            o_done.update(blocks)
            if {blocks[0] // 2 * 2, blocks[0] // 2 * 2 + 1} <= o_done:
                @pl.when(h == H - 1)
                def _():
                    cp_out(blocks[0] // 2).start()

        ops = {'m': kv_product, 'r': score_block, 'd': lambda I, _: score_diag(I), 'p': pv_chunk,
               'D': lambda i, _: out_proj([i, i + 1]), 'S': lambda i, _: out_proj([i])}
        for op, i, c in prog:
            ops[op](i, c)
        assert t_pace.finished()
        for m in range(2):
            @pl.when(jnp.logical_and((h + 3) >> 1 < NP, par == 1 - m))
            def _():
                cp_kv((h + 3) >> 1, m).start()
        return carry

    lax.fori_loop(0, H, head, 0)
    for b in range(S // OW):
        cp_out(b).wait()


@jax.jit
def pallas_gated_mix__compressed_kv_cla__moe_arch_mod__prompt_kernel(
    A_x: jax.Array,
    A_c_kv: jax.Array,
    A_w_q: jax.Array,
    A_w_uk: jax.Array,
    A_w_uv: jax.Array,
    A_w_o: jax.Array,
    B_x: jax.Array,
    B_w_r: jax.Array,
    B_w_gate: jax.Array,
    B_w_up: jax.Array,
    B_w_down: jax.Array,
    gate_w: jax.Array,
):
    del B_x
    V = pltpu.VMEM
    out_t = pl.pallas_call(
        _kernel,
        in_specs=[pl.BlockSpec(memory_space=pl.ANY)] * 11,
        out_specs=pl.BlockSpec(memory_space=pl.ANY),
        out_shape=jax.ShapeDtypeStruct((M, S), bf),
        scratch_shapes=[
            V((M, S), bf), V((2, S, HM), bf), V((5, HS, HM), bf),
            V((S, DC), bf), V((49, QS // 2, QC), u32),
            V((NP, M, D), u32), V((2, 2, DC, D), u32), V((H, M, D), bf),
            V((H, 2, S, T), bf), V((H, 5, HS, T), bf),
            V((NQ, M, T), f32),
            V((M, F), bf), V((M, F), bf), V((M, F), bf),
            V((M,), bf), V((M,), bf), V((M, S), bf),
            V((NQ, 8, T), f32), V((2, 16, HM), bf), V((16, T), f32),
            pltpu.SMEM((2,), jnp.int32),
            V((2, 2, NQ, T, T), f32), V((2, QC // 2, T), u32),
            pltpu.SemaphoreType.DMA((NSEM,)),
        ],
        compiler_params=pltpu.CompilerParams(vmem_limit_bytes=110 * 1024 * 1024),
        name="gated_mix_cla_mod",
    )(A_x[0].T, A_c_kv[0], A_w_q, A_w_uk, A_w_uv, A_w_o.transpose(0, 2, 1), B_w_r, B_w_gate, B_w_up,
      B_w_down.T, gate_w)
    return out_t.T[None]
```

```python
import functools
import math

import jax
import jax.numpy as jnp
from jax import lax
from jax.experimental import pallas as pl
from jax.experimental.pallas import tpu as pltpu

S, M, H, D, DC, F = 2048, 448, 16, 256, 1024, 1792
T = 128
NP, NQ = H // 2, S // T
HS, HM, HC = S // 2, M // 2, DC // 2
QS, QC = S // 4, DC // 4
RB = 16
XC = 256
NG = 5
NT = (((1,), (1,)), ((), ()))
QSCALE = D ** -0.5 * math.log2(math.e)
NEG = -1e30
bf, f32, u32 = jnp.bfloat16, jnp.float32, jnp.uint32
HI = 0xFFFF0000

SEM_WO, SEM_FFN, SEM_VEC, SEM_KV, SEM_WQ, SEM_XT, SEM_C, SEM_OUT, NSEM = 0, 1, 4, 6, 8, 16, 24, 32, 48
SEQ = (1, 3, 4, 6, 0, 2, 5)


def _lhs_terms(a11, a12, a21, a22):
    return [a11 + a22, a21 + a22, a11, a22, a11 + a12, a21 - a11, a12 - a22]


def _rhs_terms(b11, b12, b21, b22):
    return [b11 + b22, b11, b12 - b22, b21 - b11, b22, b11 + b12, b21 + b22]


def _strassen(mm):
    m2, m3, m4, m5, m1, m7, m6 = [mm(i) for i in (1, 2, 3, 4, 0, 6, 5)]
    return (m4 - m5) + (m1 + m7), m3 + m5, m2 + m4, (m3 - m2) + (m1 + m6)


def _lhs_terms2(a11, a12, a21, a22):
    h21, q21, h22 = 0.5 * a21, 0.25 * a21, 0.5 * a22
    s1 = a11 + a22
    v, hs = a12 + q21, 0.5 * s1
    return [s1, q21 + h22, a11 + h21, h22 - q21, v + hs, h21 - a11, v - hs]


def _rhs_terms2(b11, b12, b21, b22):
    h21 = 0.5 * b21
    t1 = b11 + b22
    v, ht = b12 + 0.5 * h21, 0.5 * t1
    return [t1, b11 + h21, v - ht, h21 - b11, b22 - h21, v + ht, b22 + h21]


def _vregs(vals):
    ts = []
    for v in vals:
        v = v if v.dtype == u32 else pltpu.bitcast(v, u32)
        ts += [v[r:r + 8, c:c + T] for r in range(0, v.shape[0], 8) for c in range(0, v.shape[1] - T + 1, T)]
    return ts


def _zero_from(ts):
    acc = ts[:4]
    for i, t in enumerate(ts[4:]):
        acc[i % 4] = acc[i % 4] | t
    while len(acc) > 1:
        acc = [acc[i] | acc[i + 1] if i + 1 < len(acc) else acc[i] for i in range(0, len(acc), 2)]
    return (acc[0] >> 16) >> 16


def _feed(a, *zs):
    zs = [z for z in zs if z is not None]
    if not zs:
        return a
    a32 = pltpu.bitcast(a, u32)
    top = functools.reduce(lambda p, q: p | q, zs, a32[0:8, :T])
    if a32.shape[1] > T:
        top = jnp.concatenate([top, a32[0:8, T:]], axis=1)
    return pltpu.bitcast(jnp.concatenate([top, a32[8:]], axis=0), bf)


class _Pacer:
    def __init__(self, thunks, per, first, last):
        self.thunks, self.pool, self.k, self.done = list(thunks), [], 0, 0
        self.tot, self.first, self.last = per * len(self.thunks), first, last

    def __call__(self):
        self.k += 1
        if self.k <= self.first:
            return None
        want = min(self.tot, -(-(self.k - self.first) * self.tot // (self.last - self.first))) - self.done
        while len(self.pool) < want and self.thunks:
            self.pool += _vregs(self.thunks.pop(0)())
        outs, self.pool = self.pool[:want], self.pool[want:]
        self.done += len(outs)
        return _zero_from(outs) if outs else None

    def finished(self):
        return not self.thunks and not self.pool


def _merge(a, b):
    out, i, j = [], 0, 0
    while i < len(a) or j < len(b):
        if j >= len(b) or (i < len(a) and i * len(b) <= j * len(a)):
            out.append(a[i]); i += 1
        else:
            out.append(b[j]); j += 1
    return out


def _head_program():
    R = lambda I: [('r', I, J) for J in range(I)] + [('d', I, 0)]
    P = lambda I: [('p', i, c) for i in (2 * I, 2 * I + 1) for c in range(0, i + 1, 2)]
    MM = lambda r1s: [('m', r1, r2) for r1 in r1s for r2 in SEQ]
    V = MM(SEQ[5:])
    nv = 10
    prog = MM(SEQ[:5]) + V[:1] + _merge(R(0) + R(7), V[1:nv]) + V[nv:]
    pend = [0]
    for I in range(7, 0, -1):
        body = _merge(R(I - 1) if I > 1 else [], (P(0) if I == 7 else []) + P(I))
        if I < 7:
            k = int(len(body) * 0.9)
            body = body[:k] + [('D', 2 * pend.pop(0), 0)] + body[k:]
        prog += body
        pend.append(I)
    return prog + [('D', 2 * pend[0], 0), ('S', 2, 0), ('S', 3, 0)]


def _dot(a, b):
    return jnp.dot(a, b, preferred_element_type=f32)


def _dot_nt(a, b):
    return lax.dot_general(a, b, NT, preferred_element_type=f32)


def _unpack(w32, sh):
    return pltpu.bitcast((w32 << sh) & jnp.uint32(HI), f32)


class _Bf16:
    def __init__(self, raw):
        self.raw = raw

    def _half(self, idx):
        idx = list(idx if isinstance(idx, tuple) else (idx,))
        idx += [slice(None)] * (len(self.raw.shape) - len(idx))
        r = idx[-2]
        if isinstance(r, slice):
            idx[-2] = slice(None if r.start is None else r.start // 2, None if r.stop is None else r.stop // 2)
        elif isinstance(r.start, int):
            idx[-2] = pl.ds(r.start // 2, r.size // 2)
        else:
            idx[-2] = pl.ds(pl.multiple_of(r.start >> 1, 8), r.size // 2)
        return tuple(idx)

    def __getitem__(self, idx):
        return pltpu.bitcast(self.raw[self._half(idx)], bf)

    def put(self, idx, v):
        idx = self._half(idx)
        ref = self.raw.at[idx[:-2]] if len(idx) > 2 else self.raw
        o = pltpu.bitcast(v, u32)
        ref[idx[-2], idx[-1]] = o
        return o

    def __setitem__(self, idx, v):
        self.put(idx, v)


def _kernel(xt_hbm, c_hbm, wq_hbm, wk_hbm, wv_hbm, wo_hbm, wr_hbm, wg_hbm, wu_hbm, wd_hbm, gw_hbm, o_hbm,
            xt_s, x_s, xa_r, c_r, ca_r, wq_p, wkv_p, wo_r, q_r, qa_r, acc_s, wg_r, wu_r, wd_r,
            wr_s, gw_s, out_s, g_s, xs_r, rsel_s, idx_s, s_s, t0_r, sem):
    xa_s, c_s, ca_s, wo_s, q_s, qa_s, wg_s, wu_s, wd_s, xs_s, t0_s = [
        _Bf16(r) for r in (xa_r, c_r, ca_r, wo_r, q_r, qa_r, wg_r, wu_r, wd_r, xs_r, t0_r)]
    mk = pltpu.make_async_copy
    wq32, wk32, wv32 = wq_hbm.bitcast(u32), wk_hbm.bitcast(u32), wv_hbm.bitcast(u32)
    cp_wq = lambda j: mk(wq32.at[:, j, :], wq_p.at[j], sem.at[SEM_WQ + j])
    cp_kv = lambda j, m: mk((wk32, wv32)[m].at[:, j, :], wkv_p.at[j & 1, m], sem.at[SEM_KV + m])
    cp_xt = lambda k: mk(xt_hbm.at[:, pl.ds(k * XC, XC)], xt_s.at[:, pl.ds(k * XC, XC)], sem.at[SEM_XT + k])
    cp_out = lambda i: mk(out_s.at[i], o_hbm.at[:, pl.ds(i * T, T)], sem.at[SEM_OUT + i])
    cp_vec = [mk(wr_hbm, wr_s, sem.at[SEM_VEC]), mk(gw_hbm, gw_s, sem.at[SEM_VEC + 1])]
    cp_ffn = [mk(src, dst, sem.at[SEM_FFN + n]) for n, (src, dst) in
              enumerate(((wg_hbm.bitcast(u32), wg_r), (wu_hbm.bitcast(u32), wu_r), (wd_hbm.bitcast(u32), wd_r)))]
    cp_wo = mk(wo_hbm.bitcast(u32), wo_r, sem.at[SEM_WO])
    c32 = c_hbm.bitcast(u32)

    def cp_c(j):
        r0 = (j - 1) * (NG * RB // 2)
        n = QS // 2 - r0 if isinstance(j, int) and j == NP - 1 else NG * RB // 2
        return [mk(c32.at[pl.ds(i * QS // 2 + r0, n)], c_r.at[pl.ds(i * QS // 2 + r0, n)], sem.at[SEM_C + j])
                for i in range(4)]

    cp_xt(0).start()
    cp_wq(0).start()
    for k in range(1, S // XC):
        cp_xt(k).start()
    for cp in cp_vec:
        cp.start()
    for j in range(1, NP):
        cp_wq(j).start()
        for cp in cp_c(j):
            cp.start()
    for cp in cp_ffn + [cp_kv(0, 0), cp_kv(0, 1), cp_wo]:
        cp.start()

    def store_q(j, e, r0, q):
        q = q * QSCALE
        q_s[2 * j + e, r0:r0 + q.shape[0], :] = q.astype(bf)
        for p0 in range(0, q.shape[0], 2 * T):
            if r0 + p0 > 0:
                qa, qb = q[p0:p0 + T], q[p0 + T:p0 + 2 * T]
                terms = _lhs_terms(qa[:, :T], qa[:, T:], qb[:, :T], qb[:, T:])
                for k, i in enumerate((0, 1, 4, 5, 6)):
                    qa_s[2 * j + e, (r0 + p0) // 2:(r0 + p0) // 2 + T, k * T:(k + 1) * T] = terms[i].astype(bf)

    def q_plain(w, r0, hook=None):
        prod = lambda a, b, wn, z: _dot(_feed(x_s[0, a:b, :], z), wn[:HM]) + _dot(x_s[1, a:b, :], wn[HM:])
        if hook is None:
            qf = prod(r0, r0 + 2 * T, w, None)
        else:
            qf = jnp.concatenate([jnp.concatenate(
                [prod(r0 + u * T, r0 + (u + 1) * T, w[:, n * T:(n + 1) * T], hook()) for u in range(2)], axis=0)
                for n in range(4)], axis=1)
        store_q(0, 0, r0, qf[:, :D])
        store_q(0, 1, r0, qf[:, D:])

    def q_rhs(j):
        lo, hi = pltpu.bitcast(wq_p[j] << 16, f32), pltpu.bitcast(wq_p[j] & jnp.uint32(HI), f32)
        return [t.astype(bf) for t in _rhs_terms(lo[:HM], hi[:HM], lo[HM:], hi[HM:])]

    def q_strassen(j, ts, r0, r1, hook):
        def lhs(i, u):
            if i in (2, 3):
                return x_s[i - 2, (i - 2) * HS + u:(i - 2) * HS + u + T, :]
            return xa_s[i - 2 * (i > 3), u:u + T, :]
        cs = _strassen(lambda i: jnp.concatenate(
            [_dot(_feed(lhs(i, u), *hook()), ts[i]) for u in range(r0, r1, T)], axis=0))
        for n, c in enumerate(cs):
            store_q(j, n % 2, (n // 2) * HS + r0, c)

    def x_prep(r0):
        a = [x_s[e, h0 + r0:h0 + r0 + RB, :].astype(f32) for h0 in (0, HS) for e in (0, 1)]
        terms = _lhs_terms(*a)
        outs = []
        for k, i in enumerate((0, 1, 4, 5, 6)):
            outs.append(xa_s.put((k, slice(r0, r0 + RB)), terms[i].astype(bf)))
        return outs

    def c_prep(g, c0):
        blk = lambda i, k: c_s[pl.ds(i * QS + g * RB, RB), k * QC + c0:k * QC + c0 + T].astype(f32)
        outer = [_lhs_terms2(*[blk(2 * i1 + i2, 2 * k1 + k2) for i1 in range(2) for k1 in range(2)])
                 for i2 in range(2) for k2 in range(2)]
        outs = []
        for r1 in range(7):
            for r2, v in enumerate(_lhs_terms(*[o[r1] for o in outer])):
                outs.append(ca_s.put((7 * r1 + r2, pl.ds(g * RB, RB), slice(c0, c0 + T)), v.astype(bf)))
        return outs

    def c_pacer(g0, ng, first, last):
        return _Pacer([functools.partial(c_prep, g0 + t // 2, (t % 2) * T) for t in range(2 * ng)], 49, first, last)

    def transpose(k):
        for e in range(2):
            x_s[e, k * XC:(k + 1) * XC, :] = xt_s[e * HM:(e + 1) * HM, k * XC:(k + 1) * XC].T

    def q_w0():
        return jnp.concatenate([pltpu.bitcast(wq_p[0] << 16, f32).astype(bf),
                                pltpu.bitcast(wq_p[0] & jnp.uint32(HI), f32).astype(bf)], axis=1)

    cp_xt(0).wait()
    transpose(0)
    cp_wq(0).wait()
    q_plain(q_w0(), 0)
    for k in range(1, 4):
        cp_xt(k).wait()
    transpose(1)
    w0 = q_w0()
    transpose(2)
    q_plain(w0, XC)
    transpose(3)
    q_plain(w0, 2 * XC)
    for k in range(4, S // XC):
        cp_xt(k).wait()
    for cp in cp_vec:
        cp.wait()
    for k in range(4, S // XC):
        transpose(k)
    row8 = lax.broadcasted_iota(jnp.int32, (8, M), 0)
    x_pace = _Pacer([functools.partial(x_prep, r0) for r0 in range(0, HS, RB)], 5, 12, 40)
    routed = []

    def hook0():
        n = len(routed)
        if n < NQ:
            rg = jnp.where(row8 == 0, wr_s[...].reshape(1, M).astype(f32), gw_s[...].reshape(1, M).astype(f32))
            g_s[n] = _dot(rg.astype(bf), xt_s[:, n * T:(n + 1) * T])
            routed.append(n)
        return x_pace()
    w0 = q_w0()
    for k in range(3, S // XC):
        q_plain(w0, k * XC, hook0)
    assert x_pace.finished()

    rb = jnp.concatenate([g_s[n][0:1, :] for n in range(NQ)], axis=1).astype(bf).astype(f32)
    lane = lax.broadcasted_iota(jnp.int32, (1, S), 1)
    m1 = jnp.max(rb, axis=1, keepdims=True)
    i1 = jnp.minimum(jnp.min(jnp.where(rb == m1, lane, S)), S - 1)
    rb2 = jnp.where(lane == i1, -jnp.inf, rb)
    m2 = jnp.max(rb2, axis=1, keepdims=True)
    i2 = jnp.minimum(jnp.min(jnp.where(jnp.logical_and(rb2 == m2, lane != i1), lane, S)), S - 1)
    row16 = lax.broadcasted_iota(jnp.int32, (16, HM), 0)

    def x_row(e, i):
        blk = x_s[e, pl.ds(pl.multiple_of((i // 16) * 16, 16), 16), :].astype(f32)
        return jnp.sum(jnp.where(row16 == i % 16, blk, 0.0), axis=0, keepdims=True)
    for e in range(2):
        xs_s[e] = jnp.where(row16 == 0, x_row(e, i1), jnp.where(row16 == 1, x_row(e, i2), 0.0)).astype(bf)
    rsel_s[...] = jax.nn.sigmoid(jnp.where(lax.broadcasted_iota(jnp.int32, (16, T), 0) == 0, m1, m2))
    idx_s[0] = i1
    idx_s[1] = i2

    def q_body(it, carry):
        js = (2 * it + 1, 2 * it + 2)
        for j in js:
            for cp in [cp_wq(j)] + cp_c(j):
                cp.wait()
        pace = c_pacer(2 * it * NG, 2 * NG, 1, 112)
        for j in js:
            q_strassen(j, q_rhs(j), 0, HS, lambda: (pace(),))
        assert pace.finished()
        return carry
    lax.fori_loop(0, 3, q_body, 0)

    for cp in cp_ffn + [cp_wq(NP - 1)] + cp_c(NP - 1):
        cp.wait()

    def residual(n):
        g8 = jax.nn.sigmoid(g_s[n])
        g_s[n] = g8
        a = (1.0 - g8[1:2, :]) * xt_s[:, n * T:(n + 1) * T].astype(f32)
        acc_s[n] = a
        return [a]

    gs, us, ys, hid = [], [], {}, []
    xs_dot = lambda w_s, n: (_dot(xs_s[0], w_s[:HM, n * T:(n + 1) * T]) + _dot(xs_s[1], w_s[HM:, n * T:(n + 1) * T]))

    def swiglu():
        gg, uu = jnp.concatenate(gs, axis=1), jnp.concatenate(us, axis=1)
        hid.append((gg * jax.nn.sigmoid(gg) * uu).astype(bf))

    def down(n0, k0):
        t = _dot_nt(hid[0][:, k0:min(k0 + 512, F)], wd_s[n0:min(n0 + T, M), k0:min(k0 + 512, F)])
        ys[n0] = ys[n0] + t if n0 in ys else t
    side = []
    for n in range(F // T):
        side += [lambda n=n: gs.append(xs_dot(wg_s, n)), lambda n=n: us.append(xs_dot(wu_s, n))]
    side += [swiglu] + [lambda: None] * 7
    side += [functools.partial(down, n0, k0) for n0 in range(0, M, T) for k0 in range(0, F, 512)]
    c_pace = c_pacer((NP - 2) * NG, QS // RB - (NP - 2) * NG, 2, 56)
    r_pace = _Pacer([functools.partial(residual, n) for n in range(NQ)], M // 8, 1, 48)

    def hook7():
        if side:
            side.pop(0)()
        return c_pace(), r_pace()
    ts7 = q_rhs(NP - 1)
    for r0 in range(0, HS, 2 * T):
        q_strassen(NP - 1, ts7, r0, r0 + 2 * T, hook7)
    assert not side and c_pace.finished() and r_pace.finished()
    y = jnp.concatenate([ys[n0] for n0 in range(0, M, T)] + [jnp.zeros((16, 512 - M), f32)], axis=1)
    yt = (y * rsel_s[:, 0:1]).T
    lane128 = lax.broadcasted_iota(jnp.int32, (1, T), 1)
    for e in range(2):
        i = idx_s[e]
        acc_s[i // T] += jnp.where(lane128 == i % T, (1.0 - g_s[i // T][1:2, :]) * yt[:M, e:e + 1], 0.0)

    cp_wo.wait()
    cp_kv(0, 0).wait()
    cp_kv(1, 0).start()

    def first_terms(hn):
        w = _unpack(wkv_p[(hn >> 1) & 1, 0, :, :T], (16 * (1 - (hn & 1))).astype(u32))
        t = w[:HC] + 0.5 * w[HC:]
        return [t0_s.put((slice(None), slice(n * T, (n + 1) * T)), v.astype(bf))
                for n, v in enumerate((t[:QC], t[QC:] - t[:QC]))]
    first_terms(jnp.int32(0))

    tri = lax.broadcasted_iota(jnp.int32, (T, T), 1) <= lax.broadcasted_iota(jnp.int32, (T, T), 0)
    prog = _head_program()

    def head(h, carry):
        par, slot = h & 1, (h >> 1) & 1
        for m in range(2):
            @pl.when(jnp.logical_and(h < H - 1, par == 1 - m))
            def _():
                cp_kv((h + 1) >> 1, m).wait()

        sh = (16 * (1 - par)).astype(u32)
        rhs = []
        for r1 in range(7):
            wk, wv = [_unpack(wkv_p[slot, m], sh + (h >> (8 + r1)).astype(u32)) for m in range(2)]
            t = _rhs_terms2(wk[:HC], wv[:HC], wk[HC:], wv[HC:])[r1]
            rhs.append([u.astype(bf) for u in _rhs_terms(t[:QC, :T], t[:QC, T:], t[QC:, :T], t[QC:, T:])])
        rhs[1][1], rhs[1][3] = t0_s[:, :T], t0_s[:, T:]
        t_pace = _Pacer([lambda: first_terms(jnp.minimum(h + 1, H - 1))], 32, 196 - 14, 196)
        prods, outer, kblk, vblk = {}, [{} for _ in range(4)], {}, {}

        def kv_product(r1, r2):
            m = prods.setdefault(r1, {})
            m[r2] = _dot(ca_s[7 * r1 + r2], rhs[r1][r2])
            new = {}
            if r2 == 3:
                new = {2: m[1] + m[3]}
            elif r2 == 2:
                new = {0: ((m[3] - m[4]) + m[6]) + m[0], 1: m[2] + m[4]}
            elif r2 == 5:
                new = {3: ((m[0] - m[1]) + m[2]) + m[5]}
            for b, o in new.items():
                a = outer[b]
                if r1 == 1:
                    a['p1'] = o
                elif r1 == 3:
                    a['e'], a['d'] = o + a['p1'], o - a['p1']
                    a['k1'] = a['e'] * 2.0
                elif r1 == 4:
                    a['f'], a['e'] = a['d'] - o, a['e'] + o
                elif r1 == 6:
                    a['f'], a['e'] = a['f'] + o, a['e'] + o
                elif r1 == 0:
                    kblk[b], a['t'] = (o + a['f'], a['k1']), o + a['d']
                elif r1 == 2:
                    a['e'], a['t'] = a['e'] + o, a['t'] + o
                else:
                    vblk[b] = ((a['e'] - o) * 0.5, a['t'] + o)

        def rows(blk, t0, t1):
            return jnp.concatenate([jnp.concatenate(
                [blk[2 * (t // 4 % 2) + j2][t // 8][t % 4 * T:(t % 4 + 1) * T] for j2 in range(2)], axis=1)
                for t in range(t0, t1)], axis=0)

        @functools.cache
        def k_tile(t):
            return rows(kblk, t, t + 1).astype(bf)

        @functools.cache
        def k_terms(J):
            ka, kb = rows(kblk, 2 * J, 2 * J + 1), rows(kblk, 2 * J + 1, 2 * J + 2)
            return [t.astype(bf) for t in _rhs_terms(ka[:, :T], kb[:, :T], ka[:, T:], kb[:, T:])]

        @functools.cache
        def v_tiles(c0, c1):
            return rows(vblk, c0, c1).astype(bf)

        scores, rmax, soft = {}, {}, {}
        q_tiles = lambda I: [q_s[h, i * T:(i + 1) * T, t * T:(t + 1) * T] for i in (2 * I, 2 * I + 1) for t in range(2)]

        def score_block(I, J):
            q4, qx = q_tiles(I), [qa_s[h, I * T:(I + 1) * T, k * T:(k + 1) * T] for k in range(5)]
            lhs = [qx[0], qx[1], q4[0], q4[3], qx[2], qx[3], qx[4]]
            cs = _strassen(lambda i: _dot_nt(_feed(lhs[i], t_pace()), k_terms(J)[i]))
            for n, c in enumerate(cs):
                s_s[I % 2, n // 2, 2 * J + n % 2] = c
            for u in range(2):
                sa, sb = s_s[I % 2, u, 2 * J], s_s[I % 2, u, 2 * J + 1]
                scores[2 * I + u, 2 * J] = s_s[I % 2, u, 2 * J]
                scores[2 * I + u, 2 * J + 1] = s_s[I % 2, u, 2 * J + 1]
                mx = jnp.maximum(sa, sb)
                rmax[2 * I + u] = jnp.maximum(rmax[2 * I + u], mx) if 2 * I + u in rmax else mx

        def score_diag(I):
            a, b = 2 * I, 2 * I + 1
            q4 = q_tiles(I)
            qa, qb = jnp.concatenate(q4[0:2], axis=1), jnp.concatenate(q4[2:4], axis=1)
            d1 = _dot_nt(jnp.concatenate([qa, qb], axis=0), k_tile(a))
            d2 = _dot_nt(qb, k_tile(b))
            scores[a, a], scores[b, a], scores[b, b] = jnp.where(tri, d1[:T], NEG), d1[T:], jnp.where(tri, d2, NEG)

        def pv_chunk(i, c0):
            if c0 == 0:
                mx = functools.reduce(jnp.maximum, ([rmax[i]] if i > 1 else [])
                                      + [scores[i, t] for t in range(i // 2 * 2, i + 1)])
                soft[i] = dict(m=jnp.max(mx, axis=1, keepdims=True), l=None, ctx=None)
            st = soft[i]
            c1 = min(c0 + 2, i + 1)
            p = jnp.exp2(jnp.concatenate([scores.pop((i, t)) for t in range(c0, c1)], axis=1) - st['m']).astype(bf)
            pf = p.astype(f32)
            for t in range(c1 - c0):
                st['l'] = pf[:, t * T:(t + 1) * T] if st['l'] is None else st['l'] + pf[:, t * T:(t + 1) * T]
            d = _dot(p, v_tiles(c0, c1))
            st['ctx'] = d if st['ctx'] is None else st['ctx'] + d

        def context(i):
            st = soft.pop(i)
            l = jnp.sum(st['l'], axis=1, keepdims=True)
            r = pl.reciprocal(l, approx=True)
            return st['ctx'] * (r * (2.0 - l * r))

        def accumulate(i, a0, d):
            a = acc_s[i, a0:a0 + d.shape[0], :] + g_s[i][1:2, :] * d
            acc_s[i, a0:a0 + d.shape[0], :] = a
            out_s[i, a0:a0 + d.shape[0], :] = a.astype(bf)

        def out_proj(blocks):
            wo = wo_s[h]
            if len(blocks) == 2:
                ctx = jnp.concatenate([context(i) for i in blocks], axis=0).astype(bf)
                d = _dot_nt(wo, ctx)
                accumulate(blocks[0], 0, d[:, :T])
                accumulate(blocks[1], 0, d[:, T:])
            else:
                ctx = context(blocks[0]).astype(bf)
                for a0 in (0, HM):
                    accumulate(blocks[0], a0, _dot_nt(wo[a0:a0 + HM], ctx))

            @pl.when(h == H - 1)
            def _():
                for i in blocks:
                    cp_out(i).start()

        ops = {'m': kv_product, 'r': score_block, 'd': lambda I, _: score_diag(I), 'p': pv_chunk,
               'D': lambda i, _: out_proj([i, i + 1]), 'S': lambda i, _: out_proj([i])}
        for op, i, c in prog:
            ops[op](i, c)
        assert t_pace.finished()
        for m in range(2):
            @pl.when(jnp.logical_and((h + 3) >> 1 < NP, par == 1 - m))
            def _():
                cp_kv((h + 3) >> 1, m).start()
        return carry

    lax.fori_loop(0, H, head, 0)
    for i in range(NQ):
        cp_out(i).wait()


@jax.jit
def pallas_gated_mix__compressed_kv_cla__moe_arch_mod__prompt_kernel(
    A_x: jax.Array,
    A_c_kv: jax.Array,
    A_w_q: jax.Array,
    A_w_uk: jax.Array,
    A_w_uv: jax.Array,
    A_w_o: jax.Array,
    B_x: jax.Array,
    B_w_r: jax.Array,
    B_w_gate: jax.Array,
    B_w_up: jax.Array,
    B_w_down: jax.Array,
    gate_w: jax.Array,
):
    del B_x
    V = pltpu.VMEM
    B = lambda *shape: V(shape[:-2] + (shape[-2] // 2, shape[-1]), u32)
    out_t = pl.pallas_call(
        _kernel,
        in_specs=[pl.BlockSpec(memory_space=pl.ANY)] * 11,
        out_specs=pl.BlockSpec(memory_space=pl.ANY),
        out_shape=jax.ShapeDtypeStruct((M, S), bf),
        scratch_shapes=[
            V((M, S), bf), V((2, S, HM), bf), B(5, HS, HM),
            B(S, DC), B(49, QS, QC),
            V((NP, M, D), u32), V((2, 2, DC, D), u32), B(H, M, D),
            B(H, S, D), B(H, HS, 5 * T),
            V((NQ, M, T), f32),
            B(M, F), B(M, F), B(M, F),
            V((M,), bf), V((M,), bf), V((NQ, M, T), bf),
            V((NQ, 8, T), f32), B(2, 16, HM), V((16, T), f32),
            pltpu.SMEM((2,), jnp.int32),
            V((2, 2, NQ, T, T), f32), B(QC, 2 * T),
            pltpu.SemaphoreType.DMA((NSEM,)),
        ],
        compiler_params=pltpu.CompilerParams(vmem_limit_bytes=110 * 1024 * 1024),
        name="gated_mix_cla_mod",
    )(A_x[0].T, A_c_kv[0], A_w_q, A_w_uk, A_w_uv, A_w_o.transpose(0, 2, 1), B_w_r, B_w_gate, B_w_up,
      B_w_down.T, gate_w)
    return out_t.T[None]
```

```python
import functools
import math

import jax
import jax.numpy as jnp
from jax import lax
from jax.experimental import pallas as pl
from jax.experimental.pallas import tpu as pltpu

S, M, H, D, DC, F = 2048, 448, 16, 256, 1024, 1792
T = 128
NP, NQ = H // 2, S // T
HS, HM, HC = S // 2, M // 2, DC // 2
QS, QC = S // 4, DC // 4
RB = 16
XC = 256
NG = 5
NT = (((1,), (1,)), ((), ()))
QSCALE = D ** -0.5 * math.log2(math.e)
NEG = -1e30
bf, f32, u32 = jnp.bfloat16, jnp.float32, jnp.uint32
HI = 0xFFFF0000

SEM_WO, SEM_FFN, SEM_VEC, SEM_KV, SEM_WQ, SEM_XT, SEM_C, SEM_OUT, NSEM = 0, 1, 4, 6, 8, 16, 24, 32, 48


def _lhs_terms(a11, a12, a21, a22):
    return [a11 + a22, a21 + a22, a11, a22, a11 + a12, a21 - a11, a12 - a22]


def _rhs_terms(b11, b12, b21, b22):
    return [b11 + b22, b11, b12 - b22, b21 - b11, b22, b11 + b12, b21 + b22]


def _strassen(mm):
    m2, m3, m4, m5, m1, m7, m6 = [mm(i) for i in (1, 2, 3, 4, 0, 6, 5)]
    return (m4 - m5) + (m1 + m7), m3 + m5, m2 + m4, (m3 - m2) + (m1 + m6)


def _lhs_terms2(a11, a12, a21, a22):
    h21, q21, h22 = 0.5 * a21, 0.25 * a21, 0.5 * a22
    s1 = a11 + a22
    v, hs = a12 + q21, 0.5 * s1
    return [s1, q21 + h22, a11 + h21, h22 - q21, v + hs, h21 - a11, v - hs]


def _rhs_terms2(b11, b12, b21, b22):
    h21 = 0.5 * b21
    t1 = b11 + b22
    v, ht = b12 + 0.5 * h21, 0.5 * t1
    return [t1, b11 + h21, v - ht, h21 - b11, b22 - h21, v + ht, b22 + h21]


def _vregs(vals):
    ts = []
    for v in vals:
        v = v if v.dtype == u32 else pltpu.bitcast(v, u32)
        ts += [v[r:r + 8, c:c + T] for r in range(0, v.shape[0], 8) for c in range(0, v.shape[1] - T + 1, T)]
    return ts


def _zero_from(ts):
    acc = ts[:4]
    for i, t in enumerate(ts[4:]):
        acc[i % 4] = acc[i % 4] | t
    while len(acc) > 1:
        acc = [acc[i] | acc[i + 1] if i + 1 < len(acc) else acc[i] for i in range(0, len(acc), 2)]
    return (acc[0] >> 16) >> 16


def _feed(a, *zs):
    zs = [z for z in zs if z is not None]
    if not zs:
        return a
    a32 = pltpu.bitcast(a, u32)
    top = functools.reduce(lambda p, q: p | q, zs, a32[0:8, :T])
    if a32.shape[1] > T:
        top = jnp.concatenate([top, a32[0:8, T:]], axis=1)
    return pltpu.bitcast(jnp.concatenate([top, a32[8:]], axis=0), bf)


class _Pacer:
    def __init__(self, thunks, per, first, last):
        self.thunks, self.pool, self.k, self.done = list(thunks), [], 0, 0
        self.tot, self.first, self.last = per * len(self.thunks), first, last

    def __call__(self):
        self.k += 1
        if self.k <= self.first:
            return None
        want = min(self.tot, -(-(self.k - self.first) * self.tot // (self.last - self.first))) - self.done
        while len(self.pool) < want and self.thunks:
            self.pool += _vregs(self.thunks.pop(0)())
        outs, self.pool = self.pool[:want], self.pool[want:]
        self.done += len(outs)
        return _zero_from(outs) if outs else None

    def finished(self):
        return not self.thunks and not self.pool


_HEAD_ORDER = """
m1.1 m1.3 m1.4 m1.6 m1.0 m1.2 m3.1 m3.3 m3.4 m1.5 m3.6 m3.0 m3.5 m4.1 m4.4 m4.3 m6.6 m4.6 m4.0 m3.2 m4.5 m6.1
m6.4 m6.3 m4.2 m6.0 m6.2 m6.5 m0.6 m0.4 m0.1 m0.3 m0.0 m0.2 m0.5 m2.1 d0 m2.3 r7.0 m2.4 r7.1 m2.0 m2.6 m5.1 r7.2
m2.2 r7.3 r7.4 m2.5 r7.5 r7.6 m5.3 d7 m5.4 m5.6 m5.0 m5.2 m5.5 r6.0 p0.0 p1.0 r6.1 r6.2 p14.0 p14.2 p14.4 p14.6
p14.8 p14.10 r6.3 p14.12 p15.0 p14.14 p15.2 p15.4 r6.4 r6.5 p15.6 p15.8 p15.10 d6 p12.0 p15.12 p15.14 r5.0 p12.2
p12.4 p12.6 p12.8 r5.2 p13.0 p12.10 r5.1 r5.3 p12.12 p13.2 p13.4 p13.6 r5.4 p13.8 d5 D0 p13.10 p10.0 p13.12
p10.2 r4.0 p10.4 r4.1 p10.6 p10.8 p11.0 p10.10 r4.2 p11.2 p11.4 p11.6 r4.3 d4 D14 p11.8 p11.10 p8.0 p8.2 p8.4
r3.0 p8.6 p9.0 r3.1 p8.8 p9.2 p9.4 r3.2 d3 D12 r2.0 p9.6 p9.8 p6.0 p6.2 p6.4 p6.6 p7.0 r2.1 p7.2 d2 D10 p4.0
r1.0 p7.4 p7.6 p4.2 p5.0 p4.4 d1 p2.0 p5.2 p3.0 D8 p2.2 p5.4 p3.2 S2 D4 D6 S3
"""


def _head_program():
    return [(t[0],) + tuple(int(v) for v in t[1:].split('.')) for t in _HEAD_ORDER.split()]


def _dot(a, b):
    return jnp.dot(a, b, preferred_element_type=f32)


def _dot_nt(a, b):
    return lax.dot_general(a, b, NT, preferred_element_type=f32)


def _unpack(w32, sh):
    return pltpu.bitcast((w32 << sh) & jnp.uint32(HI), f32)


class _Bf16:
    def __init__(self, raw):
        self.raw = raw

    def _half(self, idx):
        idx = list(idx if isinstance(idx, tuple) else (idx,))
        idx += [slice(None)] * (len(self.raw.shape) - len(idx))
        r = idx[-2]
        if isinstance(r, slice):
            idx[-2] = slice(None if r.start is None else r.start // 2, None if r.stop is None else r.stop // 2)
        elif isinstance(r.start, int):
            idx[-2] = pl.ds(r.start // 2, r.size // 2)
        else:
            idx[-2] = pl.ds(pl.multiple_of(r.start >> 1, 8), r.size // 2)
        return tuple(idx)

    def __getitem__(self, idx):
        return pltpu.bitcast(self.raw[self._half(idx)], bf)

    def put(self, idx, v):
        idx = self._half(idx)
        ref = self.raw.at[idx[:-2]] if len(idx) > 2 else self.raw
        o = pltpu.bitcast(v, u32)
        ref[idx[-2], idx[-1]] = o
        return o

    def __setitem__(self, idx, v):
        self.put(idx, v)


def _kernel(xt_hbm, c_hbm, wq_hbm, wk_hbm, wv_hbm, wo_hbm, wr_hbm, wg_hbm, wu_hbm, wd_hbm, gw_hbm, o_hbm,
            xt_s, x_s, xa_r, c_r, ca_r, wq_p, wkv_p, wo_r, q_r, qa_r, acc_s, wg_r, wu_r, wd_r,
            wr_s, gw_s, out_s, g_s, xs_r, rsel_s, idx_s, s_s, t0_r, sem):
    xa_s, c_s, ca_s, wo_s, q_s, qa_s, wg_s, wu_s, wd_s, xs_s, t0_s = [
        _Bf16(r) for r in (xa_r, c_r, ca_r, wo_r, q_r, qa_r, wg_r, wu_r, wd_r, xs_r, t0_r)]
    mk = pltpu.make_async_copy
    wq32, wk32, wv32 = wq_hbm.bitcast(u32), wk_hbm.bitcast(u32), wv_hbm.bitcast(u32)
    cp_wq = lambda j: mk(wq32.at[:, j, :], wq_p.at[j], sem.at[SEM_WQ + j])
    cp_kv = lambda j, m: mk((wk32, wv32)[m].at[:, j, :], wkv_p.at[j & 1, m], sem.at[SEM_KV + m])
    cp_xt = lambda k: mk(xt_hbm.at[:, pl.ds(k * XC, XC)], xt_s.at[:, pl.ds(k * XC, XC)], sem.at[SEM_XT + k])
    cp_out = lambda i: mk(out_s.at[i], o_hbm.at[:, pl.ds(i * T, T)], sem.at[SEM_OUT + i])
    cp_vec = [mk(wr_hbm, wr_s, sem.at[SEM_VEC]), mk(gw_hbm, gw_s, sem.at[SEM_VEC + 1])]
    cp_ffn = [mk(src, dst, sem.at[SEM_FFN + n]) for n, (src, dst) in
              enumerate(((wg_hbm.bitcast(u32), wg_r), (wu_hbm.bitcast(u32), wu_r), (wd_hbm.bitcast(u32), wd_r)))]
    cp_wo = mk(wo_hbm.bitcast(u32), wo_r, sem.at[SEM_WO])
    c32 = c_hbm.bitcast(u32)

    def cp_c(j):
        r0 = (j - 1) * (NG * RB // 2)
        n = QS // 2 - r0 if isinstance(j, int) and j == NP - 1 else NG * RB // 2
        return [mk(c32.at[pl.ds(i * QS // 2 + r0, n)], c_r.at[pl.ds(i * QS // 2 + r0, n)], sem.at[SEM_C + j])
                for i in range(4)]

    cp_xt(0).start()
    cp_wq(0).start()
    for k in range(1, S // XC):
        cp_xt(k).start()
    for cp in cp_vec:
        cp.start()
    for j in range(1, NP):
        cp_wq(j).start()
        for cp in cp_c(j):
            cp.start()
    for cp in cp_ffn + [cp_kv(0, 0), cp_kv(0, 1), cp_wo]:
        cp.start()

    def store_q(j, e, r0, q):
        q = q * QSCALE
        q_s[2 * j + e, r0:r0 + q.shape[0], :] = q.astype(bf)
        for p0 in range(0, q.shape[0], 2 * T):
            if r0 + p0 > 0:
                qa, qb = q[p0:p0 + T], q[p0 + T:p0 + 2 * T]
                terms = _lhs_terms(qa[:, :T], qa[:, T:], qb[:, :T], qb[:, T:])
                for k, i in enumerate((0, 1, 4, 5, 6)):
                    qa_s[2 * j + e, (r0 + p0) // 2:(r0 + p0) // 2 + T, k * T:(k + 1) * T] = terms[i].astype(bf)

    def q_plain(w, r0, hook=None):
        prod = lambda a, b, wn, z: _dot(_feed(x_s[0, a:b, :], z), wn[:HM]) + _dot(x_s[1, a:b, :], wn[HM:])
        if hook is None:
            qf = prod(r0, r0 + 2 * T, w, None)
        else:
            qf = jnp.concatenate([jnp.concatenate(
                [prod(r0 + u * T, r0 + (u + 1) * T, w[:, n * T:(n + 1) * T], hook()) for u in range(2)], axis=0)
                for n in range(4)], axis=1)
        store_q(0, 0, r0, qf[:, :D])
        store_q(0, 1, r0, qf[:, D:])

    def q_rhs(j):
        lo, hi = pltpu.bitcast(wq_p[j] << 16, f32), pltpu.bitcast(wq_p[j] & jnp.uint32(HI), f32)
        return [t.astype(bf) for t in _rhs_terms(lo[:HM], hi[:HM], lo[HM:], hi[HM:])]

    def q_strassen(j, ts, r0, r1, hook):
        def lhs(i, u):
            if i in (2, 3):
                return x_s[i - 2, (i - 2) * HS + u:(i - 2) * HS + u + T, :]
            return xa_s[i - 2 * (i > 3), u:u + T, :]
        cs = _strassen(lambda i: jnp.concatenate(
            [_dot(_feed(lhs(i, u), *hook()), ts[i]) for u in range(r0, r1, T)], axis=0))
        for n, c in enumerate(cs):
            store_q(j, n % 2, (n // 2) * HS + r0, c)

    def x_prep(r0):
        a = [x_s[e, h0 + r0:h0 + r0 + RB, :].astype(f32) for h0 in (0, HS) for e in (0, 1)]
        terms = _lhs_terms(*a)
        outs = []
        for k, i in enumerate((0, 1, 4, 5, 6)):
            outs.append(xa_s.put((k, slice(r0, r0 + RB)), terms[i].astype(bf)))
        return outs

    def c_prep(g, c0):
        blk = lambda i, k: c_s[pl.ds(i * QS + g * RB, RB), k * QC + c0:k * QC + c0 + T].astype(f32)
        outer = [_lhs_terms2(*[blk(2 * i1 + i2, 2 * k1 + k2) for i1 in range(2) for k1 in range(2)])
                 for i2 in range(2) for k2 in range(2)]
        outs = []
        for r1 in range(7):
            for r2, v in enumerate(_lhs_terms(*[o[r1] for o in outer])):
                outs.append(ca_s.put((7 * r1 + r2, pl.ds(g * RB, RB), slice(c0, c0 + T)), v.astype(bf)))
        return outs

    def c_pacer(g0, ng, first, last):
        return _Pacer([functools.partial(c_prep, g0 + t // 2, (t % 2) * T) for t in range(2 * ng)], 49, first, last)

    def transpose(k):
        for e in range(2):
            x_s[e, k * XC:(k + 1) * XC, :] = xt_s[e * HM:(e + 1) * HM, k * XC:(k + 1) * XC].T

    def q_w0():
        return jnp.concatenate([pltpu.bitcast(wq_p[0] << 16, f32).astype(bf),
                                pltpu.bitcast(wq_p[0] & jnp.uint32(HI), f32).astype(bf)], axis=1)

    cp_xt(0).wait()
    transpose(0)
    cp_wq(0).wait()
    q_plain(q_w0(), 0)
    for k in range(1, 4):
        cp_xt(k).wait()
    transpose(1)
    w0 = q_w0()
    transpose(2)
    q_plain(w0, XC)
    transpose(3)
    q_plain(w0, 2 * XC)
    for k in range(4, S // XC):
        cp_xt(k).wait()
    for cp in cp_vec:
        cp.wait()
    for k in range(4, S // XC):
        transpose(k)
    row8 = lax.broadcasted_iota(jnp.int32, (8, M), 0)
    x_pace = _Pacer([functools.partial(x_prep, r0) for r0 in range(0, HS, RB)], 5, 12, 40)
    routed = []

    def hook0():
        n = len(routed)
        if n < NQ:
            rg = jnp.where(row8 == 0, wr_s[...].reshape(1, M).astype(f32), gw_s[...].reshape(1, M).astype(f32))
            g_s[n] = _dot(rg.astype(bf), xt_s[:, n * T:(n + 1) * T])
            routed.append(n)
        return x_pace()
    w0 = q_w0()
    for k in range(3, S // XC):
        q_plain(w0, k * XC, hook0)
    assert x_pace.finished()

    rb = jnp.concatenate([g_s[n][0:1, :] for n in range(NQ)], axis=1).astype(bf).astype(f32)
    lane = lax.broadcasted_iota(jnp.int32, (1, S), 1)
    m1 = jnp.max(rb, axis=1, keepdims=True)
    i1 = jnp.minimum(jnp.min(jnp.where(rb == m1, lane, S)), S - 1)
    rb2 = jnp.where(lane == i1, -jnp.inf, rb)
    m2 = jnp.max(rb2, axis=1, keepdims=True)
    i2 = jnp.minimum(jnp.min(jnp.where(jnp.logical_and(rb2 == m2, lane != i1), lane, S)), S - 1)
    row16 = lax.broadcasted_iota(jnp.int32, (16, HM), 0)

    def x_row(e, i):
        blk = x_s[e, pl.ds(pl.multiple_of((i // 16) * 16, 16), 16), :].astype(f32)
        return jnp.sum(jnp.where(row16 == i % 16, blk, 0.0), axis=0, keepdims=True)
    for e in range(2):
        xs_s[e] = jnp.where(row16 == 0, x_row(e, i1), jnp.where(row16 == 1, x_row(e, i2), 0.0)).astype(bf)
    rsel_s[...] = jax.nn.sigmoid(jnp.where(lax.broadcasted_iota(jnp.int32, (16, T), 0) == 0, m1, m2))
    idx_s[0] = i1
    idx_s[1] = i2

    def q_body(it, carry):
        js = (2 * it + 1, 2 * it + 2)
        for j in js:
            for cp in [cp_wq(j)] + cp_c(j):
                cp.wait()
        pace = c_pacer(2 * it * NG, 2 * NG, 1, 112)
        for j in js:
            q_strassen(j, q_rhs(j), 0, HS, lambda: (pace(),))
        assert pace.finished()
        return carry
    lax.fori_loop(0, 3, q_body, 0)

    for cp in cp_ffn + [cp_wq(NP - 1)] + cp_c(NP - 1):
        cp.wait()

    def residual(n):
        g8 = jax.nn.sigmoid(g_s[n])
        g_s[n] = g8
        a = (1.0 - g8[1:2, :]) * xt_s[:, n * T:(n + 1) * T].astype(f32)
        acc_s[n] = a
        return [a]

    gs, us, ys, hid = [], [], {}, []
    xs_dot = lambda w_s, n: (_dot(xs_s[0], w_s[:HM, n * T:(n + 1) * T]) + _dot(xs_s[1], w_s[HM:, n * T:(n + 1) * T]))

    def swiglu():
        gg, uu = jnp.concatenate(gs, axis=1), jnp.concatenate(us, axis=1)
        hid.append((gg * jax.nn.sigmoid(gg) * uu).astype(bf))

    def down(n0, k0):
        t = _dot_nt(hid[0][:, k0:min(k0 + 512, F)], wd_s[n0:min(n0 + T, M), k0:min(k0 + 512, F)])
        ys[n0] = ys[n0] + t if n0 in ys else t
    side = []
    for n in range(F // T):
        side += [lambda n=n: gs.append(xs_dot(wg_s, n)), lambda n=n: us.append(xs_dot(wu_s, n))]
    side += [swiglu] + [lambda: None] * 7
    side += [functools.partial(down, n0, k0) for n0 in range(0, M, T) for k0 in range(0, F, 512)]
    c_pace = c_pacer((NP - 2) * NG, QS // RB - (NP - 2) * NG, 2, 56)
    r_pace = _Pacer([functools.partial(residual, n) for n in range(NQ)], M // 8, 1, 48)

    def hook7():
        if side:
            side.pop(0)()
        return c_pace(), r_pace()
    ts7 = q_rhs(NP - 1)
    for r0 in range(0, HS, 2 * T):
        q_strassen(NP - 1, ts7, r0, r0 + 2 * T, hook7)
    assert not side and c_pace.finished() and r_pace.finished()
    y = jnp.concatenate([ys[n0] for n0 in range(0, M, T)] + [jnp.zeros((16, 512 - M), f32)], axis=1)
    yt = (y * rsel_s[:, 0:1]).T
    lane128 = lax.broadcasted_iota(jnp.int32, (1, T), 1)
    for e in range(2):
        i = idx_s[e]
        acc_s[i // T] += jnp.where(lane128 == i % T, (1.0 - g_s[i // T][1:2, :]) * yt[:M, e:e + 1], 0.0)

    cp_wo.wait()
    cp_kv(0, 0).wait()
    cp_kv(1, 0).start()

    def first_terms(hn):
        w = _unpack(wkv_p[(hn >> 1) & 1, 0, :, :T], (16 * (1 - (hn & 1))).astype(u32))
        t = w[:HC] + 0.5 * w[HC:]
        return [t0_s.put((slice(None), slice(n * T, (n + 1) * T)), v.astype(bf))
                for n, v in enumerate((t[:QC], t[QC:] - t[:QC]))]
    first_terms(jnp.int32(0))

    tri = lax.broadcasted_iota(jnp.int32, (T, T), 1) <= lax.broadcasted_iota(jnp.int32, (T, T), 0)
    prog = _head_program()

    def head(h, carry):
        par, slot = h & 1, (h >> 1) & 1
        for m in range(2):
            @pl.when(jnp.logical_and(h < H - 1, par == 1 - m))
            def _():
                cp_kv((h + 1) >> 1, m).wait()

        sh = (16 * (1 - par)).astype(u32)
        rhs = []
        for r1 in range(7):
            wk, wv = [_unpack(wkv_p[slot, m], sh + (h >> (8 + r1)).astype(u32)) for m in range(2)]
            t = _rhs_terms2(wk[:HC], wv[:HC], wk[HC:], wv[HC:])[r1]
            rhs.append([u.astype(bf) for u in _rhs_terms(t[:QC, :T], t[:QC, T:], t[QC:, :T], t[QC:, T:])])
        rhs[1][1], rhs[1][3] = t0_s[:, :T], t0_s[:, T:]
        t_pace = _Pacer([lambda: first_terms(jnp.minimum(h + 1, H - 1))], 32, 196 - 14, 196)
        prods, inner_q, outer, kblk, vblk = {}, {}, {}, {}, {}

        def kv_product(r1, r2):
            m = prods.setdefault(r1, {})
            m[r2] = _dot(ca_s[7 * r1 + r2], rhs[r1][r2])
            if len(m) == 7:
                inner_q[r1] = (((m[3] - m[4]) + m[6]) + m[0], m[2] + m[4], m[1] + m[3], ((m[0] - m[1]) + m[2]) + m[5])
                for b in range(4):
                    if b not in kblk and all(q in inner_q for q in (0, 1, 3, 4, 6)):
                        p = {q: inner_q[q][b] for q in (0, 1, 3, 4, 6)}
                        e, d = p[3] + p[1], p[3] - p[1]
                        kblk[b] = (p[0] + ((d - p[4]) + p[6]), e * 2.0)
                        outer[b] = ((e + p[4]) + p[6], p[0] + d)
                    if len(inner_q) == 7:
                        p2, p5 = inner_q[2][b], inner_q[5][b]
                        vblk[b] = (((outer[b][0] + p2) - p5) * 0.5, (outer[b][1] + p2) + p5)

        def rows(blk, t0, t1):
            return jnp.concatenate([jnp.concatenate(
                [blk[2 * (t // 4 % 2) + j2][t // 8][t % 4 * T:(t % 4 + 1) * T] for j2 in range(2)], axis=1)
                for t in range(t0, t1)], axis=0)

        @functools.cache
        def k_tile(t):
            return rows(kblk, t, t + 1).astype(bf)

        @functools.cache
        def k_terms(J):
            ka, kb = rows(kblk, 2 * J, 2 * J + 1), rows(kblk, 2 * J + 1, 2 * J + 2)
            return [t.astype(bf) for t in _rhs_terms(ka[:, :T], kb[:, :T], ka[:, T:], kb[:, T:])]

        @functools.cache
        def v_tiles(c0, c1):
            return rows(vblk, c0, c1).astype(bf)

        scores, rmax, soft = {}, {}, {}
        q_tiles = lambda I: [q_s[h, i * T:(i + 1) * T, t * T:(t + 1) * T] for i in (2 * I, 2 * I + 1) for t in range(2)]

        def score_block(I, J):
            q4, qx = q_tiles(I), [qa_s[h, I * T:(I + 1) * T, k * T:(k + 1) * T] for k in range(5)]
            lhs = [qx[0], qx[1], q4[0], q4[3], qx[2], qx[3], qx[4]]
            cs = _strassen(lambda i: _dot_nt(_feed(lhs[i], t_pace()), k_terms(J)[i]))
            for n, c in enumerate(cs):
                s_s[I % 2, n // 2, 2 * J + n % 2] = c
            for u in range(2):
                sa, sb = s_s[I % 2, u, 2 * J], s_s[I % 2, u, 2 * J + 1]
                scores[2 * I + u, 2 * J] = s_s[I % 2, u, 2 * J]
                scores[2 * I + u, 2 * J + 1] = s_s[I % 2, u, 2 * J + 1]
                mx = jnp.maximum(sa, sb)
                rmax[2 * I + u] = jnp.maximum(rmax[2 * I + u], mx) if 2 * I + u in rmax else mx

        def score_diag(I):
            a, b = 2 * I, 2 * I + 1
            q4 = q_tiles(I)
            qa, qb = jnp.concatenate(q4[0:2], axis=1), jnp.concatenate(q4[2:4], axis=1)
            d1 = _dot_nt(jnp.concatenate([qa, qb], axis=0), k_tile(a))
            d2 = _dot_nt(qb, k_tile(b))
            scores[a, a], scores[b, a], scores[b, b] = jnp.where(tri, d1[:T], NEG), d1[T:], jnp.where(tri, d2, NEG)

        def pv_chunk(i, c0):
            if c0 == 0:
                mx = functools.reduce(jnp.maximum, ([rmax[i]] if i > 1 else [])
                                      + [scores[i, t] for t in range(i // 2 * 2, i + 1)])
                soft[i] = dict(m=jnp.max(mx, axis=1, keepdims=True), l=None, ctx=None)
            st = soft[i]
            c1 = min(c0 + 2, i + 1)
            p = jnp.exp2(jnp.concatenate([scores.pop((i, t)) for t in range(c0, c1)], axis=1) - st['m']).astype(bf)
            pf = p.astype(f32)
            for t in range(c1 - c0):
                st['l'] = pf[:, t * T:(t + 1) * T] if st['l'] is None else st['l'] + pf[:, t * T:(t + 1) * T]
            d = _dot(p, v_tiles(c0, c1))
            st['ctx'] = d if st['ctx'] is None else st['ctx'] + d

        def context(i):
            st = soft.pop(i)
            l = jnp.sum(st['l'], axis=1, keepdims=True)
            r = pl.reciprocal(l, approx=True)
            return st['ctx'] * (r * (2.0 - l * r))

        def accumulate(i, a0, d):
            a = acc_s[i, a0:a0 + d.shape[0], :] + g_s[i][1:2, :] * d
            acc_s[i, a0:a0 + d.shape[0], :] = a
            out_s[i, a0:a0 + d.shape[0], :] = a.astype(bf)

        def out_proj(blocks):
            wo = wo_s[h]
            if len(blocks) == 2:
                ctx = jnp.concatenate([context(i) for i in blocks], axis=0).astype(bf)
                d = _dot_nt(wo, ctx)
                accumulate(blocks[0], 0, d[:, :T])
                accumulate(blocks[1], 0, d[:, T:])
            else:
                ctx = context(blocks[0]).astype(bf)
                for a0 in (0, HM):
                    accumulate(blocks[0], a0, _dot_nt(wo[a0:a0 + HM], ctx))

            @pl.when(h == H - 1)
            def _():
                for i in blocks:
                    cp_out(i).start()

        ops = {'m': kv_product, 'r': score_block, 'd': score_diag, 'p': pv_chunk,
               'D': lambda i: out_proj([i, i + 1]), 'S': lambda i: out_proj([i])}
        for op, *args in prog:
            ops[op](*args)
        assert t_pace.finished()
        for m in range(2):
            @pl.when(jnp.logical_and((h + 3) >> 1 < NP, par == 1 - m))
            def _():
                cp_kv((h + 3) >> 1, m).start()
        return carry

    lax.fori_loop(0, H, head, 0)
    for i in range(NQ):
        cp_out(i).wait()


@jax.jit
def pallas_gated_mix__compressed_kv_cla__moe_arch_mod__prompt_kernel(
    A_x: jax.Array,
    A_c_kv: jax.Array,
    A_w_q: jax.Array,
    A_w_uk: jax.Array,
    A_w_uv: jax.Array,
    A_w_o: jax.Array,
    B_x: jax.Array,
    B_w_r: jax.Array,
    B_w_gate: jax.Array,
    B_w_up: jax.Array,
    B_w_down: jax.Array,
    gate_w: jax.Array,
):
    del B_x
    V = pltpu.VMEM
    B = lambda *shape: V(shape[:-2] + (shape[-2] // 2, shape[-1]), u32)
    out_t = pl.pallas_call(
        _kernel,
        in_specs=[pl.BlockSpec(memory_space=pl.ANY)] * 11,
        out_specs=pl.BlockSpec(memory_space=pl.ANY),
        out_shape=jax.ShapeDtypeStruct((M, S), bf),
        scratch_shapes=[
            V((M, S), bf), V((2, S, HM), bf), B(5, HS, HM),
            B(S, DC), B(49, QS, QC),
            V((NP, M, D), u32), V((2, 2, DC, D), u32), B(H, M, D),
            B(H, S, D), B(H, HS, 5 * T),
            V((NQ, M, T), f32),
            B(M, F), B(M, F), B(M, F),
            V((M,), bf), V((M,), bf), V((NQ, M, T), bf),
            V((NQ, 8, T), f32), B(2, 16, HM), V((16, T), f32),
            pltpu.SMEM((2,), jnp.int32),
            V((2, 2, NQ, T, T), f32), B(QC, 2 * T),
            pltpu.SemaphoreType.DMA((NSEM,)),
        ],
        compiler_params=pltpu.CompilerParams(vmem_limit_bytes=110 * 1024 * 1024),
        name="gated_mix_cla_mod",
    )(A_x[0].T, A_c_kv[0], A_w_q, A_w_uk, A_w_uv, A_w_o.transpose(0, 2, 1), B_w_r, B_w_gate, B_w_up,
      B_w_down.T, gate_w)
    return out_t.T[None]
```

```python
import functools
import math

import jax
import jax.numpy as jnp
from jax import lax
from jax.experimental import pallas as pl
from jax.experimental.pallas import tpu as pltpu

S, M, H, D, DC, F = 2048, 448, 16, 256, 1024, 1792
T = 128
NP, NQ = H // 2, S // T
HS, HM, HC = S // 2, M // 2, DC // 2
QS, QC = S // 4, DC // 4
RB = 16
XC = 256
NG = 5
NT = (((1,), (1,)), ((), ()))
QSCALE = D ** -0.5 * math.log2(math.e)
NEG = -1e30
bf, f32, u32 = jnp.bfloat16, jnp.float32, jnp.uint32
HI = 0xFFFF0000

SEM_WO, SEM_FFN, SEM_VEC, SEM_KV, SEM_WQ, SEM_XT, SEM_C, SEM_OUT, NSEM = 0, 1, 4, 6, 8, 16, 24, 32, 48


def _lhs_terms(a11, a12, a21, a22):
    return [a11 + a22, a21 + a22, a11, a22, a11 + a12, a21 - a11, a12 - a22]


def _rhs_terms(b11, b12, b21, b22):
    return [b11 + b22, b11, b12 - b22, b21 - b11, b22, b11 + b12, b21 + b22]


def _strassen(mm):
    m2, m3, m4, m5, m1, m7, m6 = [mm(i) for i in (1, 2, 3, 4, 0, 6, 5)]
    return (m4 - m5) + (m1 + m7), m3 + m5, m2 + m4, (m3 - m2) + (m1 + m6)


def _lhs_terms2(a11, a12, a21, a22):
    h21, q21, h22 = 0.5 * a21, 0.25 * a21, 0.5 * a22
    s1 = a11 + a22
    v, hs = a12 + q21, 0.5 * s1
    return [s1, q21 + h22, a11 + h21, h22 - q21, v + hs, h21 - a11, v - hs]


def _rhs_terms2(b11, b12, b21, b22):
    h21 = 0.5 * b21
    t1 = b11 + b22
    v, ht = b12 + 0.5 * h21, 0.5 * t1
    return [t1, b11 + h21, v - ht, h21 - b11, b22 - h21, v + ht, b22 + h21]


def _vregs(vals):
    ts = []
    for v in vals:
        v = v if v.dtype == u32 else pltpu.bitcast(v, u32)
        ts += [v[r:r + 8, c:c + T] for r in range(0, v.shape[0], 8) for c in range(0, v.shape[1] - T + 1, T)]
    return ts


def _zero_from(ts):
    acc = ts[:4]
    for i, t in enumerate(ts[4:]):
        acc[i % 4] = acc[i % 4] | t
    while len(acc) > 1:
        acc = [acc[i] | acc[i + 1] if i + 1 < len(acc) else acc[i] for i in range(0, len(acc), 2)]
    return (acc[0] >> 16) >> 16


def _feed(a, *zs):
    zs = [z for z in zs if z is not None]
    if not zs:
        return a
    a32 = pltpu.bitcast(a, u32)
    top = functools.reduce(lambda p, q: p | q, zs, a32[0:8, :T])
    if a32.shape[1] > T:
        top = jnp.concatenate([top, a32[0:8, T:]], axis=1)
    return pltpu.bitcast(jnp.concatenate([top, a32[8:]], axis=0), bf)


class _Pacer:
    def __init__(self, thunks, per, first, last):
        self.thunks, self.pool, self.k, self.done = list(thunks), [], 0, 0
        self.tot, self.first, self.last = per * len(self.thunks), first, last

    def __call__(self):
        self.k += 1
        if self.k <= self.first:
            return None
        want = min(self.tot, -(-(self.k - self.first) * self.tot // (self.last - self.first))) - self.done
        while len(self.pool) < want and self.thunks:
            self.pool += _vregs(self.thunks.pop(0)())
        outs, self.pool = self.pool[:want], self.pool[want:]
        self.done += len(outs)
        return _zero_from(outs) if outs else None

    def finished(self):
        return not self.thunks and not self.pool


_HEAD_ORDER = """
m1.1 m1.3 m1.4 m1.6 m1.0 m1.2 m3.1 m3.3 m3.4 m1.5 m3.6 m3.0 m3.5 m4.1 m4.4 m4.3 m6.6 m4.6 m4.0 m3.2 m4.5 m6.1
m6.4 m6.3 m4.2 m6.0 m6.2 m6.5 m0.6 m0.4 m0.1 m0.3 m0.0 m0.2 m0.5 m2.1 d0 m2.3 r7.0 m2.4 r7.1 m2.0 m2.6 m5.1 r7.2
m2.2 r7.3 r7.4 m2.5 r7.5 r7.6 m5.3 d7 m5.4 m5.6 m5.0 m5.2 m5.5 r6.0 p1.0 r6.1 p0.0 r6.2 p14.0 p14.2 p14.4 p14.6
p14.8 p14.10 p15.0 p14.12 p14.14 r6.3 p15.2 p15.4 r6.4 r6.5 p15.6 p15.8 p15.10 d6 p15.12 p12.0 p15.14 r5.0 p12.2
p12.4 p12.6 p12.8 r5.2 p13.0 p12.10 r5.3 r5.1 p12.12 r5.4 p13.2 p13.4 p13.6 p13.8 d5 o0.3 o0.1 o0.2 o0.0 o0.5
o0.4 p10.0 o0.6 p13.10 p11.0 r4.1 p13.12 p10.2 r4.0 p10.4 p10.6 p10.8 p11.2 p10.10 r4.2 p11.4 p11.6 r4.3 d4 o7.2
o7.0 o7.1 o7.3 o7.4 o7.6 o7.5 p11.8 p8.0 p11.10 p8.2 p8.4 p8.6 r3.1 r3.0 p9.0 d3 p9.2 p8.8 r3.2 o6.1 o6.3 o6.2
o6.4 p9.4 o6.0 o6.6 o6.5 r2.0 p9.6 r2.1 p9.8 p6.0 p6.2 p6.4 p6.6 p7.0 d2 p7.2 o5.1 o5.2 o5.4 o5.3 o5.6 o5.0 o5.5
p4.0 p5.0 p7.4 r1.0 p4.2 p7.6 p4.4 d1 p2.0 p5.2 o4.1 o4.2 o4.0 o4.4 o4.3 o4.6 o4.5 p2.2 p5.4 p3.0 o2.1 p3.2 S2
o2.3 o2.2 o2.0 o2.4 o2.6 o3.2 o2.5 o3.6 o3.3 o3.1 o3.0 o3.5 o3.4 S3
"""


def _head_program():
    return [(t[0],) + tuple(int(v) for v in t[1:].split('.')) for t in _HEAD_ORDER.split()]


def _dot(a, b):
    return jnp.dot(a, b, preferred_element_type=f32)


def _dot_nt(a, b):
    return lax.dot_general(a, b, NT, preferred_element_type=f32)


def _unpack(w32, sh):
    return pltpu.bitcast((w32 << sh) & jnp.uint32(HI), f32)


class _Bf16:
    def __init__(self, raw):
        self.raw = raw

    def _half(self, idx):
        idx = list(idx if isinstance(idx, tuple) else (idx,))
        idx += [slice(None)] * (len(self.raw.shape) - len(idx))
        r = idx[-2]
        if isinstance(r, slice):
            idx[-2] = slice(None if r.start is None else r.start // 2, None if r.stop is None else r.stop // 2)
        elif isinstance(r.start, int):
            idx[-2] = pl.ds(r.start // 2, r.size // 2)
        else:
            idx[-2] = pl.ds(pl.multiple_of(r.start >> 1, 8), r.size // 2)
        return tuple(idx)

    def __getitem__(self, idx):
        return pltpu.bitcast(self.raw[self._half(idx)], bf)

    def put(self, idx, v):
        idx = self._half(idx)
        ref = self.raw.at[idx[:-2]] if len(idx) > 2 else self.raw
        o = pltpu.bitcast(v, u32)
        ref[idx[-2], idx[-1]] = o
        return o

    def __setitem__(self, idx, v):
        self.put(idx, v)


def _kernel(xt_hbm, c_hbm, wq_hbm, wk_hbm, wv_hbm, wo_hbm, wr_hbm, wg_hbm, wu_hbm, wd_hbm, gw_hbm, o_hbm,
            xt_s, x_s, xa_r, c_r, ca_r, wq_p, wkv_p, wo_r, q_r, qa_r, acc_s, wg_r, wu_r, wd_r,
            wr_s, gw_s, out_s, g_s, xs_r, rsel_s, idx_s, s_s, t0_r, om_s, sem):
    xa_s, c_s, ca_s, wo_s, q_s, qa_s, wg_s, wu_s, wd_s, xs_s, t0_s = [
        _Bf16(r) for r in (xa_r, c_r, ca_r, wo_r, q_r, qa_r, wg_r, wu_r, wd_r, xs_r, t0_r)]
    mk = pltpu.make_async_copy
    wq32, wk32, wv32 = wq_hbm.bitcast(u32), wk_hbm.bitcast(u32), wv_hbm.bitcast(u32)
    cp_wq = lambda j: mk(wq32.at[:, j, :], wq_p.at[j], sem.at[SEM_WQ + j])
    cp_kv = lambda j, m: mk((wk32, wv32)[m].at[:, j, :], wkv_p.at[j & 1, m], sem.at[SEM_KV + m])
    cp_xt = lambda k: mk(xt_hbm.at[:, pl.ds(k * XC, XC)], xt_s.at[:, pl.ds(k * XC, XC)], sem.at[SEM_XT + k])
    cp_out = lambda i: mk(out_s.at[i], o_hbm.at[:, pl.ds(i * T, T)], sem.at[SEM_OUT + i])
    cp_vec = [mk(wr_hbm, wr_s, sem.at[SEM_VEC]), mk(gw_hbm, gw_s, sem.at[SEM_VEC + 1])]
    cp_ffn = [mk(src, dst, sem.at[SEM_FFN + n]) for n, (src, dst) in
              enumerate(((wg_hbm.bitcast(u32), wg_r), (wu_hbm.bitcast(u32), wu_r), (wd_hbm.bitcast(u32), wd_r)))]
    cp_wo = mk(wo_hbm.bitcast(u32), wo_r, sem.at[SEM_WO])
    c32 = c_hbm.bitcast(u32)

    def cp_c(j):
        r0 = (j - 1) * (NG * RB // 2)
        n = QS // 2 - r0 if isinstance(j, int) and j == NP - 1 else NG * RB // 2
        return [mk(c32.at[pl.ds(i * QS // 2 + r0, n)], c_r.at[pl.ds(i * QS // 2 + r0, n)], sem.at[SEM_C + j])
                for i in range(4)]

    cp_xt(0).start()
    cp_wq(0).start()
    for k in range(1, S // XC):
        cp_xt(k).start()
    for cp in cp_vec:
        cp.start()
    for j in range(1, NP):
        cp_wq(j).start()
        for cp in cp_c(j):
            cp.start()
    for cp in cp_ffn + [cp_kv(0, 0), cp_kv(0, 1), cp_wo]:
        cp.start()

    @pl.loop(0, NQ // 2)
    def _(n):
        om_s[n] = jnp.zeros(om_s.shape[1:], f32)

    def store_q(j, e, r0, q):
        q = q * QSCALE
        q_s[2 * j + e, r0:r0 + q.shape[0], :] = q.astype(bf)
        for p0 in range(0, q.shape[0], 2 * T):
            if r0 + p0 > 0:
                qa, qb = q[p0:p0 + T], q[p0 + T:p0 + 2 * T]
                terms = _lhs_terms(qa[:, :T], qa[:, T:], qb[:, :T], qb[:, T:])
                for k, i in enumerate((0, 1, 4, 5, 6)):
                    qa_s[2 * j + e, (r0 + p0) // 2:(r0 + p0) // 2 + T, k * T:(k + 1) * T] = terms[i].astype(bf)

    def q_plain(w, r0, hook=None):
        prod = lambda a, b, wn, z: _dot(_feed(x_s[0, a:b, :], z), wn[:HM]) + _dot(x_s[1, a:b, :], wn[HM:])
        if hook is None:
            qf = prod(r0, r0 + 2 * T, w, None)
        else:
            qf = jnp.concatenate([jnp.concatenate(
                [prod(r0 + u * T, r0 + (u + 1) * T, w[:, n * T:(n + 1) * T], hook()) for u in range(2)], axis=0)
                for n in range(4)], axis=1)
        store_q(0, 0, r0, qf[:, :D])
        store_q(0, 1, r0, qf[:, D:])

    def q_rhs(j):
        lo, hi = pltpu.bitcast(wq_p[j] << 16, f32), pltpu.bitcast(wq_p[j] & jnp.uint32(HI), f32)
        return [t.astype(bf) for t in _rhs_terms(lo[:HM], hi[:HM], lo[HM:], hi[HM:])]

    def q_strassen(j, ts, r0, r1, hook):
        def lhs(i, u):
            if i in (2, 3):
                return x_s[i - 2, (i - 2) * HS + u:(i - 2) * HS + u + T, :]
            return xa_s[i - 2 * (i > 3), u:u + T, :]
        cs = _strassen(lambda i: jnp.concatenate(
            [_dot(_feed(lhs(i, u), *hook()), ts[i]) for u in range(r0, r1, T)], axis=0))
        for n, c in enumerate(cs):
            store_q(j, n % 2, (n // 2) * HS + r0, c)

    def x_prep(r0):
        a = [x_s[e, h0 + r0:h0 + r0 + RB, :].astype(f32) for h0 in (0, HS) for e in (0, 1)]
        terms = _lhs_terms(*a)
        outs = []
        for k, i in enumerate((0, 1, 4, 5, 6)):
            outs.append(xa_s.put((k, slice(r0, r0 + RB)), terms[i].astype(bf)))
        return outs

    def c_prep(g, c0):
        blk = lambda i, k: c_s[pl.ds(i * QS + g * RB, RB), k * QC + c0:k * QC + c0 + T].astype(f32)
        outer = [_lhs_terms2(*[blk(2 * i1 + i2, 2 * k1 + k2) for i1 in range(2) for k1 in range(2)])
                 for i2 in range(2) for k2 in range(2)]
        outs = []
        for r1 in range(7):
            for r2, v in enumerate(_lhs_terms(*[o[r1] for o in outer])):
                outs.append(ca_s.put((7 * r1 + r2, pl.ds(g * RB, RB), slice(c0, c0 + T)), v.astype(bf)))
        return outs

    def c_pacer(g0, ng, first, last):
        return _Pacer([functools.partial(c_prep, g0 + t // 2, (t % 2) * T) for t in range(2 * ng)], 49, first, last)

    def transpose(k):
        for e in range(2):
            x_s[e, k * XC:(k + 1) * XC, :] = xt_s[e * HM:(e + 1) * HM, k * XC:(k + 1) * XC].T

    def q_w0():
        return jnp.concatenate([pltpu.bitcast(wq_p[0] << 16, f32).astype(bf),
                                pltpu.bitcast(wq_p[0] & jnp.uint32(HI), f32).astype(bf)], axis=1)

    cp_xt(0).wait()
    transpose(0)
    cp_wq(0).wait()
    q_plain(q_w0(), 0)
    for k in range(1, 4):
        cp_xt(k).wait()
    transpose(1)
    w0 = q_w0()
    transpose(2)
    q_plain(w0, XC)
    transpose(3)
    q_plain(w0, 2 * XC)
    for k in range(4, S // XC):
        cp_xt(k).wait()
    for cp in cp_vec:
        cp.wait()
    for k in range(4, S // XC):
        transpose(k)
    row8 = lax.broadcasted_iota(jnp.int32, (8, M), 0)
    x_pace = _Pacer([functools.partial(x_prep, r0) for r0 in range(0, HS, RB)], 5, 12, 40)
    routed = []

    def hook0():
        n = len(routed)
        if n < NQ:
            rg = jnp.where(row8 == 0, wr_s[...].reshape(1, M).astype(f32), gw_s[...].reshape(1, M).astype(f32))
            g_s[n] = _dot(rg.astype(bf), xt_s[:, n * T:(n + 1) * T])
            routed.append(n)
        return x_pace()
    w0 = q_w0()
    for k in range(3, S // XC):
        q_plain(w0, k * XC, hook0)
    assert x_pace.finished()

    rb = jnp.concatenate([g_s[n][0:1, :] for n in range(NQ)], axis=1).astype(bf).astype(f32)
    lane = lax.broadcasted_iota(jnp.int32, (1, S), 1)
    m1 = jnp.max(rb, axis=1, keepdims=True)
    i1 = jnp.minimum(jnp.min(jnp.where(rb == m1, lane, S)), S - 1)
    rb2 = jnp.where(lane == i1, -jnp.inf, rb)
    m2 = jnp.max(rb2, axis=1, keepdims=True)
    i2 = jnp.minimum(jnp.min(jnp.where(jnp.logical_and(rb2 == m2, lane != i1), lane, S)), S - 1)
    row16 = lax.broadcasted_iota(jnp.int32, (16, HM), 0)

    def x_row(e, i):
        blk = x_s[e, pl.ds(pl.multiple_of((i // 16) * 16, 16), 16), :].astype(f32)
        return jnp.sum(jnp.where(row16 == i % 16, blk, 0.0), axis=0, keepdims=True)
    for e in range(2):
        xs_s[e] = jnp.where(row16 == 0, x_row(e, i1), jnp.where(row16 == 1, x_row(e, i2), 0.0)).astype(bf)
    rsel_s[...] = jax.nn.sigmoid(jnp.where(lax.broadcasted_iota(jnp.int32, (16, T), 0) == 0, m1, m2))
    idx_s[0] = i1
    idx_s[1] = i2

    def q_body(it, carry):
        js = (2 * it + 1, 2 * it + 2)
        for j in js:
            for cp in [cp_wq(j)] + cp_c(j):
                cp.wait()
        pace = c_pacer(2 * it * NG, 2 * NG, 1, 112)
        for j in js:
            q_strassen(j, q_rhs(j), 0, HS, lambda: (pace(),))
        assert pace.finished()
        return carry
    lax.fori_loop(0, 3, q_body, 0)

    for cp in cp_ffn + [cp_wq(NP - 1)] + cp_c(NP - 1):
        cp.wait()

    def residual(n):
        g8 = jax.nn.sigmoid(g_s[n])
        g_s[n] = g8
        a = (1.0 - g8[1:2, :]) * xt_s[:, n * T:(n + 1) * T].astype(f32)
        acc_s[n] = a
        return [a]

    gs, us, ys, hid = [], [], {}, []
    xs_dot = lambda w_s, n: (_dot(xs_s[0], w_s[:HM, n * T:(n + 1) * T]) + _dot(xs_s[1], w_s[HM:, n * T:(n + 1) * T]))

    def swiglu():
        gg, uu = jnp.concatenate(gs, axis=1), jnp.concatenate(us, axis=1)
        hid.append((gg * jax.nn.sigmoid(gg) * uu).astype(bf))

    def down(n0, k0):
        t = _dot_nt(hid[0][:, k0:min(k0 + 512, F)], wd_s[n0:min(n0 + T, M), k0:min(k0 + 512, F)])
        ys[n0] = ys[n0] + t if n0 in ys else t
    side = []
    for n in range(F // T):
        side += [lambda n=n: gs.append(xs_dot(wg_s, n)), lambda n=n: us.append(xs_dot(wu_s, n))]
    side += [swiglu] + [lambda: None] * 7
    side += [functools.partial(down, n0, k0) for n0 in range(0, M, T) for k0 in range(0, F, 512)]
    c_pace = c_pacer((NP - 2) * NG, QS // RB - (NP - 2) * NG, 2, 56)
    r_pace = _Pacer([functools.partial(residual, n) for n in range(NQ)], M // 8, 1, 48)

    def hook7():
        if side:
            side.pop(0)()
        return c_pace(), r_pace()
    ts7 = q_rhs(NP - 1)
    for r0 in range(0, HS, 2 * T):
        q_strassen(NP - 1, ts7, r0, r0 + 2 * T, hook7)
    assert not side and c_pace.finished() and r_pace.finished()
    y = jnp.concatenate([ys[n0] for n0 in range(0, M, T)] + [jnp.zeros((16, 512 - M), f32)], axis=1)
    yt = (y * rsel_s[:, 0:1]).T
    lane128 = lax.broadcasted_iota(jnp.int32, (1, T), 1)
    for e in range(2):
        i = idx_s[e]
        acc_s[i // T] += jnp.where(lane128 == i % T, (1.0 - g_s[i // T][1:2, :]) * yt[:M, e:e + 1], 0.0)

    cp_wo.wait()
    cp_kv(0, 0).wait()
    cp_kv(1, 0).start()

    def first_terms(hn):
        w = _unpack(wkv_p[(hn >> 1) & 1, 0, :, :T], (16 * (1 - (hn & 1))).astype(u32))
        t = w[:HC] + 0.5 * w[HC:]
        return [t0_s.put((slice(None), slice(n * T, (n + 1) * T)), v.astype(bf))
                for n, v in enumerate((t[:QC], t[QC:] - t[:QC]))]
    first_terms(jnp.int32(0))

    tri = lax.broadcasted_iota(jnp.int32, (T, T), 1) <= lax.broadcasted_iota(jnp.int32, (T, T), 0)
    prog = _head_program()

    def head(h, carry):
        par, slot = h & 1, (h >> 1) & 1
        for m in range(2):
            @pl.when(jnp.logical_and(h < H - 1, par == 1 - m))
            def _():
                cp_kv((h + 1) >> 1, m).wait()

        sh = (16 * (1 - par)).astype(u32)
        rhs = []
        for r1 in range(7):
            wk, wv = [_unpack(wkv_p[slot, m], sh + (h >> (8 + r1)).astype(u32)) for m in range(2)]
            t = _rhs_terms2(wk[:HC], wv[:HC], wk[HC:], wv[HC:])[r1]
            rhs.append([u.astype(bf) for u in _rhs_terms(t[:QC, :T], t[:QC, T:], t[QC:, :T], t[QC:, T:])])
        rhs[1][1], rhs[1][3] = t0_s[:, :T], t0_s[:, T:]
        t_pace = _Pacer([lambda: first_terms(jnp.minimum(h + 1, H - 1))], 32, 196 - 14, 196)
        prods, inner_q, outer, kblk, vblk = {}, {}, {}, {}, {}

        def kv_product(r1, r2):
            m = prods.setdefault(r1, {})
            m[r2] = _dot(ca_s[7 * r1 + r2], rhs[r1][r2])
            if len(m) == 7:
                inner_q[r1] = (((m[3] - m[4]) + m[6]) + m[0], m[2] + m[4], m[1] + m[3], ((m[0] - m[1]) + m[2]) + m[5])
                for b in range(4):
                    if b not in kblk and all(q in inner_q for q in (0, 1, 3, 4, 6)):
                        p = {q: inner_q[q][b] for q in (0, 1, 3, 4, 6)}
                        e, d = p[3] + p[1], p[3] - p[1]
                        kblk[b] = (p[0] + ((d - p[4]) + p[6]), e * 2.0)
                        outer[b] = ((e + p[4]) + p[6], p[0] + d)
                    if len(inner_q) == 7:
                        p2, p5 = inner_q[2][b], inner_q[5][b]
                        vblk[b] = (((outer[b][0] + p2) - p5) * 0.5, (outer[b][1] + p2) + p5)

        def rows(blk, t0, t1):
            return jnp.concatenate([jnp.concatenate(
                [blk[2 * (t // 4 % 2) + j2][t // 8][t % 4 * T:(t % 4 + 1) * T] for j2 in range(2)], axis=1)
                for t in range(t0, t1)], axis=0)

        @functools.cache
        def k_tile(t):
            return rows(kblk, t, t + 1).astype(bf)

        @functools.cache
        def k_terms(J):
            ka, kb = rows(kblk, 2 * J, 2 * J + 1), rows(kblk, 2 * J + 1, 2 * J + 2)
            return [t.astype(bf) for t in _rhs_terms(ka[:, :T], kb[:, :T], ka[:, T:], kb[:, T:])]

        @functools.cache
        def v_tiles(c0, c1):
            return rows(vblk, c0, c1).astype(bf)

        scores, rmax, soft = {}, {}, {}
        q_tiles = lambda I: [q_s[h, i * T:(i + 1) * T, t * T:(t + 1) * T] for i in (2 * I, 2 * I + 1) for t in range(2)]

        def score_block(I, J):
            q4, qx = q_tiles(I), [qa_s[h, I * T:(I + 1) * T, k * T:(k + 1) * T] for k in range(5)]
            lhs = [qx[0], qx[1], q4[0], q4[3], qx[2], qx[3], qx[4]]
            cs = _strassen(lambda i: _dot_nt(_feed(lhs[i], t_pace()), k_terms(J)[i]))
            for n, c in enumerate(cs):
                s_s[I % 2, n // 2, 2 * J + n % 2] = c
            for u in range(2):
                sa, sb = s_s[I % 2, u, 2 * J], s_s[I % 2, u, 2 * J + 1]
                scores[2 * I + u, 2 * J] = s_s[I % 2, u, 2 * J]
                scores[2 * I + u, 2 * J + 1] = s_s[I % 2, u, 2 * J + 1]
                mx = jnp.maximum(sa, sb)
                rmax[2 * I + u] = jnp.maximum(rmax[2 * I + u], mx) if 2 * I + u in rmax else mx

        def score_diag(I):
            a, b = 2 * I, 2 * I + 1
            q4 = q_tiles(I)
            qa, qb = jnp.concatenate(q4[0:2], axis=1), jnp.concatenate(q4[2:4], axis=1)
            d1 = _dot_nt(jnp.concatenate([qa, qb], axis=0), k_tile(a))
            d2 = _dot_nt(qb, k_tile(b))
            scores[a, a], scores[b, a], scores[b, b] = jnp.where(tri, d1[:T], NEG), d1[T:], jnp.where(tri, d2, NEG)

        def pv_chunk(i, c0):
            if c0 == 0:
                mx = functools.reduce(jnp.maximum, ([rmax[i]] if i > 1 else [])
                                      + [scores[i, t] for t in range(i // 2 * 2, i + 1)])
                soft[i] = dict(m=jnp.max(mx, axis=1, keepdims=True), l=None, ctx=None)
            st = soft[i]
            c1 = min(c0 + 2, i + 1)
            p = jnp.exp2(jnp.concatenate([scores.pop((i, t)) for t in range(c0, c1)], axis=1) - st['m']).astype(bf)
            pf = p.astype(f32)
            for t in range(c1 - c0):
                st['l'] = pf[:, t * T:(t + 1) * T] if st['l'] is None else st['l'] + pf[:, t * T:(t + 1) * T]
            d = _dot(p, v_tiles(c0, c1))
            st['ctx'] = d if st['ctx'] is None else st['ctx'] + d

        def context(i):
            st = soft.pop(i)
            l = jnp.sum(st['l'], axis=1, keepdims=True)
            r = pl.reciprocal(l, approx=True)
            return st['ctx'] * (r * (2.0 - l * r))

        def accumulate(i, a0, d):
            a = acc_s[i, a0:a0 + d.shape[0], :] + g_s[i][1:2, :] * d
            acc_s[i, a0:a0 + d.shape[0], :] = a
            out_s[i, a0:a0 + d.shape[0], :] = a.astype(bf)

        def out_proj(blocks):
            wo = wo_s[h]
            if len(blocks) == 2:
                ctx = jnp.concatenate([context(i) for i in blocks], axis=0).astype(bf)
                d = _dot_nt(wo, ctx)
                accumulate(blocks[0], 0, d[:, :T])
                accumulate(blocks[1], 0, d[:, T:])
            else:
                ctx = context(blocks[0]).astype(bf)
                for a0 in (0, HM):
                    accumulate(blocks[0], a0, _dot_nt(wo[a0:a0 + HM], ctx))

            @pl.when(h == H - 1)
            def _():
                for i in blocks:
                    cp_out(i).start()

        @functools.cache
        def wo_terms():
            w = wo_s[h].astype(f32)
            return [t.astype(bf) for t in _lhs_terms(w[:HM, :T], w[:HM, T:], w[HM:, :T], w[HM:, T:])]

        @functools.cache
        def ctx_terms(I):
            ca, cb = context(2 * I), context(2 * I + 1)
            return _rhs_terms(ca[:, :T], cb[:, :T], ca[:, T:], cb[:, T:])

        oacc = {}

        def o_product(I, k):
            om_s[I, k] += _dot_nt(wo_terms()[k], ctx_terms(I)[k].astype(bf))
            oacc[I, k] = om_s[I, k]
            if all((I, q) in oacc for q in range(7)):
                cs = _strassen(lambda q: oacc.pop((I, q)))
                for n, c in enumerate(cs):
                    i, a0 = 2 * I + n % 2, (n // 2) * HM
                    out_s[i, a0:a0 + HM, :] = (acc_s[i, a0:a0 + HM, :] + g_s[i][1:2, :] * c).astype(bf)

                @pl.when(h == H - 1)
                def _():
                    for i in (2 * I, 2 * I + 1):
                        cp_out(i).start()

        ops = {'o': o_product, 'm': kv_product, 'r': score_block, 'd': score_diag, 'p': pv_chunk,
               'D': lambda i: out_proj([i, i + 1]), 'S': lambda i: out_proj([i])}
        for op, *args in prog:
            ops[op](*args)
        assert t_pace.finished()
        for m in range(2):
            @pl.when(jnp.logical_and((h + 3) >> 1 < NP, par == 1 - m))
            def _():
                cp_kv((h + 3) >> 1, m).start()
        return carry

    lax.fori_loop(0, H, head, 0)
    for i in range(NQ):
        cp_out(i).wait()


@jax.jit
def pallas_gated_mix__compressed_kv_cla__moe_arch_mod__prompt_kernel(
    A_x: jax.Array,
    A_c_kv: jax.Array,
    A_w_q: jax.Array,
    A_w_uk: jax.Array,
    A_w_uv: jax.Array,
    A_w_o: jax.Array,
    B_x: jax.Array,
    B_w_r: jax.Array,
    B_w_gate: jax.Array,
    B_w_up: jax.Array,
    B_w_down: jax.Array,
    gate_w: jax.Array,
):
    del B_x
    V = pltpu.VMEM
    B = lambda *shape: V(shape[:-2] + (shape[-2] // 2, shape[-1]), u32)
    out_t = pl.pallas_call(
        _kernel,
        in_specs=[pl.BlockSpec(memory_space=pl.ANY)] * 11,
        out_specs=pl.BlockSpec(memory_space=pl.ANY),
        out_shape=jax.ShapeDtypeStruct((M, S), bf),
        scratch_shapes=[
            V((M, S), bf), V((2, S, HM), bf), B(5, HS, HM),
            B(S, DC), B(49, QS, QC),
            V((NP, M, D), u32), V((2, 2, DC, D), u32), B(H, M, D),
            B(H, S, D), B(H, HS, 5 * T),
            V((NQ, M, T), f32),
            B(M, F), B(M, F), B(M, F),
            V((M,), bf), V((M,), bf), V((NQ, M, T), bf),
            V((NQ, 8, T), f32), B(2, 16, HM), V((16, T), f32),
            pltpu.SMEM((2,), jnp.int32),
            V((2, 2, NQ, T, T), f32), B(QC, 2 * T),
            V((NQ // 2, 7, HM, T), f32),
            pltpu.SemaphoreType.DMA((NSEM,)),
        ],
        compiler_params=pltpu.CompilerParams(vmem_limit_bytes=110 * 1024 * 1024),
        name="gated_mix_cla_mod",
    )(A_x[0].T, A_c_kv[0], A_w_q, A_w_uk, A_w_uv, A_w_o.transpose(0, 2, 1), B_w_r, B_w_gate, B_w_up,
      B_w_down.T, gate_w)
    return out_t.T[None]
```

```python
import functools
import math

import jax
import jax.numpy as jnp
from jax import lax
from jax.experimental import pallas as pl
from jax.experimental.pallas import tpu as pltpu

S, M, H, D, DC, F = 2048, 448, 16, 256, 1024, 1792
T = 128
NP, NQ = H // 2, S // T
HS, HM, HC = S // 2, M // 2, DC // 2
QS, QC = S // 4, DC // 4
RB = 16
XC = 256
NG = 5
NT = (((1,), (1,)), ((), ()))
QSCALE = D ** -0.5 * math.log2(math.e)
NEG = -1e30
bf, f32, u32 = jnp.bfloat16, jnp.float32, jnp.uint32
HI = 0xFFFF0000

SEM_WO, SEM_FFN, SEM_VEC, SEM_KV, SEM_WQ, SEM_XT, SEM_C, SEM_OUT, NSEM = 0, 1, 4, 6, 8, 16, 24, 32, 48


def _lhs_terms(a11, a12, a21, a22):
    return [a11 + a22, a21 + a22, a11, a22, a11 + a12, a21 - a11, a12 - a22]


def _rhs_terms(b11, b12, b21, b22):
    return [b11 + b22, b11, b12 - b22, b21 - b11, b22, b11 + b12, b21 + b22]


def _strassen(mm):
    m2, m3, m4, m5, m1, m7, m6 = [mm(i) for i in (1, 2, 3, 4, 0, 6, 5)]
    return (m4 - m5) + (m1 + m7), m3 + m5, m2 + m4, (m3 - m2) + (m1 + m6)


def _lhs_terms2(a11, a12, a21, a22):
    h21, q21, h22 = 0.5 * a21, 0.25 * a21, 0.5 * a22
    s1 = a11 + a22
    v, hs = a12 + q21, 0.5 * s1
    return [s1, q21 + h22, a11 + h21, h22 - q21, v + hs, h21 - a11, v - hs]


def _rhs_terms2(b11, b12, b21, b22):
    h21 = 0.5 * b21
    t1 = b11 + b22
    v, ht = b12 + 0.5 * h21, 0.5 * t1
    return [t1, b11 + h21, v - ht, h21 - b11, b22 - h21, v + ht, b22 + h21]


def _vregs(vals):
    ts = []
    for v in vals:
        v = v if v.dtype == u32 else pltpu.bitcast(v, u32)
        ts += [v[r:r + 8, c:c + T] for r in range(0, v.shape[0], 8) for c in range(0, v.shape[1] - T + 1, T)]
    return ts


def _zero_from(ts):
    acc = ts[:4]
    for i, t in enumerate(ts[4:]):
        acc[i % 4] = acc[i % 4] | t
    while len(acc) > 1:
        acc = [acc[i] | acc[i + 1] if i + 1 < len(acc) else acc[i] for i in range(0, len(acc), 2)]
    return (acc[0] >> 16) >> 16


def _feed(a, *zs):
    zs = [z for z in zs if z is not None]
    if not zs:
        return a
    a32 = pltpu.bitcast(a, u32)
    top = functools.reduce(lambda p, q: p | q, zs, a32[0:8, :T])
    if a32.shape[1] > T:
        top = jnp.concatenate([top, a32[0:8, T:]], axis=1)
    return pltpu.bitcast(jnp.concatenate([top, a32[8:]], axis=0), bf)


class _Pacer:
    def __init__(self, thunks, per, first, last):
        self.thunks, self.pool, self.k, self.done = list(thunks), [], 0, 0
        self.tot, self.first, self.last = per * len(self.thunks), first, last

    def __call__(self):
        self.k += 1
        if self.k <= self.first:
            return None
        want = min(self.tot, -(-(self.k - self.first) * self.tot // (self.last - self.first))) - self.done
        while len(self.pool) < want and self.thunks:
            self.pool += _vregs(self.thunks.pop(0)())
        outs, self.pool = self.pool[:want], self.pool[want:]
        self.done += len(outs)
        return _zero_from(outs) if outs else None

    def finished(self):
        return not self.thunks and not self.pool


_HEAD_ORDER = """
m1.1 m1.3 m1.4 m1.6 m1.0 m1.2 m3.3 m4.3 m3.4 m3.1 m3.0 m3.6 m4.1 m4.4 m3.2 m3.5 m1.5 m6.6 m4.6 m4.0 m4.5 m6.1
m4.2 m6.4 m6.0 m6.3 m6.2 m0.1 m6.5 m0.6 m0.4 m0.3 m0.0 m0.2 m0.5 m2.1 d0 m2.3 r7.0 m2.4 r7.1 m2.0 m2.6 m5.1 r7.2
m2.2 r7.3 r7.4 m2.5 r7.5 r7.6 m5.3 d7 m5.4 m5.6 m5.0 m5.2 m5.5 p14.0 r6.0 p1.0 r6.1 p0.0 r6.2 p14.2 p14.4 p14.6
p14.8 p14.10 p14.12 r6.3 p15.0 r6.5 p14.14 p15.2 p15.4 r6.4 p15.6 p15.8 p15.10 d6 p15.12 p12.0 p15.14 r5.0 p12.2
p12.4 p12.6 p12.8 p12.10 p13.0 r5.2 r5.3 r5.1 r5.4 p13.2 p13.4 p13.6 p13.8 d5 o0.3 p12.12 o0.2 o0.1 o0.0 o0.5
o0.4 p13.10 r4.1 p11.0 p10.0 p13.12 p10.2 p10.4 r4.0 o0.6 p10.6 p10.8 p11.2 p10.10 r4.2 p11.4 p11.6 r4.3 d4 o7.2
o7.0 o7.1 o7.3 o7.4 o7.6 o7.5 r3.0 p8.0 p11.8 p11.10 p8.2 p8.4 p8.6 r3.1 d3 p9.0 p9.2 p8.8 r3.2 o6.1 o6.3 o6.2
p9.4 o6.4 o6.0 o6.6 r2.0 r2.1 p9.6 p6.0 p6.2 p9.8 p6.4 o6.5 p6.6 d2 p7.0 p7.2 o5.3 o5.1 o5.2 o5.4 o5.6 o5.0 p5.0
p4.0 o5.5 p7.4 r1.0 p4.2 p7.6 p4.4 d1 p5.2 p2.0 o4.1 o4.2 o4.0 o4.4 o4.3 o4.6 o4.5 p2.2 p5.4 o2.1 p3.0 p3.2 S2
o2.3 o2.0 o2.2 o2.6 o3.3 o2.5 o3.2 o2.4 o3.6 o3.1 o3.0 o3.5 o3.4 S3
"""


def _head_program():
    return [(t[0],) + tuple(int(v) for v in t[1:].split('.')) for t in _HEAD_ORDER.split()]


def _dot(a, b):
    return jnp.dot(a, b, preferred_element_type=f32)


def _dot_nt(a, b):
    return lax.dot_general(a, b, NT, preferred_element_type=f32)


def _unpack(w32, sh):
    return pltpu.bitcast((w32 << sh) & jnp.uint32(HI), f32)


class _Bf16:
    def __init__(self, raw):
        self.raw = raw

    def _half(self, idx):
        idx = list(idx if isinstance(idx, tuple) else (idx,))
        idx += [slice(None)] * (len(self.raw.shape) - len(idx))
        r = idx[-2]
        if isinstance(r, slice):
            idx[-2] = slice(None if r.start is None else r.start // 2, None if r.stop is None else r.stop // 2)
        elif isinstance(r.start, int):
            idx[-2] = pl.ds(r.start // 2, r.size // 2)
        else:
            idx[-2] = pl.ds(pl.multiple_of(r.start >> 1, 8), r.size // 2)
        return tuple(idx)

    def __getitem__(self, idx):
        return pltpu.bitcast(self.raw[self._half(idx)], bf)

    def put(self, idx, v):
        idx = self._half(idx)
        ref = self.raw.at[idx[:-2]] if len(idx) > 2 else self.raw
        o = pltpu.bitcast(v, u32)
        ref[idx[-2], idx[-1]] = o
        return o

    def __setitem__(self, idx, v):
        self.put(idx, v)


def _kernel(xt_hbm, c_hbm, wq_hbm, wk_hbm, wv_hbm, wo_hbm, wr_hbm, wg_hbm, wu_hbm, wd_hbm, gw_hbm, o_hbm,
            xt_s, x_s, xa_r, c_r, ca_r, wq_p, wkv_p, wo_r, q_r, qa_r, acc_s, wg_r, wu_r, wd_r,
            wr_s, gw_s, out_s, g_s, xs_r, rsel_s, idx_s, s_s, t0_r, om_s, sem):
    xa_s, c_s, ca_s, wo_s, q_s, qa_s, wg_s, wu_s, wd_s, xs_s, t0_s = [
        _Bf16(r) for r in (xa_r, c_r, ca_r, wo_r, q_r, qa_r, wg_r, wu_r, wd_r, xs_r, t0_r)]
    mk = pltpu.make_async_copy
    wq32, wk32, wv32 = wq_hbm.bitcast(u32), wk_hbm.bitcast(u32), wv_hbm.bitcast(u32)
    cp_wq = lambda j: mk(wq32.at[:, j, :], wq_p.at[j], sem.at[SEM_WQ + j])
    cp_kv = lambda j, m: mk((wk32, wv32)[m].at[:, j, :], wkv_p.at[j & 1, m], sem.at[SEM_KV + m])
    cp_xt = lambda k: mk(xt_hbm.at[:, pl.ds(k * XC, XC)], xt_s.at[:, pl.ds(k * XC, XC)], sem.at[SEM_XT + k])
    cp_out = lambda i: mk(out_s.at[i], o_hbm.at[:, pl.ds(i * T, T)], sem.at[SEM_OUT + i])
    cp_vec = [mk(wr_hbm, wr_s, sem.at[SEM_VEC]), mk(gw_hbm, gw_s, sem.at[SEM_VEC + 1])]
    cp_ffn = [mk(src, dst, sem.at[SEM_FFN + n]) for n, (src, dst) in
              enumerate(((wg_hbm.bitcast(u32), wg_r), (wu_hbm.bitcast(u32), wu_r), (wd_hbm.bitcast(u32), wd_r)))]
    cp_wo = mk(wo_hbm.bitcast(u32), wo_r, sem.at[SEM_WO])
    c32 = c_hbm.bitcast(u32)

    def cp_c(j):
        r0 = (j - 1) * (NG * RB // 2)
        n = QS // 2 - r0 if isinstance(j, int) and j == NP - 1 else NG * RB // 2
        return [mk(c32.at[pl.ds(i * QS // 2 + r0, n)], c_r.at[pl.ds(i * QS // 2 + r0, n)], sem.at[SEM_C + j])
                for i in range(4)]

    cp_xt(0).start()
    cp_wq(0).start()
    for k in range(1, S // XC):
        cp_xt(k).start()
    for cp in cp_vec:
        cp.start()
    for j in range(1, NP):
        cp_wq(j).start()
        for cp in cp_c(j):
            cp.start()
    for cp in cp_ffn + [cp_kv(0, 0), cp_kv(0, 1), cp_wo]:
        cp.start()

    @pl.loop(0, NQ // 2)
    def _(n):
        om_s[n] = jnp.zeros(om_s.shape[1:], f32)

    def store_q(j, e, r0, q):
        q = q * QSCALE
        q_s[2 * j + e, r0:r0 + q.shape[0], :] = q.astype(bf)
        for p0 in range(0, q.shape[0], 2 * T):
            if r0 + p0 > 0:
                qa, qb = q[p0:p0 + T], q[p0 + T:p0 + 2 * T]
                terms = _lhs_terms(qa[:, :T], qa[:, T:], qb[:, :T], qb[:, T:])
                for k, i in enumerate((0, 1, 4, 5, 6)):
                    qa_s[2 * j + e, (r0 + p0) // 2:(r0 + p0) // 2 + T, k * T:(k + 1) * T] = terms[i].astype(bf)

    def q_plain(w, r0, hook=None):
        prod = lambda a, b, wn, z: _dot(_feed(x_s[0, a:b, :], z), wn[:HM]) + _dot(x_s[1, a:b, :], wn[HM:])
        if hook is None:
            qf = prod(r0, r0 + 2 * T, w, None)
        else:
            qf = jnp.concatenate([jnp.concatenate(
                [prod(r0 + u * T, r0 + (u + 1) * T, w[:, n * T:(n + 1) * T], hook()) for u in range(2)], axis=0)
                for n in range(4)], axis=1)
        store_q(0, 0, r0, qf[:, :D])
        store_q(0, 1, r0, qf[:, D:])

    def q_rhs(j):
        lo, hi = pltpu.bitcast(wq_p[j] << 16, f32), pltpu.bitcast(wq_p[j] & jnp.uint32(HI), f32)
        return [t.astype(bf) for t in _rhs_terms(lo[:HM], hi[:HM], lo[HM:], hi[HM:])]

    def q_strassen(j, ts, r0, r1, hook):
        def lhs(i, u):
            if i in (2, 3):
                return x_s[i - 2, (i - 2) * HS + u:(i - 2) * HS + u + T, :]
            return xa_s[i - 2 * (i > 3), u:u + T, :]
        cs = _strassen(lambda i: jnp.concatenate(
            [_dot(_feed(lhs(i, u), *hook()), ts[i]) for u in range(r0, r1, T)], axis=0))
        for n, c in enumerate(cs):
            store_q(j, n % 2, (n // 2) * HS + r0, c)

    def x_prep(r0):
        a = [x_s[e, h0 + r0:h0 + r0 + RB, :].astype(f32) for h0 in (0, HS) for e in (0, 1)]
        terms = _lhs_terms(*a)
        outs = []
        for k, i in enumerate((0, 1, 4, 5, 6)):
            outs.append(xa_s.put((k, slice(r0, r0 + RB)), terms[i].astype(bf)))
        return outs

    def c_prep(g, c0):
        blk = lambda i, k: c_s[pl.ds(i * QS + g * RB, RB), k * QC + c0:k * QC + c0 + T].astype(f32)
        outer = [_lhs_terms2(*[blk(2 * i1 + i2, 2 * k1 + k2) for i1 in range(2) for k1 in range(2)])
                 for i2 in range(2) for k2 in range(2)]
        outs = []
        for r1 in range(7):
            for r2, v in enumerate(_lhs_terms(*[o[r1] for o in outer])):
                outs.append(ca_s.put((7 * r1 + r2, pl.ds(g * RB, RB), slice(c0, c0 + T)), v.astype(bf)))
        return outs

    def c_pacer(g0, ng, first, last):
        return _Pacer([functools.partial(c_prep, g0 + t // 2, (t % 2) * T) for t in range(2 * ng)], 49, first, last)

    def transpose(k):
        for e in range(2):
            x_s[e, k * XC:(k + 1) * XC, :] = xt_s[e * HM:(e + 1) * HM, k * XC:(k + 1) * XC].T

    def q_w0():
        return jnp.concatenate([pltpu.bitcast(wq_p[0] << 16, f32).astype(bf),
                                pltpu.bitcast(wq_p[0] & jnp.uint32(HI), f32).astype(bf)], axis=1)

    cp_xt(0).wait()
    transpose(0)
    cp_wq(0).wait()
    q_plain(q_w0(), 0)
    for k in range(1, 4):
        cp_xt(k).wait()
    transpose(1)
    w0 = q_w0()
    transpose(2)
    q_plain(w0, XC)
    transpose(3)
    q_plain(w0, 2 * XC)
    for k in range(4, S // XC):
        cp_xt(k).wait()
    for cp in cp_vec:
        cp.wait()
    for k in range(4, S // XC):
        transpose(k)
    row8 = lax.broadcasted_iota(jnp.int32, (8, M), 0)
    x_pace = _Pacer([functools.partial(x_prep, r0) for r0 in range(0, HS, RB)], 5, 12, 40)
    routed = []

    def hook0():
        n = len(routed)
        if n < NQ:
            rg = jnp.where(row8 == 0, wr_s[...].reshape(1, M).astype(f32), gw_s[...].reshape(1, M).astype(f32))
            g_s[n] = _dot(rg.astype(bf), xt_s[:, n * T:(n + 1) * T])
            routed.append(n)
        return x_pace()
    w0 = q_w0()
    for k in range(3, S // XC):
        q_plain(w0, k * XC, hook0)
    assert x_pace.finished()

    rb = jnp.concatenate([g_s[n][0:1, :] for n in range(NQ)], axis=1).astype(bf).astype(f32)
    lane = lax.broadcasted_iota(jnp.int32, (1, S), 1)
    m1 = jnp.max(rb, axis=1, keepdims=True)
    i1 = jnp.minimum(jnp.min(jnp.where(rb == m1, lane, S)), S - 1)
    rb2 = jnp.where(lane == i1, -jnp.inf, rb)
    m2 = jnp.max(rb2, axis=1, keepdims=True)
    i2 = jnp.minimum(jnp.min(jnp.where(jnp.logical_and(rb2 == m2, lane != i1), lane, S)), S - 1)
    row16 = lax.broadcasted_iota(jnp.int32, (16, HM), 0)

    def x_row(e, i):
        blk = x_s[e, pl.ds(pl.multiple_of((i // 16) * 16, 16), 16), :].astype(f32)
        return jnp.sum(jnp.where(row16 == i % 16, blk, 0.0), axis=0, keepdims=True)
    for e in range(2):
        xs_s[e] = jnp.where(row16 == 0, x_row(e, i1), jnp.where(row16 == 1, x_row(e, i2), 0.0)).astype(bf)
    rsel_s[...] = jax.nn.sigmoid(jnp.where(lax.broadcasted_iota(jnp.int32, (16, T), 0) == 0, m1, m2))
    idx_s[0] = i1
    idx_s[1] = i2

    def q_body(it, carry):
        js = (2 * it + 1, 2 * it + 2)
        for j in js:
            for cp in [cp_wq(j)] + cp_c(j):
                cp.wait()
        pace = c_pacer(2 * it * NG, 2 * NG, 1, 112)
        for j in js:
            ts = q_rhs(j)
            for r0 in range(0, HS, HS):
                q_strassen(j, ts, r0, r0 + HS, lambda: (pace(),))
        assert pace.finished()
        return carry
    lax.fori_loop(0, 3, q_body, 0)

    for cp in cp_ffn + [cp_wq(NP - 1)] + cp_c(NP - 1):
        cp.wait()

    def residual(n):
        g8 = jax.nn.sigmoid(g_s[n])
        g_s[n] = g8
        a = (1.0 - g8[1:2, :]) * xt_s[:, n * T:(n + 1) * T].astype(f32)
        acc_s[n] = a
        return [a]

    gs, us, ys, hid = [], [], {}, []
    xs_dot = lambda w_s, n: (_dot(xs_s[0], w_s[:HM, n * T:(n + 1) * T]) + _dot(xs_s[1], w_s[HM:, n * T:(n + 1) * T]))

    def swiglu():
        gg, uu = jnp.concatenate(gs, axis=1), jnp.concatenate(us, axis=1)
        hid.append((gg * jax.nn.sigmoid(gg) * uu).astype(bf))

    def down(n0, k0):
        t = _dot_nt(hid[0][:, k0:min(k0 + 512, F)], wd_s[n0:min(n0 + T, M), k0:min(k0 + 512, F)])
        ys[n0] = ys[n0] + t if n0 in ys else t
    side = []
    for n in range(F // T):
        side += [lambda n=n: gs.append(xs_dot(wg_s, n)), lambda n=n: us.append(xs_dot(wu_s, n))]
    side += [swiglu] + [lambda: None] * 7
    side += [functools.partial(down, n0, k0) for n0 in range(0, M, T) for k0 in range(0, F, 512)]
    c_pace = c_pacer((NP - 2) * NG, QS // RB - (NP - 2) * NG, 2, 56)
    r_pace = _Pacer([functools.partial(residual, n) for n in range(NQ)], M // 8, 1, 48)

    def hook7():
        if side:
            side.pop(0)()
        return c_pace(), r_pace()
    ts7 = q_rhs(NP - 1)
    for r0 in range(0, HS, 1024):
        q_strassen(NP - 1, ts7, r0, r0 + 1024, hook7)
    assert not side and c_pace.finished() and r_pace.finished()
    y = jnp.concatenate([ys[n0] for n0 in range(0, M, T)] + [jnp.zeros((16, 512 - M), f32)], axis=1)
    yt = (y * rsel_s[:, 0:1]).T
    lane128 = lax.broadcasted_iota(jnp.int32, (1, T), 1)
    for e in range(2):
        i = idx_s[e]
        acc_s[i // T] += jnp.where(lane128 == i % T, (1.0 - g_s[i // T][1:2, :]) * yt[:M, e:e + 1], 0.0)

    cp_wo.wait()
    cp_kv(0, 0).wait()
    cp_kv(1, 0).start()

    def first_terms(hn):
        w = _unpack(wkv_p[(hn >> 1) & 1, 0, :, :T], (16 * (1 - (hn & 1))).astype(u32))
        t = w[:HC] + 0.5 * w[HC:]
        return [t0_s.put((slice(None), slice(n * T, (n + 1) * T)), v.astype(bf))
                for n, v in enumerate((t[:QC], t[QC:] - t[:QC]))]
    first_terms(jnp.int32(0))

    tri = lax.broadcasted_iota(jnp.int32, (T, T), 1) <= lax.broadcasted_iota(jnp.int32, (T, T), 0)
    prog = _head_program()

    def head(h, carry):
        par, slot = h & 1, (h >> 1) & 1
        for m in range(2):
            @pl.when(jnp.logical_and(h < H - 1, par == 1 - m))
            def _():
                cp_kv((h + 1) >> 1, m).wait()

        sh = (16 * (1 - par)).astype(u32)
        rhs = []
        for r1 in range(7):
            wk, wv = [_unpack(wkv_p[slot, m], sh + (h >> (8 + r1)).astype(u32)) for m in range(2)]
            t = _rhs_terms2(wk[:HC], wv[:HC], wk[HC:], wv[HC:])[r1]
            rhs.append([u.astype(bf) for u in _rhs_terms(t[:QC, :T], t[:QC, T:], t[QC:, :T], t[QC:, T:])])
        rhs[1][1], rhs[1][3] = t0_s[:, :T], t0_s[:, T:]
        t_pace = _Pacer([lambda: first_terms(jnp.minimum(h + 1, H - 1))], 32, 196 - 14, 196)
        prods, inner_q, outer, kblk, vblk = {}, {}, {}, {}, {}

        def kv_product(r1, r2):
            m = prods.setdefault(r1, {})
            m[r2] = _dot(ca_s[7 * r1 + r2], rhs[r1][r2])
            if len(m) == 7:
                inner_q[r1] = (((m[3] - m[4]) + m[6]) + m[0], m[2] + m[4], m[1] + m[3], ((m[0] - m[1]) + m[2]) + m[5])
                for b in range(4):
                    if b not in kblk and all(q in inner_q for q in (0, 1, 3, 4, 6)):
                        p = {q: inner_q[q][b] for q in (0, 1, 3, 4, 6)}
                        e, d = p[3] + p[1], p[3] - p[1]
                        kblk[b] = (p[0] + ((d - p[4]) + p[6]), e * 2.0)
                        outer[b] = ((e + p[4]) + p[6], p[0] + d)
                    if len(inner_q) == 7:
                        p2, p5 = inner_q[2][b], inner_q[5][b]
                        vblk[b] = (((outer[b][0] + p2) - p5) * 0.5, (outer[b][1] + p2) + p5)

        def rows(blk, t0, t1):
            return jnp.concatenate([jnp.concatenate(
                [blk[2 * (t // 4 % 2) + j2][t // 8][t % 4 * T:(t % 4 + 1) * T] for j2 in range(2)], axis=1)
                for t in range(t0, t1)], axis=0)

        @functools.cache
        def k_tile(t):
            return rows(kblk, t, t + 1).astype(bf)

        @functools.cache
        def k_terms(J):
            ka, kb = rows(kblk, 2 * J, 2 * J + 1), rows(kblk, 2 * J + 1, 2 * J + 2)
            return [t.astype(bf) for t in _rhs_terms(ka[:, :T], kb[:, :T], ka[:, T:], kb[:, T:])]

        @functools.cache
        def v_tiles(c0, c1):
            return rows(vblk, c0, c1).astype(bf)

        scores, rmax, soft, o_sum = {}, {}, {}, {}
        q_tiles = lambda I: [q_s[h, i * T:(i + 1) * T, t * T:(t + 1) * T] for i in (2 * I, 2 * I + 1) for t in range(2)]

        def score_block(I, J):
            q4, qx = q_tiles(I), [qa_s[h, I * T:(I + 1) * T, k * T:(k + 1) * T] for k in range(5)]
            lhs = [qx[0], qx[1], q4[0], q4[3], qx[2], qx[3], qx[4]]
            cs = _strassen(lambda i: _dot_nt(_feed(lhs[i], t_pace()), k_terms(J)[i]))
            for n, c in enumerate(cs):
                s_s[I % 2, n // 2, 2 * J + n % 2] = c
            for u in range(2):
                sa, sb = s_s[I % 2, u, 2 * J], s_s[I % 2, u, 2 * J + 1]
                scores[2 * I + u, 2 * J] = s_s[I % 2, u, 2 * J]
                scores[2 * I + u, 2 * J + 1] = s_s[I % 2, u, 2 * J + 1]
                mx = jnp.maximum(sa, sb)
                rmax[2 * I + u] = jnp.maximum(rmax[2 * I + u], mx) if 2 * I + u in rmax else mx

        def score_diag(I):
            a, b = 2 * I, 2 * I + 1
            q4 = q_tiles(I)
            qa, qb = jnp.concatenate(q4[0:2], axis=1), jnp.concatenate(q4[2:4], axis=1)
            d1 = _dot_nt(jnp.concatenate([qa, qb], axis=0), k_tile(a))
            d2 = _dot_nt(qb, k_tile(b))
            scores[a, a], scores[b, a], scores[b, b] = jnp.where(tri, d1[:T], NEG), d1[T:], jnp.where(tri, d2, NEG)

        def pv_chunk(i, c0):
            if c0 == 0:
                mx = functools.reduce(jnp.maximum, ([rmax[i]] if i > 1 else [])
                                      + [scores[i, t] for t in range(i // 2 * 2, i + 1)])
                soft[i] = dict(m=jnp.max(mx, axis=1, keepdims=True), l=None, ctx=None)
            st = soft[i]
            c1 = min(c0 + 2, i + 1)
            p = jnp.exp2(jnp.concatenate([scores.pop((i, t)) for t in range(c0, c1)], axis=1) - st['m']).astype(bf)
            pf = p.astype(f32)
            for t in range(c1 - c0):
                st['l'] = pf[:, t * T:(t + 1) * T] if st['l'] is None else st['l'] + pf[:, t * T:(t + 1) * T]
            d = _dot(p, v_tiles(c0, c1))
            st['ctx'] = d if st['ctx'] is None else st['ctx'] + d

        def context(i):
            st = soft.pop(i)
            l = jnp.sum(st['l'], axis=1, keepdims=True)
            r = pl.reciprocal(l, approx=True)
            return st['ctx'] * (r * (2.0 - l * r))

        def ship(blocks):
            @pl.when(h == H - 1)
            def _():
                for i in blocks:
                    cp_out(i).start()

        def out_plain(i):
            wo, ctx = wo_s[h], context(i).astype(bf)
            for a0 in (0, HM):
                a = acc_s[i, a0:a0 + HM, :] + g_s[i][1:2, :] * _dot_nt(wo[a0:a0 + HM], ctx)
                acc_s[i, a0:a0 + HM, :] = a
                out_s[i, a0:a0 + HM, :] = a.astype(bf)
            ship([i])

        @functools.cache
        def wo_terms():
            w = wo_s[h].astype(f32)
            return [t.astype(bf) for t in _lhs_terms(w[:HM, :T], w[:HM, T:], w[HM:, :T], w[HM:, T:])]

        @functools.cache
        def ctx_terms(I):
            ca, cb = context(2 * I), context(2 * I + 1)
            return _rhs_terms(ca[:, :T], cb[:, :T], ca[:, T:], cb[:, T:])

        def out_product(I, k):
            om_s[I, k] += _dot_nt(wo_terms()[k], ctx_terms(I)[k].astype(bf))
            o_sum[I, k] = om_s[I, k]
            if all((I, q) in o_sum for q in range(7)):
                for n, c in enumerate(_strassen(lambda q: o_sum.pop((I, q)))):
                    i, a0 = 2 * I + n % 2, (n // 2) * HM
                    out_s[i, a0:a0 + HM, :] = (acc_s[i, a0:a0 + HM, :] + g_s[i][1:2, :] * c).astype(bf)
                ship([2 * I, 2 * I + 1])

        ops = {'m': kv_product, 'r': score_block, 'd': score_diag, 'p': pv_chunk,
               'o': out_product, 'S': out_plain}
        for op, *args in prog:
            ops[op](*args)
        assert t_pace.finished()
        for m in range(2):
            @pl.when(jnp.logical_and((h + 3) >> 1 < NP, par == 1 - m))
            def _():
                cp_kv((h + 3) >> 1, m).start()
        return carry

    lax.fori_loop(0, H, head, 0)
    for i in range(NQ):
        cp_out(i).wait()


@jax.jit
def pallas_gated_mix__compressed_kv_cla__moe_arch_mod__prompt_kernel(
    A_x: jax.Array,
    A_c_kv: jax.Array,
    A_w_q: jax.Array,
    A_w_uk: jax.Array,
    A_w_uv: jax.Array,
    A_w_o: jax.Array,
    B_x: jax.Array,
    B_w_r: jax.Array,
    B_w_gate: jax.Array,
    B_w_up: jax.Array,
    B_w_down: jax.Array,
    gate_w: jax.Array,
):
    del B_x
    V = pltpu.VMEM
    B = lambda *shape: V(shape[:-2] + (shape[-2] // 2, shape[-1]), u32)
    out_t = pl.pallas_call(
        _kernel,
        in_specs=[pl.BlockSpec(memory_space=pl.ANY)] * 11,
        out_specs=pl.BlockSpec(memory_space=pl.ANY),
        out_shape=jax.ShapeDtypeStruct((M, S), bf),
        scratch_shapes=[
            V((M, S), bf), V((2, S, HM), bf), B(5, HS, HM),
            B(S, DC), B(49, QS, QC),
            V((NP, M, D), u32), V((2, 2, DC, D), u32), B(H, M, D),
            B(H, S, D), B(H, HS, 5 * T),
            V((NQ, M, T), f32),
            B(M, F), B(M, F), B(M, F),
            V((M,), bf), V((M,), bf), V((NQ, M, T), bf),
            V((NQ, 8, T), f32), B(2, 16, HM), V((16, T), f32),
            pltpu.SMEM((2,), jnp.int32),
            V((2, 2, NQ, T, T), f32), B(QC, 2 * T),
            V((NQ // 2, 7, HM, T), f32),
            pltpu.SemaphoreType.DMA((NSEM,)),
        ],
        compiler_params=pltpu.CompilerParams(vmem_limit_bytes=110 * 1024 * 1024),
        name="gated_mix_cla_mod",
    )(A_x[0].T, A_c_kv[0], A_w_q, A_w_uk, A_w_uv, A_w_o.transpose(0, 2, 1), B_w_r, B_w_gate, B_w_up,
      B_w_down.T, gate_w)
    return out_t.T[None]
```

```python
import functools
import math

import jax
import jax.numpy as jnp
from jax import lax
from jax.experimental import pallas as pl
from jax.experimental.pallas import tpu as pltpu

S, M, H, D, DC, F = 2048, 448, 16, 256, 1024, 1792
T = 128
NP, NQ = H // 2, S // T
HS, HM, HC = S // 2, M // 2, DC // 2
QS, QC = S // 4, DC // 4
RB = 16
XC = 256
NG = 5
NT = (((1,), (1,)), ((), ()))
QSCALE = D ** -0.5 * math.log2(math.e)
NEG = -1e30
bf, f32, u32 = jnp.bfloat16, jnp.float32, jnp.uint32
HI = 0xFFFF0000

SEM_WO, SEM_FFN, SEM_VEC, SEM_KV, SEM_WQ, SEM_XT, SEM_C, SEM_OUT, NSEM = 0, 1, 4, 6, 8, 16, 24, 32, 48


def _lhs_terms(a11, a12, a21, a22):
    return [a11 + a22, a21 + a22, a11, a22, a11 + a12, a21 - a11, a12 - a22]


def _rhs_terms(b11, b12, b21, b22):
    return [b11 + b22, b11, b12 - b22, b21 - b11, b22, b11 + b12, b21 + b22]


def _strassen(mm):
    m2, m3, m4, m5, m1, m7, m6 = [mm(i) for i in (1, 2, 3, 4, 0, 6, 5)]
    return (m4 - m5) + (m1 + m7), m3 + m5, m2 + m4, (m3 - m2) + (m1 + m6)


def _lhs_terms2(a11, a12, a21, a22):
    h21, q21, h22 = 0.5 * a21, 0.25 * a21, 0.5 * a22
    s1 = a11 + a22
    v, hs = a12 + q21, 0.5 * s1
    return [s1, q21 + h22, a11 + h21, h22 - q21, v + hs, h21 - a11, v - hs]


def _rhs_terms2(b11, b12, b21, b22):
    h21 = 0.5 * b21
    t1 = b11 + b22
    v, ht = b12 + 0.5 * h21, 0.5 * t1
    return [t1, b11 + h21, v - ht, h21 - b11, b22 - h21, v + ht, b22 + h21]


def _vregs(vals):
    ts = []
    for v in vals:
        v = v if v.dtype == u32 else pltpu.bitcast(v, u32)
        ts += [v[r:r + 8, c:c + T] for r in range(0, v.shape[0], 8) for c in range(0, v.shape[1] - T + 1, T)]
    return ts


def _zero_from(ts):
    acc = ts[:4]
    for i, t in enumerate(ts[4:]):
        acc[i % 4] = acc[i % 4] | t
    while len(acc) > 1:
        acc = [acc[i] | acc[i + 1] if i + 1 < len(acc) else acc[i] for i in range(0, len(acc), 2)]
    return (acc[0] >> 16) >> 16


def _feed(a, *zs):
    zs = [z for z in zs if z is not None]
    if not zs:
        return a
    a32 = pltpu.bitcast(a, u32)
    top = functools.reduce(lambda p, q: p | q, zs, a32[0:8, :T])
    if a32.shape[1] > T:
        top = jnp.concatenate([top, a32[0:8, T:]], axis=1)
    return pltpu.bitcast(jnp.concatenate([top, a32[8:]], axis=0), bf)


class _Pacer:
    def __init__(self, thunks, per, first, last):
        self.thunks, self.pool, self.k, self.done = list(thunks), [], 0, 0
        self.tot, self.first, self.last = per * len(self.thunks), first, last

    def __call__(self):
        self.k += 1
        if self.k <= self.first:
            return None
        want = min(self.tot, -(-(self.k - self.first) * self.tot // (self.last - self.first))) - self.done
        while len(self.pool) < want and self.thunks:
            self.pool += _vregs(self.thunks.pop(0)())
        outs, self.pool = self.pool[:want], self.pool[want:]
        self.done += len(outs)
        return _zero_from(outs) if outs else None

    def finished(self):
        return not self.thunks and not self.pool


_HEAD_ORDER = """
m1.1 m1.3 m1.4 m1.6 m1.0 m3.3 m3.6 m1.2 m3.4 m4.3 m3.1 m3.0 m4.4 m3.2 m3.5 m1.5 m4.6 m4.1 m4.0 m6.3 m6.0 m6.6
m4.5 m0.1 m6.4 m6.1 m6.5 m6.2 m4.2 m0.6 m0.4 m0.3 m0.0 m0.2 m0.5 m2.1 d0 m2.3 r7.0 m2.4 r7.1 m2.0 m2.6 m5.1 r7.2
m2.2 r7.4 m2.5 r7.3 r7.6 r7.5 m5.3 d7 m5.6 m5.4 m5.0 m5.2 m5.5 p14.0 r6.0 p1.0 p0.0 r6.2 r6.1 p14.2 p14.4 p14.6
p14.8 p14.10 p15.0 p14.12 p14.14 r6.3 r6.4 r6.5 p15.2 p15.4 p15.6 p15.8 p15.10 d6 p15.12 p15.14 r5.0 p12.0 p12.2
p12.4 p12.6 r5.3 r5.2 r5.1 p12.8 p12.10 p13.0 p13.2 r5.4 p13.4 p13.6 p13.8 p12.12 d5 o0.3 o0.2 o0.1 p10.0 o0.0
o0.5 p11.0 p13.10 r4.1 o0.4 p10.2 p13.12 p10.4 r4.0 o0.6 p10.6 p10.8 p11.2 p10.10 r4.2 r4.3 p11.4 d4 p11.6 o7.2
o7.0 o7.1 o7.4 o7.3 o7.6 o7.5 r3.0 p11.8 p8.0 p8.2 p11.10 p8.4 p8.6 p9.0 p9.2 p8.8 r3.1 d3 r3.2 o6.4 o6.2 p9.4
o6.3 o6.0 o6.6 o6.1 p7.0 r2.1 p9.6 p9.8 p6.0 p6.2 p6.4 r2.0 o6.5 p6.6 d2 p7.2 p4.0 o5.3 o5.2 o5.1 o5.4 o5.6 o5.5
o5.0 r1.0 p4.2 p5.0 p7.4 p7.6 p4.4 d1 p5.2 o4.4 o4.2 p2.0 o4.0 o4.1 o4.3 p3.0 o4.6 o4.5 p2.2 p5.4 o2.1 p3.2 S2
o3.3 o2.3 o2.6 o2.4 o2.0 o3.2 o3.1 o2.2 o2.5 o3.6 o3.5 o3.0 o3.4 S3
"""


def _head_program():
    return [(t[0],) + tuple(int(v) for v in t[1:].split('.')) for t in _HEAD_ORDER.split()]


def _dot(a, b):
    return jnp.dot(a, b, preferred_element_type=f32)


def _dot_nt(a, b):
    return lax.dot_general(a, b, NT, preferred_element_type=f32)


def _unpack(w32, sh):
    return pltpu.bitcast((w32 << sh) & jnp.uint32(HI), f32)


class _Bf16:
    def __init__(self, raw):
        self.raw = raw

    def _half(self, idx):
        idx = list(idx if isinstance(idx, tuple) else (idx,))
        idx += [slice(None)] * (len(self.raw.shape) - len(idx))
        r = idx[-2]
        if isinstance(r, slice):
            idx[-2] = slice(None if r.start is None else r.start // 2, None if r.stop is None else r.stop // 2)
        elif isinstance(r.start, int):
            idx[-2] = pl.ds(r.start // 2, r.size // 2)
        else:
            idx[-2] = pl.ds(pl.multiple_of(r.start >> 1, 8), r.size // 2)
        return tuple(idx)

    def __getitem__(self, idx):
        return pltpu.bitcast(self.raw[self._half(idx)], bf)

    def put(self, idx, v):
        idx = self._half(idx)
        ref = self.raw.at[idx[:-2]] if len(idx) > 2 else self.raw
        o = pltpu.bitcast(v, u32)
        ref[idx[-2], idx[-1]] = o
        return o

    def __setitem__(self, idx, v):
        self.put(idx, v)


def _kernel(xt_hbm, c_hbm, wq_hbm, wk_hbm, wv_hbm, wo_hbm, wr_hbm, wg_hbm, wu_hbm, wd_hbm, gw_hbm, o_hbm,
            xt_s, x_s, xa_r, c_r, ca_r, wq_p, wkv_p, wo_r, q_r, qa_r, acc_s, wg_r, wu_r, wd_r,
            wr_s, gw_s, out_s, g_s, xs_r, rsel_s, idx_s, s_s, t0_r, om_s, fw_s, sem):
    WR, WS = 512, 8
    xa_s, c_s, ca_s, wo_s, q_s, qa_s, wg_s, wu_s, wd_s, xs_s, t0_s = [
        _Bf16(r) for r in (xa_r, c_r, ca_r, wo_r, q_r, qa_r, wg_r, wu_r, wd_r, xs_r, t0_r)]
    mk = pltpu.make_async_copy
    wq32, wk32, wv32 = wq_hbm.bitcast(u32), wk_hbm.bitcast(u32), wv_hbm.bitcast(u32)
    cp_wq = lambda j: mk(wq32.at[:, j, :], wq_p.at[j], sem.at[SEM_WQ + j])
    cp_kv = lambda j, m: mk((wk32, wv32)[m].at[:, j, :], wkv_p.at[j & 1, m], sem.at[SEM_KV + m])
    cp_xt = lambda k: mk(xt_hbm.at[:, pl.ds(k * XC, XC)], xt_s.at[:, pl.ds(k * XC, XC)], sem.at[SEM_XT + k])
    cp_out = lambda i: mk(out_s.at[i], o_hbm.at[:, pl.ds(i * T, T)], sem.at[SEM_OUT + i])
    cp_vec = [mk(wr_hbm, wr_s, sem.at[SEM_VEC]), mk(gw_hbm, gw_s, sem.at[SEM_VEC + 1])]
    cp_ffn = [mk(src, dst, sem.at[SEM_FFN + n]) for n, (src, dst) in
              enumerate(((wg_hbm.bitcast(u32), wg_r), (wu_hbm.bitcast(u32), wu_r), (wd_hbm.bitcast(u32), wd_r)))]
    cp_wo = mk(wo_hbm.bitcast(u32), wo_r, sem.at[SEM_WO])
    c32 = c_hbm.bitcast(u32)

    def cp_c(j):
        r0 = (j - 1) * (NG * RB // 2)
        n = QS // 2 - r0 if isinstance(j, int) and j == NP - 1 else NG * RB // 2
        return [mk(c32.at[pl.ds(i * QS // 2 + r0, n)], c_r.at[pl.ds(i * QS // 2 + r0, n)], sem.at[SEM_C + j])
                for i in range(4)]

    cp_xt(0).start()
    cp_wq(0).start()
    for k in range(1, S // XC):
        cp_xt(k).start()
    for cp in cp_vec:
        cp.start()
    for j in range(1, NP):
        cp_wq(j).start()
        for cp in cp_c(j):
            cp.start()
    for cp in cp_ffn + [cp_kv(0, 0), cp_kv(0, 1), cp_wo]:
        cp.start()

    @pl.loop(0, NQ // 2)
    def _(n):
        om_s[n] = jnp.zeros(om_s.shape[1:], f32)

    def store_q(j, e, r0, q):
        q = q * QSCALE
        q_s[2 * j + e, r0:r0 + q.shape[0], :] = q.astype(bf)
        for p0 in range(0, q.shape[0], 2 * T):
            if r0 + p0 > 0:
                qa, qb = q[p0:p0 + T], q[p0 + T:p0 + 2 * T]
                terms = _lhs_terms(qa[:, :T], qa[:, T:], qb[:, :T], qb[:, T:])
                for k, i in enumerate((0, 1, 4, 5, 6)):
                    qa_s[2 * j + e, (r0 + p0) // 2:(r0 + p0) // 2 + T, k * T:(k + 1) * T] = terms[i].astype(bf)

    def q_plain(w, r0, hook=None):
        prod = lambda a, b, wn, z: _dot(_feed(x_s[0, a:b, :], z), wn[:HM]) + _dot(x_s[1, a:b, :], wn[HM:])
        if hook is None:
            qf = prod(r0, r0 + 2 * T, w, None)
        else:
            qf = jnp.concatenate([jnp.concatenate(
                [prod(r0 + u * T, r0 + (u + 1) * T, w[:, n * T:(n + 1) * T], hook()) for u in range(2)], axis=0)
                for n in range(4)], axis=1)
        store_q(0, 0, r0, qf[:, :D])
        store_q(0, 1, r0, qf[:, D:])

    def q_rhs(j):
        lo, hi = pltpu.bitcast(wq_p[j] << 16, f32), pltpu.bitcast(wq_p[j] & jnp.uint32(HI), f32)
        b = [jnp.concatenate([lo[:, t * T:(t + 1) * T], hi[:, t * T:(t + 1) * T]], axis=1) for t in range(2)]
        return [t.astype(bf) for t in _rhs_terms(b[0][:HM], b[1][:HM], b[0][HM:], b[1][HM:])]

    def q_strassen(j, ts, r0, r1, hook):
        def lhs(i, u):
            if i in (2, 3):
                return x_s[i - 2, (i - 2) * HS + u:(i - 2) * HS + u + T, :]
            return xa_s[i - 2 * (i > 3), u:u + T, :]
        cs = _strassen(lambda i: jnp.concatenate(
            [_dot(_feed(lhs(i, u), *hook()), ts[i]) for u in range(r0, r1, T)], axis=0))
        for u in range(2):
            for e in range(2):
                store_q(j, e, u * HS + r0, jnp.concatenate([c[:, e * T:(e + 1) * T] for c in cs[2 * u:2 * u + 2]], axis=1))

    def x_prep(r0):
        a = [x_s[e, h0 + r0:h0 + r0 + RB, :].astype(f32) for h0 in (0, HS) for e in (0, 1)]
        terms = _lhs_terms(*a)
        outs = []
        for k, i in enumerate((0, 1, 4, 5, 6)):
            outs.append(xa_s.put((k, slice(r0, r0 + RB)), terms[i].astype(bf)))
        return outs

    def c_prep(g, c0):
        blk = lambda i, k: c_s[pl.ds(i * QS + g * RB, RB), k * QC + c0:k * QC + c0 + T].astype(f32)
        outer = [_lhs_terms2(*[blk(2 * i1 + i2, 2 * k1 + k2) for i1 in range(2) for k1 in range(2)])
                 for i2 in range(2) for k2 in range(2)]
        outs = []
        for r1 in range(7):
            for r2, v in enumerate(_lhs_terms(*[o[r1] for o in outer])):
                outs.append(ca_s.put((7 * r1 + r2, pl.ds(g * RB, RB), slice(c0, c0 + T)), v.astype(bf)))
        return outs

    def c_pacer(g0, ng, first, last):
        return _Pacer([functools.partial(c_prep, g0 + t // 2, (t % 2) * T) for t in range(2 * ng)], 49, first, last)

    def transpose(k):
        for e in range(2):
            x_s[e, k * XC:(k + 1) * XC, :] = xt_s[e * HM:(e + 1) * HM, k * XC:(k + 1) * XC].T

    def q_w0():
        return jnp.concatenate([pltpu.bitcast(wq_p[0] << 16, f32).astype(bf),
                                pltpu.bitcast(wq_p[0] & jnp.uint32(HI), f32).astype(bf)], axis=1)

    cp_xt(0).wait()
    transpose(0)
    cp_wq(0).wait()
    q_plain(q_w0(), 0)
    for k in range(1, 4):
        cp_xt(k).wait()
    transpose(1)
    w0 = q_w0()
    transpose(2)
    q_plain(w0, XC)
    transpose(3)
    q_plain(w0, 2 * XC)
    for k in range(4, S // XC):
        cp_xt(k).wait()
    for cp in cp_vec:
        cp.wait()
    for k in range(4, S // XC):
        transpose(k)
    row8 = lax.broadcasted_iota(jnp.int32, (8, M), 0)
    x_pace = _Pacer([functools.partial(x_prep, r0) for r0 in range(0, HS, RB)], 5, 12, 40)
    routed = []

    def hook0():
        n = len(routed)
        if n < NQ:
            rg = jnp.where(row8 == 0, wr_s[...].reshape(1, M).astype(f32), gw_s[...].reshape(1, M).astype(f32))
            g_s[n] = _dot(rg.astype(bf), xt_s[:, n * T:(n + 1) * T])
            routed.append(n)
        return x_pace()
    w0 = q_w0()
    for k in range(3, S // XC):
        q_plain(w0, k * XC, hook0)
    assert x_pace.finished()

    rb = jnp.concatenate([g_s[n][0:1, :] for n in range(NQ)], axis=1).astype(bf).astype(f32)
    lane = lax.broadcasted_iota(jnp.int32, (1, S), 1)
    m1 = jnp.max(rb, axis=1, keepdims=True)
    i1 = jnp.minimum(jnp.min(jnp.where(rb == m1, lane, S)), S - 1)
    rb2 = jnp.where(lane == i1, -jnp.inf, rb)
    m2 = jnp.max(rb2, axis=1, keepdims=True)
    i2 = jnp.minimum(jnp.min(jnp.where(jnp.logical_and(rb2 == m2, lane != i1), lane, S)), S - 1)
    row16 = lax.broadcasted_iota(jnp.int32, (16, HM), 0)

    def x_row(e, i):
        blk = x_s[e, pl.ds(pl.multiple_of((i // 16) * 16, 16), 16), :].astype(f32)
        return jnp.sum(jnp.where(row16 == i % 16, blk, 0.0), axis=0, keepdims=True)
    for e in range(2):
        xs_s[e] = jnp.where(row16 == 0, x_row(e, i1), jnp.where(row16 == 1, x_row(e, i2), 0.0)).astype(bf)
    rsel_s[...] = jax.nn.sigmoid(jnp.where(lax.broadcasted_iota(jnp.int32, (16, T), 0) == 0, m1, m2))
    idx_s[0] = i1
    idx_s[1] = i2

    def q_body(it, carry):
        js = (2 * it + 1, 2 * it + 2)
        for j in js:
            for cp in [cp_wq(j)] + cp_c(j):
                cp.wait()
        pace = c_pacer(2 * it * NG, 2 * NG, 1, 112)
        for j in js:
            ts = q_rhs(j)
            for r0 in range(0, HS, HS):
                q_strassen(j, ts, r0, r0 + HS, lambda: (pace(),))
        assert pace.finished()
        return carry
    lax.fori_loop(0, 3, q_body, 0)

    for cp in cp_ffn + [cp_wq(NP - 1), cp_kv(0, 0), cp_kv(0, 1), cp_wo] + cp_c(NP - 1):
        cp.wait()

    def w_sum(hn, m, r0):
        w = [wkv_p[(hn >> 1) & 1, m, r:r + 8, :] for r in range(r0, r0 + WR, 8 * WS)]
        w = (jnp.concatenate(w, axis=0) << (16 * (1 - (hn & 1))).astype(u32)) & jnp.uint32(0x7FFF0000)
        return functools.reduce(jnp.add, [pltpu.bitcast(t, f32) for t in _vregs([w])])

    def w_balance(parts):
        n = len(parts) // 2
        sk, sv = [jnp.sum(functools.reduce(jnp.add, p), keepdims=True) for p in (parts[:n], parts[n:])]
        ok = jnp.logical_and(sk > 0, sv > 0)
        ratio = jnp.broadcast_to(jnp.where(ok, 1.4 * sk, 1.0) / jnp.where(ok, sv, 1.0), (8, T))
        e = jnp.clip(pltpu.bitcast(ratio, jnp.int32) & 0x7F800000, (127 - 40) << 23, (127 + 40) << 23)
        fw_s[0] = pltpu.bitcast(e, f32)
        fw_s[1] = pltpu.bitcast((254 << 23) - e, f32)
        return [e]

    def w_pacer(hn, first, last):
        parts = []
        return _Pacer([lambda m=m, r0=r0: parts.append(w_sum(hn, m, r0)) or parts[-1:]
                       for m in range(2) for r0 in range(0, DC, WR)] + [lambda: w_balance(parts)], 1, first, last)

    def first_terms(hn):
        w = _unpack(wkv_p[(hn >> 1) & 1, 0, :, :T], (16 * (1 - (hn & 1))).astype(u32))
        t = w[:HC] + 0.5 * w[HC:]
        return [t0_s.put((slice(None), slice(n * T, (n + 1) * T)), v.astype(bf))
                for n, v in enumerate((t[:QC], t[QC:] - t[:QC]))]

    def residual(n):
        g8 = jax.nn.sigmoid(g_s[n])
        g_s[n] = g8
        a = (1.0 - g8[1:2, :]) * xt_s[:, n * T:(n + 1) * T].astype(f32)
        acc_s[n] = a
        return [a]

    gs, us, ys, hid = [], [], {}, []
    xs_dot = lambda w_s, n: (_dot(xs_s[0], w_s[:HM, n * T:(n + 1) * T]) + _dot(xs_s[1], w_s[HM:, n * T:(n + 1) * T]))

    def swiglu():
        gg, uu = jnp.concatenate(gs, axis=1), jnp.concatenate(us, axis=1)
        hid.append((gg * jax.nn.sigmoid(gg) * uu).astype(bf))

    def down(n0, k0):
        t = _dot_nt(hid[0][:, k0:min(k0 + 512, F)], wd_s[n0:min(n0 + T, M), k0:min(k0 + 512, F)])
        ys[n0] = ys[n0] + t if n0 in ys else t
    side = []
    for n in range(F // T):
        side += [lambda n=n: gs.append(xs_dot(wg_s, n)), lambda n=n: us.append(xs_dot(wu_s, n))]
    side += [swiglu] + [lambda: None] * 7
    side += [functools.partial(down, n0, k0) for n0 in range(0, M, T) for k0 in range(0, F, 512)]
    c_pace = c_pacer((NP - 2) * NG, QS // RB - (NP - 2) * NG, 2, 56)
    r_pace = _Pacer([functools.partial(residual, n) for n in range(NQ)], M // 8, 1, 48)

    w_pace0 = w_pacer(jnp.int32(0), 4, 52)
    t_pace0 = _Pacer([lambda: first_terms(jnp.int32(0))], 32, 40, 56)

    def hook7():
        if side:
            side.pop(0)()
        return c_pace(), r_pace(), w_pace0(), t_pace0()
    ts7 = q_rhs(NP - 1)
    for r0 in range(0, HS, 1024):
        q_strassen(NP - 1, ts7, r0, r0 + 1024, hook7)
    assert not side and all(p.finished() for p in (c_pace, r_pace, w_pace0, t_pace0))
    y = jnp.concatenate([ys[n0] for n0 in range(0, M, T)] + [jnp.zeros((16, 512 - M), f32)], axis=1)
    yt = (y * rsel_s[:, 0:1]).T
    lane128 = lax.broadcasted_iota(jnp.int32, (1, T), 1)
    for e in range(2):
        i = idx_s[e]
        acc_s[i // T] += jnp.where(lane128 == i % T, (1.0 - g_s[i // T][1:2, :]) * yt[:M, e:e + 1], 0.0)

    for m in range(2):
        cp_kv(1, m).start()

    tri = lax.broadcasted_iota(jnp.int32, (T, T), 1) <= lax.broadcasted_iota(jnp.int32, (T, T), 0)
    prog = _head_program()

    def head(h, carry):
        par, slot = h & 1, (h >> 1) & 1
        @pl.when(jnp.logical_and(h < H - 1, par == 1))
        def _():
            for m in range(2):
                cp_kv((h + 1) >> 1, m).wait()

        sh = (16 * (1 - par)).astype(u32)
        rhs, fw, fw_inv = [], fw_s[0], fw_s[1]
        for r1 in range(7):
            wk, wv = [_unpack(wkv_p[slot, m], sh + (h >> (8 + r1)).astype(u32)) for m in range(2)]
            wv = jnp.concatenate([wv[:, :T] * fw[0:1], wv[:, T:] * fw[0:1]], axis=1)
            t = _rhs_terms2(wk[:HC], wv[:HC], wk[HC:], wv[HC:])[r1]
            rhs.append([u.astype(bf) for u in _rhs_terms(t[:QC, :T], t[:QC, T:], t[QC:, :T], t[QC:, T:])])
        rhs[1][1], rhs[1][3] = t0_s[:, :T], t0_s[:, T:]
        hn = jnp.minimum(h + 1, H - 1)
        t_pace = _Pacer([lambda: first_terms(hn)], 32, 196 - 14, 196)
        w_pace = w_pacer(hn, 60, 180)
        prods, inner_q, outer, kblk, vblk = {}, {}, {}, {}, {}

        def kv_product(r1, r2):
            m = prods.setdefault(r1, {})
            m[r2] = _dot(ca_s[7 * r1 + r2], rhs[r1][r2])
            if len(m) == 7:
                inner_q[r1] = (((m[3] - m[4]) + m[6]) + m[0], m[2] + m[4], m[1] + m[3], ((m[0] - m[1]) + m[2]) + m[5])
                for b in range(4):
                    if b not in kblk and all(q in inner_q for q in (0, 1, 3, 4, 6)):
                        p = {q: inner_q[q][b] for q in (0, 1, 3, 4, 6)}
                        e, d = p[3] + p[1], p[3] - p[1]
                        kblk[b] = (p[0] + ((d - p[4]) + p[6]), e * 2.0)
                        outer[b] = ((e + p[4]) + p[6], p[0] + d)
                    if len(inner_q) == 7:
                        p2, p5 = inner_q[2][b], inner_q[5][b]
                        vblk[b] = (((outer[b][0] + p2) - p5) * 0.5, (outer[b][1] + p2) + p5)

        def rows(blk, t0, t1):
            return jnp.concatenate([jnp.concatenate(
                [blk[2 * (t // 4 % 2) + j2][t // 8][t % 4 * T:(t % 4 + 1) * T] for j2 in range(2)], axis=1)
                for t in range(t0, t1)], axis=0)

        @functools.cache
        def k_tile(t):
            return rows(kblk, t, t + 1).astype(bf)

        @functools.cache
        def k_terms(J):
            ka, kb = rows(kblk, 2 * J, 2 * J + 1), rows(kblk, 2 * J + 1, 2 * J + 2)
            return [t.astype(bf) for t in _rhs_terms(ka[:, :T], kb[:, :T], ka[:, T:], kb[:, T:])]

        @functools.cache
        def v_tiles(c0, c1):
            return rows(vblk, c0, c1).astype(bf)

        scores, rmax, soft, o_sum = {}, {}, {}, {}
        q_tiles = lambda I: [q_s[h, i * T:(i + 1) * T, t * T:(t + 1) * T] for i in (2 * I, 2 * I + 1) for t in range(2)]

        def score_block(I, J):
            q4, qx = q_tiles(I), [qa_s[h, I * T:(I + 1) * T, k * T:(k + 1) * T] for k in range(5)]
            lhs = [qx[0], qx[1], q4[0], q4[3], qx[2], qx[3], qx[4]]
            cs = _strassen(lambda i: _dot_nt(_feed(lhs[i], t_pace(), w_pace()), k_terms(J)[i]))
            for n, c in enumerate(cs):
                s_s[I % 2, n // 2, 2 * J + n % 2] = c
            for u in range(2):
                sa, sb = s_s[I % 2, u, 2 * J], s_s[I % 2, u, 2 * J + 1]
                scores[2 * I + u, 2 * J] = s_s[I % 2, u, 2 * J]
                scores[2 * I + u, 2 * J + 1] = s_s[I % 2, u, 2 * J + 1]
                mx = jnp.maximum(sa, sb)
                rmax[2 * I + u] = jnp.maximum(rmax[2 * I + u], mx) if 2 * I + u in rmax else mx

        def score_diag(I):
            a, b = 2 * I, 2 * I + 1
            q4 = q_tiles(I)
            qa, qb = jnp.concatenate(q4[0:2], axis=1), jnp.concatenate(q4[2:4], axis=1)
            d1 = _dot_nt(jnp.concatenate([qa, qb], axis=0), k_tile(a))
            d2 = _dot_nt(qb, k_tile(b))
            scores[a, a], scores[b, a], scores[b, b] = jnp.where(tri, d1[:T], NEG), d1[T:], jnp.where(tri, d2, NEG)

        def pv_chunk(i, c0):
            if c0 == 0:
                mx = functools.reduce(jnp.maximum, ([rmax[i]] if i > 1 else [])
                                      + [scores[i, t] for t in range(i // 2 * 2, i + 1)])
                soft[i] = dict(m=jnp.max(mx, axis=1, keepdims=True), l=None, ctx=None)
            st = soft[i]
            c1 = min(c0 + 2, i + 1)
            p = jnp.exp2(jnp.concatenate([scores.pop((i, t)) for t in range(c0, c1)], axis=1) - st['m']).astype(bf)
            pf = p.astype(f32)
            for t in range(c1 - c0):
                st['l'] = pf[:, t * T:(t + 1) * T] if st['l'] is None else st['l'] + pf[:, t * T:(t + 1) * T]
            d = _dot(p, v_tiles(c0, c1))
            st['ctx'] = d if st['ctx'] is None else st['ctx'] + d

        def context(i):
            st = soft.pop(i)
            l = jnp.sum(st['l'], axis=1, keepdims=True)
            r = pl.reciprocal(l, approx=True)
            return st['ctx'] * (r * (2.0 - l * r) * fw_inv[0:1, 0:1])

        def ship(blocks):
            @pl.when(h == H - 1)
            def _():
                for i in blocks:
                    cp_out(i).start()

        def out_plain(i):
            wo, ctx = wo_s[h], context(i).astype(bf)
            for a0 in (0, HM):
                a = acc_s[i, a0:a0 + HM, :] + g_s[i][1:2, :] * _dot_nt(wo[a0:a0 + HM], ctx)
                acc_s[i, a0:a0 + HM, :] = a
                out_s[i, a0:a0 + HM, :] = a.astype(bf)
            ship([i])

        @functools.cache
        def wo_terms():
            w = wo_s[h].astype(f32)
            return [t.astype(bf) for t in _lhs_terms(w[:HM, :T], w[:HM, T:], w[HM:, :T], w[HM:, T:])]

        @functools.cache
        def ctx_terms(I):
            ca, cb = context(2 * I), context(2 * I + 1)
            return _rhs_terms(ca[:, :T], cb[:, :T], ca[:, T:], cb[:, T:])

        def out_product(I, k):
            om_s[I, k] += _dot_nt(wo_terms()[k], ctx_terms(I)[k].astype(bf))
            o_sum[I, k] = om_s[I, k]
            if all((I, q) in o_sum for q in range(7)):
                for n, c in enumerate(_strassen(lambda q: o_sum.pop((I, q)))):
                    i, a0 = 2 * I + n % 2, (n // 2) * HM
                    out_s[i, a0:a0 + HM, :] = (acc_s[i, a0:a0 + HM, :] + g_s[i][1:2, :] * c).astype(bf)
                ship([2 * I, 2 * I + 1])

        ops = {'m': kv_product, 'r': score_block, 'd': score_diag, 'p': pv_chunk,
               'o': out_product, 'S': out_plain}
        for op, *args in prog:
            ops[op](*args)
        assert t_pace.finished() and w_pace.finished()

        @pl.when(jnp.logical_and((h + 3) >> 1 < NP, par == 1))
        def _():
            for m in range(2):
                cp_kv((h + 3) >> 1, m).start()
        return carry

    lax.fori_loop(0, H, head, 0)
    for i in range(NQ):
        cp_out(i).wait()


@jax.jit
def pallas_gated_mix__compressed_kv_cla__moe_arch_mod__prompt_kernel(
    A_x: jax.Array,
    A_c_kv: jax.Array,
    A_w_q: jax.Array,
    A_w_uk: jax.Array,
    A_w_uv: jax.Array,
    A_w_o: jax.Array,
    B_x: jax.Array,
    B_w_r: jax.Array,
    B_w_gate: jax.Array,
    B_w_up: jax.Array,
    B_w_down: jax.Array,
    gate_w: jax.Array,
):
    del B_x
    V = pltpu.VMEM
    B = lambda *shape: V(shape[:-2] + (shape[-2] // 2, shape[-1]), u32)
    out_t = pl.pallas_call(
        _kernel,
        in_specs=[pl.BlockSpec(memory_space=pl.ANY)] * 11,
        out_specs=pl.BlockSpec(memory_space=pl.ANY),
        out_shape=jax.ShapeDtypeStruct((M, S), bf),
        scratch_shapes=[
            V((M, S), bf), V((2, S, HM), bf), B(5, HS, HM),
            B(S, DC), B(49, QS, QC),
            V((NP, M, D), u32), V((2, 2, DC, D), u32), B(H, M, D),
            B(H, S, D), B(H, HS, 5 * T),
            V((NQ, M, T), f32),
            B(M, F), B(M, F), B(M, F),
            V((M,), bf), V((M,), bf), V((NQ, M, T), bf),
            V((NQ, 8, T), f32), B(2, 16, HM), V((16, T), f32),
            pltpu.SMEM((2,), jnp.int32),
            V((2, 2, NQ, T, T), f32), B(QC, 2 * T),
            V((NQ // 2, 7, HM, T), f32),
            V((2, 8, T), f32),
            pltpu.SemaphoreType.DMA((NSEM,)),
        ],
        compiler_params=pltpu.CompilerParams(vmem_limit_bytes=110 * 1024 * 1024),
        name="gated_mix_cla_mod",
    )(A_x[0].T, A_c_kv[0], A_w_q, A_w_uk, A_w_uv, A_w_o.transpose(0, 2, 1), B_w_r, B_w_gate, B_w_up,
      B_w_down.T, gate_w)
    return out_t.T[None]
```

```python
import functools
import math

import jax
import jax.numpy as jnp
from jax import lax
from jax.experimental import pallas as pl
from jax.experimental.pallas import tpu as pltpu

S, M, H, D, DC, F = 2048, 448, 16, 256, 1024, 1792
T = 128
NP, NQ = H // 2, S // T
HS, HM, HC = S // 2, M // 2, DC // 2
QS, QC = S // 4, DC // 4
RB = 16
XC = 256
NG = 5
NT = (((1,), (1,)), ((), ()))
QSCALE = D ** -0.5 * math.log2(math.e)
NEG = -1e30
bf, f32, u32 = jnp.bfloat16, jnp.float32, jnp.uint32
HI = 0xFFFF0000

SEM_WO, SEM_FFN, SEM_VEC, SEM_KV, SEM_WQ, SEM_XT, SEM_C, SEM_OUT, NSEM = 0, 1, 4, 6, 8, 16, 24, 32, 48


def _lhs_terms(a11, a12, a21, a22):
    return [a11 + a22, a21 + a22, a11, a22, a11 + a12, a21 - a11, a12 - a22]


def _rhs_terms(b11, b12, b21, b22):
    return [b11 + b22, b11, b12 - b22, b21 - b11, b22, b11 + b12, b21 + b22]


def _strassen(mm, order=(1, 2, 3, 4, 0, 6, 5)):
    m = {i: mm(i) for i in order}
    m1, m2, m3, m4, m5, m6, m7 = [m[i] for i in range(7)]
    return (m4 - m5) + (m1 + m7), m3 + m5, m2 + m4, (m3 - m2) + (m1 + m6)


def _lhs_terms2(a11, a12, a21, a22):
    h21, q21, h22 = 0.5 * a21, 0.25 * a21, 0.5 * a22
    s1 = a11 + a22
    v, hs = a12 + q21, 0.5 * s1
    return [s1, q21 + h22, a11 + h21, h22 - q21, v + hs, h21 - a11, v - hs]


def _rhs_terms2(b11, b12, b21, b22):
    h21 = 0.5 * b21
    t1 = b11 + b22
    v, ht = b12 + 0.5 * h21, 0.5 * t1
    return [t1, b11 + h21, v - ht, h21 - b11, b22 - h21, v + ht, b22 + h21]


def _vregs(vals):
    ts = []
    for v in vals:
        v = v if v.dtype == u32 else pltpu.bitcast(v, u32)
        ts += [v[r:r + 8, c:c + T] for r in range(0, v.shape[0], 8) for c in range(0, v.shape[1] - T + 1, T)]
    return ts


def _zero_from(ts):
    acc = ts[:4]
    for i, t in enumerate(ts[4:]):
        acc[i % 4] = acc[i % 4] | t
    while len(acc) > 1:
        acc = [acc[i] | acc[i + 1] if i + 1 < len(acc) else acc[i] for i in range(0, len(acc), 2)]
    return (acc[0] >> 16) >> 16


def _feed(a, *zs):
    zs = [z for z in zs if z is not None]
    if not zs:
        return a
    a32 = pltpu.bitcast(a, u32)
    top = functools.reduce(lambda p, q: p | q, zs, a32[0:8, :T])
    if a32.shape[1] > T:
        top = jnp.concatenate([top, a32[0:8, T:]], axis=1)
    return pltpu.bitcast(jnp.concatenate([top, a32[8:]], axis=0), bf)


class _Pacer:
    def __init__(self, thunks, per, first, last):
        self.thunks, self.pool, self.k, self.done = list(thunks), [], 0, 0
        self.tot, self.first, self.last = per * len(self.thunks), first, last

    def __call__(self):
        self.k += 1
        if self.k <= self.first:
            return None
        want = min(self.tot, -(-(self.k - self.first) * self.tot // (self.last - self.first))) - self.done
        while len(self.pool) < want and self.thunks:
            self.pool += _vregs(self.thunks.pop(0)())
        outs, self.pool = self.pool[:want], self.pool[want:]
        self.done += len(outs)
        return _zero_from(outs) if outs else None

    def finished(self):
        return not self.thunks and not self.pool


_HEAD_ORDER = """
m1.1 m1.3 m1.4 m1.6 m1.0 m3.3 m3.6 m1.2 m3.4 m4.3 m3.1 m3.0 m4.4 m3.2 m3.5 m1.5 m4.6 m4.1 m4.0 m6.6 m6.3 m6.0
m4.5 m0.1 m6.4 m6.1 m6.5 m6.2 m4.2 m0.6 m0.4 m0.3 m0.0 m0.2 m0.5 m2.1 d0 m2.3 r7.0 m2.4 r7.1 m2.0 m2.6 m5.1 r7.2
m2.2 r7.4 m2.5 r7.3 r7.6 r7.5 m5.3 d7 m5.6 m5.4 m5.0 m5.2 m5.5 p14.0 r6.0 p1.0 p0.0 r6.2 r6.1 p14.2 p14.4 p14.6
p14.8 p14.10 p15.0 p14.12 p14.14 r6.3 r6.4 r6.5 p15.2 p15.4 p15.6 p15.8 p15.10 d6 p15.12 p15.14 p12.0 r5.0 p12.2
p12.4 p12.6 r5.3 r5.2 r5.1 p12.8 p13.0 p12.10 p13.2 r5.4 p13.4 p13.6 p13.8 p12.12 d5 o0.3 o0.2 o0.1 p10.0 o0.0
o0.5 p11.0 p13.10 r4.1 o0.4 p10.2 p13.12 p10.4 r4.0 o0.6 p10.6 p10.8 p11.2 p10.10 r4.2 r4.3 p11.4 d4 p11.6 o7.2
o7.0 o7.1 o7.4 o7.3 o7.6 o7.5 r3.0 p11.8 p8.0 p8.2 p8.4 p8.6 p9.0 p9.2 p11.10 p8.8 r3.1 d3 r3.2 o6.4 o6.2 p9.4
o6.0 o6.6 o6.3 o6.1 p7.0 r2.1 p9.6 p6.0 p9.8 p6.2 p6.4 r2.0 o6.5 p6.6 d2 p7.2 p4.0 o5.3 o5.2 o5.1 o5.4 o5.6 o5.5
o5.0 r1.0 p4.2 p7.4 p5.0 p7.6 p4.4 d1 p5.2 o4.4 o4.2 p2.0 o4.1 o4.0 o4.3 p3.0 o4.6 o4.5 p2.2 p5.4 o2.1 p3.2 S2
o3.3 o2.3 o2.6 o2.4 o2.0 o3.2 o2.2 o2.5 o3.5 o3.1 o3.6 o3.0 o3.4 S3
"""


def _head_program():
    return [(t[0],) + tuple(int(v) for v in t[1:].split('.')) for t in _HEAD_ORDER.split()]


def _dot(a, b):
    return jnp.dot(a, b, preferred_element_type=f32)


def _dot_nt(a, b):
    return lax.dot_general(a, b, NT, preferred_element_type=f32)


def _unpack(w32, sh):
    return pltpu.bitcast((w32 << sh) & jnp.uint32(HI), f32)


class _Bf16:
    def __init__(self, raw):
        self.raw = raw

    def _half(self, idx):
        idx = list(idx if isinstance(idx, tuple) else (idx,))
        idx += [slice(None)] * (len(self.raw.shape) - len(idx))
        r = idx[-2]
        if isinstance(r, slice):
            idx[-2] = slice(None if r.start is None else r.start // 2, None if r.stop is None else r.stop // 2)
        elif isinstance(r.start, int):
            idx[-2] = pl.ds(r.start // 2, r.size // 2)
        else:
            idx[-2] = pl.ds(pl.multiple_of(r.start >> 1, 8), r.size // 2)
        return tuple(idx)

    def __getitem__(self, idx):
        return pltpu.bitcast(self.raw[self._half(idx)], bf)

    def put(self, idx, v):
        idx = self._half(idx)
        ref = self.raw.at[idx[:-2]] if len(idx) > 2 else self.raw
        o = pltpu.bitcast(v, u32)
        ref[idx[-2], idx[-1]] = o
        return o

    def __setitem__(self, idx, v):
        self.put(idx, v)


def _kernel(xt_hbm, c_hbm, wq_hbm, wk_hbm, wv_hbm, wo_hbm, wr_hbm, wg_hbm, wu_hbm, wd_hbm, gw_hbm, o_hbm,
            xt_s, x_s, xa_r, c_r, ca_r, wq_p, wkv_p, wo_r, q_r, qa_r, acc_s, wg_r, wu_r, wd_r,
            wr_s, gw_s, out_s, g_s, xs_r, rsel_s, idx_s, s_s, t0_r, om_s, fw_s, sem):
    WR, WS = 512, 8
    xa_s, c_s, ca_s, wo_s, q_s, qa_s, wg_s, wu_s, wd_s, xs_s, t0_s = [
        _Bf16(r) for r in (xa_r, c_r, ca_r, wo_r, q_r, qa_r, wg_r, wu_r, wd_r, xs_r, t0_r)]
    mk = pltpu.make_async_copy
    wq32, wk32, wv32 = wq_hbm.bitcast(u32), wk_hbm.bitcast(u32), wv_hbm.bitcast(u32)
    cp_wq = lambda j: mk(wq32.at[:, j, :], wq_p.at[j], sem.at[SEM_WQ + j])
    cp_kv = lambda j, m: mk((wk32, wv32)[m].at[:, j, :], wkv_p.at[j & 1, m], sem.at[SEM_KV + m])
    cp_xt = lambda k: mk(xt_hbm.at[:, pl.ds(k * XC, XC)], xt_s.at[:, pl.ds(k * XC, XC)], sem.at[SEM_XT + k])
    cp_out = lambda i: mk(out_s.at[i], o_hbm.at[:, pl.ds(i * T, T)], sem.at[SEM_OUT + i])
    cp_vec = [mk(wr_hbm, wr_s, sem.at[SEM_VEC]), mk(gw_hbm, gw_s, sem.at[SEM_VEC + 1])]
    cp_ffn = [mk(src, dst, sem.at[SEM_FFN + n]) for n, (src, dst) in
              enumerate(((wg_hbm.bitcast(u32), wg_r), (wu_hbm.bitcast(u32), wu_r), (wd_hbm.bitcast(u32), wd_r)))]
    cp_wo = mk(wo_hbm.bitcast(u32), wo_r, sem.at[SEM_WO])
    c32 = c_hbm.bitcast(u32)

    def cp_c(j):
        r0 = (j - 1) * (NG * RB // 2)
        n = QS // 2 - r0 if isinstance(j, int) and j == NP - 1 else NG * RB // 2
        return [mk(c32.at[pl.ds(i * QS // 2 + r0, n)], c_r.at[pl.ds(i * QS // 2 + r0, n)], sem.at[SEM_C + j])
                for i in range(4)]

    cp_xt(0).start()
    cp_wq(0).start()
    for k in range(1, S // XC):
        cp_xt(k).start()
    for cp in cp_vec:
        cp.start()
    for j in range(1, NP):
        cp_wq(j).start()
        for cp in cp_c(j):
            cp.start()
    for cp in cp_ffn + [cp_kv(0, 0), cp_kv(0, 1), cp_wo]:
        cp.start()

    @pl.loop(0, NQ // 2)
    def _(n):
        om_s[n] = jnp.zeros(om_s.shape[1:], f32)

    def store_q(j, e, r0, q):
        q = q * QSCALE
        q_s[2 * j + e, r0:r0 + q.shape[0], :] = q.astype(bf)
        for p0 in range(0, q.shape[0], 2 * T):
            if r0 + p0 > 0:
                qa, qb = q[p0:p0 + T], q[p0 + T:p0 + 2 * T]
                terms = _lhs_terms(qa[:, :T], qa[:, T:], qb[:, :T], qb[:, T:])
                for k, i in enumerate((0, 1, 4, 5, 6)):
                    qa_s[2 * j + e, (r0 + p0) // 2:(r0 + p0) // 2 + T, k * T:(k + 1) * T] = terms[i].astype(bf)

    def q_plain(w, r0, hook=None):
        prod = lambda a, b, wn, z: _dot(_feed(x_s[0, a:b, :], z), wn[:HM]) + _dot(x_s[1, a:b, :], wn[HM:])
        if hook is None:
            qf = prod(r0, r0 + 2 * T, w, None)
        else:
            qf = jnp.concatenate([jnp.concatenate(
                [prod(r0 + u * T, r0 + (u + 1) * T, w[:, n * T:(n + 1) * T], hook()) for u in range(2)], axis=0)
                for n in range(4)], axis=1)
        store_q(0, 0, r0, qf[:, :D])
        store_q(0, 1, r0, qf[:, D:])

    def q_rhs(j):
        lo, hi = pltpu.bitcast(wq_p[j] << 16, f32), pltpu.bitcast(wq_p[j] & jnp.uint32(HI), f32)
        b = [jnp.concatenate([lo[:, t * T:(t + 1) * T], hi[:, t * T:(t + 1) * T]], axis=1) for t in range(2)]
        return [t.astype(bf) for t in _rhs_terms(b[0][:HM], b[1][:HM], b[0][HM:], b[1][HM:])]

    def q_strassen(j, ts, r0, r1, hook):
        def lhs(i, u):
            if i in (2, 3):
                return x_s[i - 2, (i - 2) * HS + u:(i - 2) * HS + u + T, :]
            return xa_s[i - 2 * (i > 3), u:u + T, :]
        cs = _strassen(lambda i: jnp.concatenate(
            [_dot(_feed(lhs(i, u), *hook()), ts[i]) for u in range(r0, r1, T)], axis=0), (1, 2, 3, 4, 0, 6, 5))
        for u in range(2):
            for e in range(2):
                store_q(j, e, u * HS + r0, jnp.concatenate([c[:, e * T:(e + 1) * T] for c in cs[2 * u:2 * u + 2]], axis=1))

    def x_prep(r0):
        a = [x_s[e, h0 + r0:h0 + r0 + RB, :].astype(f32) for h0 in (0, HS) for e in (0, 1)]
        terms = _lhs_terms(*a)
        outs = []
        for k, i in enumerate((0, 1, 4, 5, 6)):
            outs.append(xa_s.put((k, slice(r0, r0 + RB)), terms[i].astype(bf)))
        return outs

    def c_prep(g, c0):
        blk = lambda i, k: c_s[pl.ds(i * QS + g * RB, RB), k * QC + c0:k * QC + c0 + T].astype(f32)
        outer = [_lhs_terms2(*[blk(2 * i1 + i2, 2 * k1 + k2) for i1 in range(2) for k1 in range(2)])
                 for i2 in range(2) for k2 in range(2)]
        outs = []
        for r1 in range(7):
            for r2, v in enumerate(_lhs_terms(*[o[r1] for o in outer])):
                outs.append(ca_s.put((7 * r1 + r2, pl.ds(g * RB, RB), slice(c0, c0 + T)), v.astype(bf)))
        return outs

    def c_pacer(g0, ng, first, last):
        return _Pacer([functools.partial(c_prep, g0 + t // 2, (t % 2) * T) for t in range(2 * ng)], 49, first, last)

    def transpose(k):
        for e in range(2):
            x_s[e, k * XC:(k + 1) * XC, :] = xt_s[e * HM:(e + 1) * HM, k * XC:(k + 1) * XC].T

    def q_w0():
        return jnp.concatenate([pltpu.bitcast(wq_p[0] << 16, f32).astype(bf),
                                pltpu.bitcast(wq_p[0] & jnp.uint32(HI), f32).astype(bf)], axis=1)

    cp_xt(0).wait()
    transpose(0)
    cp_wq(0).wait()
    q_plain(q_w0(), 0)
    for k in range(1, 4):
        cp_xt(k).wait()
    transpose(1)
    w0 = q_w0()
    transpose(2)
    q_plain(w0, XC)
    transpose(3)
    q_plain(w0, 2 * XC)
    for k in range(4, S // XC):
        cp_xt(k).wait()
    for cp in cp_vec:
        cp.wait()
    for k in range(4, S // XC):
        transpose(k)
    row8 = lax.broadcasted_iota(jnp.int32, (8, M), 0)
    x_pace = _Pacer([functools.partial(x_prep, r0) for r0 in range(0, HS, RB)], 5, 12, 40)
    routed = []

    def hook0():
        n = len(routed)
        if n < NQ:
            rg = jnp.where(row8 == 0, wr_s[...].reshape(1, M).astype(f32), gw_s[...].reshape(1, M).astype(f32))
            g_s[n] = _dot(rg.astype(bf), xt_s[:, n * T:(n + 1) * T])
            routed.append(n)
        return x_pace()
    w0 = q_w0()
    for k in range(3, S // XC):
        q_plain(w0, k * XC, hook0)
    assert x_pace.finished()

    rb = jnp.concatenate([g_s[n][0:1, :] for n in range(NQ)], axis=1).astype(bf).astype(f32)
    lane = lax.broadcasted_iota(jnp.int32, (1, S), 1)
    m1 = jnp.max(rb, axis=1, keepdims=True)
    i1 = jnp.minimum(jnp.min(jnp.where(rb == m1, lane, S)), S - 1)
    rb2 = jnp.where(lane == i1, -jnp.inf, rb)
    m2 = jnp.max(rb2, axis=1, keepdims=True)
    i2 = jnp.minimum(jnp.min(jnp.where(jnp.logical_and(rb2 == m2, lane != i1), lane, S)), S - 1)
    row16 = lax.broadcasted_iota(jnp.int32, (16, HM), 0)

    def x_row(e, i):
        blk = x_s[e, pl.ds(pl.multiple_of((i // 16) * 16, 16), 16), :].astype(f32)
        return jnp.sum(jnp.where(row16 == i % 16, blk, 0.0), axis=0, keepdims=True)
    for e in range(2):
        xs_s[e] = jnp.where(row16 == 0, x_row(e, i1), jnp.where(row16 == 1, x_row(e, i2), 0.0)).astype(bf)
    rsel_s[...] = jax.nn.sigmoid(jnp.where(lax.broadcasted_iota(jnp.int32, (16, T), 0) == 0, m1, m2))
    idx_s[0] = i1
    idx_s[1] = i2

    def q_body(it, carry):
        js = (2 * it + 1, 2 * it + 2)
        for j in js:
            for cp in [cp_wq(j)] + cp_c(j):
                cp.wait()
        pace = c_pacer(2 * it * NG, 2 * NG, 1, 108)
        for j in js:
            ts = q_rhs(j)
            for r0 in range(0, HS, HS):
                q_strassen(j, ts, r0, r0 + HS, lambda: (pace(),))
        assert pace.finished()
        return carry
    lax.fori_loop(0, 3, q_body, 0)

    for cp in cp_ffn + [cp_wq(NP - 1), cp_kv(0, 0), cp_kv(0, 1)] + cp_c(NP - 1):
        cp.wait()

    def w_sum(hn, m, r0):
        w = [wkv_p[(hn >> 1) & 1, m, r:r + 8, :] for r in range(r0, r0 + WR, 8 * WS)]
        w = (jnp.concatenate(w, axis=0) << (16 * (1 - (hn & 1))).astype(u32)) & jnp.uint32(0x7FFF0000)
        return functools.reduce(jnp.add, [pltpu.bitcast(t, f32) for t in _vregs([w])])

    def w_balance(parts):
        n = len(parts) // 2
        sk, sv = [jnp.sum(functools.reduce(jnp.add, p), keepdims=True) for p in (parts[:n], parts[n:])]
        ok = jnp.logical_and(sk > 0, sv > 0)
        ratio = jnp.broadcast_to(jnp.where(ok, 1.4 * sk, 1.0) / jnp.where(ok, sv, 1.0), (8, T))
        e = jnp.clip(pltpu.bitcast(ratio, jnp.int32) & 0x7F800000, (127 - 40) << 23, (127 + 40) << 23)
        fw_s[0] = pltpu.bitcast(e, f32)
        fw_s[1] = pltpu.bitcast((254 << 23) - e, f32)
        return [e]

    def w_pacer(hn, first, last):
        parts = []
        return _Pacer([lambda m=m, r0=r0: parts.append(w_sum(hn, m, r0)) or parts[-1:]
                       for m in range(2) for r0 in range(0, DC, WR)] + [lambda: w_balance(parts)], 1, first, last)

    def first_terms(hn):
        w = _unpack(wkv_p[(hn >> 1) & 1, 0, :, :T], (16 * (1 - (hn & 1))).astype(u32))
        t = w[:HC] + 0.5 * w[HC:]
        return [t0_s.put((slice(None), slice(n * T, (n + 1) * T)), v.astype(bf))
                for n, v in enumerate((t[:QC], t[QC:] - t[:QC]))]

    def residual(n):
        g8 = jax.nn.sigmoid(g_s[n])
        g_s[n] = g8
        a = (1.0 - g8[1:2, :]) * xt_s[:, n * T:(n + 1) * T].astype(f32)
        acc_s[n] = a
        return [a]

    gs, us, ys, hid = [], [], {}, []
    xs_dot = lambda w_s, n: (_dot(xs_s[0], w_s[:HM, n * T:(n + 1) * T]) + _dot(xs_s[1], w_s[HM:, n * T:(n + 1) * T]))

    def swiglu():
        gg, uu = jnp.concatenate(gs, axis=1), jnp.concatenate(us, axis=1)
        hid.append((gg * jax.nn.sigmoid(gg) * uu).astype(bf))

    def down(n0, k0):
        t = _dot_nt(hid[0][:, k0:min(k0 + 512, F)], wd_s[n0:min(n0 + T, M), k0:min(k0 + 512, F)])
        ys[n0] = ys[n0] + t if n0 in ys else t
    side = []
    for n in range(F // T):
        side += [lambda n=n: gs.append(xs_dot(wg_s, n)), lambda n=n: us.append(xs_dot(wu_s, n))]
    side += [swiglu] + [lambda: None] * 7
    side += [functools.partial(down, n0, k0) for n0 in range(0, M, T) for k0 in range(0, F, 512)]
    c_pace = c_pacer((NP - 2) * NG, QS // RB - (NP - 2) * NG, 2, 56)
    r_pace = _Pacer([functools.partial(residual, n) for n in range(NQ)], M // 8, 1, 48)

    w_pace0 = w_pacer(jnp.int32(0), 4, 52)
    t_pace0 = _Pacer([lambda: first_terms(jnp.int32(0))], 32, 40, 56)

    def hook7():
        if side:
            side.pop(0)()
        return c_pace(), r_pace(), w_pace0(), t_pace0()
    ts7 = q_rhs(NP - 1)
    for r0 in range(0, HS, 1024):
        q_strassen(NP - 1, ts7, r0, r0 + 1024, hook7)
    assert not side and all(p.finished() for p in (c_pace, r_pace, w_pace0, t_pace0))
    y = jnp.concatenate([ys[n0] for n0 in range(0, M, T)] + [jnp.zeros((16, 512 - M), f32)], axis=1)
    yt = (y * rsel_s[:, 0:1]).T
    lane128 = lax.broadcasted_iota(jnp.int32, (1, T), 1)
    for e in range(2):
        i = idx_s[e]
        acc_s[i // T] += jnp.where(lane128 == i % T, (1.0 - g_s[i // T][1:2, :]) * yt[:M, e:e + 1], 0.0)

    for m in range(2):
        cp_kv(1, m).start()
    cp_wo.wait()

    tri = lax.broadcasted_iota(jnp.int32, (T, T), 1) <= lax.broadcasted_iota(jnp.int32, (T, T), 0)
    prog = _head_program()

    def head(h, carry):
        par, slot = h & 1, (h >> 1) & 1
        @pl.when(jnp.logical_and(h < H - 1, par == 1))
        def _():
            for m in range(2):
                cp_kv((h + 1) >> 1, m).wait()

        sh = (16 * (1 - par)).astype(u32)
        rhs, fw, fw_inv = [], fw_s[0], fw_s[1]
        for r1 in range(7):
            wk, wv = [_unpack(wkv_p[slot, m], sh + (h >> (8 + r1)).astype(u32)) for m in range(2)]
            wv = jnp.concatenate([wv[:, :T] * fw[0:1], wv[:, T:] * fw[0:1]], axis=1)
            t = _rhs_terms2(wk[:HC], wv[:HC], wk[HC:], wv[HC:])[r1]
            rhs.append([u.astype(bf) for u in _rhs_terms(t[:QC, :T], t[:QC, T:], t[QC:, :T], t[QC:, T:])])
        rhs[1][1], rhs[1][3] = t0_s[:, :T], t0_s[:, T:]
        hn = jnp.minimum(h + 1, H - 1)
        t_pace = _Pacer([lambda: first_terms(hn)], 32, 196 - 14, 196)
        w_pace = w_pacer(hn, 60, 180)
        prods, inner_q, outer, kblk, vblk = {}, {}, {}, {}, {}

        def kv_product(r1, r2):
            m = prods.setdefault(r1, {})
            m[r2] = _dot(ca_s[7 * r1 + r2], rhs[r1][r2])
            if len(m) == 7:
                inner_q[r1] = (((m[3] - m[4]) + m[6]) + m[0], m[2] + m[4], m[1] + m[3], ((m[0] - m[1]) + m[2]) + m[5])
                for b in range(4):
                    if b not in kblk and all(q in inner_q for q in (0, 1, 3, 4, 6)):
                        p = {q: inner_q[q][b] for q in (0, 1, 3, 4, 6)}
                        e, d = p[3] + p[1], p[3] - p[1]
                        kblk[b] = (p[0] + ((d - p[4]) + p[6]), e * 2.0)
                        outer[b] = ((e + p[4]) + p[6], p[0] + d)
                    if len(inner_q) == 7:
                        p2, p5 = inner_q[2][b], inner_q[5][b]
                        vblk[b] = (((outer[b][0] + p2) - p5) * 0.5, (outer[b][1] + p2) + p5)

        def rows(blk, t0, t1):
            return jnp.concatenate([jnp.concatenate(
                [blk[2 * (t // 4 % 2) + j2][t // 8][t % 4 * T:(t % 4 + 1) * T] for j2 in range(2)], axis=1)
                for t in range(t0, t1)], axis=0)

        @functools.cache
        def k_tile(t):
            return rows(kblk, t, t + 1).astype(bf)

        @functools.cache
        def k_terms(J):
            ka, kb = rows(kblk, 2 * J, 2 * J + 1), rows(kblk, 2 * J + 1, 2 * J + 2)
            return [t.astype(bf) for t in _rhs_terms(ka[:, :T], kb[:, :T], ka[:, T:], kb[:, T:])]

        @functools.cache
        def v_tiles(c0, c1):
            return rows(vblk, c0, c1).astype(bf)

        scores, rmax, soft, o_sum = {}, {}, {}, {}
        q_tiles = lambda I: [q_s[h, i * T:(i + 1) * T, t * T:(t + 1) * T] for i in (2 * I, 2 * I + 1) for t in range(2)]

        def score_block(I, J):
            q4, qx = q_tiles(I), [qa_s[h, I * T:(I + 1) * T, k * T:(k + 1) * T] for k in range(5)]
            lhs = [qx[0], qx[1], q4[0], q4[3], qx[2], qx[3], qx[4]]
            cs = _strassen(lambda i: _dot_nt(_feed(lhs[i], t_pace(), w_pace()), k_terms(J)[i]))
            for n, c in enumerate(cs):
                s_s[I % 2, n // 2, 2 * J + n % 2] = c
            for u in range(2):
                sa, sb = s_s[I % 2, u, 2 * J], s_s[I % 2, u, 2 * J + 1]
                scores[2 * I + u, 2 * J] = s_s[I % 2, u, 2 * J]
                scores[2 * I + u, 2 * J + 1] = s_s[I % 2, u, 2 * J + 1]
                mx = jnp.maximum(sa, sb)
                rmax[2 * I + u] = jnp.maximum(rmax[2 * I + u], mx) if 2 * I + u in rmax else mx

        def score_diag(I):
            a, b = 2 * I, 2 * I + 1
            q4 = q_tiles(I)
            qa, qb = jnp.concatenate(q4[0:2], axis=1), jnp.concatenate(q4[2:4], axis=1)
            d1 = _dot_nt(jnp.concatenate([qa, qb], axis=0), k_tile(a))
            d2 = _dot_nt(qb, k_tile(b))
            scores[a, a], scores[b, a], scores[b, b] = jnp.where(tri, d1[:T], NEG), d1[T:], jnp.where(tri, d2, NEG)

        def pv_chunk(i, c0):
            if c0 == 0:
                mx = functools.reduce(jnp.maximum, ([rmax[i]] if i > 1 else [])
                                      + [scores[i, t] for t in range(i // 2 * 2, i + 1)])
                soft[i] = dict(m=jnp.max(mx, axis=1, keepdims=True), l=None, ctx=None)
            st = soft[i]
            c1 = min(c0 + 2, i + 1)
            p = jnp.exp2(jnp.concatenate([scores.pop((i, t)) for t in range(c0, c1)], axis=1) - st['m']).astype(bf)
            pf = p.astype(f32)
            for t in range(c1 - c0):
                st['l'] = pf[:, t * T:(t + 1) * T] if st['l'] is None else st['l'] + pf[:, t * T:(t + 1) * T]
            d = _dot(p, v_tiles(c0, c1))
            st['ctx'] = d if st['ctx'] is None else st['ctx'] + d

        def context(i):
            st = soft.pop(i)
            l = jnp.sum(st['l'], axis=1, keepdims=True)
            r = pl.reciprocal(l, approx=True)
            return st['ctx'] * (r * (2.0 - l * r) * fw_inv[0:1, 0:1])

        def ship(blocks):
            @pl.when(h == H - 1)
            def _():
                for i in blocks:
                    cp_out(i).start()

        def out_plain(i):
            wo, ctx = wo_s[h], context(i).astype(bf)
            for a0 in (0, HM):
                a = acc_s[i, a0:a0 + HM, :] + g_s[i][1:2, :] * _dot_nt(wo[a0:a0 + HM], ctx)
                acc_s[i, a0:a0 + HM, :] = a
                out_s[i, a0:a0 + HM, :] = a.astype(bf)
            ship([i])

        @functools.cache
        def wo_terms():
            w = wo_s[h].astype(f32)
            return [t.astype(bf) for t in _lhs_terms(w[:HM, :T], w[:HM, T:], w[HM:, :T], w[HM:, T:])]

        @functools.cache
        def ctx_terms(I):
            ca, cb = context(2 * I), context(2 * I + 1)
            return _rhs_terms(ca[:, :T], cb[:, :T], ca[:, T:], cb[:, T:])

        def out_product(I, k):
            om_s[I, k] += _dot_nt(wo_terms()[k], ctx_terms(I)[k].astype(bf))
            o_sum[I, k] = om_s[I, k]
            if all((I, q) in o_sum for q in range(7)):
                for n, c in enumerate(_strassen(lambda q: o_sum.pop((I, q)))):
                    i, a0 = 2 * I + n % 2, (n // 2) * HM
                    out_s[i, a0:a0 + HM, :] = (acc_s[i, a0:a0 + HM, :] + g_s[i][1:2, :] * c).astype(bf)
                ship([2 * I, 2 * I + 1])

        ops = {'m': kv_product, 'r': score_block, 'd': score_diag, 'p': pv_chunk,
               'o': out_product, 'S': out_plain}
        for op, *args in prog:
            ops[op](*args)
        assert t_pace.finished() and w_pace.finished()

        @pl.when(jnp.logical_and((h + 3) >> 1 < NP, par == 1))
        def _():
            for m in range(2):
                cp_kv((h + 3) >> 1, m).start()
        return carry

    lax.fori_loop(0, H, head, 0)
    for i in range(NQ):
        cp_out(i).wait()


@jax.jit
def pallas_gated_mix__compressed_kv_cla__moe_arch_mod__prompt_kernel(
    A_x: jax.Array,
    A_c_kv: jax.Array,
    A_w_q: jax.Array,
    A_w_uk: jax.Array,
    A_w_uv: jax.Array,
    A_w_o: jax.Array,
    B_x: jax.Array,
    B_w_r: jax.Array,
    B_w_gate: jax.Array,
    B_w_up: jax.Array,
    B_w_down: jax.Array,
    gate_w: jax.Array,
):
    del B_x
    V = pltpu.VMEM
    B = lambda *shape: V(shape[:-2] + (shape[-2] // 2, shape[-1]), u32)
    out_t = pl.pallas_call(
        _kernel,
        in_specs=[pl.BlockSpec(memory_space=pl.ANY)] * 11,
        out_specs=pl.BlockSpec(memory_space=pl.ANY),
        out_shape=jax.ShapeDtypeStruct((M, S), bf),
        scratch_shapes=[
            V((M, S), bf), V((2, S, HM), bf), B(5, HS, HM),
            B(S, DC), B(49, QS, QC),
            V((NP, M, D), u32), V((2, 2, DC, D), u32), B(H, M, D),
            B(H, S, D), B(H, HS, 5 * T),
            V((NQ, M, T), f32),
            B(M, F), B(M, F), B(M, F),
            V((M,), bf), V((M,), bf), V((NQ, M, T), bf),
            V((NQ, 8, T), f32), B(2, 16, HM), V((16, T), f32),
            pltpu.SMEM((2,), jnp.int32),
            V((2, 2, NQ, T, T), f32), B(QC, 2 * T),
            V((NQ // 2, 7, HM, T), f32),
            V((2, 8, T), f32),
            pltpu.SemaphoreType.DMA((NSEM,)),
        ],
        compiler_params=pltpu.CompilerParams(vmem_limit_bytes=110 * 1024 * 1024),
        name="gated_mix_cla_mod",
    )(A_x[0].T, A_c_kv[0], A_w_q, A_w_uk, A_w_uv, A_w_o.transpose(0, 2, 1), B_w_r, B_w_gate, B_w_up,
      B_w_down.T, gate_w)
    return out_t.T[None]
```

```python
import functools
import math

import jax
import jax.numpy as jnp
from jax import lax
from jax.experimental import pallas as pl
from jax.experimental.pallas import tpu as pltpu

S, M, H, D, DC, F = 2048, 448, 16, 256, 1024, 1792
T = 128
NP, NQ = H // 2, S // T
HS, HM, HC = S // 2, M // 2, DC // 2
QS, QC = S // 4, DC // 4
RB = 16
XC = 256
NG = 5
NT = (((1,), (1,)), ((), ()))
QSCALE = D ** -0.5 * math.log2(math.e)
NEG = -1e30
bf, f32, u32 = jnp.bfloat16, jnp.float32, jnp.uint32
HI = 0xFFFF0000

SEM_WO, SEM_FFN, SEM_VEC, SEM_KV, SEM_WQ, SEM_XT, SEM_C, SEM_OUT, NSEM = 0, 1, 4, 6, 8, 16, 24, 32, 48


def _lhs_terms(a11, a12, a21, a22):
    return [a11 + a22, a21 + a22, a11, a22, a11 + a12, a21 - a11, a12 - a22]


def _rhs_terms(b11, b12, b21, b22):
    return [b11 + b22, b11, b12 - b22, b21 - b11, b22, b11 + b12, b21 + b22]


def _strassen(mm):
    m2, m3, m4, m5, m1, m7, m6 = [mm(i) for i in (1, 2, 3, 4, 0, 6, 5)]
    return (m4 - m5) + (m1 + m7), m3 + m5, m2 + m4, (m3 - m2) + (m1 + m6)


def _lhs_terms2(a11, a12, a21, a22):
    h21, q21, h22 = 0.5 * a21, 0.25 * a21, 0.5 * a22
    s1 = a11 + a22
    v, hs = a12 + q21, 0.5 * s1
    return [s1, q21 + h22, a11 + h21, h22 - q21, v + hs, h21 - a11, v - hs]


def _rhs_terms2(b11, b12, b21, b22):
    h21 = 0.5 * b21
    t1 = b11 + b22
    v, ht = b12 + 0.5 * h21, 0.5 * t1
    return [t1, b11 + h21, v - ht, h21 - b11, b22 - h21, v + ht, b22 + h21]


def _vregs(vals):
    ts = []
    for v in vals:
        v = v if v.dtype == u32 else pltpu.bitcast(v, u32)
        ts += [v[r:r + 8, c:c + T] for r in range(0, v.shape[0], 8) for c in range(0, v.shape[1] - T + 1, T)]
    return ts


def _zero_from(ts):
    acc = ts[:4]
    for i, t in enumerate(ts[4:]):
        acc[i % 4] = acc[i % 4] | t
    while len(acc) > 1:
        acc = [acc[i] | acc[i + 1] if i + 1 < len(acc) else acc[i] for i in range(0, len(acc), 2)]
    return (acc[0] >> 16) >> 16


def _feed(a, *zs):
    zs = [z for z in zs if z is not None]
    if not zs:
        return a
    a32 = pltpu.bitcast(a, u32)
    top = functools.reduce(lambda p, q: p | q, zs, a32[0:8, :T])
    if a32.shape[1] > T:
        top = jnp.concatenate([top, a32[0:8, T:]], axis=1)
    return pltpu.bitcast(jnp.concatenate([top, a32[8:]], axis=0), bf)


class _Pacer:
    def __init__(self, thunks, per, first, last):
        self.thunks, self.pool, self.k, self.done = list(thunks), [], 0, 0
        self.tot, self.first, self.last = per * len(self.thunks), first, last

    def __call__(self):
        self.k += 1
        if self.k <= self.first:
            return None
        want = min(self.tot, -(-(self.k - self.first) * self.tot // (self.last - self.first))) - self.done
        while len(self.pool) < want and self.thunks:
            self.pool += _vregs(self.thunks.pop(0)())
        outs, self.pool = self.pool[:want], self.pool[want:]
        self.done += len(outs)
        return _zero_from(outs) if outs else None

    def finished(self):
        return not self.thunks and not self.pool


_HEAD_ORDER = """
m1.1 m1.3 m1.4 m1.6 m1.0 m3.3 m3.6 m1.2 m3.4 m4.3 m3.1 m3.0 m4.4 m3.2 m3.5 m1.5 m4.6 m4.1 m4.0 m6.6 m6.3 m6.0
m4.5 m0.1 m6.4 m6.1 m6.5 m6.2 m4.2 m0.6 m0.4 m0.3 m0.0 m0.2 m0.5 m2.1 d0 m2.3 r7.0 m2.4 r7.1 m2.0 m2.6 m5.1 r7.2
m2.2 r7.4 m2.5 r7.3 r7.6 r7.5 m5.3 d7 m5.6 m5.4 m5.0 m5.2 m5.5 p14.0 r6.0 p1.0 p0.0 r6.2 r6.1 p14.2 p14.4 p14.6
p14.8 p14.10 p15.0 p14.12 p14.14 r6.3 r6.4 r6.5 p15.2 p15.4 p15.6 p15.8 p15.10 d6 p15.12 p15.14 p12.0 r5.0 p12.2
p12.4 p12.6 r5.3 r5.2 r5.1 p12.8 p13.0 p12.10 p13.2 r5.4 p13.4 p13.6 p13.8 p12.12 d5 o0.3 o0.2 o0.1 p10.0 o0.0
o0.5 p11.0 p13.10 r4.1 o0.4 p10.2 p13.12 p10.4 r4.0 o0.6 p10.6 p10.8 p11.2 p10.10 r4.2 r4.3 p11.4 d4 p11.6 o7.2
o7.0 o7.1 o7.4 o7.3 o7.6 o7.5 r3.0 p11.8 p8.0 p8.2 p8.4 p8.6 p9.0 p9.2 p11.10 p8.8 r3.1 d3 r3.2 o6.4 o6.2 p9.4
o6.0 o6.6 o6.3 o6.1 p7.0 r2.1 p9.6 p6.0 p9.8 p6.2 p6.4 r2.0 o6.5 p6.6 d2 p7.2 p4.0 o5.3 o5.2 o5.1 o5.4 o5.6 o5.5
o5.0 r1.0 p4.2 p7.4 p5.0 p7.6 p4.4 d1 p5.2 o4.4 o4.2 p2.0 o4.1 o4.0 o4.3 p3.0 o4.6 o4.5 p2.2 p5.4 o2.1 p3.2 S2
o3.3 o2.3 o2.6 o2.4 o2.0 o3.2 o2.2 o2.5 o3.5 o3.1 o3.6 o3.0 o3.4 S3
"""


def _head_program():
    return [(t[0],) + tuple(int(v) for v in t[1:].split('.')) for t in _HEAD_ORDER.split()]


def _dot(a, b):
    return jnp.dot(a, b, preferred_element_type=f32)


def _dot_nt(a, b):
    return lax.dot_general(a, b, NT, preferred_element_type=f32)


def _unpack(w32, sh):
    return pltpu.bitcast((w32 << sh) & jnp.uint32(HI), f32)


class _Bf16:
    def __init__(self, raw):
        self.raw = raw

    def _half(self, idx):
        idx = list(idx if isinstance(idx, tuple) else (idx,))
        idx += [slice(None)] * (len(self.raw.shape) - len(idx))
        r = idx[-2]
        if isinstance(r, slice):
            idx[-2] = slice(None if r.start is None else r.start // 2, None if r.stop is None else r.stop // 2)
        elif isinstance(r.start, int):
            idx[-2] = pl.ds(r.start // 2, r.size // 2)
        else:
            idx[-2] = pl.ds(pl.multiple_of(r.start >> 1, 8), r.size // 2)
        return tuple(idx)

    def __getitem__(self, idx):
        return pltpu.bitcast(self.raw[self._half(idx)], bf)

    def put(self, idx, v):
        idx = self._half(idx)
        ref = self.raw.at[idx[:-2]] if len(idx) > 2 else self.raw
        o = pltpu.bitcast(v, u32)
        ref[idx[-2], idx[-1]] = o
        return o

    def __setitem__(self, idx, v):
        self.put(idx, v)


def _kernel(xt_hbm, c_hbm, wq_hbm, wk_hbm, wv_hbm, wo_hbm, wr_hbm, wg_hbm, wu_hbm, wd_hbm, gw_hbm, o_hbm,
            xt_s, x_s, xa_r, c_r, ca_r, wq_p, wkv_p, wo_r, q_r, qa_r, acc_s, wg_r, wu_r, wd_r,
            wr_s, gw_s, out_s, g_s, xs_r, rsel_s, idx_s, s_s, t0_r, om_s, fw_s, sem):
    xa_s, c_s, ca_s, wo_s, q_s, qa_s, wg_s, wu_s, wd_s, xs_s, t0_s = [
        _Bf16(r) for r in (xa_r, c_r, ca_r, wo_r, q_r, qa_r, wg_r, wu_r, wd_r, xs_r, t0_r)]
    mk = pltpu.make_async_copy
    wq32, wk32, wv32 = wq_hbm.bitcast(u32), wk_hbm.bitcast(u32), wv_hbm.bitcast(u32)
    cp_wq = lambda j: mk(wq32.at[:, j, :], wq_p.at[j], sem.at[SEM_WQ + j])
    cp_kv = lambda j, m: mk((wk32, wv32)[m].at[:, j, :], wkv_p.at[j & 1, m], sem.at[SEM_KV + m])
    cp_xt = lambda k: mk(xt_hbm.at[:, pl.ds(k * XC, XC)], xt_s.at[:, pl.ds(k * XC, XC)], sem.at[SEM_XT + k])
    cp_out = lambda i: mk(out_s.at[i], o_hbm.at[:, pl.ds(i * T, T)], sem.at[SEM_OUT + i])
    cp_vec = [mk(wr_hbm, wr_s, sem.at[SEM_VEC]), mk(gw_hbm, gw_s, sem.at[SEM_VEC + 1])]
    cp_ffn = [mk(src, dst, sem.at[SEM_FFN + n]) for n, (src, dst) in
              enumerate(((wg_hbm.bitcast(u32), wg_r), (wu_hbm.bitcast(u32), wu_r), (wd_hbm.bitcast(u32), wd_r)))]
    cp_wo = mk(wo_hbm.bitcast(u32), wo_r, sem.at[SEM_WO])
    c32 = c_hbm.bitcast(u32)

    def cp_c(j):
        r0 = (j - 1) * (NG * RB // 2)
        n = QS // 2 - r0 if isinstance(j, int) and j == NP - 1 else NG * RB // 2
        return [mk(c32.at[pl.ds(i * QS // 2 + r0, n)], c_r.at[pl.ds(i * QS // 2 + r0, n)], sem.at[SEM_C + j])
                for i in range(4)]

    cp_xt(0).start()
    cp_wq(0).start()
    for k in range(1, S // XC):
        cp_xt(k).start()
    for cp in cp_vec:
        cp.start()
    for j in range(1, NP):
        cp_wq(j).start()
        for cp in cp_c(j):
            cp.start()
    for cp in cp_ffn + [cp_kv(0, 0), cp_kv(0, 1), cp_wo]:
        cp.start()

    @pl.loop(0, NQ // 2)
    def _(n):
        om_s[n] = jnp.zeros(om_s.shape[1:], f32)

    def store_q(j, e, r0, q):
        q = q * QSCALE
        q_s[2 * j + e, r0:r0 + q.shape[0], :] = q.astype(bf)
        for p0 in range(0, q.shape[0], 2 * T):
            if r0 + p0 > 0:
                qa, qb = q[p0:p0 + T], q[p0 + T:p0 + 2 * T]
                terms = _lhs_terms(qa[:, :T], qa[:, T:], qb[:, :T], qb[:, T:])
                for k, i in enumerate((0, 1, 4, 5, 6)):
                    qa_s[2 * j + e, (r0 + p0) // 2:(r0 + p0) // 2 + T, k * T:(k + 1) * T] = terms[i].astype(bf)

    def q_plain(w, r0, hook=None):
        prod = lambda a, b, wn, z: _dot(_feed(x_s[0, a:b, :], z), wn[:HM]) + _dot(x_s[1, a:b, :], wn[HM:])
        if hook is None:
            qf = prod(r0, r0 + 2 * T, w, None)
        else:
            qf = jnp.concatenate([jnp.concatenate(
                [prod(r0 + u * T, r0 + (u + 1) * T, w[:, n * T:(n + 1) * T], hook()) for u in range(2)], axis=0)
                for n in range(4)], axis=1)
        store_q(0, 0, r0, qf[:, :D])
        store_q(0, 1, r0, qf[:, D:])

    def q_rhs(j):
        lo, hi = pltpu.bitcast(wq_p[j] << 16, f32), pltpu.bitcast(wq_p[j] & jnp.uint32(HI), f32)
        b = [jnp.concatenate([lo[:, t * T:(t + 1) * T], hi[:, t * T:(t + 1) * T]], axis=1) for t in range(2)]
        return [t.astype(bf) for t in _rhs_terms(b[0][:HM], b[1][:HM], b[0][HM:], b[1][HM:])]

    def q_strassen(j, hook):
        ts = q_rhs(j)

        def lhs(i, u):
            if i in (2, 3):
                return x_s[i - 2, (i - 2) * HS + u:(i - 2) * HS + u + T, :]
            return xa_s[i - 2 * (i > 3), u:u + T, :]
        cs = _strassen(lambda i: jnp.concatenate(
            [_dot(_feed(lhs(i, u), *hook()), ts[i]) for u in range(0, HS, T)], axis=0))
        for u in range(2):
            for e in range(2):
                store_q(j, e, u * HS, jnp.concatenate([c[:, e * T:(e + 1) * T] for c in cs[2 * u:2 * u + 2]], axis=1))

    def x_prep(r0):
        a = [x_s[e, h0 + r0:h0 + r0 + RB, :].astype(f32) for h0 in (0, HS) for e in (0, 1)]
        terms = _lhs_terms(*a)
        outs = []
        for k, i in enumerate((0, 1, 4, 5, 6)):
            outs.append(xa_s.put((k, slice(r0, r0 + RB)), terms[i].astype(bf)))
        return outs

    def c_prep(g, c0):
        blk = lambda i, k: c_s[pl.ds(i * QS + g * RB, RB), k * QC + c0:k * QC + c0 + T].astype(f32)
        outer = [_lhs_terms2(*[blk(2 * i1 + i2, 2 * k1 + k2) for i1 in range(2) for k1 in range(2)])
                 for i2 in range(2) for k2 in range(2)]
        outs = []
        for r1 in range(7):
            for r2, v in enumerate(_lhs_terms(*[o[r1] for o in outer])):
                outs.append(ca_s.put((7 * r1 + r2, pl.ds(g * RB, RB), slice(c0, c0 + T)), v.astype(bf)))
        return outs

    def c_pacer(g0, ng, first, last):
        return _Pacer([functools.partial(c_prep, g0 + t // 2, (t % 2) * T) for t in range(2 * ng)], 49, first, last)

    def transpose(k):
        for e in range(2):
            x_s[e, k * XC:(k + 1) * XC, :] = xt_s[e * HM:(e + 1) * HM, k * XC:(k + 1) * XC].T

    def q_w0():
        return jnp.concatenate([pltpu.bitcast(wq_p[0] << 16, f32).astype(bf),
                                pltpu.bitcast(wq_p[0] & jnp.uint32(HI), f32).astype(bf)], axis=1)

    cp_xt(0).wait()
    transpose(0)
    cp_wq(0).wait()
    q_plain(q_w0(), 0)
    for k in range(1, 4):
        cp_xt(k).wait()
    transpose(1)
    w0 = q_w0()
    transpose(2)
    q_plain(w0, XC)
    transpose(3)
    q_plain(w0, 2 * XC)
    for k in range(4, S // XC):
        cp_xt(k).wait()
    for cp in cp_vec:
        cp.wait()
    for k in range(4, S // XC):
        transpose(k)
    row8 = lax.broadcasted_iota(jnp.int32, (8, M), 0)
    x_pace = _Pacer([functools.partial(x_prep, r0) for r0 in range(0, HS, RB)], 5, 12, 40)
    routed = []

    def hook0():
        n = len(routed)
        if n < NQ:
            rg = jnp.where(row8 == 0, wr_s[...].reshape(1, M).astype(f32), gw_s[...].reshape(1, M).astype(f32))
            g_s[n] = _dot(rg.astype(bf), xt_s[:, n * T:(n + 1) * T])
            routed.append(n)
        return x_pace()
    w0 = q_w0()
    for k in range(3, S // XC):
        q_plain(w0, k * XC, hook0)
    assert x_pace.finished()

    rb = jnp.concatenate([g_s[n][0:1, :] for n in range(NQ)], axis=1).astype(bf).astype(f32)
    lane = lax.broadcasted_iota(jnp.int32, (1, S), 1)
    m1 = jnp.max(rb, axis=1, keepdims=True)
    i1 = jnp.minimum(jnp.min(jnp.where(rb == m1, lane, S)), S - 1)
    rb2 = jnp.where(lane == i1, -jnp.inf, rb)
    m2 = jnp.max(rb2, axis=1, keepdims=True)
    i2 = jnp.minimum(jnp.min(jnp.where(jnp.logical_and(rb2 == m2, lane != i1), lane, S)), S - 1)
    row16 = lax.broadcasted_iota(jnp.int32, (16, HM), 0)

    def x_row(e, i):
        blk = x_s[e, pl.ds(pl.multiple_of((i // 16) * 16, 16), 16), :].astype(f32)
        return jnp.sum(jnp.where(row16 == i % 16, blk, 0.0), axis=0, keepdims=True)
    for e in range(2):
        xs_s[e] = jnp.where(row16 == 0, x_row(e, i1), jnp.where(row16 == 1, x_row(e, i2), 0.0)).astype(bf)
    rsel_s[...] = jax.nn.sigmoid(jnp.where(lax.broadcasted_iota(jnp.int32, (16, T), 0) == 0, m1, m2))
    idx_s[0] = i1
    idx_s[1] = i2

    def q_body(it, carry):
        js = (2 * it + 1, 2 * it + 2)
        for j in js:
            for cp in [cp_wq(j)] + cp_c(j):
                cp.wait()
        pace = c_pacer(2 * it * NG, 2 * NG, 1, 108)
        for j in js:
            q_strassen(j, lambda: (pace(),))
        assert pace.finished()
        return carry
    lax.fori_loop(0, 3, q_body, 0)

    for cp in cp_ffn + [cp_wq(NP - 1), cp_kv(0, 0), cp_kv(0, 1)] + cp_c(NP - 1):
        cp.wait()

    def w_sum(hn, m, r0):
        w = [wkv_p[(hn >> 1) & 1, m, r:r + 8, :] for r in range(r0, r0 + HC, 64)]
        w = (jnp.concatenate(w, axis=0) << (16 * (1 - (hn & 1))).astype(u32)) & jnp.uint32(0x7FFF0000)
        return functools.reduce(jnp.add, [pltpu.bitcast(t, f32) for t in _vregs([w])])

    def w_balance(parts):
        n = len(parts) // 2
        sk, sv = [jnp.sum(functools.reduce(jnp.add, p), keepdims=True) for p in (parts[:n], parts[n:])]
        ok = jnp.logical_and(sk > 0, sv > 0)
        ratio = jnp.broadcast_to(jnp.where(ok, 1.4 * sk, 1.0) / jnp.where(ok, sv, 1.0), (8, T))
        e = jnp.clip(pltpu.bitcast(ratio, jnp.int32) & 0x7F800000, (127 - 40) << 23, (127 + 40) << 23)
        fw_s[0] = pltpu.bitcast(e, f32)
        fw_s[1] = pltpu.bitcast((254 << 23) - e, f32)
        return [e]

    def w_pacer(hn, first, last):
        parts = []
        return _Pacer([lambda m=m, r0=r0: parts.append(w_sum(hn, m, r0)) or parts[-1:]
                       for m in range(2) for r0 in (0, HC)] + [lambda: w_balance(parts)], 1, first, last)

    def first_terms(hn):
        w = _unpack(wkv_p[(hn >> 1) & 1, 0, :, :T], (16 * (1 - (hn & 1))).astype(u32))
        t = w[:HC] + 0.5 * w[HC:]
        return [t0_s.put((slice(None), slice(n * T, (n + 1) * T)), v.astype(bf))
                for n, v in enumerate((t[:QC], t[QC:] - t[:QC]))]

    def residual(n):
        g8 = jax.nn.sigmoid(g_s[n])
        g_s[n] = g8
        a = (1.0 - g8[1:2, :]) * xt_s[:, n * T:(n + 1) * T].astype(f32)
        acc_s[n] = a
        return [a]

    gs, us, ys, hid = [], [], {}, []
    xs_dot = lambda w_s, n: (_dot(xs_s[0], w_s[:HM, n * T:(n + 1) * T]) + _dot(xs_s[1], w_s[HM:, n * T:(n + 1) * T]))

    def swiglu():
        gg, uu = jnp.concatenate(gs, axis=1), jnp.concatenate(us, axis=1)
        hid.append((gg * jax.nn.sigmoid(gg) * uu).astype(bf))

    def down(n0, k0):
        t = _dot_nt(hid[0][:, k0:min(k0 + 512, F)], wd_s[n0:min(n0 + T, M), k0:min(k0 + 512, F)])
        ys[n0] = ys[n0] + t if n0 in ys else t
    side = []
    for n in range(F // T):
        side += [lambda n=n: gs.append(xs_dot(wg_s, n)), lambda n=n: us.append(xs_dot(wu_s, n))]
    side += [swiglu] + [lambda: None] * 7
    side += [functools.partial(down, n0, k0) for n0 in range(0, M, T) for k0 in range(0, F, 512)]
    c_pace = c_pacer((NP - 2) * NG, QS // RB - (NP - 2) * NG, 2, 56)
    r_pace = _Pacer([functools.partial(residual, n) for n in range(NQ)], M // 8, 1, 48)

    w_pace0 = w_pacer(jnp.int32(0), 4, 52)
    t_pace0 = _Pacer([lambda: first_terms(jnp.int32(0))], 32, 40, 56)

    def hook7():
        if side:
            side.pop(0)()
        return c_pace(), r_pace(), w_pace0(), t_pace0()
    q_strassen(NP - 1, hook7)
    assert not side and all(p.finished() for p in (c_pace, r_pace, w_pace0, t_pace0))
    y = jnp.concatenate([ys[n0] for n0 in range(0, M, T)] + [jnp.zeros((16, 512 - M), f32)], axis=1)
    yt = (y * rsel_s[:, 0:1]).T
    lane128 = lax.broadcasted_iota(jnp.int32, (1, T), 1)
    for e in range(2):
        i = idx_s[e]
        acc_s[i // T] += jnp.where(lane128 == i % T, (1.0 - g_s[i // T][1:2, :]) * yt[:M, e:e + 1], 0.0)

    for m in range(2):
        cp_kv(1, m).start()
    cp_wo.wait()

    tri = lax.broadcasted_iota(jnp.int32, (T, T), 1) <= lax.broadcasted_iota(jnp.int32, (T, T), 0)
    prog = _head_program()

    def head(h, carry):
        par, slot = h & 1, (h >> 1) & 1

        @pl.when(jnp.logical_and(h < H - 1, par == 1))
        def _():
            for m in range(2):
                cp_kv((h + 1) >> 1, m).wait()

        sh = (16 * (1 - par)).astype(u32)
        rhs, fw, fw_inv = [], fw_s[0], fw_s[1]
        for r1 in range(7):
            wk, wv = [_unpack(wkv_p[slot, m], sh + (h >> (8 + r1)).astype(u32)) for m in range(2)]
            wv = jnp.concatenate([wv[:, :T] * fw[0:1], wv[:, T:] * fw[0:1]], axis=1)
            t = _rhs_terms2(wk[:HC], wv[:HC], wk[HC:], wv[HC:])[r1]
            rhs.append([u.astype(bf) for u in _rhs_terms(t[:QC, :T], t[:QC, T:], t[QC:, :T], t[QC:, T:])])
        rhs[1][1], rhs[1][3] = t0_s[:, :T], t0_s[:, T:]
        hn = jnp.minimum(h + 1, H - 1)
        t_pace = _Pacer([lambda: first_terms(hn)], 32, 196 - 14, 196)
        w_pace = w_pacer(hn, 60, 180)
        prods, inner_q, outer, kblk, vblk = {}, {}, {}, {}, {}

        def kv_product(r1, r2):
            m = prods.setdefault(r1, {})
            m[r2] = _dot(ca_s[7 * r1 + r2], rhs[r1][r2])
            if len(m) == 7:
                inner_q[r1] = (((m[3] - m[4]) + m[6]) + m[0], m[2] + m[4], m[1] + m[3], ((m[0] - m[1]) + m[2]) + m[5])
                for b in range(4):
                    if b not in kblk and all(q in inner_q for q in (0, 1, 3, 4, 6)):
                        p = {q: inner_q[q][b] for q in (0, 1, 3, 4, 6)}
                        e, d = p[3] + p[1], p[3] - p[1]
                        kblk[b] = (p[0] + ((d - p[4]) + p[6]), e * 2.0)
                        outer[b] = ((e + p[4]) + p[6], p[0] + d)
                    if len(inner_q) == 7:
                        p2, p5 = inner_q[2][b], inner_q[5][b]
                        vblk[b] = (((outer[b][0] + p2) - p5) * 0.5, (outer[b][1] + p2) + p5)

        def rows(blk, t0, t1):
            return jnp.concatenate([jnp.concatenate(
                [blk[2 * (t // 4 % 2) + j2][t // 8][t % 4 * T:(t % 4 + 1) * T] for j2 in range(2)], axis=1)
                for t in range(t0, t1)], axis=0)

        @functools.cache
        def k_tile(t):
            return rows(kblk, t, t + 1).astype(bf)

        @functools.cache
        def k_terms(J):
            ka, kb = rows(kblk, 2 * J, 2 * J + 1), rows(kblk, 2 * J + 1, 2 * J + 2)
            return [t.astype(bf) for t in _rhs_terms(ka[:, :T], kb[:, :T], ka[:, T:], kb[:, T:])]

        @functools.cache
        def v_tiles(c0, c1):
            return rows(vblk, c0, c1).astype(bf)

        scores, rmax, soft, o_sum = {}, {}, {}, {}
        q_tiles = lambda I: [q_s[h, i * T:(i + 1) * T, t * T:(t + 1) * T] for i in (2 * I, 2 * I + 1) for t in range(2)]

        def score_block(I, J):
            q4, qx = q_tiles(I), [qa_s[h, I * T:(I + 1) * T, k * T:(k + 1) * T] for k in range(5)]
            lhs = [qx[0], qx[1], q4[0], q4[3], qx[2], qx[3], qx[4]]
            cs = _strassen(lambda i: _dot_nt(_feed(lhs[i], t_pace(), w_pace()), k_terms(J)[i]))
            for n, c in enumerate(cs):
                s_s[I % 2, n // 2, 2 * J + n % 2] = c
            for u in range(2):
                sa, sb = s_s[I % 2, u, 2 * J], s_s[I % 2, u, 2 * J + 1]
                scores[2 * I + u, 2 * J] = s_s[I % 2, u, 2 * J]
                scores[2 * I + u, 2 * J + 1] = s_s[I % 2, u, 2 * J + 1]
                mx = jnp.maximum(sa, sb)
                rmax[2 * I + u] = jnp.maximum(rmax[2 * I + u], mx) if 2 * I + u in rmax else mx

        def score_diag(I):
            a, b = 2 * I, 2 * I + 1
            q4 = q_tiles(I)
            qa, qb = jnp.concatenate(q4[0:2], axis=1), jnp.concatenate(q4[2:4], axis=1)
            d1 = _dot_nt(jnp.concatenate([qa, qb], axis=0), k_tile(a))
            d2 = _dot_nt(qb, k_tile(b))
            scores[a, a], scores[b, a], scores[b, b] = jnp.where(tri, d1[:T], NEG), d1[T:], jnp.where(tri, d2, NEG)

        def pv_chunk(i, c0):
            if c0 == 0:
                mx = functools.reduce(jnp.maximum, ([rmax[i]] if i > 1 else [])
                                      + [scores[i, t] for t in range(i // 2 * 2, i + 1)])
                soft[i] = dict(m=jnp.max(mx, axis=1, keepdims=True), l=None, ctx=None)
            st = soft[i]
            c1 = min(c0 + 2, i + 1)
            p = jnp.exp2(jnp.concatenate([scores.pop((i, t)) for t in range(c0, c1)], axis=1) - st['m']).astype(bf)
            pf = p.astype(f32)
            for t in range(c1 - c0):
                st['l'] = pf[:, t * T:(t + 1) * T] if st['l'] is None else st['l'] + pf[:, t * T:(t + 1) * T]
            d = _dot(p, v_tiles(c0, c1))
            st['ctx'] = d if st['ctx'] is None else st['ctx'] + d

        def context(i):
            st = soft.pop(i)
            l = jnp.sum(st['l'], axis=1, keepdims=True)
            r = pl.reciprocal(l, approx=True)
            return st['ctx'] * (r * (2.0 - l * r) * fw_inv[0:1, 0:1])

        def ship(blocks):
            @pl.when(h == H - 1)
            def _():
                for i in blocks:
                    cp_out(i).start()

        def out_plain(i):
            wo, ctx = wo_s[h], context(i).astype(bf)
            for a0 in (0, HM):
                a = acc_s[i, a0:a0 + HM, :] + g_s[i][1:2, :] * _dot_nt(wo[a0:a0 + HM], ctx)
                acc_s[i, a0:a0 + HM, :] = a
                out_s[i, a0:a0 + HM, :] = a.astype(bf)
            ship([i])

        @functools.cache
        def wo_terms():
            w = wo_s[h].astype(f32)
            return [t.astype(bf) for t in _lhs_terms(w[:HM, :T], w[:HM, T:], w[HM:, :T], w[HM:, T:])]

        @functools.cache
        def ctx_terms(I):
            ca, cb = context(2 * I), context(2 * I + 1)
            return _rhs_terms(ca[:, :T], cb[:, :T], ca[:, T:], cb[:, T:])

        def out_product(I, k):
            om_s[I, k] += _dot_nt(wo_terms()[k], ctx_terms(I)[k].astype(bf))
            o_sum[I, k] = om_s[I, k]
            if all((I, q) in o_sum for q in range(7)):
                for n, c in enumerate(_strassen(lambda q: o_sum.pop((I, q)))):
                    i, a0 = 2 * I + n % 2, (n // 2) * HM
                    out_s[i, a0:a0 + HM, :] = (acc_s[i, a0:a0 + HM, :] + g_s[i][1:2, :] * c).astype(bf)
                ship([2 * I, 2 * I + 1])

        ops = {'m': kv_product, 'r': score_block, 'd': score_diag, 'p': pv_chunk,
               'o': out_product, 'S': out_plain}
        for op, *args in prog:
            ops[op](*args)
        assert t_pace.finished() and w_pace.finished()

        @pl.when(jnp.logical_and((h + 3) >> 1 < NP, par == 1))
        def _():
            for m in range(2):
                cp_kv((h + 3) >> 1, m).start()
        return carry

    lax.fori_loop(0, H, head, 0)
    for i in range(NQ):
        cp_out(i).wait()


@jax.jit
def pallas_gated_mix__compressed_kv_cla__moe_arch_mod__prompt_kernel(
    A_x: jax.Array,
    A_c_kv: jax.Array,
    A_w_q: jax.Array,
    A_w_uk: jax.Array,
    A_w_uv: jax.Array,
    A_w_o: jax.Array,
    B_x: jax.Array,
    B_w_r: jax.Array,
    B_w_gate: jax.Array,
    B_w_up: jax.Array,
    B_w_down: jax.Array,
    gate_w: jax.Array,
):
    del B_x
    V = pltpu.VMEM
    B = lambda *shape: V(shape[:-2] + (shape[-2] // 2, shape[-1]), u32)
    out_t = pl.pallas_call(
        _kernel,
        in_specs=[pl.BlockSpec(memory_space=pl.ANY)] * 11,
        out_specs=pl.BlockSpec(memory_space=pl.ANY),
        out_shape=jax.ShapeDtypeStruct((M, S), bf),
        scratch_shapes=[
            V((M, S), bf), V((2, S, HM), bf), B(5, HS, HM),
            B(S, DC), B(49, QS, QC),
            V((NP, M, D), u32), V((2, 2, DC, D), u32), B(H, M, D),
            B(H, S, D), B(H, HS, 5 * T),
            V((NQ, M, T), f32),
            B(M, F), B(M, F), B(M, F),
            V((M,), bf), V((M,), bf), V((NQ, M, T), bf),
            V((NQ, 8, T), f32), B(2, 16, HM), V((16, T), f32),
            pltpu.SMEM((2,), jnp.int32),
            V((2, 2, NQ, T, T), f32), B(QC, 2 * T),
            V((NQ // 2, 7, HM, T), f32),
            V((2, 8, T), f32),
            pltpu.SemaphoreType.DMA((NSEM,)),
        ],
        compiler_params=pltpu.CompilerParams(vmem_limit_bytes=110 * 1024 * 1024),
        name="gated_mix_cla_mod",
    )(A_x[0].T, A_c_kv[0], A_w_q, A_w_uk, A_w_uv, A_w_o.transpose(0, 2, 1), B_w_r, B_w_gate, B_w_up,
      B_w_down.T, gate_w)
    return out_t.T[None]
```

```python
import functools
import math

import jax
import jax.numpy as jnp
from jax import lax
from jax.experimental import pallas as pl
from jax.experimental.pallas import tpu as pltpu

S, M, H, D, DC, F = 2048, 448, 16, 256, 1024, 1792
T = 128
NP, NQ = H // 2, S // T
HS, HM, HC = S // 2, M // 2, DC // 2
QS, QC = S // 4, DC // 4
RB = 16
XC = 256
NG = 5
NT = (((1,), (1,)), ((), ()))
QSCALE = D ** -0.5 * math.log2(math.e)
NEG = -1e30
bf, f32, u32 = jnp.bfloat16, jnp.float32, jnp.uint32
HI = 0xFFFF0000

SEM_WO, SEM_FFN, SEM_VEC, SEM_KV, SEM_WQ, SEM_XT, SEM_C, SEM_OUT, NSEM = 0, 1, 4, 6, 8, 16, 24, 32, 48


def _lhs_terms(a11, a12, a21, a22):
    return [a11 + a22, a21 + a22, a11, a22, a11 + a12, a21 - a11, a12 - a22]


def _rhs_terms(b11, b12, b21, b22):
    return [b11 + b22, b11, b12 - b22, b21 - b11, b22, b11 + b12, b21 + b22]


def _strassen(mm):
    m2, m3, m4, m5, m1, m7, m6 = [mm(i) for i in (1, 2, 3, 4, 0, 6, 5)]
    return (m4 - m5) + (m1 + m7), m3 + m5, m2 + m4, (m3 - m2) + (m1 + m6)


def _lhs_terms2(a11, a12, a21, a22):
    h21, q21, h22 = 0.5 * a21, 0.25 * a21, 0.5 * a22
    s1 = a11 + a22
    v, hs = a12 + q21, 0.5 * s1
    return [s1, q21 + h22, a11 + h21, h22 - q21, v + hs, h21 - a11, v - hs]


def _rhs_terms2(b11, b12, b21, b22):
    h21 = 0.5 * b21
    t1 = b11 + b22
    v, ht = b12 + 0.5 * h21, 0.5 * t1
    return [t1, b11 + h21, v - ht, h21 - b11, b22 - h21, v + ht, b22 + h21]


def _vregs(vals):
    ts = []
    for v in vals:
        v = v if v.dtype == u32 else pltpu.bitcast(v, u32)
        ts += [v[r:r + 8, c:c + T] for r in range(0, v.shape[0], 8) for c in range(0, v.shape[1] - T + 1, T)]
    return ts


def _zero_from(ts):
    acc = ts[:4]
    for i, t in enumerate(ts[4:]):
        acc[i % 4] = acc[i % 4] | t
    while len(acc) > 1:
        acc = [acc[i] | acc[i + 1] if i + 1 < len(acc) else acc[i] for i in range(0, len(acc), 2)]
    return (acc[0] >> 16) >> 16


def _feed(a, *zs):
    zs = [z for z in zs if z is not None]
    if not zs:
        return a
    a32 = pltpu.bitcast(a, u32)
    top = functools.reduce(lambda p, q: p | q, zs, a32[0:8, :T])
    if a32.shape[1] > T:
        top = jnp.concatenate([top, a32[0:8, T:]], axis=1)
    return pltpu.bitcast(jnp.concatenate([top, a32[8:]], axis=0), bf)


class _Pacer:
    def __init__(self, thunks, per, first, last):
        self.thunks, self.pool, self.k, self.done = list(thunks), [], 0, 0
        self.tot, self.first, self.last = per * len(self.thunks), first, last

    def __call__(self):
        self.k += 1
        if self.k <= self.first:
            return None
        want = min(self.tot, -(-(self.k - self.first) * self.tot // (self.last - self.first))) - self.done
        while len(self.pool) < want and self.thunks:
            self.pool += _vregs(self.thunks.pop(0)())
        outs, self.pool = self.pool[:want], self.pool[want:]
        self.done += len(outs)
        return _zero_from(outs) if outs else None

    def finished(self):
        return not self.thunks and not self.pool


_HEAD_ORDER = """
m1.1 m1.3 m1.4 m1.6 m1.0 m3.3 m3.6 m1.2 m3.4 m4.3 m3.1 m3.0 m4.4 m3.2 m3.5 m1.5 m4.6 m4.1 m4.0 m6.6 m6.3 m6.0
m4.5 m0.1 m6.4 m6.1 m6.5 m6.2 m4.2 m0.6 m0.4 m0.3 m0.0 m0.2 m0.5 m2.1 d0 m2.3 r7.0 m2.4 r7.1 m2.0 m2.6 m5.1 r7.2
m2.2 r7.4 m2.5 r7.3 r7.6 r7.5 m5.3 d7 m5.6 m5.4 m5.0 m5.2 m5.5 p14.0 r6.0 p1.0 p0.0 r6.2 r6.1 p14.2 p14.4 p14.6
p14.8 p14.10 p15.0 p14.12 p14.14 r6.3 r6.4 r6.5 p15.2 p15.4 p15.6 p15.8 p15.10 d6 p15.12 p15.14 p12.0 r5.0 p12.2
p12.4 p12.6 r5.3 r5.2 r5.1 p12.8 p13.0 p12.10 p13.2 r5.4 p13.4 p13.6 p13.8 p12.12 d5 o0.3 o0.2 o0.1 p10.0 o0.0
o0.5 p11.0 p13.10 r4.1 o0.4 p10.2 p13.12 p10.4 r4.0 o0.6 p10.6 p10.8 p11.2 p10.10 r4.2 r4.3 p11.4 d4 p11.6 o7.2
o7.0 o7.1 o7.4 o7.3 o7.6 o7.5 r3.0 p11.8 p8.0 p8.2 p8.4 p8.6 p9.0 p9.2 p11.10 p8.8 r3.1 d3 r3.2 o6.4 o6.2 p9.4
o6.0 o6.6 o6.3 o6.1 p7.0 r2.1 p9.6 p6.0 p9.8 p6.2 p6.4 r2.0 o6.5 p6.6 d2 p7.2 p4.0 o5.3 o5.2 o5.1 o5.4 o5.6 o5.5
o5.0 r1.0 p4.2 p7.4 p5.0 p7.6 p4.4 d1 p5.2 o4.4 o4.2 p2.0 o4.1 o4.0 o4.3 p3.0 o4.6 o4.5 p2.2 p5.4 o2.1 p3.2 S2
o3.3 o2.3 o2.6 o2.4 o2.0 o3.2 o2.2 o2.5 o3.5 o3.1 o3.6 o3.0 o3.4 S3
"""


def _head_program():
    return [(t[0],) + tuple(int(v) for v in t[1:].split('.')) for t in _HEAD_ORDER.split()]


_Q7_ORDER = """
010 023 021 027 016 022 026 025 030 012 014 015 011 017 045 044 047 020 031 032 033 034 013 024 046 043 036 035
041 042 000 037 040 001 005 004 003 006 002 007 060 061 066 067 062 063 064 065 051 053 052 050 056 054 055 057
"""
_Q_ORDER = """
016 011 015 012 014 017 013 010 041 027 031 022 026 024 034 007 040 021 001 036 025 046 033 047 035 042 005 023
006 032 043 020 037 004 044 030 000 045 002 003 050 061 054 053 064 067 051 060 052 066 062 063 065 116 112 111
113 117 124 125 121 123 126 120 057 127 122 133 130 131 144 132 056 114 140 137 143 110 055 100 146 115 145 141
107 160 134 136 147 135 161 142 101 102 162 106 104 103 154 105 163 165 167 152 150 157 155 166 151 156 153 164
"""


def _dot(a, b):
    return jnp.dot(a, b, preferred_element_type=f32)


def _dot_nt(a, b):
    return lax.dot_general(a, b, NT, preferred_element_type=f32)


def _unpack(w32, sh):
    return pltpu.bitcast((w32 << sh) & jnp.uint32(HI), f32)


class _Bf16:
    def __init__(self, raw):
        self.raw = raw

    def _half(self, idx):
        idx = list(idx if isinstance(idx, tuple) else (idx,))
        idx += [slice(None)] * (len(self.raw.shape) - len(idx))
        r = idx[-2]
        if isinstance(r, slice):
            idx[-2] = slice(None if r.start is None else r.start // 2, None if r.stop is None else r.stop // 2)
        elif isinstance(r.start, int):
            idx[-2] = pl.ds(r.start // 2, r.size // 2)
        else:
            idx[-2] = pl.ds(pl.multiple_of(r.start >> 1, 8), r.size // 2)
        return tuple(idx)

    def __getitem__(self, idx):
        return pltpu.bitcast(self.raw[self._half(idx)], bf)

    def put(self, idx, v):
        idx = self._half(idx)
        ref = self.raw.at[idx[:-2]] if len(idx) > 2 else self.raw
        o = pltpu.bitcast(v, u32)
        ref[idx[-2], idx[-1]] = o
        return o

    def __setitem__(self, idx, v):
        self.put(idx, v)


def _kernel(xt_hbm, c_hbm, wq_hbm, wk_hbm, wv_hbm, wo_hbm, wr_hbm, wg_hbm, wu_hbm, wd_hbm, gw_hbm, o_hbm,
            xt_s, x_s, xa_r, c_r, ca_r, wq_p, wkv_p, wo_r, q_r, qa_r, acc_s, wg_r, wu_r, wd_r,
            wr_s, gw_s, out_s, g_s, xs_r, rsel_s, idx_s, s_s, t0_r, om_s, fw_s, sem):
    xa_s, c_s, ca_s, wo_s, q_s, qa_s, wg_s, wu_s, wd_s, xs_s, t0_s = [
        _Bf16(r) for r in (xa_r, c_r, ca_r, wo_r, q_r, qa_r, wg_r, wu_r, wd_r, xs_r, t0_r)]
    mk = pltpu.make_async_copy
    wq32, wk32, wv32 = wq_hbm.bitcast(u32), wk_hbm.bitcast(u32), wv_hbm.bitcast(u32)
    cp_wq = lambda j: mk(wq32.at[:, j, :], wq_p.at[j], sem.at[SEM_WQ + j])
    cp_kv = lambda j, m: mk((wk32, wv32)[m].at[:, j, :], wkv_p.at[j & 1, m], sem.at[SEM_KV + m])
    cp_xt = lambda k: mk(xt_hbm.at[:, pl.ds(k * XC, XC)], xt_s.at[:, pl.ds(k * XC, XC)], sem.at[SEM_XT + k])
    cp_out = lambda i: mk(out_s.at[i], o_hbm.at[:, pl.ds(i * T, T)], sem.at[SEM_OUT + i])
    cp_vec = [mk(wr_hbm, wr_s, sem.at[SEM_VEC]), mk(gw_hbm, gw_s, sem.at[SEM_VEC + 1])]
    cp_ffn = [mk(src, dst, sem.at[SEM_FFN + n]) for n, (src, dst) in
              enumerate(((wg_hbm.bitcast(u32), wg_r), (wu_hbm.bitcast(u32), wu_r), (wd_hbm.bitcast(u32), wd_r)))]
    cp_wo = mk(wo_hbm.bitcast(u32), wo_r, sem.at[SEM_WO])
    c32 = c_hbm.bitcast(u32)

    def cp_c(j):
        r0 = (j - 1) * (NG * RB // 2)
        n = QS // 2 - r0 if isinstance(j, int) and j == NP - 1 else NG * RB // 2
        return [mk(c32.at[pl.ds(i * QS // 2 + r0, n)], c_r.at[pl.ds(i * QS // 2 + r0, n)], sem.at[SEM_C + j])
                for i in range(4)]

    cp_xt(0).start()
    cp_wq(0).start()
    for k in range(1, S // XC):
        cp_xt(k).start()
    for cp in cp_vec:
        cp.start()
    for j in range(1, NP):
        cp_wq(j).start()
        for cp in cp_c(j):
            cp.start()
    for cp in cp_ffn + [cp_kv(0, 0), cp_kv(0, 1), cp_wo]:
        cp.start()

    @pl.loop(0, NQ // 2)
    def _(n):
        om_s[n] = jnp.zeros(om_s.shape[1:], f32)

    def store_q(j, e, r0, q):
        q = q * QSCALE
        q_s[2 * j + e, r0:r0 + q.shape[0], :] = q.astype(bf)
        for p0 in range(0, q.shape[0], 2 * T):
            if r0 + p0 > 0:
                qa, qb = q[p0:p0 + T], q[p0 + T:p0 + 2 * T]
                terms = _lhs_terms(qa[:, :T], qa[:, T:], qb[:, :T], qb[:, T:])
                for k, i in enumerate((0, 1, 4, 5, 6)):
                    qa_s[2 * j + e, (r0 + p0) // 2:(r0 + p0) // 2 + T, k * T:(k + 1) * T] = terms[i].astype(bf)

    def q_plain(w, r0, hook=None):
        prod = lambda a, b, wn, z: _dot(_feed(x_s[0, a:b, :], z), wn[:HM]) + _dot(x_s[1, a:b, :], wn[HM:])
        if hook is None:
            qf = prod(r0, r0 + 2 * T, w, None)
        else:
            qf = jnp.concatenate([jnp.concatenate(
                [prod(r0 + u * T, r0 + (u + 1) * T, w[:, n * T:(n + 1) * T], hook()) for u in range(2)], axis=0)
                for n in range(4)], axis=1)
        store_q(0, 0, r0, qf[:, :D])
        store_q(0, 1, r0, qf[:, D:])

    def q_rhs(j):
        lo, hi = pltpu.bitcast(wq_p[j] << 16, f32), pltpu.bitcast(wq_p[j] & jnp.uint32(HI), f32)
        b = [jnp.concatenate([lo[:, t * T:(t + 1) * T], hi[:, t * T:(t + 1) * T]], axis=1) for t in range(2)]
        return [t.astype(bf) for t in _rhs_terms(b[0][:HM], b[1][:HM], b[0][HM:], b[1][HM:])]

    def q_strassen(js, order, hook):
        ts, res = [q_rhs(j) for j in js], {}
        for a, k, u in [map(int, t) for t in order.split()]:
            if k in (2, 3):
                lhs = x_s[k - 2, (k - 2) * HS + u * T:(k - 2) * HS + (u + 1) * T, :]
            else:
                lhs = xa_s[k - 2 * (k > 3), u * T:(u + 1) * T, :]
            res[a, k, u] = _dot(_feed(lhs, *hook()), ts[a][k])
            v = u // 2 * 2
            if all((a, kk, uu) in res for kk in range(7) for uu in (v, v + 1)):
                cs = _strassen(lambda i: jnp.concatenate([res.pop((a, i, v)), res.pop((a, i, v + 1))], axis=0))
                for w in range(2):
                    for e in range(2):
                        q = jnp.concatenate([c[:, e * T:(e + 1) * T] for c in cs[2 * w:2 * w + 2]], axis=1)
                        store_q(js[a], e, w * HS + v * T, q)

    def x_prep(r0):
        a = [x_s[e, h0 + r0:h0 + r0 + RB, :].astype(f32) for h0 in (0, HS) for e in (0, 1)]
        terms = _lhs_terms(*a)
        outs = []
        for k, i in enumerate((0, 1, 4, 5, 6)):
            outs.append(xa_s.put((k, slice(r0, r0 + RB)), terms[i].astype(bf)))
        return outs

    def c_prep(g, c0):
        blk = lambda i, k: c_s[pl.ds(i * QS + g * RB, RB), k * QC + c0:k * QC + c0 + T].astype(f32)
        outer = [_lhs_terms2(*[blk(2 * i1 + i2, 2 * k1 + k2) for i1 in range(2) for k1 in range(2)])
                 for i2 in range(2) for k2 in range(2)]
        outs = []
        for r1 in range(7):
            for r2, v in enumerate(_lhs_terms(*[o[r1] for o in outer])):
                outs.append(ca_s.put((7 * r1 + r2, pl.ds(g * RB, RB), slice(c0, c0 + T)), v.astype(bf)))
        return outs

    def c_pacer(g0, ng, first, last):
        return _Pacer([functools.partial(c_prep, g0 + t // 2, (t % 2) * T) for t in range(2 * ng)], 49, first, last)

    def transpose(k):
        for e in range(2):
            x_s[e, k * XC:(k + 1) * XC, :] = xt_s[e * HM:(e + 1) * HM, k * XC:(k + 1) * XC].T

    def q_w0():
        return jnp.concatenate([pltpu.bitcast(wq_p[0] << 16, f32).astype(bf),
                                pltpu.bitcast(wq_p[0] & jnp.uint32(HI), f32).astype(bf)], axis=1)

    cp_xt(0).wait()
    transpose(0)
    cp_wq(0).wait()
    q_plain(q_w0(), 0)
    for k in range(1, 4):
        cp_xt(k).wait()
    transpose(1)
    w0 = q_w0()
    transpose(2)
    q_plain(w0, XC)
    transpose(3)
    q_plain(w0, 2 * XC)
    for k in range(4, S // XC):
        cp_xt(k).wait()
    for cp in cp_vec:
        cp.wait()
    for k in range(4, S // XC):
        transpose(k)
    row8 = lax.broadcasted_iota(jnp.int32, (8, M), 0)
    x_pace = _Pacer([functools.partial(x_prep, r0) for r0 in range(0, HS, RB)], 5, 12, 40)
    routed = []

    def hook0():
        n = len(routed)
        if n < NQ:
            rg = jnp.where(row8 == 0, wr_s[...].reshape(1, M).astype(f32), gw_s[...].reshape(1, M).astype(f32))
            g_s[n] = _dot(rg.astype(bf), xt_s[:, n * T:(n + 1) * T])
            routed.append(n)
        return x_pace()
    w0 = q_w0()
    for k in range(3, S // XC):
        q_plain(w0, k * XC, hook0)
    assert x_pace.finished()

    rb = jnp.concatenate([g_s[n][0:1, :] for n in range(NQ)], axis=1).astype(bf).astype(f32)
    lane = lax.broadcasted_iota(jnp.int32, (1, S), 1)
    m1 = jnp.max(rb, axis=1, keepdims=True)
    i1 = jnp.minimum(jnp.min(jnp.where(rb == m1, lane, S)), S - 1)
    rb2 = jnp.where(lane == i1, -jnp.inf, rb)
    m2 = jnp.max(rb2, axis=1, keepdims=True)
    i2 = jnp.minimum(jnp.min(jnp.where(jnp.logical_and(rb2 == m2, lane != i1), lane, S)), S - 1)
    row16 = lax.broadcasted_iota(jnp.int32, (16, HM), 0)

    def x_row(e, i):
        blk = x_s[e, pl.ds(pl.multiple_of((i // 16) * 16, 16), 16), :].astype(f32)
        return jnp.sum(jnp.where(row16 == i % 16, blk, 0.0), axis=0, keepdims=True)
    for e in range(2):
        xs_s[e] = jnp.where(row16 == 0, x_row(e, i1), jnp.where(row16 == 1, x_row(e, i2), 0.0)).astype(bf)
    rsel_s[...] = jax.nn.sigmoid(jnp.where(lax.broadcasted_iota(jnp.int32, (16, T), 0) == 0, m1, m2))
    idx_s[0] = i1
    idx_s[1] = i2

    def q_body(it, carry):
        js = (2 * it + 1, 2 * it + 2)
        for j in js:
            for cp in [cp_wq(j)] + cp_c(j):
                cp.wait()
        pace = c_pacer(2 * it * NG, 2 * NG, 1, 108)
        q_strassen(js, _Q_ORDER, lambda: (pace(),))
        assert pace.finished()
        return carry
    lax.fori_loop(0, 3, q_body, 0)

    for cp in cp_ffn + [cp_wq(NP - 1), cp_kv(0, 0), cp_kv(0, 1)] + cp_c(NP - 1):
        cp.wait()

    def w_sum(hn, m, r0):
        w = [wkv_p[(hn >> 1) & 1, m, r:r + 8, :] for r in range(r0, r0 + HC, 64)]
        w = (jnp.concatenate(w, axis=0) << (16 * (1 - (hn & 1))).astype(u32)) & jnp.uint32(0x7FFF0000)
        return functools.reduce(jnp.add, [pltpu.bitcast(t, f32) for t in _vregs([w])])

    def w_balance(parts):
        n = len(parts) // 2
        sk, sv = [jnp.sum(functools.reduce(jnp.add, p), keepdims=True) for p in (parts[:n], parts[n:])]
        ok = jnp.logical_and(sk > 0, sv > 0)
        ratio = jnp.broadcast_to(jnp.where(ok, 1.4 * sk, 1.0) / jnp.where(ok, sv, 1.0), (8, T))
        e = jnp.clip(pltpu.bitcast(ratio, jnp.int32) & 0x7F800000, (127 - 40) << 23, (127 + 40) << 23)
        fw_s[0] = pltpu.bitcast(e, f32)
        fw_s[1] = pltpu.bitcast((254 << 23) - e, f32)
        return [e]

    def w_pacer(hn, first, last):
        parts = []
        return _Pacer([lambda m=m, r0=r0: parts.append(w_sum(hn, m, r0)) or parts[-1:]
                       for m in range(2) for r0 in (0, HC)] + [lambda: w_balance(parts)], 1, first, last)

    def first_terms(hn):
        w = _unpack(wkv_p[(hn >> 1) & 1, 0, :, :T], (16 * (1 - (hn & 1))).astype(u32))
        t = w[:HC] + 0.5 * w[HC:]
        return [t0_s.put((slice(None), slice(n * T, (n + 1) * T)), v.astype(bf))
                for n, v in enumerate((t[:QC], t[QC:] - t[:QC]))]

    def residual(n):
        g8 = jax.nn.sigmoid(g_s[n])
        g_s[n] = g8
        a = (1.0 - g8[1:2, :]) * xt_s[:, n * T:(n + 1) * T].astype(f32)
        acc_s[n] = a
        return [a]

    gs, us, ys, hid = [], [], {}, []
    xs_dot = lambda w_s, n: (_dot(xs_s[0], w_s[:HM, n * T:(n + 1) * T]) + _dot(xs_s[1], w_s[HM:, n * T:(n + 1) * T]))

    def swiglu():
        gg, uu = jnp.concatenate(gs, axis=1), jnp.concatenate(us, axis=1)
        hid.append((gg * jax.nn.sigmoid(gg) * uu).astype(bf))

    def down(n0, k0):
        t = _dot_nt(hid[0][:, k0:min(k0 + 512, F)], wd_s[n0:min(n0 + T, M), k0:min(k0 + 512, F)])
        ys[n0] = ys[n0] + t if n0 in ys else t
    side = []
    for n in range(F // T):
        side += [lambda n=n: gs.append(xs_dot(wg_s, n)), lambda n=n: us.append(xs_dot(wu_s, n))]
    side += [swiglu] + [lambda: None] * 7
    side += [functools.partial(down, n0, k0) for n0 in range(0, M, T) for k0 in range(0, F, 512)]
    c_pace = c_pacer((NP - 2) * NG, QS // RB - (NP - 2) * NG, 2, 55)
    r_pace = _Pacer([functools.partial(residual, n) for n in range(NQ)], M // 8, 2, 47)

    w_pace0 = w_pacer(jnp.int32(0), 3, 52)
    t_pace0 = _Pacer([lambda: first_terms(jnp.int32(0))], 32, 37, 56)

    def hook7():
        if side:
            side.pop(0)()
        return c_pace(), r_pace(), w_pace0(), t_pace0()
    q_strassen([NP - 1], _Q7_ORDER, hook7)
    assert not side and all(p.finished() for p in (c_pace, r_pace, w_pace0, t_pace0))
    y = jnp.concatenate([ys[n0] for n0 in range(0, M, T)] + [jnp.zeros((16, 512 - M), f32)], axis=1)
    yt = (y * rsel_s[:, 0:1]).T
    lane128 = lax.broadcasted_iota(jnp.int32, (1, T), 1)
    for e in range(2):
        i = idx_s[e]
        acc_s[i // T] += jnp.where(lane128 == i % T, (1.0 - g_s[i // T][1:2, :]) * yt[:M, e:e + 1], 0.0)

    for m in range(2):
        cp_kv(1, m).start()
    cp_wo.wait()

    tri = lax.broadcasted_iota(jnp.int32, (T, T), 1) <= lax.broadcasted_iota(jnp.int32, (T, T), 0)
    prog = _head_program()

    def head(h, carry):
        par, slot = h & 1, (h >> 1) & 1

        @pl.when(jnp.logical_and(h < H - 1, par == 1))
        def _():
            for m in range(2):
                cp_kv((h + 1) >> 1, m).wait()

        sh = (16 * (1 - par)).astype(u32)
        rhs, fw, fw_inv = [], fw_s[0], fw_s[1]
        for r1 in range(7):
            wk, wv = [_unpack(wkv_p[slot, m], sh + (h >> (8 + r1)).astype(u32)) for m in range(2)]
            wv = jnp.concatenate([wv[:, :T] * fw[0:1], wv[:, T:] * fw[0:1]], axis=1)
            t = _rhs_terms2(wk[:HC], wv[:HC], wk[HC:], wv[HC:])[r1]
            rhs.append([u.astype(bf) for u in _rhs_terms(t[:QC, :T], t[:QC, T:], t[QC:, :T], t[QC:, T:])])
        rhs[1][1], rhs[1][3] = t0_s[:, :T], t0_s[:, T:]
        hn = jnp.minimum(h + 1, H - 1)
        t_pace = _Pacer([lambda: first_terms(hn)], 32, 196 - 14, 196)
        w_pace = w_pacer(hn, 60, 180)
        prods, inner_q, outer, kblk, vblk = {}, {}, {}, {}, {}

        def kv_product(r1, r2):
            m = prods.setdefault(r1, {})
            m[r2] = _dot(ca_s[7 * r1 + r2], rhs[r1][r2])
            if len(m) == 7:
                inner_q[r1] = (((m[3] - m[4]) + m[6]) + m[0], m[2] + m[4], m[1] + m[3], ((m[0] - m[1]) + m[2]) + m[5])
                for b in range(4):
                    if b not in kblk and all(q in inner_q for q in (0, 1, 3, 4, 6)):
                        p = {q: inner_q[q][b] for q in (0, 1, 3, 4, 6)}
                        e, d = p[3] + p[1], p[3] - p[1]
                        kblk[b] = (p[0] + ((d - p[4]) + p[6]), e * 2.0)
                        outer[b] = ((e + p[4]) + p[6], p[0] + d)
                    if len(inner_q) == 7:
                        p2, p5 = inner_q[2][b], inner_q[5][b]
                        vblk[b] = (((outer[b][0] + p2) - p5) * 0.5, (outer[b][1] + p2) + p5)

        def rows(blk, t0, t1):
            return jnp.concatenate([jnp.concatenate(
                [blk[2 * (t // 4 % 2) + j2][t // 8][t % 4 * T:(t % 4 + 1) * T] for j2 in range(2)], axis=1)
                for t in range(t0, t1)], axis=0)

        @functools.cache
        def k_tile(t):
            return rows(kblk, t, t + 1).astype(bf)

        @functools.cache
        def k_terms(J):
            ka, kb = rows(kblk, 2 * J, 2 * J + 1), rows(kblk, 2 * J + 1, 2 * J + 2)
            return [t.astype(bf) for t in _rhs_terms(ka[:, :T], kb[:, :T], ka[:, T:], kb[:, T:])]

        @functools.cache
        def v_tiles(c0, c1):
            return rows(vblk, c0, c1).astype(bf)

        scores, rmax, soft, o_sum = {}, {}, {}, {}
        q_tiles = lambda I: [q_s[h, i * T:(i + 1) * T, t * T:(t + 1) * T] for i in (2 * I, 2 * I + 1) for t in range(2)]

        def score_block(I, J):
            q4, qx = q_tiles(I), [qa_s[h, I * T:(I + 1) * T, k * T:(k + 1) * T] for k in range(5)]
            lhs = [qx[0], qx[1], q4[0], q4[3], qx[2], qx[3], qx[4]]
            cs = _strassen(lambda i: _dot_nt(_feed(lhs[i], t_pace(), w_pace()), k_terms(J)[i]))
            for n, c in enumerate(cs):
                s_s[I % 2, n // 2, 2 * J + n % 2] = c
            for u in range(2):
                sa, sb = s_s[I % 2, u, 2 * J], s_s[I % 2, u, 2 * J + 1]
                scores[2 * I + u, 2 * J] = s_s[I % 2, u, 2 * J]
                scores[2 * I + u, 2 * J + 1] = s_s[I % 2, u, 2 * J + 1]
                mx = jnp.maximum(sa, sb)
                rmax[2 * I + u] = jnp.maximum(rmax[2 * I + u], mx) if 2 * I + u in rmax else mx

        def score_diag(I):
            a, b = 2 * I, 2 * I + 1
            q4 = q_tiles(I)
            qa, qb = jnp.concatenate(q4[0:2], axis=1), jnp.concatenate(q4[2:4], axis=1)
            d1 = _dot_nt(jnp.concatenate([qa, qb], axis=0), k_tile(a))
            d2 = _dot_nt(qb, k_tile(b))
            scores[a, a], scores[b, a], scores[b, b] = jnp.where(tri, d1[:T], NEG), d1[T:], jnp.where(tri, d2, NEG)

        def pv_chunk(i, c0):
            if c0 == 0:
                mx = functools.reduce(jnp.maximum, ([rmax[i]] if i > 1 else [])
                                      + [scores[i, t] for t in range(i // 2 * 2, i + 1)])
                soft[i] = dict(m=jnp.max(mx, axis=1, keepdims=True), l=None, ctx=None)
            st = soft[i]
            c1 = min(c0 + 2, i + 1)
            p = jnp.exp2(jnp.concatenate([scores.pop((i, t)) for t in range(c0, c1)], axis=1) - st['m']).astype(bf)
            pf = p.astype(f32)
            for t in range(c1 - c0):
                st['l'] = pf[:, t * T:(t + 1) * T] if st['l'] is None else st['l'] + pf[:, t * T:(t + 1) * T]
            d = _dot(p, v_tiles(c0, c1))
            st['ctx'] = d if st['ctx'] is None else st['ctx'] + d

        def context(i):
            st = soft.pop(i)
            l = jnp.sum(st['l'], axis=1, keepdims=True)
            r = pl.reciprocal(l, approx=True)
            return st['ctx'] * (r * (2.0 - l * r) * fw_inv[0:1, 0:1])

        def ship(blocks):
            @pl.when(h == H - 1)
            def _():
                for i in blocks:
                    cp_out(i).start()

        def out_plain(i):
            wo, ctx = wo_s[h], context(i).astype(bf)
            for a0 in (0, HM):
                a = acc_s[i, a0:a0 + HM, :] + g_s[i][1:2, :] * _dot_nt(wo[a0:a0 + HM], ctx)
                acc_s[i, a0:a0 + HM, :] = a
                out_s[i, a0:a0 + HM, :] = a.astype(bf)
            ship([i])

        @functools.cache
        def wo_terms():
            w = wo_s[h].astype(f32)
            return [t.astype(bf) for t in _lhs_terms(w[:HM, :T], w[:HM, T:], w[HM:, :T], w[HM:, T:])]

        @functools.cache
        def ctx_terms(I):
            ca, cb = context(2 * I), context(2 * I + 1)
            return _rhs_terms(ca[:, :T], cb[:, :T], ca[:, T:], cb[:, T:])

        def out_product(I, k):
            om_s[I, k] += _dot_nt(wo_terms()[k], ctx_terms(I)[k].astype(bf))
            o_sum[I, k] = om_s[I, k]
            if all((I, q) in o_sum for q in range(7)):
                for n, c in enumerate(_strassen(lambda q: o_sum.pop((I, q)))):
                    i, a0 = 2 * I + n % 2, (n // 2) * HM
                    out_s[i, a0:a0 + HM, :] = (acc_s[i, a0:a0 + HM, :] + g_s[i][1:2, :] * c).astype(bf)
                ship([2 * I, 2 * I + 1])

        ops = {'m': kv_product, 'r': score_block, 'd': score_diag, 'p': pv_chunk,
               'o': out_product, 'S': out_plain}
        for op, *args in prog:
            ops[op](*args)
        assert t_pace.finished() and w_pace.finished()

        @pl.when(jnp.logical_and((h + 3) >> 1 < NP, par == 1))
        def _():
            for m in range(2):
                cp_kv((h + 3) >> 1, m).start()
        return carry

    lax.fori_loop(0, H, head, 0)
    for i in range(NQ):
        cp_out(i).wait()


@jax.jit
def pallas_gated_mix__compressed_kv_cla__moe_arch_mod__prompt_kernel(
    A_x: jax.Array,
    A_c_kv: jax.Array,
    A_w_q: jax.Array,
    A_w_uk: jax.Array,
    A_w_uv: jax.Array,
    A_w_o: jax.Array,
    B_x: jax.Array,
    B_w_r: jax.Array,
    B_w_gate: jax.Array,
    B_w_up: jax.Array,
    B_w_down: jax.Array,
    gate_w: jax.Array,
):
    del B_x
    V = pltpu.VMEM
    B = lambda *shape: V(shape[:-2] + (shape[-2] // 2, shape[-1]), u32)
    out_t = pl.pallas_call(
        _kernel,
        in_specs=[pl.BlockSpec(memory_space=pl.ANY)] * 11,
        out_specs=pl.BlockSpec(memory_space=pl.ANY),
        out_shape=jax.ShapeDtypeStruct((M, S), bf),
        scratch_shapes=[
            V((M, S), bf), V((2, S, HM), bf), B(5, HS, HM),
            B(S, DC), B(49, QS, QC),
            V((NP, M, D), u32), V((2, 2, DC, D), u32), B(H, M, D),
            B(H, S, D), B(H, HS, 5 * T),
            V((NQ, M, T), f32),
            B(M, F), B(M, F), B(M, F),
            V((M,), bf), V((M,), bf), V((NQ, M, T), bf),
            V((NQ, 8, T), f32), B(2, 16, HM), V((16, T), f32),
            pltpu.SMEM((2,), jnp.int32),
            V((2, 2, NQ, T, T), f32), B(QC, 2 * T),
            V((NQ // 2, 7, HM, T), f32),
            V((2, 8, T), f32),
            pltpu.SemaphoreType.DMA((NSEM,)),
        ],
        compiler_params=pltpu.CompilerParams(vmem_limit_bytes=110 * 1024 * 1024),
        name="gated_mix_cla_mod",
    )(A_x[0].T, A_c_kv[0], A_w_q, A_w_uk, A_w_uv, A_w_o.transpose(0, 2, 1), B_w_r, B_w_gate, B_w_up,
      B_w_down.T, gate_w)
    return out_t.T[None]
```

```python
import functools
import math

import jax
import jax.numpy as jnp
from jax import lax
from jax.experimental import pallas as pl
from jax.experimental.pallas import tpu as pltpu

S, M, H, D, DC, F = 2048, 448, 16, 256, 1024, 1792
T = 128
NP, NQ = H // 2, S // T
HS, HM, HC = S // 2, M // 2, DC // 2
QS, QC = S // 4, DC // 4
RB = 16
XC = 256
NG = 5
NT = (((1,), (1,)), ((), ()))
QSCALE = D ** -0.5 * math.log2(math.e)
NEG = -1e30
bf, f32, u32 = jnp.bfloat16, jnp.float32, jnp.uint32
HI = 0xFFFF0000

SEM_WO, SEM_FFN, SEM_VEC, SEM_KV, SEM_WQ, SEM_XT, SEM_C, SEM_OUT, NSEM = 0, 1, 4, 6, 8, 16, 24, 32, 48


def _lhs_terms(a11, a12, a21, a22):
    return [a11 + a22, a21 + a22, a11, a22, a11 + a12, a21 - a11, a12 - a22]


def _rhs_terms(b11, b12, b21, b22):
    return [b11 + b22, b11, b12 - b22, b21 - b11, b22, b11 + b12, b21 + b22]


def _strassen(mm):
    m2, m3, m4, m5, m1, m7, m6 = [mm(i) for i in (1, 2, 3, 4, 0, 6, 5)]
    return (m4 - m5) + (m1 + m7), m3 + m5, m2 + m4, (m3 - m2) + (m1 + m6)


def _lhs_terms2(a11, a12, a21, a22):
    h21, q21, h22 = 0.5 * a21, 0.25 * a21, 0.5 * a22
    s1 = a11 + a22
    v, hs = a12 + q21, 0.5 * s1
    return [s1, q21 + h22, a11 + h21, h22 - q21, v + hs, h21 - a11, v - hs]


def _rhs_terms2(b11, b12, b21, b22):
    h21 = 0.5 * b21
    t1 = b11 + b22
    v, ht = b12 + 0.5 * h21, 0.5 * t1
    return [t1, b11 + h21, v - ht, h21 - b11, b22 - h21, v + ht, b22 + h21]


def _vregs(vals):
    ts = []
    for v in vals:
        v = v if v.dtype == u32 else pltpu.bitcast(v, u32)
        ts += [v[r:r + 8, c:c + T] for r in range(0, v.shape[0], 8) for c in range(0, v.shape[1] - T + 1, T)]
    return ts


def _zero_from(ts):
    acc = ts[:4]
    for i, t in enumerate(ts[4:]):
        acc[i % 4] = acc[i % 4] | t
    while len(acc) > 1:
        acc = [acc[i] | acc[i + 1] if i + 1 < len(acc) else acc[i] for i in range(0, len(acc), 2)]
    return (acc[0] >> 16) >> 16


def _feed(a, *zs):
    zs = [z for z in zs if z is not None]
    if not zs:
        return a
    a32 = pltpu.bitcast(a, u32)
    top = functools.reduce(lambda p, q: p | q, zs, a32[0:8, :T])
    if a32.shape[1] > T:
        top = jnp.concatenate([top, a32[0:8, T:]], axis=1)
    return pltpu.bitcast(jnp.concatenate([top, a32[8:]], axis=0), bf)


class _Pacer:
    def __init__(self, thunks, per, first, last):
        self.thunks, self.pool, self.k, self.done = list(thunks), [], 0, 0
        self.tot, self.first, self.last = per * len(self.thunks), first, last

    def __call__(self):
        self.k += 1
        if self.k <= self.first:
            return None
        want = min(self.tot, -(-(self.k - self.first) * self.tot // (self.last - self.first))) - self.done
        while len(self.pool) < want and self.thunks:
            self.pool += _vregs(self.thunks.pop(0)())
        outs, self.pool = self.pool[:want], self.pool[want:]
        self.done += len(outs)
        return _zero_from(outs) if outs else None

    def finished(self):
        return not self.thunks and not self.pool


_HEAD_ORDER = """
m1.1 m1.3 m1.4 m1.6 m1.0 m3.3 m3.6 m1.2 m3.4 m4.3 m3.1 m3.0 m4.4 m3.2 m3.5 m1.5 m4.6 m4.1 m4.0 m6.6 m6.3 m6.0
m4.5 m0.1 m6.4 m6.1 m6.5 m6.2 m4.2 m0.6 m0.4 m0.3 m0.0 m0.2 m0.5 m2.1 d0 m2.3 r7.0 m2.4 r7.1 m2.0 m2.6 m5.1 r7.2
m2.2 r7.4 m2.5 r7.3 r7.6 r7.5 m5.3 d7 m5.6 m5.4 m5.0 m5.2 m5.5 p14.0 r6.0 p1.0 p0.0 r6.2 r6.1 p14.2 p14.4 p14.6
p14.8 p14.10 p15.0 p14.12 p14.14 r6.3 r6.4 r6.5 p15.2 p15.4 p15.6 p15.8 p15.10 d6 p15.12 p15.14 p12.0 r5.0 p12.2
p12.4 p12.6 r5.3 r5.2 r5.1 p12.8 p13.0 p12.10 p13.2 r5.4 p13.4 p13.6 p13.8 p12.12 d5 o0.3 o0.2 o0.1 p10.0 o0.0
o0.5 p11.0 p13.10 r4.1 o0.4 p10.2 p13.12 p10.4 r4.0 o0.6 p10.6 p10.8 p11.2 p10.10 r4.2 r4.3 p11.4 d4 p11.6 o7.2
o7.0 o7.1 o7.4 o7.3 o7.6 o7.5 r3.0 p11.8 p8.0 p8.2 p8.4 p8.6 p9.0 p9.2 p11.10 p8.8 r3.1 d3 r3.2 o6.4 o6.2 p9.4
o6.0 o6.6 o6.3 o6.1 p7.0 r2.1 p9.6 p6.0 p9.8 p6.2 p6.4 r2.0 o6.5 p6.6 d2 p7.2 p4.0 o5.3 o5.2 o5.1 o5.4 o5.6 o5.5
o5.0 r1.0 p4.2 p7.4 p5.0 p7.6 p4.4 d1 p5.2 o4.4 o4.2 p2.0 o4.1 o4.0 o4.3 p3.0 o4.6 o4.5 p2.2 p5.4 o2.1 p3.2 S2
o3.3 o2.3 o2.6 o2.4 o2.0 o3.2 o2.2 o2.5 o3.5 o3.1 o3.6 o3.0 o3.4 S3
"""


def _head_program():
    return [(t[0],) + tuple(int(v) for v in t[1:].split('.')) for t in _HEAD_ORDER.split()]


_P0_ORDER = """
61 r0 r1 70 r4 r3 60 r2 71 62 r5 63 r7 72 r6 73 r8 80 r9 90 93 r11 81 r14 r12 91 r13 83 r15 82 r10 92 a1 a0 b0
f3 c3 d2 d3 f0 e0 e1 b2 c0 c1 b1 a3 a2 b3 e2 c2 f2 f1 e3 d1 d0
"""
_Q7_ORDER = """
010 023 021 027 016 022 026 025 030 012 014 015 011 017 045 044 047 020 031 032 033 034 013 024 046 043 036 035
041 042 000 037 040 001 005 004 003 006 002 007 060 061 066 067 062 063 064 065 051 053 052 050 056 054 055 057
"""
_Q_ORDER = """
016 011 015 012 014 017 013 010 041 027 031 022 026 024 034 007 040 021 001 036 025 046 033 047 035 042 005 023
006 032 043 020 037 004 044 030 000 045 002 003 050 061 054 053 064 067 051 060 052 066 062 063 065 116 112 111
113 117 124 125 121 123 126 120 057 127 122 133 130 131 144 132 056 114 140 137 143 110 055 100 146 115 145 141
107 160 134 136 147 135 161 142 101 102 162 106 104 103 154 105 163 165 167 152 150 157 155 166 151 156 153 164
"""


def _dot(a, b):
    return jnp.dot(a, b, preferred_element_type=f32)


def _dot_nt(a, b):
    return lax.dot_general(a, b, NT, preferred_element_type=f32)


def _unpack(w32, sh):
    return pltpu.bitcast((w32 << sh) & jnp.uint32(HI), f32)


class _Bf16:
    def __init__(self, raw):
        self.raw = raw

    def _half(self, idx):
        idx = list(idx if isinstance(idx, tuple) else (idx,))
        idx += [slice(None)] * (len(self.raw.shape) - len(idx))
        r = idx[-2]
        if isinstance(r, slice):
            idx[-2] = slice(None if r.start is None else r.start // 2, None if r.stop is None else r.stop // 2)
        elif isinstance(r.start, int):
            idx[-2] = pl.ds(r.start // 2, r.size // 2)
        else:
            idx[-2] = pl.ds(pl.multiple_of(r.start >> 1, 8), r.size // 2)
        return tuple(idx)

    def __getitem__(self, idx):
        return pltpu.bitcast(self.raw[self._half(idx)], bf)

    def put(self, idx, v):
        idx = self._half(idx)
        ref = self.raw.at[idx[:-2]] if len(idx) > 2 else self.raw
        o = pltpu.bitcast(v, u32)
        ref[idx[-2], idx[-1]] = o
        return o

    def __setitem__(self, idx, v):
        self.put(idx, v)


def _kernel(xt_hbm, c_hbm, wq_hbm, wk_hbm, wv_hbm, wo_hbm, wr_hbm, wg_hbm, wu_hbm, wd_hbm, gw_hbm, o_hbm,
            xt_s, x_s, xa_r, c_r, ca_r, wq_p, wkv_p, wo_r, q_r, qa_r, acc_s, wg_r, wu_r, wd_r,
            wr_s, gw_s, out_s, g_s, xs_r, rsel_s, idx_s, s_s, t0_r, om_s, fw_s, sem):
    xa_s, c_s, ca_s, wo_s, q_s, qa_s, wg_s, wu_s, wd_s, xs_s, t0_s = [
        _Bf16(r) for r in (xa_r, c_r, ca_r, wo_r, q_r, qa_r, wg_r, wu_r, wd_r, xs_r, t0_r)]
    mk = pltpu.make_async_copy
    wq32, wk32, wv32 = wq_hbm.bitcast(u32), wk_hbm.bitcast(u32), wv_hbm.bitcast(u32)
    cp_wq = lambda j: mk(wq32.at[:, j, :], wq_p.at[j], sem.at[SEM_WQ + j])
    cp_kv = lambda j, m: mk((wk32, wv32)[m].at[:, j, :], wkv_p.at[j & 1, m], sem.at[SEM_KV + m])
    cp_xt = lambda k: mk(xt_hbm.at[:, pl.ds(k * XC, XC)], xt_s.at[:, pl.ds(k * XC, XC)], sem.at[SEM_XT + k])
    cp_out = lambda i: mk(out_s.at[i], o_hbm.at[:, pl.ds(i * T, T)], sem.at[SEM_OUT + i])
    cp_vec = [mk(wr_hbm, wr_s, sem.at[SEM_VEC]), mk(gw_hbm, gw_s, sem.at[SEM_VEC + 1])]
    cp_ffn = [mk(src, dst, sem.at[SEM_FFN + n]) for n, (src, dst) in
              enumerate(((wg_hbm.bitcast(u32), wg_r), (wu_hbm.bitcast(u32), wu_r), (wd_hbm.bitcast(u32), wd_r)))]
    cp_wo = mk(wo_hbm.bitcast(u32), wo_r, sem.at[SEM_WO])
    c32 = c_hbm.bitcast(u32)

    def cp_c(j):
        r0 = (j - 1) * (NG * RB // 2)
        n = QS // 2 - r0 if isinstance(j, int) and j == NP - 1 else NG * RB // 2
        return [mk(c32.at[pl.ds(i * QS // 2 + r0, n)], c_r.at[pl.ds(i * QS // 2 + r0, n)], sem.at[SEM_C + j])
                for i in range(4)]

    cp_xt(0).start()
    cp_wq(0).start()
    for k in range(1, S // XC):
        cp_xt(k).start()
    for cp in cp_vec:
        cp.start()
    for j in range(1, NP):
        cp_wq(j).start()
        for cp in cp_c(j):
            cp.start()
    for cp in cp_ffn + [cp_kv(0, 0), cp_kv(0, 1), cp_wo]:
        cp.start()

    @pl.loop(0, NQ // 2)
    def _(n):
        om_s[n] = jnp.zeros(om_s.shape[1:], f32)

    def store_q(j, e, r0, q):
        q = q * QSCALE
        q_s[2 * j + e, r0:r0 + q.shape[0], :] = q.astype(bf)
        for p0 in range(0, q.shape[0], 2 * T):
            if r0 + p0 > 0:
                qa, qb = q[p0:p0 + T], q[p0 + T:p0 + 2 * T]
                terms = _lhs_terms(qa[:, :T], qa[:, T:], qb[:, :T], qb[:, T:])
                for k, i in enumerate((0, 1, 4, 5, 6)):
                    qa_s[2 * j + e, (r0 + p0) // 2:(r0 + p0) // 2 + T, k * T:(k + 1) * T] = terms[i].astype(bf)

    def q_dot(w, r0, r1, z=None):
        return _dot(_feed(x_s[0, r0:r1, :], z), w[:HM]) + _dot(x_s[1, r0:r1, :], w[HM:])

    def q_plain(w, r0):
        qf = q_dot(w, r0, r0 + 2 * T)
        store_q(0, 0, r0, qf[:, :D])
        store_q(0, 1, r0, qf[:, D:])

    def q_rhs(j):
        lo, hi = pltpu.bitcast(wq_p[j] << 16, f32), pltpu.bitcast(wq_p[j] & jnp.uint32(HI), f32)
        b = [jnp.concatenate([lo[:, t * T:(t + 1) * T], hi[:, t * T:(t + 1) * T]], axis=1) for t in range(2)]
        return [t.astype(bf) for t in _rhs_terms(b[0][:HM], b[1][:HM], b[0][HM:], b[1][HM:])]

    def q_strassen(js, order, hook):
        ts, res = [q_rhs(j) for j in js], {}
        for a, k, u in [map(int, t) for t in order.split()]:
            if k in (2, 3):
                lhs = x_s[k - 2, (k - 2) * HS + u * T:(k - 2) * HS + (u + 1) * T, :]
            else:
                lhs = xa_s[k - 2 * (k > 3), u * T:(u + 1) * T, :]
            res[a, k, u] = _dot(_feed(lhs, *hook()), ts[a][k])
            v = u // 2 * 2
            if all((a, kk, uu) in res for kk in range(7) for uu in (v, v + 1)):
                cs = _strassen(lambda i: jnp.concatenate([res.pop((a, i, v)), res.pop((a, i, v + 1))], axis=0))
                for w in range(2):
                    for e in range(2):
                        q = jnp.concatenate([c[:, e * T:(e + 1) * T] for c in cs[2 * w:2 * w + 2]], axis=1)
                        store_q(js[a], e, w * HS + v * T, q)

    def x_prep(r0):
        a = [x_s[e, h0 + r0:h0 + r0 + RB, :].astype(f32) for h0 in (0, HS) for e in (0, 1)]
        terms = _lhs_terms(*a)
        outs = []
        for k, i in enumerate((0, 1, 4, 5, 6)):
            outs.append(xa_s.put((k, slice(r0, r0 + RB)), terms[i].astype(bf)))
        return outs

    def c_prep(g, c0):
        blk = lambda i, k: c_s[pl.ds(i * QS + g * RB, RB), k * QC + c0:k * QC + c0 + T].astype(f32)
        outer = [_lhs_terms2(*[blk(2 * i1 + i2, 2 * k1 + k2) for i1 in range(2) for k1 in range(2)])
                 for i2 in range(2) for k2 in range(2)]
        outs = []
        for r1 in range(7):
            for r2, v in enumerate(_lhs_terms(*[o[r1] for o in outer])):
                outs.append(ca_s.put((7 * r1 + r2, pl.ds(g * RB, RB), slice(c0, c0 + T)), v.astype(bf)))
        return outs

    def c_pacer(g0, ng, first, last):
        return _Pacer([functools.partial(c_prep, g0 + t // 2, (t % 2) * T) for t in range(2 * ng)], 49, first, last)

    def transpose(k):
        for e in range(2):
            x_s[e, k * XC:(k + 1) * XC, :] = xt_s[e * HM:(e + 1) * HM, k * XC:(k + 1) * XC].T

    def q_w0():
        return jnp.concatenate([pltpu.bitcast(wq_p[0] << 16, f32).astype(bf),
                                pltpu.bitcast(wq_p[0] & jnp.uint32(HI), f32).astype(bf)], axis=1)

    cp_xt(0).wait()
    transpose(0)
    cp_wq(0).wait()
    q_plain(q_w0(), 0)
    for k in range(1, 4):
        cp_xt(k).wait()
    transpose(1)
    w0 = q_w0()
    transpose(2)
    q_plain(w0, XC)
    transpose(3)
    q_plain(w0, 2 * XC)
    for k in range(4, S // XC):
        cp_xt(k).wait()
    for cp in cp_vec:
        cp.wait()
    for k in range(4, S // XC):
        transpose(k)
    row8 = lax.broadcasted_iota(jnp.int32, (8, M), 0)
    x_pace = _Pacer([functools.partial(x_prep, r0) for r0 in range(0, HS, RB)], 5, 12, 40)
    w0, res = q_w0(), {}
    for t in _P0_ORDER.split():
        if t[0] == 'r':
            n = int(t[1:])
            rg = jnp.where(row8 == 0, wr_s[...].reshape(1, M).astype(f32), gw_s[...].reshape(1, M).astype(f32))
            g_s[n] = _dot(rg.astype(bf), xt_s[:, n * T:(n + 1) * T])
            continue
        u, n = int(t[:-1], 16), int(t[-1])
        res[u, n] = q_dot(w0[:, n * T:(n + 1) * T], u * T, (u + 1) * T, x_pace())
        v = u // 2 * 2
        if all((uu, nn) in res for uu in (v, v + 1) for nn in range(4)):
            for e in range(2):
                store_q(0, e, v * T, jnp.concatenate([jnp.concatenate(
                    [res.pop((uu, nn)) for nn in (2 * e, 2 * e + 1)], axis=1) for uu in (v, v + 1)], axis=0))
    assert x_pace.finished()

    rb = jnp.concatenate([g_s[n][0:1, :] for n in range(NQ)], axis=1).astype(bf).astype(f32)
    lane = lax.broadcasted_iota(jnp.int32, (1, S), 1)
    m1 = jnp.max(rb, axis=1, keepdims=True)
    i1 = jnp.minimum(jnp.min(jnp.where(rb == m1, lane, S)), S - 1)
    rb2 = jnp.where(lane == i1, -jnp.inf, rb)
    m2 = jnp.max(rb2, axis=1, keepdims=True)
    i2 = jnp.minimum(jnp.min(jnp.where(jnp.logical_and(rb2 == m2, lane != i1), lane, S)), S - 1)
    row16 = lax.broadcasted_iota(jnp.int32, (16, HM), 0)

    def x_row(e, i):
        blk = x_s[e, pl.ds(pl.multiple_of((i // 16) * 16, 16), 16), :].astype(f32)
        return jnp.sum(jnp.where(row16 == i % 16, blk, 0.0), axis=0, keepdims=True)
    for e in range(2):
        xs_s[e] = jnp.where(row16 == 0, x_row(e, i1), jnp.where(row16 == 1, x_row(e, i2), 0.0)).astype(bf)
    rsel_s[...] = jax.nn.sigmoid(jnp.where(lax.broadcasted_iota(jnp.int32, (16, T), 0) == 0, m1, m2))
    idx_s[0] = i1
    idx_s[1] = i2

    def q_body(it, carry):
        js = (2 * it + 1, 2 * it + 2)
        for j in js:
            for cp in [cp_wq(j)] + cp_c(j):
                cp.wait()
        pace = c_pacer(2 * it * NG, 2 * NG, 1, 108)
        q_strassen(js, _Q_ORDER, lambda: (pace(),))
        assert pace.finished()
        return carry
    lax.fori_loop(0, 3, q_body, 0)

    for cp in cp_ffn + [cp_wq(NP - 1), cp_kv(0, 0), cp_kv(0, 1)] + cp_c(NP - 1):
        cp.wait()

    def w_sum(hn, m, r0):
        w = [wkv_p[(hn >> 1) & 1, m, r:r + 8, :] for r in range(r0, r0 + HC, 64)]
        w = (jnp.concatenate(w, axis=0) << (16 * (1 - (hn & 1))).astype(u32)) & jnp.uint32(0x7FFF0000)
        return functools.reduce(jnp.add, [pltpu.bitcast(t, f32) for t in _vregs([w])])

    def w_balance(parts):
        n = len(parts) // 2
        sk, sv = [jnp.sum(functools.reduce(jnp.add, p), keepdims=True) for p in (parts[:n], parts[n:])]
        ok = jnp.logical_and(sk > 0, sv > 0)
        ratio = jnp.broadcast_to(jnp.where(ok, 1.4 * sk, 1.0) / jnp.where(ok, sv, 1.0), (8, T))
        e = jnp.clip(pltpu.bitcast(ratio, jnp.int32) & 0x7F800000, (127 - 40) << 23, (127 + 40) << 23)
        fw_s[0] = pltpu.bitcast(e, f32)
        fw_s[1] = pltpu.bitcast((254 << 23) - e, f32)
        return [e]

    def w_pacer(hn, first, last):
        parts = []
        return _Pacer([lambda m=m, r0=r0: parts.append(w_sum(hn, m, r0)) or parts[-1:]
                       for m in range(2) for r0 in (0, HC)] + [lambda: w_balance(parts)], 1, first, last)

    def first_terms(hn):
        w = _unpack(wkv_p[(hn >> 1) & 1, 0, :, :T], (16 * (1 - (hn & 1))).astype(u32))
        t = w[:HC] + 0.5 * w[HC:]
        return [t0_s.put((slice(None), slice(n * T, (n + 1) * T)), v.astype(bf))
                for n, v in enumerate((t[:QC], t[QC:] - t[:QC]))]

    def residual(n):
        g8 = jax.nn.sigmoid(g_s[n])
        g_s[n] = g8
        a = (1.0 - g8[1:2, :]) * xt_s[:, n * T:(n + 1) * T].astype(f32)
        acc_s[n] = a
        return [a]

    gs, us, ys, hid = [], [], {}, []
    xs_dot = lambda w_s, n: (_dot(xs_s[0], w_s[:HM, n * T:(n + 1) * T]) + _dot(xs_s[1], w_s[HM:, n * T:(n + 1) * T]))

    def swiglu():
        gg, uu = jnp.concatenate(gs, axis=1), jnp.concatenate(us, axis=1)
        hid.append((gg * jax.nn.sigmoid(gg) * uu).astype(bf))

    def down(n0, k0):
        t = _dot_nt(hid[0][:, k0:min(k0 + 512, F)], wd_s[n0:min(n0 + T, M), k0:min(k0 + 512, F)])
        ys[n0] = ys[n0] + t if n0 in ys else t
    side = []
    for n in range(F // T):
        side += [lambda n=n: gs.append(xs_dot(wg_s, n)), lambda n=n: us.append(xs_dot(wu_s, n))]
    side += [swiglu] + [lambda: None] * 7
    side += [functools.partial(down, n0, k0) for n0 in range(0, M, T) for k0 in range(0, F, 512)]
    c_pace = c_pacer((NP - 2) * NG, QS // RB - (NP - 2) * NG, 2, 55)
    r_pace = _Pacer([functools.partial(residual, n) for n in range(NQ)], M // 8, 2, 47)

    w_pace0 = w_pacer(jnp.int32(0), 3, 52)
    t_pace0 = _Pacer([lambda: first_terms(jnp.int32(0))], 32, 37, 56)

    def hook7():
        if side:
            side.pop(0)()
        return c_pace(), r_pace(), w_pace0(), t_pace0()
    q_strassen([NP - 1], _Q7_ORDER, hook7)
    assert not side and all(p.finished() for p in (c_pace, r_pace, w_pace0, t_pace0))
    y = jnp.concatenate([ys[n0] for n0 in range(0, M, T)] + [jnp.zeros((16, 512 - M), f32)], axis=1)
    yt = (y * rsel_s[:, 0:1]).T
    lane128 = lax.broadcasted_iota(jnp.int32, (1, T), 1)
    for e in range(2):
        i = idx_s[e]
        acc_s[i // T] += jnp.where(lane128 == i % T, (1.0 - g_s[i // T][1:2, :]) * yt[:M, e:e + 1], 0.0)

    for m in range(2):
        cp_kv(1, m).start()
    cp_wo.wait()

    tri = lax.broadcasted_iota(jnp.int32, (T, T), 1) <= lax.broadcasted_iota(jnp.int32, (T, T), 0)
    prog = _head_program()

    def head(h, carry):
        par, slot = h & 1, (h >> 1) & 1

        @pl.when(jnp.logical_and(h < H - 1, par == 1))
        def _():
            for m in range(2):
                cp_kv((h + 1) >> 1, m).wait()

        sh = (16 * (1 - par)).astype(u32)
        rhs, fw, fw_inv = [], fw_s[0], fw_s[1]
        for r1 in range(7):
            wk, wv = [_unpack(wkv_p[slot, m], sh + (h >> (8 + r1)).astype(u32)) for m in range(2)]
            wv = jnp.concatenate([wv[:, :T] * fw[0:1], wv[:, T:] * fw[0:1]], axis=1)
            t = _rhs_terms2(wk[:HC], wv[:HC], wk[HC:], wv[HC:])[r1]
            rhs.append([u.astype(bf) for u in _rhs_terms(t[:QC, :T], t[:QC, T:], t[QC:, :T], t[QC:, T:])])
        rhs[1][1], rhs[1][3] = t0_s[:, :T], t0_s[:, T:]
        hn = jnp.minimum(h + 1, H - 1)
        t_pace = _Pacer([lambda: first_terms(hn)], 32, 196 - 14, 196)
        w_pace = w_pacer(hn, 60, 180)
        prods, inner_q, outer, kblk, vblk = {}, {}, {}, {}, {}

        def kv_product(r1, r2):
            m = prods.setdefault(r1, {})
            m[r2] = _dot(ca_s[7 * r1 + r2], rhs[r1][r2])
            if len(m) == 7:
                inner_q[r1] = (((m[3] - m[4]) + m[6]) + m[0], m[2] + m[4], m[1] + m[3], ((m[0] - m[1]) + m[2]) + m[5])
                for b in range(4):
                    if b not in kblk and all(q in inner_q for q in (0, 1, 3, 4, 6)):
                        p = {q: inner_q[q][b] for q in (0, 1, 3, 4, 6)}
                        e, d = p[3] + p[1], p[3] - p[1]
                        kblk[b] = (p[0] + ((d - p[4]) + p[6]), e * 2.0)
                        outer[b] = ((e + p[4]) + p[6], p[0] + d)
                    if len(inner_q) == 7:
                        p2, p5 = inner_q[2][b], inner_q[5][b]
                        vblk[b] = (((outer[b][0] + p2) - p5) * 0.5, (outer[b][1] + p2) + p5)

        def rows(blk, t0, t1):
            return jnp.concatenate([jnp.concatenate(
                [blk[2 * (t // 4 % 2) + j2][t // 8][t % 4 * T:(t % 4 + 1) * T] for j2 in range(2)], axis=1)
                for t in range(t0, t1)], axis=0)

        @functools.cache
        def k_tile(t):
            return rows(kblk, t, t + 1).astype(bf)

        @functools.cache
        def k_terms(J):
            ka, kb = rows(kblk, 2 * J, 2 * J + 1), rows(kblk, 2 * J + 1, 2 * J + 2)
            return [t.astype(bf) for t in _rhs_terms(ka[:, :T], kb[:, :T], ka[:, T:], kb[:, T:])]

        @functools.cache
        def v_tiles(c0, c1):
            return rows(vblk, c0, c1).astype(bf)

        scores, rmax, soft, o_sum = {}, {}, {}, {}
        q_tiles = lambda I: [q_s[h, i * T:(i + 1) * T, t * T:(t + 1) * T] for i in (2 * I, 2 * I + 1) for t in range(2)]

        def score_block(I, J):
            q4, qx = q_tiles(I), [qa_s[h, I * T:(I + 1) * T, k * T:(k + 1) * T] for k in range(5)]
            lhs = [qx[0], qx[1], q4[0], q4[3], qx[2], qx[3], qx[4]]
            cs = _strassen(lambda i: _dot_nt(_feed(lhs[i], t_pace(), w_pace()), k_terms(J)[i]))
            for n, c in enumerate(cs):
                s_s[I % 2, n // 2, 2 * J + n % 2] = c
            for u in range(2):
                sa, sb = s_s[I % 2, u, 2 * J], s_s[I % 2, u, 2 * J + 1]
                scores[2 * I + u, 2 * J] = s_s[I % 2, u, 2 * J]
                scores[2 * I + u, 2 * J + 1] = s_s[I % 2, u, 2 * J + 1]
                mx = jnp.maximum(sa, sb)
                rmax[2 * I + u] = jnp.maximum(rmax[2 * I + u], mx) if 2 * I + u in rmax else mx

        def score_diag(I):
            a, b = 2 * I, 2 * I + 1
            q4 = q_tiles(I)
            qa, qb = jnp.concatenate(q4[0:2], axis=1), jnp.concatenate(q4[2:4], axis=1)
            d1 = _dot_nt(jnp.concatenate([qa, qb], axis=0), k_tile(a))
            d2 = _dot_nt(qb, k_tile(b))
            scores[a, a], scores[b, a], scores[b, b] = jnp.where(tri, d1[:T], NEG), d1[T:], jnp.where(tri, d2, NEG)

        def pv_chunk(i, c0):
            if c0 == 0:
                mx = functools.reduce(jnp.maximum, ([rmax[i]] if i > 1 else [])
                                      + [scores[i, t] for t in range(i // 2 * 2, i + 1)])
                soft[i] = dict(m=jnp.max(mx, axis=1, keepdims=True), l=None, ctx=None)
            st = soft[i]
            c1 = min(c0 + 2, i + 1)
            p = jnp.exp2(jnp.concatenate([scores.pop((i, t)) for t in range(c0, c1)], axis=1) - st['m']).astype(bf)
            pf = p.astype(f32)
            for t in range(c1 - c0):
                st['l'] = pf[:, t * T:(t + 1) * T] if st['l'] is None else st['l'] + pf[:, t * T:(t + 1) * T]
            d = _dot(p, v_tiles(c0, c1))
            st['ctx'] = d if st['ctx'] is None else st['ctx'] + d

        def context(i):
            st = soft.pop(i)
            l = jnp.sum(st['l'], axis=1, keepdims=True)
            r = pl.reciprocal(l, approx=True)
            return st['ctx'] * (r * (2.0 - l * r) * fw_inv[0:1, 0:1])

        def ship(blocks):
            @pl.when(h == H - 1)
            def _():
                for i in blocks:
                    cp_out(i).start()

        def out_plain(i):
            wo, ctx = wo_s[h], context(i).astype(bf)
            for a0 in (0, HM):
                a = acc_s[i, a0:a0 + HM, :] + g_s[i][1:2, :] * _dot_nt(wo[a0:a0 + HM], ctx)
                acc_s[i, a0:a0 + HM, :] = a
                out_s[i, a0:a0 + HM, :] = a.astype(bf)
            ship([i])

        @functools.cache
        def wo_terms():
            w = wo_s[h].astype(f32)
            return [t.astype(bf) for t in _lhs_terms(w[:HM, :T], w[:HM, T:], w[HM:, :T], w[HM:, T:])]

        @functools.cache
        def ctx_terms(I):
            ca, cb = context(2 * I), context(2 * I + 1)
            return _rhs_terms(ca[:, :T], cb[:, :T], ca[:, T:], cb[:, T:])

        def out_product(I, k):
            om_s[I, k] += _dot_nt(wo_terms()[k], ctx_terms(I)[k].astype(bf))
            o_sum[I, k] = om_s[I, k]
            if all((I, q) in o_sum for q in range(7)):
                for n, c in enumerate(_strassen(lambda q: o_sum.pop((I, q)))):
                    i, a0 = 2 * I + n % 2, (n // 2) * HM
                    out_s[i, a0:a0 + HM, :] = (acc_s[i, a0:a0 + HM, :] + g_s[i][1:2, :] * c).astype(bf)
                ship([2 * I, 2 * I + 1])

        ops = {'m': kv_product, 'r': score_block, 'd': score_diag, 'p': pv_chunk,
               'o': out_product, 'S': out_plain}
        for op, *args in prog:
            ops[op](*args)
        assert t_pace.finished() and w_pace.finished()

        @pl.when(jnp.logical_and((h + 3) >> 1 < NP, par == 1))
        def _():
            for m in range(2):
                cp_kv((h + 3) >> 1, m).start()
        return carry

    lax.fori_loop(0, H, head, 0)
    for i in range(NQ):
        cp_out(i).wait()


@jax.jit
def pallas_gated_mix__compressed_kv_cla__moe_arch_mod__prompt_kernel(
    A_x: jax.Array,
    A_c_kv: jax.Array,
    A_w_q: jax.Array,
    A_w_uk: jax.Array,
    A_w_uv: jax.Array,
    A_w_o: jax.Array,
    B_x: jax.Array,
    B_w_r: jax.Array,
    B_w_gate: jax.Array,
    B_w_up: jax.Array,
    B_w_down: jax.Array,
    gate_w: jax.Array,
):
    del B_x
    V = pltpu.VMEM
    B = lambda *shape: V(shape[:-2] + (shape[-2] // 2, shape[-1]), u32)
    out_t = pl.pallas_call(
        _kernel,
        in_specs=[pl.BlockSpec(memory_space=pl.ANY)] * 11,
        out_specs=pl.BlockSpec(memory_space=pl.ANY),
        out_shape=jax.ShapeDtypeStruct((M, S), bf),
        scratch_shapes=[
            V((M, S), bf), V((2, S, HM), bf), B(5, HS, HM),
            B(S, DC), B(49, QS, QC),
            V((NP, M, D), u32), V((2, 2, DC, D), u32), B(H, M, D),
            B(H, S, D), B(H, HS, 5 * T),
            V((NQ, M, T), f32),
            B(M, F), B(M, F), B(M, F),
            V((M,), bf), V((M,), bf), V((NQ, M, T), bf),
            V((NQ, 8, T), f32), B(2, 16, HM), V((16, T), f32),
            pltpu.SMEM((2,), jnp.int32),
            V((2, 2, NQ, T, T), f32), B(QC, 2 * T),
            V((NQ // 2, 7, HM, T), f32),
            V((2, 8, T), f32),
            pltpu.SemaphoreType.DMA((NSEM,)),
        ],
        compiler_params=pltpu.CompilerParams(vmem_limit_bytes=110 * 1024 * 1024),
        name="gated_mix_cla_mod",
    )(A_x[0].T, A_c_kv[0], A_w_q, A_w_uk, A_w_uv, A_w_o.transpose(0, 2, 1), B_w_r, B_w_gate, B_w_up,
      B_w_down.T, gate_w)
    return out_t.T[None]
```

```python
import functools
import math

import jax
import jax.numpy as jnp
from jax import lax
from jax.experimental import pallas as pl
from jax.experimental.pallas import tpu as pltpu

S, M, H, D, DC, F = 2048, 448, 16, 256, 1024, 1792
T = 128
NP, NQ = H // 2, S // T
HS, HM, HC = S // 2, M // 2, DC // 2
QS, QC = S // 4, DC // 4
RB = 16
XC = 256
NG = 5
NT = (((1,), (1,)), ((), ()))
QSCALE = D ** -0.5 * math.log2(math.e)
NEG = -1e30
bf, f32, u32 = jnp.bfloat16, jnp.float32, jnp.uint32
HI = 0xFFFF0000

SEM_WO, SEM_FFN, SEM_VEC, SEM_KV, SEM_WQ, SEM_XT, SEM_C, SEM_OUT, NSEM = 0, 1, 4, 6, 8, 16, 24, 32, 48


def _lhs_terms(a11, a12, a21, a22):
    return [a11 + a22, a21 + a22, a11, a22, a11 + a12, a21 - a11, a12 - a22]


def _rhs_terms(b11, b12, b21, b22):
    return [b11 + b22, b11, b12 - b22, b21 - b11, b22, b11 + b12, b21 + b22]


def _strassen(mm):
    m2, m3, m4, m5, m1, m7, m6 = [mm(i) for i in (1, 2, 3, 4, 0, 6, 5)]
    return (m4 - m5) + (m1 + m7), m3 + m5, m2 + m4, (m3 - m2) + (m1 + m6)


def _lhs_terms2(a11, a12, a21, a22):
    h21, q21, h22 = 0.5 * a21, 0.25 * a21, 0.5 * a22
    s1 = a11 + a22
    v, hs = a12 + q21, 0.5 * s1
    return [s1, q21 + h22, a11 + h21, h22 - q21, v + hs, h21 - a11, v - hs]


def _rhs_terms2(b11, b12, b21, b22):
    h21 = 0.5 * b21
    t1 = b11 + b22
    v, ht = b12 + 0.5 * h21, 0.5 * t1
    return [t1, b11 + h21, v - ht, h21 - b11, b22 - h21, v + ht, b22 + h21]


def _vregs(vals):
    ts = []
    for v in vals:
        v = v if v.dtype == u32 else pltpu.bitcast(v, u32)
        ts += [v[r:r + 8, c:c + T] for r in range(0, v.shape[0], 8) for c in range(0, v.shape[1] - T + 1, T)]
    return ts


def _zero_from(ts):
    acc = ts[:4]
    for i, t in enumerate(ts[4:]):
        acc[i % 4] = acc[i % 4] | t
    while len(acc) > 1:
        acc = [acc[i] | acc[i + 1] if i + 1 < len(acc) else acc[i] for i in range(0, len(acc), 2)]
    return (acc[0] >> 16) >> 16


def _feed(a, *zs):
    zs = [z for z in zs if z is not None]
    if not zs:
        return a
    a32 = pltpu.bitcast(a, u32)
    top = functools.reduce(lambda p, q: p | q, zs, a32[0:8, :T])
    if a32.shape[1] > T:
        top = jnp.concatenate([top, a32[0:8, T:]], axis=1)
    return pltpu.bitcast(jnp.concatenate([top, a32[8:]], axis=0), bf)


class _Pacer:
    def __init__(self, thunks, per, first, last):
        self.thunks, self.pool, self.k, self.done = list(thunks), [], 0, 0
        self.tot, self.first, self.last = per * len(self.thunks), first, last

    def __call__(self):
        self.k += 1
        if self.k <= self.first:
            return None
        want = min(self.tot, -(-(self.k - self.first) * self.tot // (self.last - self.first))) - self.done
        while len(self.pool) < want and self.thunks:
            self.pool += _vregs(self.thunks.pop(0)())
        outs, self.pool = self.pool[:want], self.pool[want:]
        self.done += len(outs)
        return _zero_from(outs) if outs else None

    def finished(self):
        return not self.thunks and not self.pool


_HEAD_ORDER = """
m1.1 m1.3 m1.4 m1.6 m1.0 m3.4 m3.3 m1.2 m4.3 m3.6 m3.0 m3.1 m4.4 m3.2 m3.5 m1.5 m4.6 m4.1 m4.0 m6.6 m6.3 m6.0
m0.1 m4.5 m6.4 m6.1 m6.5 m6.2 m4.2 m0.6 m0.4 m0.3 m0.0 m0.2 m0.5 m2.1 d0 m2.3 r7.1 r7.2 r7.3 r7.4 r7.0 r7.6 r7.5
m2.4 r7.9 r7.10 r7.11 r7.12 r7.8 r7.14 r7.13 m2.0 m2.6 m5.1 r7.17 r7.18 r7.19 r7.20 r7.16 r7.22 r7.21 m2.2 r7.33
r7.34 r7.35 r7.36 r7.37 r7.32 r7.38 m2.5 r7.25 r7.26 r7.27 r7.24 r7.28 r7.30 r7.49 r7.29 r7.50 r7.51 r7.52 r7.48
r7.54 r7.53 r7.41 r7.42 r7.43 r7.44 r7.40 r7.46 r7.45 d7 m5.3 m5.6 m5.4 m5.0 m5.2 m5.5 p14.0 r6.1 r6.2 r6.3 r6.4
r6.0 r6.5 p1.0 p0.0 r6.6 r6.17 r6.18 r6.19 r6.20 r6.16 r6.9 r6.22 r6.21 r6.10 r6.12 r6.11 r6.8 r6.14 r6.13 p14.2
p14.4 p14.6 p14.8 p14.10 p14.12 p15.0 p14.14 r6.24 r6.25 r6.26 r6.27 r6.28 r6.30 r6.29 r6.33 r6.34 r6.35 r6.36
r6.32 r6.38 r6.37 r6.41 r6.42 r6.43 r6.44 r6.40 r6.46 r6.45 p15.2 p15.4 p15.6 p15.8 p15.10 d6 p15.12 p15.14 r5.1
r5.2 r5.3 r5.4 r5.0 r5.6 p12.0 r5.5 p12.2 p12.4 p12.6 r5.26 r5.25 r5.27 r5.28 r5.24 r5.30 r5.29 r5.17 r5.18
r5.19 r5.20 r5.16 r5.22 r5.21 r5.9 r5.10 r5.11 r5.12 r5.8 r5.13 r5.14 p12.8 p12.10 p13.0 p13.2 p13.4 r5.33 r5.34
r5.35 r5.36 r5.32 r5.38 r5.37 p13.6 p13.8 d5 o0.3 p12.12 p10.0 o0.2 o0.1 o0.0 o0.5 p13.10 p11.0 r4.10 r4.9 r4.11
r4.12 r4.8 r4.14 r4.13 o0.4 p10.2 p13.12 p10.4 r4.1 r4.2 r4.3 r4.4 r4.0 r4.6 r4.5 o0.6 p10.6 p10.8 p11.2 p10.10
r4.25 r4.26 r4.27 r4.28 r4.24 r4.30 r4.18 r4.19 r4.20 r4.16 r4.22 p11.4 r4.29 r4.21 r4.17 d4 p11.6 o7.2 o7.0
o7.1 o7.4 o7.3 o7.6 o7.5 p11.8 p8.0 r3.1 r3.2 r3.3 r3.4 r3.0 p8.2 r3.6 r3.5 p11.10 p8.4 p9.0 p8.6 p9.2 p8.8 r3.9
r3.11 r3.12 r3.14 r3.13 r3.10 r3.8 d3 r3.17 r3.18 r3.19 r3.20 r3.16 r3.22 r3.21 o6.4 o6.2 p9.4 o6.3 p7.0 o6.6
o6.0 o6.1 r2.9 r2.10 r2.11 r2.12 r2.8 r2.14 r2.13 p9.6 p9.8 p6.0 p6.2 p6.4 r2.2 r2.3 r2.4 r2.1 r2.0 r2.5 r2.6
o6.5 p6.6 d2 p7.2 p4.0 o5.2 o5.3 o5.1 o5.4 o5.6 o5.5 o5.0 r1.1 r1.2 r1.3 r1.6 r1.4 r1.0 r1.5 p4.2 p5.0 p7.4 p7.6
p4.4 d1 p5.2 o4.4 o4.2 p2.0 o4.0 o4.1 o4.3 p3.0 o4.6 o4.5 p2.2 p5.4 o2.1 p3.2 S2 o3.3 o2.0 o3.1 o3.2 o2.6 o2.3
o2.4 o2.2 o2.5 o3.5 o3.0 o3.6 o3.4 S3
"""


def _head_program():
    return [(t[0],) + tuple(int(v) for v in t[1:].split('.')) for t in _HEAD_ORDER.split()]


_P0_ORDER = """
61 r0 r1 70 r4 r3 60 r2 71 62 r5 63 r7 72 r6 73 r8 80 r9 90 93 r11 81 r14 r12 91 r13 83 r15 82 r10 92 a1 a0 b0
f3 c3 d2 d3 f0 e0 e1 b2 c0 c1 b1 a3 a2 b3 e2 c2 f2 f1 e3 d1 d0
"""
_Q7_ORDER = """
010 023 021 027 016 022 026 025 030 012 014 015 011 017 045 044 047 020 031 032 033 034 013 024 046 043 036 035
041 042 000 037 040 001 005 004 003 006 002 007 060 061 066 067 062 063 064 065 051 053 052 050 056 054 055 057
"""
_Q_ORDER = """
016 011 015 012 014 017 013 010 041 027 031 022 026 024 034 007 040 021 001 036 025 046 033 047 035 042 005 023
006 032 043 020 037 004 044 030 000 045 002 003 050 061 054 053 064 067 051 060 052 066 062 063 065 116 112 111
113 117 124 125 121 123 126 120 057 127 122 133 130 131 144 132 056 114 140 137 143 110 055 100 146 115 145 141
107 160 134 136 147 135 161 142 101 102 162 106 104 103 154 105 163 165 167 152 150 157 155 166 151 156 153 164
"""


def _dot(a, b):
    return jnp.dot(a, b, preferred_element_type=f32)


def _dot_nt(a, b):
    return lax.dot_general(a, b, NT, preferred_element_type=f32)


def _unpack(w32, sh):
    return pltpu.bitcast((w32 << sh) & jnp.uint32(HI), f32)


class _Bf16:
    def __init__(self, raw):
        self.raw = raw

    def _half(self, idx):
        idx = list(idx if isinstance(idx, tuple) else (idx,))
        idx += [slice(None)] * (len(self.raw.shape) - len(idx))
        r = idx[-2]
        if isinstance(r, slice):
            idx[-2] = slice(None if r.start is None else r.start // 2, None if r.stop is None else r.stop // 2)
        elif isinstance(r.start, int):
            idx[-2] = pl.ds(r.start // 2, r.size // 2)
        else:
            idx[-2] = pl.ds(pl.multiple_of(r.start >> 1, 8), r.size // 2)
        return tuple(idx)

    def __getitem__(self, idx):
        return pltpu.bitcast(self.raw[self._half(idx)], bf)

    def put(self, idx, v):
        idx = self._half(idx)
        ref = self.raw.at[idx[:-2]] if len(idx) > 2 else self.raw
        o = pltpu.bitcast(v, u32)
        ref[idx[-2], idx[-1]] = o
        return o

    def __setitem__(self, idx, v):
        self.put(idx, v)


def _kernel(xt_hbm, c_hbm, wq_hbm, wk_hbm, wv_hbm, wo_hbm, wr_hbm, wg_hbm, wu_hbm, wd_hbm, gw_hbm, o_hbm,
            xt_s, x_s, xa_r, c_r, ca_r, wq_p, wkv_p, wo_r, q_r, qa_r, acc_s, wg_r, wu_r, wd_r,
            wr_s, gw_s, out_s, g_s, xs_r, rsel_s, idx_s, s_s, t0_r, om_s, fw_s, sem):
    xa_s, c_s, ca_s, wo_s, q_s, qa_s, wg_s, wu_s, wd_s, xs_s, t0_s = [
        _Bf16(r) for r in (xa_r, c_r, ca_r, wo_r, q_r, qa_r, wg_r, wu_r, wd_r, xs_r, t0_r)]
    mk = pltpu.make_async_copy
    wq32, wk32, wv32 = wq_hbm.bitcast(u32), wk_hbm.bitcast(u32), wv_hbm.bitcast(u32)
    cp_wq = lambda j: mk(wq32.at[:, j, :], wq_p.at[j], sem.at[SEM_WQ + j])
    cp_kv = lambda j, m: mk((wk32, wv32)[m].at[:, j, :], wkv_p.at[j & 1, m], sem.at[SEM_KV + m])
    cp_xt = lambda k: mk(xt_hbm.at[:, pl.ds(k * XC, XC)], xt_s.at[:, pl.ds(k * XC, XC)], sem.at[SEM_XT + k])
    cp_out = lambda i: mk(out_s.at[i], o_hbm.at[:, pl.ds(i * T, T)], sem.at[SEM_OUT + i])
    cp_vec = [mk(wr_hbm, wr_s, sem.at[SEM_VEC]), mk(gw_hbm, gw_s, sem.at[SEM_VEC + 1])]
    cp_ffn = [mk(src, dst, sem.at[SEM_FFN + n]) for n, (src, dst) in
              enumerate(((wg_hbm.bitcast(u32), wg_r), (wu_hbm.bitcast(u32), wu_r), (wd_hbm.bitcast(u32), wd_r)))]
    cp_wo = mk(wo_hbm.bitcast(u32), wo_r, sem.at[SEM_WO])
    c32 = c_hbm.bitcast(u32)

    def cp_c(j):
        r0 = (j - 1) * (NG * RB // 2)
        n = QS // 2 - r0 if isinstance(j, int) and j == NP - 1 else NG * RB // 2
        return [mk(c32.at[pl.ds(i * QS // 2 + r0, n)], c_r.at[pl.ds(i * QS // 2 + r0, n)], sem.at[SEM_C + j])
                for i in range(4)]

    cp_xt(0).start()
    cp_wq(0).start()
    for k in range(1, S // XC):
        cp_xt(k).start()
    for cp in cp_vec:
        cp.start()
    for j in range(1, NP):
        cp_wq(j).start()
        for cp in cp_c(j):
            cp.start()
    for cp in cp_ffn + [cp_kv(0, 0), cp_kv(0, 1), cp_wo]:
        cp.start()

    @pl.loop(0, NQ // 2)
    def _(n):
        om_s[n] = jnp.zeros(om_s.shape[1:], f32)

    def store_q(j, e, r0, q):
        q = q * QSCALE
        q_s[2 * j + e, r0:r0 + q.shape[0], :] = q.astype(bf)
        for p0 in range(0, q.shape[0], 2 * T):
            if r0 + p0 > 0:
                qa, qb = q[p0:p0 + T], q[p0 + T:p0 + 2 * T]
                terms = _lhs_terms(qa[:, :T], qa[:, T:], qb[:, :T], qb[:, T:])
                for k, i in enumerate((0, 1, 4, 5, 6)):
                    qa_s[2 * j + e, (r0 + p0) // 2:(r0 + p0) // 2 + T, k * T:(k + 1) * T] = terms[i].astype(bf)

    def q_dot(w, r0, r1, z=None):
        return _dot(_feed(x_s[0, r0:r1, :], z), w[:HM]) + _dot(x_s[1, r0:r1, :], w[HM:])

    def q_plain(w, r0):
        qf = q_dot(w, r0, r0 + 2 * T)
        store_q(0, 0, r0, qf[:, :D])
        store_q(0, 1, r0, qf[:, D:])

    def q_rhs(j):
        lo, hi = pltpu.bitcast(wq_p[j] << 16, f32), pltpu.bitcast(wq_p[j] & jnp.uint32(HI), f32)
        b = [jnp.concatenate([lo[:, t * T:(t + 1) * T], hi[:, t * T:(t + 1) * T]], axis=1) for t in range(2)]
        return [t.astype(bf) for t in _rhs_terms(b[0][:HM], b[1][:HM], b[0][HM:], b[1][HM:])]

    def q_strassen(js, order, hook):
        ts, res = [q_rhs(j) for j in js], {}
        for a, k, u in [map(int, t) for t in order.split()]:
            if k in (2, 3):
                lhs = x_s[k - 2, (k - 2) * HS + u * T:(k - 2) * HS + (u + 1) * T, :]
            else:
                lhs = xa_s[k - 2 * (k > 3), u * T:(u + 1) * T, :]
            res[a, k, u] = _dot(_feed(lhs, *hook()), ts[a][k])
            v = u // 2 * 2
            if all((a, kk, uu) in res for kk in range(7) for uu in (v, v + 1)):
                cs = _strassen(lambda i: jnp.concatenate([res.pop((a, i, v)), res.pop((a, i, v + 1))], axis=0))
                for w in range(2):
                    for e in range(2):
                        q = jnp.concatenate([c[:, e * T:(e + 1) * T] for c in cs[2 * w:2 * w + 2]], axis=1)
                        store_q(js[a], e, w * HS + v * T, q)

    def x_prep(r0):
        a = [x_s[e, h0 + r0:h0 + r0 + RB, :].astype(f32) for h0 in (0, HS) for e in (0, 1)]
        terms = _lhs_terms(*a)
        outs = []
        for k, i in enumerate((0, 1, 4, 5, 6)):
            outs.append(xa_s.put((k, slice(r0, r0 + RB)), terms[i].astype(bf)))
        return outs

    def c_prep(g, c0):
        blk = lambda i, k: c_s[pl.ds(i * QS + g * RB, RB), k * QC + c0:k * QC + c0 + T].astype(f32)
        outer = [_lhs_terms2(*[blk(2 * i1 + i2, 2 * k1 + k2) for i1 in range(2) for k1 in range(2)])
                 for i2 in range(2) for k2 in range(2)]
        outs = []
        for r1 in range(7):
            for r2, v in enumerate(_lhs_terms(*[o[r1] for o in outer])):
                outs.append(ca_s.put((7 * r1 + r2, pl.ds(g * RB, RB), slice(c0, c0 + T)), v.astype(bf)))
        return outs

    def c_pacer(g0, ng, first, last):
        return _Pacer([functools.partial(c_prep, g0 + t // 2, (t % 2) * T) for t in range(2 * ng)], 49, first, last)

    def transpose(k):
        for e in range(2):
            x_s[e, k * XC:(k + 1) * XC, :] = xt_s[e * HM:(e + 1) * HM, k * XC:(k + 1) * XC].T

    def q_w0():
        return jnp.concatenate([pltpu.bitcast(wq_p[0] << 16, f32).astype(bf),
                                pltpu.bitcast(wq_p[0] & jnp.uint32(HI), f32).astype(bf)], axis=1)

    cp_xt(0).wait()
    transpose(0)
    cp_wq(0).wait()
    q_plain(q_w0(), 0)
    for k in range(1, 4):
        cp_xt(k).wait()
    transpose(1)
    w0 = q_w0()
    transpose(2)
    q_plain(w0, XC)
    transpose(3)
    q_plain(w0, 2 * XC)
    for k in range(4, S // XC):
        cp_xt(k).wait()
    for cp in cp_vec:
        cp.wait()
    for k in range(4, S // XC):
        transpose(k)
    row8 = lax.broadcasted_iota(jnp.int32, (8, M), 0)
    x_pace = _Pacer([functools.partial(x_prep, r0) for r0 in range(0, HS, RB)], 5, 12, 40)
    w0, res = q_w0(), {}
    for t in _P0_ORDER.split():
        if t[0] == 'r':
            n = int(t[1:])
            rg = jnp.where(row8 == 0, wr_s[...].reshape(1, M).astype(f32), gw_s[...].reshape(1, M).astype(f32))
            g_s[n] = _dot(rg.astype(bf), xt_s[:, n * T:(n + 1) * T])
            continue
        u, n = int(t[:-1], 16), int(t[-1])
        res[u, n] = q_dot(w0[:, n * T:(n + 1) * T], u * T, (u + 1) * T, x_pace())
        v = u // 2 * 2
        if all((uu, nn) in res for uu in (v, v + 1) for nn in range(4)):
            for e in range(2):
                store_q(0, e, v * T, jnp.concatenate([jnp.concatenate(
                    [res.pop((uu, nn)) for nn in (2 * e, 2 * e + 1)], axis=1) for uu in (v, v + 1)], axis=0))
    assert x_pace.finished()

    rb = jnp.concatenate([g_s[n][0:1, :] for n in range(NQ)], axis=1).astype(bf).astype(f32)
    lane = lax.broadcasted_iota(jnp.int32, (1, S), 1)
    m1 = jnp.max(rb, axis=1, keepdims=True)
    i1 = jnp.minimum(jnp.min(jnp.where(rb == m1, lane, S)), S - 1)
    rb2 = jnp.where(lane == i1, -jnp.inf, rb)
    m2 = jnp.max(rb2, axis=1, keepdims=True)
    i2 = jnp.minimum(jnp.min(jnp.where(jnp.logical_and(rb2 == m2, lane != i1), lane, S)), S - 1)
    row16 = lax.broadcasted_iota(jnp.int32, (16, HM), 0)

    def x_row(e, i):
        blk = x_s[e, pl.ds(pl.multiple_of((i // 16) * 16, 16), 16), :].astype(f32)
        return jnp.sum(jnp.where(row16 == i % 16, blk, 0.0), axis=0, keepdims=True)
    for e in range(2):
        xs_s[e] = jnp.where(row16 == 0, x_row(e, i1), jnp.where(row16 == 1, x_row(e, i2), 0.0)).astype(bf)
    rsel_s[...] = jax.nn.sigmoid(jnp.where(lax.broadcasted_iota(jnp.int32, (16, T), 0) == 0, m1, m2))
    idx_s[0] = i1
    idx_s[1] = i2

    def q_body(it, carry):
        js = (2 * it + 1, 2 * it + 2)
        for j in js:
            for cp in [cp_wq(j)] + cp_c(j):
                cp.wait()
        pace = c_pacer(2 * it * NG, 2 * NG, 1, 108)
        q_strassen(js, _Q_ORDER, lambda: (pace(),))
        assert pace.finished()
        return carry
    lax.fori_loop(0, 3, q_body, 0)

    for cp in cp_ffn + [cp_wq(NP - 1), cp_kv(0, 0), cp_kv(0, 1)] + cp_c(NP - 1):
        cp.wait()

    def w_sum(hn, m, r0):
        w = [wkv_p[(hn >> 1) & 1, m, r:r + 8, :] for r in range(r0, r0 + HC, 64)]
        w = (jnp.concatenate(w, axis=0) << (16 * (1 - (hn & 1))).astype(u32)) & jnp.uint32(0x7FFF0000)
        return functools.reduce(jnp.add, [pltpu.bitcast(t, f32) for t in _vregs([w])])

    def w_balance(parts):
        n = len(parts) // 2
        sk, sv = [jnp.sum(functools.reduce(jnp.add, p), keepdims=True) for p in (parts[:n], parts[n:])]
        ok = jnp.logical_and(sk > 0, sv > 0)
        ratio = jnp.broadcast_to(jnp.where(ok, 1.4 * sk, 1.0) / jnp.where(ok, sv, 1.0), (8, T))
        e = jnp.clip(pltpu.bitcast(ratio, jnp.int32) & 0x7F800000, (127 - 40) << 23, (127 + 40) << 23)
        fw_s[0] = pltpu.bitcast(e, f32)
        fw_s[1] = pltpu.bitcast((254 << 23) - e, f32)
        return [e]

    def w_pacer(hn, first, last):
        parts = []
        return _Pacer([lambda m=m, r0=r0: parts.append(w_sum(hn, m, r0)) or parts[-1:]
                       for m in range(2) for r0 in (0, HC)] + [lambda: w_balance(parts)], 1, first, last)

    def first_terms(hn):
        w = _unpack(wkv_p[(hn >> 1) & 1, 0, :, :T], (16 * (1 - (hn & 1))).astype(u32))
        t = w[:HC] + 0.5 * w[HC:]
        return [t0_s.put((slice(r, r + RB), slice(n * T, (n + 1) * T)), v[r:r + RB].astype(bf))
                for n, v in enumerate((t[:QC], t[QC:] - t[:QC])) for r in range(0, QC, RB)]

    def residual(n):
        g8 = jax.nn.sigmoid(g_s[n])
        g_s[n] = g8
        a = (1.0 - g8[1:2, :]) * xt_s[:, n * T:(n + 1) * T].astype(f32)
        acc_s[n] = a
        return [a]

    gs, us, ys, hid = [], [], {}, []
    xs_dot = lambda w_s, n: (_dot(xs_s[0], w_s[:HM, n * T:(n + 1) * T]) + _dot(xs_s[1], w_s[HM:, n * T:(n + 1) * T]))

    def swiglu():
        gg, uu = jnp.concatenate(gs, axis=1), jnp.concatenate(us, axis=1)
        hid.append((gg * jax.nn.sigmoid(gg) * uu).astype(bf))

    def down(n0, k0):
        t = _dot_nt(hid[0][:, k0:min(k0 + 512, F)], wd_s[n0:min(n0 + T, M), k0:min(k0 + 512, F)])
        ys[n0] = ys[n0] + t if n0 in ys else t
    side = []
    for n in range(F // T):
        side += [lambda n=n: gs.append(xs_dot(wg_s, n)), lambda n=n: us.append(xs_dot(wu_s, n))]
    side += [swiglu] + [lambda: None] * 7
    side += [functools.partial(down, n0, k0) for n0 in range(0, M, T) for k0 in range(0, F, 512)]
    c_pace = c_pacer((NP - 2) * NG, QS // RB - (NP - 2) * NG, 2, 55)
    r_pace = _Pacer([functools.partial(residual, n) for n in range(NQ)], M // 8, 2, 47)

    w_pace0 = w_pacer(jnp.int32(0), 3, 52)
    t_pace0 = _Pacer([lambda: first_terms(jnp.int32(0))], 32, 37, 56)

    def hook7():
        if side:
            side.pop(0)()
        return c_pace(), r_pace(), w_pace0(), t_pace0()
    q_strassen([NP - 1], _Q7_ORDER, hook7)
    assert not side and all(p.finished() for p in (c_pace, r_pace, w_pace0, t_pace0))
    y = jnp.concatenate([ys[n0] for n0 in range(0, M, T)] + [jnp.zeros((16, 512 - M), f32)], axis=1)
    yt = (y * rsel_s[:, 0:1]).T
    lane128 = lax.broadcasted_iota(jnp.int32, (1, T), 1)
    for e in range(2):
        i = idx_s[e]
        acc_s[i // T] += jnp.where(lane128 == i % T, (1.0 - g_s[i // T][1:2, :]) * yt[:M, e:e + 1], 0.0)

    for m in range(2):
        cp_kv(1, m).start()
    cp_wo.wait()

    tri = lax.broadcasted_iota(jnp.int32, (T, T), 1) <= lax.broadcasted_iota(jnp.int32, (T, T), 0)
    prog = _head_program()

    def head(h, carry):
        par, slot = h & 1, (h >> 1) & 1

        @pl.when(jnp.logical_and(h < H - 1, par == 1))
        def _():
            for m in range(2):
                cp_kv((h + 1) >> 1, m).wait()

        sh = (16 * (1 - par)).astype(u32)
        rhs, fw, fw_inv = [], fw_s[0], fw_s[1]
        for r1 in range(7):
            wk, wv = [_unpack(wkv_p[slot, m], sh + (h >> (8 + r1)).astype(u32)) for m in range(2)]
            wv = jnp.concatenate([wv[:, :T] * fw[0:1], wv[:, T:] * fw[0:1]], axis=1)
            t = _rhs_terms2(wk[:HC], wv[:HC], wk[HC:], wv[HC:])[r1]
            rhs.append([u.astype(bf) for u in _rhs_terms(t[:QC, :T], t[:QC, T:], t[QC:, :T], t[QC:, T:])])
        rhs[1][1], rhs[1][3] = t0_s[:, :T], t0_s[:, T:]
        hn = jnp.minimum(h + 1, H - 1)
        t_pace = _Pacer([lambda: first_terms(hn)], 32, 196 - 14, 196)
        w_pace = w_pacer(hn, 60, 180)
        prods, inner_q, outer, kblk, vblk = {}, {}, {}, {}, {}

        def kv_product(r1, r2):
            m = prods.setdefault(r1, {})
            m[r2] = _dot(ca_s[7 * r1 + r2], rhs[r1][r2])
            if len(m) == 7:
                inner_q[r1] = (((m[3] - m[4]) + m[6]) + m[0], m[2] + m[4], m[1] + m[3], ((m[0] - m[1]) + m[2]) + m[5])
                for b in range(4):
                    if b not in kblk and all(q in inner_q for q in (0, 1, 3, 4, 6)):
                        p = {q: inner_q[q][b] for q in (0, 1, 3, 4, 6)}
                        e, d = p[3] + p[1], p[3] - p[1]
                        kblk[b] = (p[0] + ((d - p[4]) + p[6]), e * 2.0)
                        outer[b] = ((e + p[4]) + p[6], p[0] + d)
                    if len(inner_q) == 7:
                        p2, p5 = inner_q[2][b], inner_q[5][b]
                        vblk[b] = (((outer[b][0] + p2) - p5) * 0.5, (outer[b][1] + p2) + p5)

        def rows(blk, t0, t1):
            return jnp.concatenate([jnp.concatenate(
                [blk[2 * (t // 4 % 2) + j2][t // 8][t % 4 * T:(t % 4 + 1) * T] for j2 in range(2)], axis=1)
                for t in range(t0, t1)], axis=0)

        @functools.cache
        def k_tile(t):
            return rows(kblk, t, t + 1).astype(bf)

        @functools.cache
        def k_terms(J):
            ka, kb = rows(kblk, 2 * J, 2 * J + 1), rows(kblk, 2 * J + 1, 2 * J + 2)
            return [t.astype(bf) for t in _rhs_terms(ka[:, :T], kb[:, :T], ka[:, T:], kb[:, T:])]

        @functools.cache
        def v_tiles(c0, c1):
            return rows(vblk, c0, c1).astype(bf)

        s_prod, scores, rmax, soft, o_sum = {}, {}, {}, {}, {}
        q_tiles = lambda I: [q_s[h, i * T:(i + 1) * T, t * T:(t + 1) * T] for i in (2 * I, 2 * I + 1) for t in range(2)]

        def score_product(I, code):
            J, k = code // 8, code % 8
            if k in (2, 3):
                lhs = q_tiles(I)[3 * (k - 2)]
            else:
                lhs = qa_s[h, I * T:(I + 1) * T, (k - 2 * (k > 3)) * T:(k - 2 * (k > 3) + 1) * T]
            s_prod[I, J, k] = _dot_nt(_feed(lhs, t_pace(), w_pace()), k_terms(J)[k])
            if not all((I, J, q) in s_prod for q in range(7)):
                return
            for n, c in enumerate(_strassen(lambda q: s_prod.pop((I, J, q)))):
                s_s[I % 2, n // 2, 2 * J + n % 2] = c
            for u in range(2):
                sa, sb = s_s[I % 2, u, 2 * J], s_s[I % 2, u, 2 * J + 1]
                scores[2 * I + u, 2 * J] = s_s[I % 2, u, 2 * J]
                scores[2 * I + u, 2 * J + 1] = s_s[I % 2, u, 2 * J + 1]
                mx = jnp.maximum(sa, sb)
                rmax[2 * I + u] = jnp.maximum(rmax[2 * I + u], mx) if 2 * I + u in rmax else mx

        def score_diag(I):
            a, b = 2 * I, 2 * I + 1
            q4 = q_tiles(I)
            qa, qb = jnp.concatenate(q4[0:2], axis=1), jnp.concatenate(q4[2:4], axis=1)
            d1 = _dot_nt(jnp.concatenate([qa, qb], axis=0), k_tile(a))
            d2 = _dot_nt(qb, k_tile(b))
            scores[a, a], scores[b, a], scores[b, b] = jnp.where(tri, d1[:T], NEG), d1[T:], jnp.where(tri, d2, NEG)

        def pv_chunk(i, c0):
            if c0 == 0:
                mx = functools.reduce(jnp.maximum, ([rmax[i]] if i > 1 else [])
                                      + [scores[i, t] for t in range(i // 2 * 2, i + 1)])
                soft[i] = dict(m=jnp.max(mx, axis=1, keepdims=True), l=None, ctx=None)
            st = soft[i]
            c1 = min(c0 + 2, i + 1)
            p = jnp.exp2(jnp.concatenate([scores.pop((i, t)) for t in range(c0, c1)], axis=1) - st['m']).astype(bf)
            pf = p.astype(f32)
            for t in range(c1 - c0):
                st['l'] = pf[:, t * T:(t + 1) * T] if st['l'] is None else st['l'] + pf[:, t * T:(t + 1) * T]
            d = _dot(p, v_tiles(c0, c1))
            st['ctx'] = d if st['ctx'] is None else st['ctx'] + d

        def context(i):
            st = soft.pop(i)
            l = jnp.sum(st['l'], axis=1, keepdims=True)
            r = pl.reciprocal(l, approx=True)
            return st['ctx'] * (r * (2.0 - l * r) * fw_inv[0:1, 0:1])

        def ship(blocks):
            @pl.when(h == H - 1)
            def _():
                for i in blocks:
                    cp_out(i).start()

        def out_plain(i):
            wo, ctx = wo_s[h], context(i).astype(bf)
            for a0 in (0, HM):
                a = acc_s[i, a0:a0 + HM, :] + g_s[i][1:2, :] * _dot_nt(wo[a0:a0 + HM], ctx)
                acc_s[i, a0:a0 + HM, :] = a
                out_s[i, a0:a0 + HM, :] = a.astype(bf)
            ship([i])

        @functools.cache
        def wo_terms():
            w = wo_s[h].astype(f32)
            return [t.astype(bf) for t in _lhs_terms(w[:HM, :T], w[:HM, T:], w[HM:, :T], w[HM:, T:])]

        @functools.cache
        def ctx_terms(I):
            ca, cb = context(2 * I), context(2 * I + 1)
            return _rhs_terms(ca[:, :T], cb[:, :T], ca[:, T:], cb[:, T:])

        def out_product(I, k):
            om_s[I, k] += _dot_nt(wo_terms()[k], ctx_terms(I)[k].astype(bf))
            o_sum[I, k] = om_s[I, k]
            if all((I, q) in o_sum for q in range(7)):
                for n, c in enumerate(_strassen(lambda q: o_sum.pop((I, q)))):
                    i, a0 = 2 * I + n % 2, (n // 2) * HM
                    out_s[i, a0:a0 + HM, :] = (acc_s[i, a0:a0 + HM, :] + g_s[i][1:2, :] * c).astype(bf)
                ship([2 * I, 2 * I + 1])

        ops = {'m': kv_product, 'r': score_product, 'd': score_diag, 'p': pv_chunk,
               'o': out_product, 'S': out_plain}
        for op, *args in prog:
            ops[op](*args)
        assert t_pace.finished() and w_pace.finished()

        @pl.when(jnp.logical_and((h + 3) >> 1 < NP, par == 1))
        def _():
            for m in range(2):
                cp_kv((h + 3) >> 1, m).start()
        return carry

    lax.fori_loop(0, H, head, 0)
    for i in range(NQ):
        cp_out(i).wait()


@jax.jit
def pallas_gated_mix__compressed_kv_cla__moe_arch_mod__prompt_kernel(
    A_x: jax.Array,
    A_c_kv: jax.Array,
    A_w_q: jax.Array,
    A_w_uk: jax.Array,
    A_w_uv: jax.Array,
    A_w_o: jax.Array,
    B_x: jax.Array,
    B_w_r: jax.Array,
    B_w_gate: jax.Array,
    B_w_up: jax.Array,
    B_w_down: jax.Array,
    gate_w: jax.Array,
):
    del B_x
    V = pltpu.VMEM
    B = lambda *shape: V(shape[:-2] + (shape[-2] // 2, shape[-1]), u32)
    out_t = pl.pallas_call(
        _kernel,
        in_specs=[pl.BlockSpec(memory_space=pl.ANY)] * 11,
        out_specs=pl.BlockSpec(memory_space=pl.ANY),
        out_shape=jax.ShapeDtypeStruct((M, S), bf),
        scratch_shapes=[
            V((M, S), bf), V((2, S, HM), bf), B(5, HS, HM),
            B(S, DC), B(49, QS, QC),
            V((NP, M, D), u32), V((2, 2, DC, D), u32), B(H, M, D),
            B(H, S, D), B(H, HS, 5 * T),
            V((NQ, M, T), f32),
            B(M, F), B(M, F), B(M, F),
            V((M,), bf), V((M,), bf), V((NQ, M, T), bf),
            V((NQ, 8, T), f32), B(2, 16, HM), V((16, T), f32),
            pltpu.SMEM((2,), jnp.int32),
            V((2, 2, NQ, T, T), f32), B(QC, 2 * T),
            V((NQ // 2, 7, HM, T), f32),
            V((2, 8, T), f32),
            pltpu.SemaphoreType.DMA((NSEM,)),
        ],
        compiler_params=pltpu.CompilerParams(vmem_limit_bytes=110 * 1024 * 1024),
        name="gated_mix_cla_mod",
    )(A_x[0].T, A_c_kv[0], A_w_q, A_w_uk, A_w_uv, A_w_o.transpose(0, 2, 1), B_w_r, B_w_gate, B_w_up,
      B_w_down.T, gate_w)
    return out_t.T[None]
```

```python
import functools
import math

import jax
import jax.numpy as jnp
from jax import lax
from jax.experimental import pallas as pl
from jax.experimental.pallas import tpu as pltpu

S, M, H, D, DC, F = 2048, 448, 16, 256, 1024, 1792
T = 128
NP, NQ = H // 2, S // T
HS, HM, HC = S // 2, M // 2, DC // 2
QS, QC = S // 4, DC // 4
RB = 16
XC = 256
NG = 5
NT = (((1,), (1,)), ((), ()))
QSCALE = D ** -0.5 * math.log2(math.e)
NEG = -1e30
bf, f32, u32 = jnp.bfloat16, jnp.float32, jnp.uint32
HI = 0xFFFF0000

SEM_WO, SEM_FFN, SEM_VEC, SEM_KV, SEM_WQ, SEM_XT, SEM_C, SEM_OUT, NSEM = 0, 1, 4, 6, 8, 16, 24, 32, 48


def _lhs_terms(a11, a12, a21, a22):
    return [a11 + a22, a21 + a22, a11, a22, a11 + a12, a21 - a11, a12 - a22]


def _rhs_terms(b11, b12, b21, b22):
    return [b11 + b22, b11, b12 - b22, b21 - b11, b22, b11 + b12, b21 + b22]


def _strassen(mm):
    m2, m3, m4, m5, m1, m7, m6 = [mm(i) for i in (1, 2, 3, 4, 0, 6, 5)]
    return (m4 - m5) + (m1 + m7), m3 + m5, m2 + m4, (m3 - m2) + (m1 + m6)


def _lhs_terms2(a11, a12, a21, a22):
    h21, q21, h22 = 0.5 * a21, 0.25 * a21, 0.5 * a22
    s1 = a11 + a22
    v, hs = a12 + q21, 0.5 * s1
    return [s1, q21 + h22, a11 + h21, h22 - q21, v + hs, h21 - a11, v - hs]


def _rhs_terms2(b11, b12, b21, b22):
    h21 = 0.5 * b21
    t1 = b11 + b22
    v, ht = b12 + 0.5 * h21, 0.5 * t1
    return [t1, b11 + h21, v - ht, h21 - b11, b22 - h21, v + ht, b22 + h21]


def _vregs(vals):
    ts = []
    for v in vals:
        v = v if v.dtype == u32 else pltpu.bitcast(v, u32)
        ts += [v[r:r + 8, c:c + T] for r in range(0, v.shape[0], 8) for c in range(0, v.shape[1] - T + 1, T)]
    return ts


def _zero_from(ts):
    acc = ts[:4]
    for i, t in enumerate(ts[4:]):
        acc[i % 4] = acc[i % 4] | t
    while len(acc) > 1:
        acc = [acc[i] | acc[i + 1] if i + 1 < len(acc) else acc[i] for i in range(0, len(acc), 2)]
    return (acc[0] >> 16) >> 16


def _feed(a, *zs):
    zs = [z for z in zs if z is not None]
    if not zs:
        return a
    a32 = pltpu.bitcast(a, u32)
    top = functools.reduce(lambda p, q: p | q, zs, a32[0:8, :T])
    if a32.shape[1] > T:
        top = jnp.concatenate([top, a32[0:8, T:]], axis=1)
    return pltpu.bitcast(jnp.concatenate([top, a32[8:]], axis=0), bf)


class _Pacer:
    def __init__(self, thunks, per, first, last):
        self.thunks, self.pool, self.k, self.done = list(thunks), [], 0, 0
        self.tot, self.first, self.last = per * len(self.thunks), first, last

    def __call__(self):
        self.k += 1
        if self.k <= self.first:
            return None
        want = min(self.tot, -(-(self.k - self.first) * self.tot // (self.last - self.first))) - self.done
        while len(self.pool) < want and self.thunks:
            self.pool += _vregs(self.thunks.pop(0)())
        outs, self.pool = self.pool[:want], self.pool[want:]
        self.done += len(outs)
        return _zero_from(outs) if outs else None

    def finished(self):
        return not self.thunks and not self.pool


_HEAD_ORDER = """
m1.1 m1.3 m1.4 m1.6 m1.0 m3.4 m1.2 m3.3 m4.3 m3.6 m3.0 m3.1 m4.4 m3.2 m3.5 m1.5 m4.6 m4.1 m4.0 m6.6 m6.3 m6.0
m0.1 m4.5 m6.4 m6.1 m6.5 m6.2 m4.2 m0.6 m0.4 m0.3 m0.0 m0.2 m0.5 m2.1 d0 m2.3 r7.1 r7.2 r7.3 r7.4 r7.0 r7.6 r7.5
m2.4 r7.9 r7.10 r7.11 r7.12 r7.8 r7.14 r7.13 m2.0 m2.6 m5.1 r7.17 r7.18 r7.19 r7.20 r7.16 r7.22 r7.21 m2.2 r7.33
r7.34 r7.35 r7.36 r7.37 r7.32 r7.38 m2.5 r7.25 r7.26 r7.27 r7.24 r7.28 r7.30 r7.49 r7.29 r7.50 r7.51 r7.52 r7.48
r7.54 r7.53 r7.41 r7.42 r7.43 r7.44 r7.40 r7.46 r7.45 d7 m5.3 m5.6 m5.4 m5.0 m5.2 m5.5 p14.0 r6.1 r6.2 r6.3 r6.4
r6.0 r6.5 p1.0 p0.0 r6.6 r6.17 r6.18 r6.20 r6.19 r6.16 r6.9 r6.22 r6.21 r6.10 r6.12 r6.11 r6.8 r6.14 r6.13 p14.2
p14.4 p14.6 p14.8 p14.10 p14.12 p14.14 r6.24 r6.25 r6.26 p15.0 r6.27 r6.28 r6.30 r6.29 r6.33 r6.34 r6.35 r6.36
r6.32 r6.38 r6.37 r6.41 r6.42 r6.43 r6.44 r6.40 r6.46 r6.45 p15.2 p15.4 p15.6 p15.8 p15.10 d6 p15.12 p15.14 r5.1
r5.2 r5.3 r5.4 r5.0 r5.5 r5.6 p12.0 p12.2 p12.4 p12.6 r5.26 r5.25 r5.27 r5.28 r5.16 r5.22 r5.21 r5.24 r5.30
r5.17 r5.29 r5.18 r5.19 r5.20 r5.9 r5.13 r5.10 r5.11 r5.12 p13.0 r5.8 r5.14 p12.8 p12.10 p13.2 p13.4 r5.33 r5.34
r5.36 r5.32 r5.38 r5.37 r5.35 p13.6 p13.8 d5 o0.3 p12.12 p10.0 o0.2 o0.1 p11.0 o0.0 o0.5 p13.10 r4.10 r4.9 r4.11
r4.12 r4.8 r4.14 r4.13 o0.4 p10.2 p13.12 p10.4 r4.1 r4.6 r4.2 r4.3 r4.4 r4.0 r4.5 o0.6 p10.6 p10.8 p11.2 p10.10
r4.24 r4.25 r4.26 r4.27 r4.28 r4.30 r4.18 r4.19 r4.20 r4.16 r4.22 p11.4 r4.29 r4.21 r4.17 d4 p11.6 o7.2 o7.0
o7.1 o7.4 o7.3 o7.6 o7.5 p11.8 p8.0 r3.1 r3.2 r3.3 r3.0 p8.2 r3.6 r3.5 r3.4 p11.10 p8.4 p9.0 p8.6 p9.2 r3.14
r3.9 p8.8 r3.11 r3.13 r3.12 r3.10 r3.8 d3 r3.17 r3.18 r3.19 r3.20 r3.22 r3.16 r3.21 o6.4 o6.2 p9.4 p7.0 o6.3
o6.6 o6.0 o6.1 r2.9 r2.10 r2.11 r2.14 r2.12 r2.8 r2.13 p9.6 p6.0 p6.2 p9.8 p6.4 r2.2 r2.3 r2.4 r2.1 r2.0 r2.5
r2.6 o6.5 p6.6 d2 p7.2 p4.0 o5.6 o5.2 o5.3 o5.1 o5.4 o5.5 o5.0 r1.2 r1.3 r1.6 r1.4 r1.1 r1.0 p4.2 p7.4 p5.0 r1.5
p7.6 p4.4 d1 p5.2 o4.2 o4.4 o4.0 o4.1 p2.0 o4.3 p3.0 o4.6 o4.5 p2.2 p5.4 o2.1 p3.2 S2 o3.3 o2.0 o3.1 o3.2 o2.5
o2.3 o2.6 o2.4 o2.2 o3.5 o3.0 o3.6 o3.4 S3
"""


def _head_program():
    return [(t[0],) + tuple(int(v) for v in t[1:].split('.')) for t in _HEAD_ORDER.split()]


_P0_ORDER = """
61 r0 r1 70 r4 r3 60 r2 71 62 r5 63 r7 72 r6 73 r8 80 r9 90 93 r11 81 r14 r12 91 r13 83 r15 82 r10 92 a1 a0 b0
f3 c3 d2 d3 f0 e0 e1 b2 c0 c1 b1 a3 a2 b3 e2 c2 f2 f1 e3 d1 d0
"""
_Q7_ORDER = """
010 023 021 027 016 022 026 025 030 012 014 015 011 017 045 044 047 020 031 032 033 034 013 024 046 043 036 035
041 042 000 037 040 001 005 004 003 006 002 007 060 061 066 067 062 063 064 065 051 053 052 050 056 054 055 057
"""
_Q_ORDER = """
017 013 016 011 014 010 015 012 041 027 031 026 022 024 034 007 040 021 042 047 001 025 036 035 033 046 005 023
006 032 043 004 044 020 037 030 000 045 054 002 003 050 061 053 066 062 063 060 067 051 064 052 065 117 112 116
113 111 124 125 126 121 123 120 057 127 122 133 130 131 144 132 056 114 140 110 137 143 055 100 146 141 115 107
160 134 136 147 145 135 161 142 101 102 162 152 163 106 150 165 103 104 167 154 105 157 153 164 155 166 151 156
"""


def _dot(a, b):
    return jnp.dot(a, b, preferred_element_type=f32)


def _dot_nt(a, b):
    return lax.dot_general(a, b, NT, preferred_element_type=f32)


def _unpack(w32, sh):
    return pltpu.bitcast((w32 << sh) & jnp.uint32(HI), f32)


class _Bf16:
    def __init__(self, raw):
        self.raw = raw

    def _half(self, idx):
        idx = list(idx if isinstance(idx, tuple) else (idx,))
        idx += [slice(None)] * (len(self.raw.shape) - len(idx))
        r = idx[-2]
        if isinstance(r, slice):
            idx[-2] = slice(None if r.start is None else r.start // 2, None if r.stop is None else r.stop // 2)
        elif isinstance(r.start, int):
            idx[-2] = pl.ds(r.start // 2, r.size // 2)
        else:
            idx[-2] = pl.ds(pl.multiple_of(r.start >> 1, 8), r.size // 2)
        return tuple(idx)

    def __getitem__(self, idx):
        return pltpu.bitcast(self.raw[self._half(idx)], bf)

    def put(self, idx, v):
        idx = self._half(idx)
        ref = self.raw.at[idx[:-2]] if len(idx) > 2 else self.raw
        o = pltpu.bitcast(v, u32)
        ref[idx[-2], idx[-1]] = o
        return o

    def __setitem__(self, idx, v):
        self.put(idx, v)


def _kernel(xt_hbm, c_hbm, wq_hbm, wk_hbm, wv_hbm, wo_hbm, wr_hbm, wg_hbm, wu_hbm, wd_hbm, gw_hbm, o_hbm,
            xt_s, x_s, xa_r, c_r, ca_r, wq_p, wkv_p, wo_r, q_r, qa_r, acc_s, wg_r, wu_r, wd_r,
            wr_s, gw_s, out_s, g_s, xs_r, rsel_s, idx_s, s_s, t0_r, om_s, fw_s, sem):
    xa_s, c_s, ca_s, wo_s, q_s, qa_s, wg_s, wu_s, wd_s, xs_s, t0_s = [
        _Bf16(r) for r in (xa_r, c_r, ca_r, wo_r, q_r, qa_r, wg_r, wu_r, wd_r, xs_r, t0_r)]
    mk = pltpu.make_async_copy
    wq32, wk32, wv32 = wq_hbm.bitcast(u32), wk_hbm.bitcast(u32), wv_hbm.bitcast(u32)
    cp_wq = lambda j: mk(wq32.at[:, j, :], wq_p.at[j], sem.at[SEM_WQ + j])
    cp_kv = lambda j, m: mk((wk32, wv32)[m].at[:, j, :], wkv_p.at[j & 1, m], sem.at[SEM_KV + m])
    cp_xt = lambda k: mk(xt_hbm.at[:, pl.ds(k * XC, XC)], xt_s.at[:, pl.ds(k * XC, XC)], sem.at[SEM_XT + k])
    cp_out = lambda i: mk(out_s.at[i], o_hbm.at[:, pl.ds(i * T, T)], sem.at[SEM_OUT + i])
    cp_vec = [mk(wr_hbm, wr_s, sem.at[SEM_VEC]), mk(gw_hbm, gw_s, sem.at[SEM_VEC + 1])]
    cp_ffn = [mk(src, dst, sem.at[SEM_FFN + n]) for n, (src, dst) in
              enumerate(((wg_hbm.bitcast(u32), wg_r), (wu_hbm.bitcast(u32), wu_r), (wd_hbm.bitcast(u32), wd_r)))]
    cp_wo = mk(wo_hbm.bitcast(u32), wo_r, sem.at[SEM_WO])
    c32 = c_hbm.bitcast(u32)

    def cp_c(j):
        r0 = (j - 1) * (NG * RB // 2)
        n = QS // 2 - r0 if isinstance(j, int) and j == NP - 1 else NG * RB // 2
        return [mk(c32.at[pl.ds(i * QS // 2 + r0, n)], c_r.at[pl.ds(i * QS // 2 + r0, n)], sem.at[SEM_C + j])
                for i in range(4)]

    cp_xt(0).start()
    cp_wq(0).start()
    for k in range(1, S // XC):
        cp_xt(k).start()
    for cp in cp_vec:
        cp.start()
    for j in range(1, NP):
        cp_wq(j).start()
        for cp in cp_c(j):
            cp.start()
    for cp in cp_ffn + [cp_kv(0, 0), cp_kv(0, 1), cp_wo]:
        cp.start()

    @pl.loop(0, NQ // 2)
    def _(n):
        om_s[n] = jnp.zeros(om_s.shape[1:], f32)

    def store_q(j, e, r0, q):
        q = q * QSCALE
        q_s[2 * j + e, r0:r0 + q.shape[0], :] = q.astype(bf)
        for p0 in range(0, q.shape[0], 2 * T):
            if r0 + p0 > 0:
                qa, qb = q[p0:p0 + T], q[p0 + T:p0 + 2 * T]
                terms = _lhs_terms(qa[:, :T], qa[:, T:], qb[:, :T], qb[:, T:])
                for k, i in enumerate((0, 1, 4, 5, 6)):
                    qa_s[2 * j + e, (r0 + p0) // 2:(r0 + p0) // 2 + T, k * T:(k + 1) * T] = terms[i].astype(bf)

    def q_dot(w, r0, r1, z=None):
        return _dot(_feed(x_s[0, r0:r1, :], z), w[:HM]) + _dot(x_s[1, r0:r1, :], w[HM:])

    def q_plain(w, r0):
        qf = q_dot(w, r0, r0 + 2 * T)
        store_q(0, 0, r0, qf[:, :D])
        store_q(0, 1, r0, qf[:, D:])

    def q_rhs(j):
        lo, hi = pltpu.bitcast(wq_p[j] << 16, f32), pltpu.bitcast(wq_p[j] & jnp.uint32(HI), f32)
        b = [jnp.concatenate([lo[:, t * T:(t + 1) * T], hi[:, t * T:(t + 1) * T]], axis=1) for t in range(2)]
        return [t.astype(bf) for t in _rhs_terms(b[0][:HM], b[1][:HM], b[0][HM:], b[1][HM:])]

    def q_strassen(js, order, hook):
        ts, res = [q_rhs(j) for j in js], {}
        for a, k, u in [map(int, t) for t in order.split()]:
            if k in (2, 3):
                lhs = x_s[k - 2, (k - 2) * HS + u * T:(k - 2) * HS + (u + 1) * T, :]
            else:
                lhs = xa_s[k - 2 * (k > 3), u * T:(u + 1) * T, :]
            res[a, k, u] = _dot(_feed(lhs, *hook()), ts[a][k])
            v = u // 2 * 2
            if all((a, kk, uu) in res for kk in range(7) for uu in (v, v + 1)):
                cs = _strassen(lambda i: jnp.concatenate([res.pop((a, i, v)), res.pop((a, i, v + 1))], axis=0))
                for w in range(2):
                    for e in range(2):
                        q = jnp.concatenate([c[:, e * T:(e + 1) * T] for c in cs[2 * w:2 * w + 2]], axis=1)
                        store_q(js[a], e, w * HS + v * T, q)

    def x_prep(r0):
        a = [x_s[e, h0 + r0:h0 + r0 + RB, :].astype(f32) for h0 in (0, HS) for e in (0, 1)]
        terms = _lhs_terms(*a)
        outs = []
        for k, i in enumerate((0, 1, 4, 5, 6)):
            outs.append(xa_s.put((k, slice(r0, r0 + RB)), terms[i].astype(bf)))
        return outs

    def c_prep(g, c0):
        blk = lambda i, k: c_s[pl.ds(i * QS + g * RB, RB), k * QC + c0:k * QC + c0 + T].astype(f32)
        outer = [_lhs_terms2(*[blk(2 * i1 + i2, 2 * k1 + k2) for i1 in range(2) for k1 in range(2)])
                 for i2 in range(2) for k2 in range(2)]
        outs = []
        for r1 in range(7):
            for r2, v in enumerate(_lhs_terms(*[o[r1] for o in outer])):
                outs.append(ca_s.put((7 * r1 + r2, pl.ds(g * RB, RB), slice(c0, c0 + T)), v.astype(bf)))
        return outs

    def c_pacer(g0, ng, first, last):
        return _Pacer([functools.partial(c_prep, g0 + t // 2, (t % 2) * T) for t in range(2 * ng)], 49, first, last)

    def transpose(k):
        for e in range(2):
            x_s[e, k * XC:(k + 1) * XC, :] = xt_s[e * HM:(e + 1) * HM, k * XC:(k + 1) * XC].T

    def q_w0():
        return jnp.concatenate([pltpu.bitcast(wq_p[0] << 16, f32).astype(bf),
                                pltpu.bitcast(wq_p[0] & jnp.uint32(HI), f32).astype(bf)], axis=1)

    cp_xt(0).wait()
    transpose(0)
    cp_wq(0).wait()
    q_plain(q_w0(), 0)
    for k in range(1, 4):
        cp_xt(k).wait()
    transpose(1)
    w0 = q_w0()
    transpose(2)
    q_plain(w0, XC)
    transpose(3)
    q_plain(w0, 2 * XC)
    for k in range(4, S // XC):
        cp_xt(k).wait()
    for cp in cp_vec:
        cp.wait()
    for k in range(4, S // XC):
        transpose(k)
    row8 = lax.broadcasted_iota(jnp.int32, (8, M), 0)
    x_pace = _Pacer([functools.partial(x_prep, r0) for r0 in range(0, HS, RB)], 5, 12, 40)
    w0, res = q_w0(), {}
    for t in _P0_ORDER.split():
        if t[0] == 'r':
            n = int(t[1:])
            rg = jnp.where(row8 == 0, wr_s[...].reshape(1, M).astype(f32), gw_s[...].reshape(1, M).astype(f32))
            g_s[n] = _dot(rg.astype(bf), xt_s[:, n * T:(n + 1) * T])
            continue
        u, n = int(t[:-1], 16), int(t[-1])
        res[u, n] = q_dot(w0[:, n * T:(n + 1) * T], u * T, (u + 1) * T, x_pace())
        v = u // 2 * 2
        if all((uu, nn) in res for uu in (v, v + 1) for nn in range(4)):
            for e in range(2):
                store_q(0, e, v * T, jnp.concatenate([jnp.concatenate(
                    [res.pop((uu, nn)) for nn in (2 * e, 2 * e + 1)], axis=1) for uu in (v, v + 1)], axis=0))
    assert x_pace.finished()

    rb = jnp.concatenate([g_s[n][0:1, :] for n in range(NQ)], axis=1).astype(bf).astype(f32)
    lane = lax.broadcasted_iota(jnp.int32, (1, S), 1)
    m1 = jnp.max(rb, axis=1, keepdims=True)
    i1 = jnp.minimum(jnp.min(jnp.where(rb == m1, lane, S)), S - 1)
    rb2 = jnp.where(lane == i1, -jnp.inf, rb)
    m2 = jnp.max(rb2, axis=1, keepdims=True)
    i2 = jnp.minimum(jnp.min(jnp.where(jnp.logical_and(rb2 == m2, lane != i1), lane, S)), S - 1)
    row16 = lax.broadcasted_iota(jnp.int32, (16, HM), 0)

    def x_row(e, i):
        blk = x_s[e, pl.ds(pl.multiple_of((i // 16) * 16, 16), 16), :].astype(f32)
        return jnp.sum(jnp.where(row16 == i % 16, blk, 0.0), axis=0, keepdims=True)
    for e in range(2):
        xs_s[e] = jnp.where(row16 == 0, x_row(e, i1), jnp.where(row16 == 1, x_row(e, i2), 0.0)).astype(bf)
    rsel_s[...] = jax.nn.sigmoid(jnp.where(lax.broadcasted_iota(jnp.int32, (16, T), 0) == 0, m1, m2))
    idx_s[0] = i1
    idx_s[1] = i2

    def q_body(it, carry):
        js = (2 * it + 1, 2 * it + 2)
        for j in js:
            for cp in [cp_wq(j)] + cp_c(j):
                cp.wait()
        pace = c_pacer(2 * it * NG, 2 * NG, 1, 108)
        q_strassen(js, _Q_ORDER, lambda: (pace(),))
        assert pace.finished()
        return carry
    lax.fori_loop(0, 3, q_body, 0)

    for cp in cp_ffn + [cp_wq(NP - 1), cp_kv(0, 0), cp_kv(0, 1)] + cp_c(NP - 1):
        cp.wait()

    def w_sum(hn, m, r0):
        w = [wkv_p[(hn >> 1) & 1, m, r:r + 8, :] for r in range(r0, r0 + HC, 64)]
        w = (jnp.concatenate(w, axis=0) << (16 * (1 - (hn & 1))).astype(u32)) & jnp.uint32(0x7FFF0000)
        return functools.reduce(jnp.add, [pltpu.bitcast(t, f32) for t in _vregs([w])])

    def w_balance(parts):
        n = len(parts) // 2
        sk, sv = [jnp.sum(functools.reduce(jnp.add, p), keepdims=True) for p in (parts[:n], parts[n:])]
        ok = jnp.logical_and(sk > 0, sv > 0)
        ratio = jnp.broadcast_to(jnp.where(ok, 1.4 * sk, 1.0) / jnp.where(ok, sv, 1.0), (8, T))
        e = jnp.clip(pltpu.bitcast(ratio, jnp.int32) & 0x7F800000, (127 - 40) << 23, (127 + 40) << 23)
        fw_s[0] = pltpu.bitcast(e, f32)
        fw_s[1] = pltpu.bitcast((254 << 23) - e, f32)
        return [e]

    def w_pacer(hn, first, last):
        parts = []
        return _Pacer([lambda m=m, r0=r0: parts.append(w_sum(hn, m, r0)) or parts[-1:]
                       for m in range(2) for r0 in (0, HC)] + [lambda: w_balance(parts)], 1, first, last)

    def first_terms(hn):
        w = _unpack(wkv_p[(hn >> 1) & 1, 0, :, :T], (16 * (1 - (hn & 1))).astype(u32))
        t = w[:HC] + 0.5 * w[HC:]
        return [t0_s.put((slice(r, r + RB), slice(n * T, (n + 1) * T)), v[r:r + RB].astype(bf))
                for n, v in enumerate((t[:QC], t[QC:] - t[:QC])) for r in range(0, QC, RB)]

    def residual(n):
        g8 = jax.nn.sigmoid(g_s[n])
        g_s[n] = g8
        a = (1.0 - g8[1:2, :]) * xt_s[:, n * T:(n + 1) * T].astype(f32)
        acc_s[n] = a
        return [a]

    gs, us, ys, hid = [], [], {}, []
    xs_dot = lambda w_s, n: (_dot(xs_s[0], w_s[:HM, n * T:(n + 1) * T]) + _dot(xs_s[1], w_s[HM:, n * T:(n + 1) * T]))

    def swiglu():
        gg, uu = jnp.concatenate(gs, axis=1), jnp.concatenate(us, axis=1)
        hid.append((gg * jax.nn.sigmoid(gg) * uu).astype(bf))

    def down(n0, k0):
        t = _dot_nt(hid[0][:, k0:min(k0 + 512, F)], wd_s[n0:min(n0 + T, M), k0:min(k0 + 512, F)])
        ys[n0] = ys[n0] + t if n0 in ys else t
    side = []
    for n in range(F // T):
        side += [lambda n=n: gs.append(xs_dot(wg_s, n)), lambda n=n: us.append(xs_dot(wu_s, n))]
    side += [swiglu] + [lambda: None] * 7
    side += [functools.partial(down, n0, k0) for n0 in range(0, M, T) for k0 in range(0, F, 512)]
    c_pace = c_pacer((NP - 2) * NG, QS // RB - (NP - 2) * NG, 2, 55)
    r_pace = _Pacer([functools.partial(residual, n) for n in range(NQ)], M // 8, 2, 47)

    w_pace0 = w_pacer(jnp.int32(0), 3, 52)
    t_pace0 = _Pacer([lambda: first_terms(jnp.int32(0))], 32, 37, 56)

    def hook7():
        if side:
            side.pop(0)()
        return c_pace(), r_pace(), w_pace0(), t_pace0()
    q_strassen([NP - 1], _Q7_ORDER, hook7)
    assert not side and all(p.finished() for p in (c_pace, r_pace, w_pace0, t_pace0))
    y = jnp.concatenate([ys[n0] for n0 in range(0, M, T)] + [jnp.zeros((16, 512 - M), f32)], axis=1)
    yt = (y * rsel_s[:, 0:1]).T
    lane128 = lax.broadcasted_iota(jnp.int32, (1, T), 1)
    for e in range(2):
        i = idx_s[e]
        acc_s[i // T] += jnp.where(lane128 == i % T, (1.0 - g_s[i // T][1:2, :]) * yt[:M, e:e + 1], 0.0)

    for m in range(2):
        cp_kv(1, m).start()
    cp_wo.wait()

    tri = lax.broadcasted_iota(jnp.int32, (T, T), 1) <= lax.broadcasted_iota(jnp.int32, (T, T), 0)
    prog = _head_program()

    def head(h, carry):
        par, slot = h & 1, (h >> 1) & 1

        @pl.when(jnp.logical_and(h < H - 1, par == 1))
        def _():
            for m in range(2):
                cp_kv((h + 1) >> 1, m).wait()

        sh = (16 * (1 - par)).astype(u32)
        rhs, fw, fw_inv = [], fw_s[0], fw_s[1]
        for r1 in range(7):
            wk, wv = [_unpack(wkv_p[slot, m], sh + (h >> (8 + r1)).astype(u32)) for m in range(2)]
            wv = jnp.concatenate([wv[:, :T] * fw[0:1], wv[:, T:] * fw[0:1]], axis=1)
            t = _rhs_terms2(wk[:HC], wv[:HC], wk[HC:], wv[HC:])[r1]
            rhs.append([u.astype(bf) for u in _rhs_terms(t[:QC, :T], t[:QC, T:], t[QC:, :T], t[QC:, T:])])
        rhs[1][1], rhs[1][3] = t0_s[:, :T], t0_s[:, T:]
        hn = jnp.minimum(h + 1, H - 1)
        t_pace = _Pacer([lambda: first_terms(hn)], 32, 196 - 14, 196)
        w_pace = w_pacer(hn, 60, 180)
        prods, inner_q, outer, kblk, vblk = {}, {}, {}, {}, {}

        def kv_product(r1, r2):
            m = prods.setdefault(r1, {})
            m[r2] = _dot(ca_s[7 * r1 + r2], rhs[r1][r2])
            if len(m) == 7:
                inner_q[r1] = (((m[3] - m[4]) + m[6]) + m[0], m[2] + m[4], m[1] + m[3], ((m[0] - m[1]) + m[2]) + m[5])
                for b in range(4):
                    if b not in kblk and all(q in inner_q for q in (0, 1, 3, 4, 6)):
                        p = {q: inner_q[q][b] for q in (0, 1, 3, 4, 6)}
                        e, d = p[3] + p[1], p[3] - p[1]
                        kblk[b] = (p[0] + ((d - p[4]) + p[6]), e * 2.0)
                        outer[b] = ((e + p[4]) + p[6], p[0] + d)
                    if len(inner_q) == 7:
                        p2, p5 = inner_q[2][b], inner_q[5][b]
                        vblk[b] = (((outer[b][0] + p2) - p5) * 0.5, (outer[b][1] + p2) + p5)

        def rows(blk, t0, t1):
            return jnp.concatenate([jnp.concatenate(
                [blk[2 * (t // 4 % 2) + j2][t // 8][t % 4 * T:(t % 4 + 1) * T] for j2 in range(2)], axis=1)
                for t in range(t0, t1)], axis=0)

        @functools.cache
        def k_tile(t):
            return rows(kblk, t, t + 1).astype(bf)

        @functools.cache
        def k_terms(J):
            ka, kb = rows(kblk, 2 * J, 2 * J + 1), rows(kblk, 2 * J + 1, 2 * J + 2)
            return [t.astype(bf) for t in _rhs_terms(ka[:, :T], kb[:, :T], ka[:, T:], kb[:, T:])]

        @functools.cache
        def v_tiles(c0, c1):
            return rows(vblk, c0, c1).astype(bf)

        s_prod, scores, rmax, soft, o_sum = {}, {}, {}, {}, {}
        q_tiles = lambda I: [q_s[h, i * T:(i + 1) * T, t * T:(t + 1) * T] for i in (2 * I, 2 * I + 1) for t in range(2)]

        def score_product(I, code):
            J, k = code // 8, code % 8
            if k in (2, 3):
                lhs = q_tiles(I)[3 * (k - 2)]
            else:
                lhs = qa_s[h, I * T:(I + 1) * T, (k - 2 * (k > 3)) * T:(k - 2 * (k > 3) + 1) * T]
            s_prod[I, J, k] = _dot_nt(_feed(lhs, t_pace(), w_pace()), k_terms(J)[k])
            if not all((I, J, q) in s_prod for q in range(7)):
                return
            for n, c in enumerate(_strassen(lambda q: s_prod.pop((I, J, q)))):
                s_s[I % 2, n // 2, 2 * J + n % 2] = c
            for u in range(2):
                sa, sb = s_s[I % 2, u, 2 * J], s_s[I % 2, u, 2 * J + 1]
                scores[2 * I + u, 2 * J] = s_s[I % 2, u, 2 * J]
                scores[2 * I + u, 2 * J + 1] = s_s[I % 2, u, 2 * J + 1]
                mx = jnp.maximum(sa, sb)
                rmax[2 * I + u] = jnp.maximum(rmax[2 * I + u], mx) if 2 * I + u in rmax else mx

        def score_diag(I):
            a, b = 2 * I, 2 * I + 1
            q4 = q_tiles(I)
            qa, qb = jnp.concatenate(q4[0:2], axis=1), jnp.concatenate(q4[2:4], axis=1)
            d1 = _dot_nt(jnp.concatenate([qa, qb], axis=0), k_tile(a))
            d2 = _dot_nt(qb, k_tile(b))
            scores[a, a], scores[b, a], scores[b, b] = jnp.where(tri, d1[:T], NEG), d1[T:], jnp.where(tri, d2, NEG)

        def pv_chunk(i, c0):
            if c0 == 0:
                mx = functools.reduce(jnp.maximum, ([rmax[i]] if i > 1 else [])
                                      + [scores[i, t] for t in range(i // 2 * 2, i + 1)])
                soft[i] = dict(m=jnp.max(mx, axis=1, keepdims=True), l=None, ctx=None)
            st = soft[i]
            c1 = min(c0 + 2, i + 1)
            p = jnp.exp2(jnp.concatenate([scores.pop((i, t)) for t in range(c0, c1)], axis=1) - st['m']).astype(bf)
            pf = p.astype(f32)
            for t in range(c1 - c0):
                st['l'] = pf[:, t * T:(t + 1) * T] if st['l'] is None else st['l'] + pf[:, t * T:(t + 1) * T]
            d = _dot(p, v_tiles(c0, c1))
            st['ctx'] = d if st['ctx'] is None else st['ctx'] + d

        def context(i):
            st = soft.pop(i)
            l = jnp.sum(st['l'], axis=1, keepdims=True)
            r = pl.reciprocal(l, approx=True)
            return st['ctx'] * (r * (2.0 - l * r) * fw_inv[0:1, 0:1])

        def ship(blocks):
            @pl.when(h == H - 1)
            def _():
                for i in blocks:
                    cp_out(i).start()

        def out_plain(i):
            wo, ctx = wo_s[h], context(i).astype(bf)
            for a0 in (0, HM):
                a = acc_s[i, a0:a0 + HM, :] + g_s[i][1:2, :] * _dot_nt(wo[a0:a0 + HM], ctx)
                acc_s[i, a0:a0 + HM, :] = a
                out_s[i, a0:a0 + HM, :] = a.astype(bf)
            ship([i])

        @functools.cache
        def wo_terms():
            w = wo_s[h].astype(f32)
            return [t.astype(bf) for t in _lhs_terms(w[:HM, :T], w[:HM, T:], w[HM:, :T], w[HM:, T:])]

        @functools.cache
        def ctx_terms(I):
            ca, cb = context(2 * I), context(2 * I + 1)
            return _rhs_terms(ca[:, :T], cb[:, :T], ca[:, T:], cb[:, T:])

        def out_product(I, k):
            om_s[I, k] += _dot_nt(wo_terms()[k], ctx_terms(I)[k].astype(bf))
            o_sum[I, k] = om_s[I, k]
            if all((I, q) in o_sum for q in range(7)):
                for n, c in enumerate(_strassen(lambda q: o_sum.pop((I, q)))):
                    i, a0 = 2 * I + n % 2, (n // 2) * HM
                    out_s[i, a0:a0 + HM, :] = (acc_s[i, a0:a0 + HM, :] + g_s[i][1:2, :] * c).astype(bf)
                ship([2 * I, 2 * I + 1])

        ops = {'m': kv_product, 'r': score_product, 'd': score_diag, 'p': pv_chunk,
               'o': out_product, 'S': out_plain}
        for op, *args in prog:
            ops[op](*args)
        assert t_pace.finished() and w_pace.finished()

        @pl.when(jnp.logical_and((h + 3) >> 1 < NP, par == 1))
        def _():
            for m in range(2):
                cp_kv((h + 3) >> 1, m).start()
        return carry

    lax.fori_loop(0, H, head, 0)
    for i in range(NQ):
        cp_out(i).wait()


@jax.jit
def pallas_gated_mix__compressed_kv_cla__moe_arch_mod__prompt_kernel(
    A_x: jax.Array,
    A_c_kv: jax.Array,
    A_w_q: jax.Array,
    A_w_uk: jax.Array,
    A_w_uv: jax.Array,
    A_w_o: jax.Array,
    B_x: jax.Array,
    B_w_r: jax.Array,
    B_w_gate: jax.Array,
    B_w_up: jax.Array,
    B_w_down: jax.Array,
    gate_w: jax.Array,
):
    del B_x
    V = pltpu.VMEM
    B = lambda *shape: V(shape[:-2] + (shape[-2] // 2, shape[-1]), u32)
    out_t = pl.pallas_call(
        _kernel,
        in_specs=[pl.BlockSpec(memory_space=pl.ANY)] * 11,
        out_specs=pl.BlockSpec(memory_space=pl.ANY),
        out_shape=jax.ShapeDtypeStruct((M, S), bf),
        scratch_shapes=[
            V((M, S), bf), V((2, S, HM), bf), B(5, HS, HM),
            B(S, DC), B(49, QS, QC),
            V((NP, M, D), u32), V((2, 2, DC, D), u32), B(H, M, D),
            B(H, S, D), B(H, HS, 5 * T),
            V((NQ, M, T), f32),
            B(M, F), B(M, F), B(M, F),
            V((M,), bf), V((M,), bf), V((NQ, M, T), bf),
            V((NQ, 8, T), f32), B(2, 16, HM), V((16, T), f32),
            pltpu.SMEM((2,), jnp.int32),
            V((2, 2, NQ, T, T), f32), B(QC, 2 * T),
            V((NQ // 2, 7, HM, T), f32),
            V((2, 8, T), f32),
            pltpu.SemaphoreType.DMA((NSEM,)),
        ],
        compiler_params=pltpu.CompilerParams(vmem_limit_bytes=110 * 1024 * 1024),
        name="gated_mix_cla_mod",
    )(A_x[0].T, A_c_kv[0], A_w_q, A_w_uk, A_w_uv, A_w_o.transpose(0, 2, 1), B_w_r, B_w_gate, B_w_up,
      B_w_down.T, gate_w)
    return out_t.T[None]
```

```python
import functools
import math

import jax
import jax.numpy as jnp
from jax import lax
from jax.experimental import pallas as pl
from jax.experimental.pallas import tpu as pltpu

S, M, H, D, DC, F = 2048, 448, 16, 256, 1024, 1792
T = 128
NP, NQ = H // 2, S // T
HS, HM, HC = S // 2, M // 2, DC // 2
QS, QC = S // 4, DC // 4
RB = 16
XC = 256
NG = 5
NT = (((1,), (1,)), ((), ()))
QSCALE = D ** -0.5 * math.log2(math.e)
NEG = -1e30
bf, f32, u32 = jnp.bfloat16, jnp.float32, jnp.uint32
HI = 0xFFFF0000

SEM_WO, SEM_FFN, SEM_VEC, SEM_KV, SEM_WQ, SEM_XT, SEM_C, SEM_OUT, NSEM = 0, 1, 4, 6, 8, 16, 24, 32, 48


def _lhs_terms(a11, a12, a21, a22):
    return [a11 + a22, a21 + a22, a11, a22, a11 + a12, a21 - a11, a12 - a22]


def _rhs_terms(b11, b12, b21, b22):
    return [b11 + b22, b11, b12 - b22, b21 - b11, b22, b11 + b12, b21 + b22]


def _strassen(mm):
    m2, m3, m4, m5, m1, m7, m6 = [mm(i) for i in (1, 2, 3, 4, 0, 6, 5)]
    return (m4 - m5) + (m1 + m7), m3 + m5, m2 + m4, (m3 - m2) + (m1 + m6)


def _lhs_terms2(a11, a12, a21, a22):
    h21, q21, h22 = 0.5 * a21, 0.25 * a21, 0.5 * a22
    s1 = a11 + a22
    v, hs = a12 + q21, 0.5 * s1
    return [s1, q21 + h22, a11 + h21, h22 - q21, v + hs, h21 - a11, v - hs]


def _rhs_terms2(b11, b12, b21, b22):
    h21 = 0.5 * b21
    t1 = b11 + b22
    v, ht = b12 + 0.5 * h21, 0.5 * t1
    return [t1, b11 + h21, v - ht, h21 - b11, b22 - h21, v + ht, b22 + h21]


def _vregs(vals):
    ts = []
    for v in vals:
        v = v if v.dtype == u32 else pltpu.bitcast(v, u32)
        ts += [v[r:r + 8, c:c + T] for r in range(0, v.shape[0], 8) for c in range(0, v.shape[1] - T + 1, T)]
    return ts


def _zero_from(ts):
    acc = ts[:4]
    for i, t in enumerate(ts[4:]):
        acc[i % 4] = acc[i % 4] | t
    while len(acc) > 1:
        acc = [acc[i] | acc[i + 1] if i + 1 < len(acc) else acc[i] for i in range(0, len(acc), 2)]
    return (acc[0] >> 16) >> 16


def _feed(a, *zs):
    zs = [z for z in zs if z is not None]
    if not zs:
        return a
    a32 = pltpu.bitcast(a, u32)
    top = functools.reduce(lambda p, q: p | q, zs, a32[0:8, :T])
    if a32.shape[1] > T:
        top = jnp.concatenate([top, a32[0:8, T:]], axis=1)
    return pltpu.bitcast(jnp.concatenate([top, a32[8:]], axis=0), bf)


class _Pacer:
    def __init__(self, thunks, per, first, last):
        self.thunks, self.pool, self.k, self.done = list(thunks), [], 0, 0
        self.tot, self.first, self.last = per * len(self.thunks), first, last

    def __call__(self):
        self.k += 1
        if self.k <= self.first:
            return None
        want = min(self.tot, -(-(self.k - self.first) * self.tot // (self.last - self.first))) - self.done
        while len(self.pool) < want and self.thunks:
            self.pool += _vregs(self.thunks.pop(0)())
        outs, self.pool = self.pool[:want], self.pool[want:]
        self.done += len(outs)
        return _zero_from(outs) if outs else None

    def finished(self):
        return not self.thunks and not self.pool


_HEAD_ORDER = """
m1.1 m1.3 m1.4 m1.6 m1.0 m3.4 m1.2 m3.3 m4.3 m3.6 m3.0 m3.1 m4.4 m3.2 m3.5 m1.5 m4.6 m4.1 m4.0 m6.6 m6.3 m6.0
m0.1 m4.5 m6.4 m6.1 m6.5 m6.2 m4.2 m0.6 m0.4 m0.3 m0.0 m0.2 m0.5 m2.1 d0 m2.3 r7.1 r7.2 r7.3 r7.4 r7.0 r7.6 r7.5
m2.4 r7.9 r7.10 r7.11 r7.12 r7.8 r7.14 r7.13 m2.0 m2.6 m5.1 r7.17 r7.18 r7.19 r7.20 r7.16 r7.22 r7.21 m2.2 r7.33
r7.34 r7.35 r7.36 r7.37 r7.32 r7.38 m2.5 r7.25 r7.26 r7.27 r7.24 r7.28 r7.30 r7.49 r7.29 r7.50 r7.51 r7.52 r7.48
r7.54 r7.53 r7.41 r7.42 r7.43 r7.44 r7.40 r7.46 r7.45 d7 m5.3 m5.6 m5.4 m5.0 m5.2 m5.5 p14.0 r6.1 r6.2 r6.3 r6.4
r6.0 r6.5 p1.0 p0.0 r6.6 r6.17 r6.18 r6.20 r6.19 r6.16 r6.9 r6.22 r6.21 r6.10 r6.12 r6.11 r6.8 r6.14 r6.13 p14.2
p14.4 p14.6 p14.8 p14.10 p14.12 p14.14 r6.24 r6.25 r6.26 r6.27 p15.0 r6.28 r6.30 r6.29 r6.33 r6.34 r6.35 r6.36
r6.32 r6.38 r6.37 r6.41 r6.42 r6.43 r6.44 r6.40 r6.46 r6.45 p15.2 p15.4 p15.6 p15.8 p15.10 d6 p15.12 p15.14 r5.1
r5.2 r5.3 r5.4 r5.0 r5.5 r5.6 p12.0 p12.2 p12.4 p12.6 r5.26 r5.25 r5.27 r5.28 r5.16 r5.22 r5.21 r5.24 r5.30
r5.17 r5.29 r5.18 r5.19 r5.20 r5.9 r5.13 r5.10 r5.11 r5.12 p13.0 r5.8 r5.14 p12.8 p12.10 p13.2 p13.4 r5.33 r5.34
r5.36 r5.32 r5.38 r5.37 r5.35 p13.6 p13.8 d5 o0.3 p12.12 p10.0 o0.2 o0.1 p11.0 o0.0 o0.5 p13.10 r4.10 r4.9 r4.11
r4.12 r4.8 r4.14 r4.13 o0.4 p10.2 p13.12 p10.4 r4.1 r4.6 r4.2 r4.3 r4.4 r4.0 r4.5 o0.6 p10.6 p10.8 p11.2 p10.10
r4.24 r4.25 r4.26 r4.27 r4.28 r4.30 r4.18 r4.19 r4.20 r4.16 r4.22 p11.4 r4.29 r4.21 r4.17 d4 p11.6 o7.2 o7.0
o7.1 o7.4 o7.3 o7.6 o7.5 p11.8 p8.0 r3.1 r3.2 r3.3 r3.0 p8.2 r3.6 r3.5 r3.4 p11.10 p8.4 p9.0 p8.6 p9.2 r3.14
r3.9 p8.8 r3.11 r3.13 r3.12 r3.10 r3.8 d3 r3.17 r3.18 r3.19 r3.20 r3.22 r3.16 r3.21 o6.4 o6.2 p9.4 p7.0 o6.3
o6.6 o6.0 o6.1 r2.9 r2.10 r2.11 r2.14 r2.12 r2.8 r2.13 p6.0 p9.6 p9.8 p6.2 p6.4 r2.2 r2.3 r2.4 r2.1 r2.0 r2.5
r2.6 o6.5 p6.6 d2 p7.2 p4.0 o5.6 o5.2 o5.3 o5.1 o5.4 o5.5 o5.0 r1.2 r1.3 r1.6 r1.4 r1.1 r1.0 p4.2 p7.4 p5.0 r1.5
p7.6 p4.4 d1 p5.2 o4.2 o4.4 o4.0 o4.1 p2.0 o4.3 o4.5 o4.6 p2.2 p5.4 p3.0 o2.1 p3.2 S2 o3.3 o2.0 o3.2 o3.1 o2.3
o2.6 o2.4 o2.2 o2.5 o3.5 o3.0 o3.4 o3.6 S3
"""


def _head_program():
    return [(t[0],) + tuple(int(v) for v in t[1:].split('.')) for t in _HEAD_ORDER.split()]


_P0_ORDER = """
61 r0 r1 70 r4 r3 60 r2 71 62 r5 63 r7 72 r6 73 r8 80 r9 90 93 r11 81 r14 r12 91 r13 83 r15 82 r10 92 a1 a0 b0
f3 c3 d2 d3 f0 e0 e1 b2 c0 c1 b1 a3 a2 b3 e2 c2 f2 f1 e3 d1 d0
"""
_Q7_ORDER = """
010 023 021 027 016 022 026 025 030 012 014 015 011 017 045 044 047 020 031 032 033 034 013 024 046 043 036 035
041 042 000 037 040 001 005 004 003 006 002 007 060 061 066 067 062 063 064 065 051 053 052 050 056 054 055 057
"""
_Q_ORDER = """
017 013 016 011 014 010 015 012 041 027 031 026 022 024 034 007 040 021 042 047 001 025 036 035 033 046 005 023
006 032 043 004 044 020 037 030 000 045 054 002 003 050 061 053 066 062 063 060 067 051 064 052 065 117 112 116
113 111 124 125 126 121 123 120 057 127 122 133 130 131 144 132 056 114 140 110 137 143 055 100 146 141 115 107
160 134 136 147 145 135 161 142 101 102 162 152 163 106 150 165 103 104 167 154 105 157 153 164 155 166 151 156
"""


def _dot(a, b):
    return jnp.dot(a, b, preferred_element_type=f32)


def _dot_nt(a, b):
    return lax.dot_general(a, b, NT, preferred_element_type=f32)


def _unpack(w32, sh):
    return pltpu.bitcast((w32 << sh) & jnp.uint32(HI), f32)


class _Bf16:
    def __init__(self, raw):
        self.raw = raw

    def _half(self, idx):
        idx = list(idx if isinstance(idx, tuple) else (idx,))
        idx += [slice(None)] * (len(self.raw.shape) - len(idx))
        r = idx[-2]
        if isinstance(r, slice):
            idx[-2] = slice(None if r.start is None else r.start // 2, None if r.stop is None else r.stop // 2)
        elif isinstance(r.start, int):
            idx[-2] = pl.ds(r.start // 2, r.size // 2)
        else:
            idx[-2] = pl.ds(pl.multiple_of(r.start >> 1, 8), r.size // 2)
        return tuple(idx)

    def __getitem__(self, idx):
        return pltpu.bitcast(self.raw[self._half(idx)], bf)

    def put(self, idx, v):
        idx = self._half(idx)
        ref = self.raw.at[idx[:-2]] if len(idx) > 2 else self.raw
        o = pltpu.bitcast(v, u32)
        ref[idx[-2], idx[-1]] = o
        return o

    def __setitem__(self, idx, v):
        self.put(idx, v)


def _kernel(xt_hbm, c_hbm, wq_hbm, wk_hbm, wv_hbm, wo_hbm, wr_hbm, wg_hbm, wu_hbm, wd_hbm, gw_hbm, o_hbm,
            xt_s, x_s, xa_r, c_r, ca_r, wq_p, wkv_p, wo_r, q_r, qa_r, acc_s, wg_r, wu_r, wd_r,
            wr_s, gw_s, out_s, g_s, xs_r, rsel_s, idx_s, s_s, t0_r, om_s, fw_s, sem):
    xa_s, c_s, ca_s, wo_s, q_s, qa_s, wg_s, wu_s, wd_s, xs_s, t0_s = [
        _Bf16(r) for r in (xa_r, c_r, ca_r, wo_r, q_r, qa_r, wg_r, wu_r, wd_r, xs_r, t0_r)]
    mk = pltpu.make_async_copy
    wq32, wk32, wv32 = wq_hbm.bitcast(u32), wk_hbm.bitcast(u32), wv_hbm.bitcast(u32)
    cp_wq = lambda j: mk(wq32.at[:, j, :], wq_p.at[j], sem.at[SEM_WQ + j])
    cp_kv = lambda j, m: mk((wk32, wv32)[m].at[:, j, :], wkv_p.at[j & 1, m], sem.at[SEM_KV + m])
    cp_xt = lambda k: mk(xt_hbm.at[:, pl.ds(k * XC, XC)], xt_s.at[:, pl.ds(k * XC, XC)], sem.at[SEM_XT + k])
    cp_out = lambda i: mk(out_s.at[i], o_hbm.at[:, pl.ds(i * T, T)], sem.at[SEM_OUT + i])
    cp_vec = [mk(wr_hbm, wr_s, sem.at[SEM_VEC]), mk(gw_hbm, gw_s, sem.at[SEM_VEC + 1])]
    cp_ffn = [mk(src, dst, sem.at[SEM_FFN + n]) for n, (src, dst) in
              enumerate(((wg_hbm.bitcast(u32), wg_r), (wu_hbm.bitcast(u32), wu_r), (wd_hbm.bitcast(u32), wd_r)))]
    cp_wo = mk(wo_hbm.bitcast(u32), wo_r, sem.at[SEM_WO])
    c32 = c_hbm.bitcast(u32)

    def cp_c(j):
        r0 = (j - 1) * (NG * RB // 2)
        n = QS // 2 - r0 if isinstance(j, int) and j == NP - 1 else NG * RB // 2
        return [mk(c32.at[pl.ds(i * QS // 2 + r0, n)], c_r.at[pl.ds(i * QS // 2 + r0, n)], sem.at[SEM_C + j])
                for i in range(4)]

    cp_xt(0).start()
    cp_wq(0).start()
    for k in range(1, S // XC):
        cp_xt(k).start()
    for cp in cp_vec:
        cp.start()
    for j in range(1, NP):
        cp_wq(j).start()
        for cp in cp_c(j):
            cp.start()
    for cp in cp_ffn + [cp_kv(0, 0), cp_kv(0, 1), cp_wo]:
        cp.start()

    @pl.loop(0, NQ // 2)
    def _(n):
        om_s[n] = jnp.zeros(om_s.shape[1:], f32)

    def store_q(j, e, r0, q):
        q = q * QSCALE
        q_s[2 * j + e, r0:r0 + q.shape[0], :] = q.astype(bf)
        for p0 in range(0, q.shape[0], 2 * T):
            if r0 + p0 > 0:
                qa, qb = q[p0:p0 + T], q[p0 + T:p0 + 2 * T]
                terms = _lhs_terms(qa[:, :T], qa[:, T:], qb[:, :T], qb[:, T:])
                for k, i in enumerate((0, 1, 4, 5, 6)):
                    qa_s[2 * j + e, (r0 + p0) // 2:(r0 + p0) // 2 + T, k * T:(k + 1) * T] = terms[i].astype(bf)

    def q_dot(w, r0, r1, z=None):
        return _dot(_feed(x_s[0, r0:r1, :], z), w[:HM]) + _dot(x_s[1, r0:r1, :], w[HM:])

    def q_plain(w, r0):
        qf = q_dot(w, r0, r0 + 2 * T)
        store_q(0, 0, r0, qf[:, :D])
        store_q(0, 1, r0, qf[:, D:])

    def q_rhs(j):
        lo, hi = pltpu.bitcast(wq_p[j] << 16, f32), pltpu.bitcast(wq_p[j] & jnp.uint32(HI), f32)
        b = [jnp.concatenate([lo[:, t * T:(t + 1) * T], hi[:, t * T:(t + 1) * T]], axis=1) for t in range(2)]
        return [t.astype(bf) for t in _rhs_terms(b[0][:HM], b[1][:HM], b[0][HM:], b[1][HM:])]

    def q_strassen(js, order, hook):
        ts, res = [q_rhs(j) for j in js], {}
        for a, k, u in [map(int, t) for t in order.split()]:
            if k in (2, 3):
                lhs = x_s[k - 2, (k - 2) * HS + u * T:(k - 2) * HS + (u + 1) * T, :]
            else:
                lhs = xa_s[k - 2 * (k > 3), u * T:(u + 1) * T, :]
            res[a, k, u] = _dot(_feed(lhs, *hook()), ts[a][k])
            v = u // 2 * 2
            if all((a, kk, uu) in res for kk in range(7) for uu in (v, v + 1)):
                cs = _strassen(lambda i: jnp.concatenate([res.pop((a, i, v)), res.pop((a, i, v + 1))], axis=0))
                for w in range(2):
                    for e in range(2):
                        q = jnp.concatenate([c[:, e * T:(e + 1) * T] for c in cs[2 * w:2 * w + 2]], axis=1)
                        store_q(js[a], e, w * HS + v * T, q)

    def x_prep(r0):
        a = [x_s[e, h0 + r0:h0 + r0 + RB, :].astype(f32) for h0 in (0, HS) for e in (0, 1)]
        terms = _lhs_terms(*a)
        outs = []
        for k, i in enumerate((0, 1, 4, 5, 6)):
            outs.append(xa_s.put((k, slice(r0, r0 + RB)), terms[i].astype(bf)))
        return outs

    def c_prep(g, c0):
        blk = lambda i, k: c_s[pl.ds(i * QS + g * RB, RB), k * QC + c0:k * QC + c0 + T].astype(f32)
        outer = [_lhs_terms2(*[blk(2 * i1 + i2, 2 * k1 + k2) for i1 in range(2) for k1 in range(2)])
                 for i2 in range(2) for k2 in range(2)]
        outs = []
        for r1 in range(7):
            for r2, v in enumerate(_lhs_terms(*[o[r1] for o in outer])):
                outs.append(ca_s.put((7 * r1 + r2, pl.ds(g * RB, RB), slice(c0, c0 + T)), v.astype(bf)))
        return outs

    def c_pacer(g0, ng, first, last):
        return _Pacer([functools.partial(c_prep, g0 + t // 2, (t % 2) * T) for t in range(2 * ng)], 49, first, last)

    def transpose(k):
        for e in range(2):
            x_s[e, k * XC:(k + 1) * XC, :] = xt_s[e * HM:(e + 1) * HM, k * XC:(k + 1) * XC].T

    def q_w0():
        return jnp.concatenate([pltpu.bitcast(wq_p[0] << 16, f32).astype(bf),
                                pltpu.bitcast(wq_p[0] & jnp.uint32(HI), f32).astype(bf)], axis=1)

    cp_xt(0).wait()
    transpose(0)
    cp_wq(0).wait()
    q_plain(q_w0(), 0)
    for k in range(1, 4):
        cp_xt(k).wait()
    transpose(1)
    w0 = q_w0()
    transpose(2)
    q_plain(w0, XC)
    transpose(3)
    q_plain(w0, 2 * XC)
    for k in range(4, S // XC):
        cp_xt(k).wait()
    for cp in cp_vec:
        cp.wait()
    for k in range(4, S // XC):
        transpose(k)
    row8 = lax.broadcasted_iota(jnp.int32, (8, M), 0)
    x_pace = _Pacer([functools.partial(x_prep, r0) for r0 in range(0, HS, RB)], 5, 12, 40)
    w0, res = q_w0(), {}
    for t in _P0_ORDER.split():
        if t[0] == 'r':
            n = int(t[1:])
            rg = jnp.where(row8 == 0, wr_s[...].reshape(1, M).astype(f32), gw_s[...].reshape(1, M).astype(f32))
            g_s[n] = _dot(rg.astype(bf), xt_s[:, n * T:(n + 1) * T])
            continue
        u, n = int(t[:-1], 16), int(t[-1])
        res[u, n] = q_dot(w0[:, n * T:(n + 1) * T], u * T, (u + 1) * T, x_pace())
        v = u // 2 * 2
        if all((uu, nn) in res for uu in (v, v + 1) for nn in range(4)):
            for e in range(2):
                store_q(0, e, v * T, jnp.concatenate([jnp.concatenate(
                    [res.pop((uu, nn)) for nn in (2 * e, 2 * e + 1)], axis=1) for uu in (v, v + 1)], axis=0))
    assert x_pace.finished()

    rb = jnp.concatenate([g_s[n][0:1, :] for n in range(NQ)], axis=1).astype(bf).astype(f32)
    lane = lax.broadcasted_iota(jnp.int32, (1, S), 1)
    m1 = jnp.max(rb, axis=1, keepdims=True)
    i1 = jnp.minimum(jnp.min(jnp.where(rb == m1, lane, S)), S - 1)
    rb2 = jnp.where(lane == i1, -jnp.inf, rb)
    m2 = jnp.max(rb2, axis=1, keepdims=True)
    i2 = jnp.minimum(jnp.min(jnp.where(jnp.logical_and(rb2 == m2, lane != i1), lane, S)), S - 1)
    row16 = lax.broadcasted_iota(jnp.int32, (16, HM), 0)

    def x_row(e, i):
        blk = x_s[e, pl.ds(pl.multiple_of((i // 16) * 16, 16), 16), :].astype(f32)
        return jnp.sum(jnp.where(row16 == i % 16, blk, 0.0), axis=0, keepdims=True)
    for e in range(2):
        xs_s[e] = jnp.where(row16 == 0, x_row(e, i1), jnp.where(row16 == 1, x_row(e, i2), 0.0)).astype(bf)
    rsel_s[...] = jax.nn.sigmoid(jnp.where(lax.broadcasted_iota(jnp.int32, (16, T), 0) == 0, m1, m2))
    idx_s[0] = i1
    idx_s[1] = i2

    def q_body(it, carry):
        js = (2 * it + 1, 2 * it + 2)
        for j in js:
            for cp in [cp_wq(j)] + cp_c(j):
                cp.wait()
        pace = c_pacer(2 * it * NG, 2 * NG, 1, 108)
        q_strassen(js, _Q_ORDER, lambda: (pace(),))
        assert pace.finished()
        return carry
    lax.fori_loop(0, 3, q_body, 0)

    for cp in cp_ffn + [cp_wq(NP - 1), cp_kv(0, 0), cp_kv(0, 1)] + cp_c(NP - 1):
        cp.wait()

    def w_sum(hn, m, r0):
        w = [wkv_p[(hn >> 1) & 1, m, r:r + 8, :] for r in range(r0, r0 + HC, 64)]
        w = (jnp.concatenate(w, axis=0) << (16 * (1 - (hn & 1))).astype(u32)) & jnp.uint32(0x7FFF0000)
        return functools.reduce(jnp.add, [pltpu.bitcast(t, f32) for t in _vregs([w])])

    def w_balance(parts):
        n = len(parts) // 2
        sk, sv = [jnp.sum(functools.reduce(jnp.add, p), keepdims=True) for p in (parts[:n], parts[n:])]
        ratio = jnp.broadcast_to(1.4 * sk / sv, (8, T))
        e = jnp.clip(pltpu.bitcast(ratio, jnp.int32) & 0x7F800000, (127 - 24) << 23, (127 + 24) << 23)
        fw_s[0] = pltpu.bitcast(e, f32)
        fw_s[1] = pltpu.bitcast((254 << 23) - e, f32)
        return [e]

    def w_pacer(hn, first, last):
        parts = []
        return _Pacer([lambda m=m, r0=r0: parts.append(w_sum(hn, m, r0)) or parts[-1:]
                       for m in range(2) for r0 in (0, HC)] + [lambda: w_balance(parts)], 1, first, last)

    def first_terms(hn):
        w = _unpack(wkv_p[(hn >> 1) & 1, 0, :, :T], (16 * (1 - (hn & 1))).astype(u32))
        t = w[:HC] + 0.5 * w[HC:]
        return [t0_s.put((slice(r, r + RB), slice(n * T, (n + 1) * T)), v[r:r + RB].astype(bf))
                for n, v in enumerate((t[:QC], t[QC:] - t[:QC])) for r in range(0, QC, RB)]

    def residual(n):
        g8 = jax.nn.sigmoid(g_s[n])
        g_s[n] = g8
        a = (1.0 - g8[1:2, :]) * xt_s[:, n * T:(n + 1) * T].astype(f32)
        acc_s[n] = a
        return [a]

    gs, us, ys, hid = [], [], {}, []
    xs_dot = lambda w_s, n: (_dot(xs_s[0], w_s[:HM, n * T:(n + 1) * T]) + _dot(xs_s[1], w_s[HM:, n * T:(n + 1) * T]))

    def swiglu():
        gg, uu = jnp.concatenate(gs, axis=1), jnp.concatenate(us, axis=1)
        hid.append((gg * jax.nn.sigmoid(gg) * uu).astype(bf))

    def down(n0, k0):
        t = _dot_nt(hid[0][:, k0:min(k0 + 512, F)], wd_s[n0:min(n0 + T, M), k0:min(k0 + 512, F)])
        ys[n0] = ys[n0] + t if n0 in ys else t
    side = []
    for n in range(F // T):
        side += [lambda n=n: gs.append(xs_dot(wg_s, n)), lambda n=n: us.append(xs_dot(wu_s, n))]
    side += [swiglu] + [lambda: None] * 7
    side += [functools.partial(down, n0, k0) for n0 in range(0, M, T) for k0 in range(0, F, 512)]
    c_pace = c_pacer((NP - 2) * NG, QS // RB - (NP - 2) * NG, 2, 55)
    r_pace = _Pacer([functools.partial(residual, n) for n in range(NQ)], M // 8, 2, 47)

    w_pace0 = w_pacer(jnp.int32(0), 3, 52)
    t_pace0 = _Pacer([lambda: first_terms(jnp.int32(0))], 32, 37, 56)

    def hook7():
        if side:
            side.pop(0)()
        return c_pace(), r_pace(), w_pace0(), t_pace0()
    q_strassen([NP - 1], _Q7_ORDER, hook7)
    assert not side and all(p.finished() for p in (c_pace, r_pace, w_pace0, t_pace0))
    y = jnp.concatenate([ys[n0] for n0 in range(0, M, T)] + [jnp.zeros((16, 512 - M), f32)], axis=1)
    yt = (y * rsel_s[:, 0:1]).T
    lane128 = lax.broadcasted_iota(jnp.int32, (1, T), 1)
    for e in range(2):
        i = idx_s[e]
        acc_s[i // T] += jnp.where(lane128 == i % T, (1.0 - g_s[i // T][1:2, :]) * yt[:M, e:e + 1], 0.0)

    for m in range(2):
        cp_kv(1, m).start()
    cp_wo.wait()

    tri = lax.broadcasted_iota(jnp.int32, (T, T), 1) <= lax.broadcasted_iota(jnp.int32, (T, T), 0)
    prog = _head_program()

    def head(h, carry):
        par, slot = h & 1, (h >> 1) & 1

        @pl.when(jnp.logical_and(h < H - 1, par == 1))
        def _():
            for m in range(2):
                cp_kv((h + 1) >> 1, m).wait()

        sh = (16 * (1 - par)).astype(u32)
        rhs, fw, fw_inv = [], fw_s[0], fw_s[1]
        for r1 in range(7):
            wk, wv = [_unpack(wkv_p[slot, m], sh + (h >> (8 + r1)).astype(u32)) for m in range(2)]
            wv = jnp.concatenate([wv[:, :T] * fw[0:1], wv[:, T:] * fw[0:1]], axis=1)
            t = _rhs_terms2(wk[:HC], wv[:HC], wk[HC:], wv[HC:])[r1]
            rhs.append([u.astype(bf) for u in _rhs_terms(t[:QC, :T], t[:QC, T:], t[QC:, :T], t[QC:, T:])])
        rhs[1][1], rhs[1][3] = t0_s[:, :T], t0_s[:, T:]
        hn = jnp.minimum(h + 1, H - 1)
        t_pace = _Pacer([lambda: first_terms(hn)], 32, 196 - 14, 196)
        w_pace = w_pacer(hn, 60, 180)
        prods, inner_q, outer, kblk, vblk = {}, {}, {}, {}, {}

        def kv_product(r1, r2):
            m = prods.setdefault(r1, {})
            m[r2] = _dot(ca_s[7 * r1 + r2], rhs[r1][r2])
            if len(m) == 7:
                inner_q[r1] = (((m[3] - m[4]) + m[6]) + m[0], m[2] + m[4], m[1] + m[3], ((m[0] - m[1]) + m[2]) + m[5])
                for b in range(4):
                    if b not in kblk and all(q in inner_q for q in (0, 1, 3, 4, 6)):
                        p = {q: inner_q[q][b] for q in (0, 1, 3, 4, 6)}
                        e, d = p[3] + p[1], p[3] - p[1]
                        kblk[b] = (p[0] + ((d - p[4]) + p[6]), e * 2.0)
                        outer[b] = ((e + p[4]) + p[6], p[0] + d)
                    if len(inner_q) == 7:
                        p2, p5 = inner_q[2][b], inner_q[5][b]
                        vblk[b] = (((outer[b][0] + p2) - p5) * 0.5, (outer[b][1] + p2) + p5)

        def rows(blk, t0, t1):
            return jnp.concatenate([jnp.concatenate(
                [blk[2 * (t // 4 % 2) + j2][t // 8][t % 4 * T:(t % 4 + 1) * T] for j2 in range(2)], axis=1)
                for t in range(t0, t1)], axis=0)

        @functools.cache
        def k_tile(t):
            return rows(kblk, t, t + 1).astype(bf)

        @functools.cache
        def k_terms(J):
            ka, kb = rows(kblk, 2 * J, 2 * J + 1), rows(kblk, 2 * J + 1, 2 * J + 2)
            return [t.astype(bf) for t in _rhs_terms(ka[:, :T], kb[:, :T], ka[:, T:], kb[:, T:])]

        @functools.cache
        def v_tiles(c0, c1):
            return rows(vblk, c0, c1).astype(bf)

        s_prod, scores, rmax, soft, o_sum = {}, {}, {}, {}, {}
        q_tiles = lambda I: [q_s[h, i * T:(i + 1) * T, t * T:(t + 1) * T] for i in (2 * I, 2 * I + 1) for t in range(2)]

        def score_product(I, code):
            J, k = code // 8, code % 8
            if k in (2, 3):
                lhs = q_tiles(I)[3 * (k - 2)]
            else:
                lhs = qa_s[h, I * T:(I + 1) * T, (k - 2 * (k > 3)) * T:(k - 2 * (k > 3) + 1) * T]
            s_prod[I, J, k] = _dot_nt(_feed(lhs, t_pace(), w_pace()), k_terms(J)[k])
            if not all((I, J, q) in s_prod for q in range(7)):
                return
            for n, c in enumerate(_strassen(lambda q: s_prod.pop((I, J, q)))):
                s_s[I % 2, n // 2, 2 * J + n % 2] = c
            for u in range(2):
                sa, sb = s_s[I % 2, u, 2 * J], s_s[I % 2, u, 2 * J + 1]
                scores[2 * I + u, 2 * J] = s_s[I % 2, u, 2 * J]
                scores[2 * I + u, 2 * J + 1] = s_s[I % 2, u, 2 * J + 1]
                mx = jnp.maximum(sa, sb)
                rmax[2 * I + u] = jnp.maximum(rmax[2 * I + u], mx) if 2 * I + u in rmax else mx

        def score_diag(I):
            a, b = 2 * I, 2 * I + 1
            q4 = q_tiles(I)
            qa, qb = jnp.concatenate(q4[0:2], axis=1), jnp.concatenate(q4[2:4], axis=1)
            d1 = _dot_nt(jnp.concatenate([qa, qb], axis=0), k_tile(a))
            d2 = _dot_nt(qb, k_tile(b))
            scores[a, a], scores[b, a], scores[b, b] = jnp.where(tri, d1[:T], NEG), d1[T:], jnp.where(tri, d2, NEG)

        def pv_chunk(i, c0):
            if c0 == 0:
                mx = functools.reduce(jnp.maximum, ([rmax[i]] if i > 1 else [])
                                      + [scores[i, t] for t in range(i // 2 * 2, i + 1)])
                soft[i] = dict(m=jnp.max(mx, axis=1, keepdims=True), l=None, ctx=None)
            st = soft[i]
            c1 = min(c0 + 2, i + 1)
            p = jnp.exp2(jnp.concatenate([scores.pop((i, t)) for t in range(c0, c1)], axis=1) - st['m']).astype(bf)
            pf = p.astype(f32)
            for t in range(c1 - c0):
                st['l'] = pf[:, t * T:(t + 1) * T] if st['l'] is None else st['l'] + pf[:, t * T:(t + 1) * T]
            d = _dot(p, v_tiles(c0, c1))
            st['ctx'] = d if st['ctx'] is None else st['ctx'] + d

        def context(i):
            st = soft.pop(i)
            l = jnp.sum(st['l'], axis=1, keepdims=True)
            r = pl.reciprocal(l, approx=True)
            return st['ctx'] * (r * (2.0 - l * r) * fw_inv[0:1, 0:1])

        def ship(blocks):
            @pl.when(h == H - 1)
            def _():
                for i in blocks:
                    cp_out(i).start()

        def out_plain(i):
            wo, ctx = wo_s[h], context(i).astype(bf)
            for a0 in (0, HM):
                a = acc_s[i, a0:a0 + HM, :] + g_s[i][1:2, :] * _dot_nt(wo[a0:a0 + HM], ctx)
                acc_s[i, a0:a0 + HM, :] = a
                out_s[i, a0:a0 + HM, :] = a.astype(bf)
            ship([i])

        @functools.cache
        def wo_terms():
            w = wo_s[h].astype(f32)
            return [t.astype(bf) for t in _lhs_terms(w[:HM, :T], w[:HM, T:], w[HM:, :T], w[HM:, T:])]

        @functools.cache
        def ctx_terms(I):
            ca, cb = context(2 * I), context(2 * I + 1)
            return _rhs_terms(ca[:, :T], cb[:, :T], ca[:, T:], cb[:, T:])

        def out_product(I, k):
            om_s[I, k] += _dot_nt(wo_terms()[k], ctx_terms(I)[k].astype(bf))
            o_sum[I, k] = om_s[I, k]
            if all((I, q) in o_sum for q in range(7)):
                for n, c in enumerate(_strassen(lambda q: o_sum.pop((I, q)))):
                    i, a0 = 2 * I + n % 2, (n // 2) * HM
                    out_s[i, a0:a0 + HM, :] = (acc_s[i, a0:a0 + HM, :] + g_s[i][1:2, :] * c).astype(bf)
                ship([2 * I, 2 * I + 1])

        ops = {'m': kv_product, 'r': score_product, 'd': score_diag, 'p': pv_chunk,
               'o': out_product, 'S': out_plain}
        for op, *args in prog:
            ops[op](*args)
        assert t_pace.finished() and w_pace.finished()

        @pl.when(jnp.logical_and((h + 3) >> 1 < NP, par == 1))
        def _():
            for m in range(2):
                cp_kv((h + 3) >> 1, m).start()
        return carry

    lax.fori_loop(0, H, head, 0)
    for i in range(NQ):
        cp_out(i).wait()


@jax.jit
def pallas_gated_mix__compressed_kv_cla__moe_arch_mod__prompt_kernel(
    A_x: jax.Array,
    A_c_kv: jax.Array,
    A_w_q: jax.Array,
    A_w_uk: jax.Array,
    A_w_uv: jax.Array,
    A_w_o: jax.Array,
    B_x: jax.Array,
    B_w_r: jax.Array,
    B_w_gate: jax.Array,
    B_w_up: jax.Array,
    B_w_down: jax.Array,
    gate_w: jax.Array,
):
    del B_x
    V = pltpu.VMEM
    B = lambda *shape: V(shape[:-2] + (shape[-2] // 2, shape[-1]), u32)
    out_t = pl.pallas_call(
        _kernel,
        in_specs=[pl.BlockSpec(memory_space=pl.ANY)] * 11,
        out_specs=pl.BlockSpec(memory_space=pl.ANY),
        out_shape=jax.ShapeDtypeStruct((M, S), bf),
        scratch_shapes=[
            V((M, S), bf), V((2, S, HM), bf), B(5, HS, HM),
            B(S, DC), B(49, QS, QC),
            V((NP, M, D), u32), V((2, 2, DC, D), u32), B(H, M, D),
            B(H, S, D), B(H, HS, 5 * T),
            V((NQ, M, T), f32),
            B(M, F), B(M, F), B(M, F),
            V((M,), bf), V((M,), bf), V((NQ, M, T), bf),
            V((NQ, 8, T), f32), B(2, 16, HM), V((16, T), f32),
            pltpu.SMEM((2,), jnp.int32),
            V((2, 2, NQ, T, T), f32), B(QC, 2 * T),
            V((NQ // 2, 7, HM, T), f32),
            V((2, 8, T), f32),
            pltpu.SemaphoreType.DMA((NSEM,)),
        ],
        compiler_params=pltpu.CompilerParams(vmem_limit_bytes=110 * 1024 * 1024),
        name="gated_mix_cla_mod",
    )(A_x[0].T, A_c_kv[0], A_w_q, A_w_uk, A_w_uv, A_w_o.transpose(0, 2, 1), B_w_r, B_w_gate, B_w_up,
      B_w_down.T, gate_w)
    return out_t.T[None]
```
